```python
import jax
import jax.numpy as jnp

def _softmax(x, axis=-1):
    return jax.nn.softmax(x, axis=axis)

def _gelu(x):
    return jax.nn.gelu(x, approximate=True)

def _silu(x):
    return jax.nn.silu(x)

def _sigmoid(x):
    return jax.nn.sigmoid(x)

def _layernorm(x, axis=-1, eps=1e-05):
    m = jnp.mean(x, axis=axis, keepdims=True)
    v = jnp.var(x, axis=axis, keepdims=True)
    return (x - m) / jnp.sqrt(v + eps)

def _scatter_add(tgt, idx, src, axis=0):
    return tgt.at[idx].add(src)

def _segment_sum(src, seg, n):
    return jax.ops.segment_sum(src, seg, n)

class _Rng:

    def __init__(self, key):
        self._k = key

    def _next(self):
        self._k, sub = jax.random.split(self._k)
        return sub

    def normal(self, shape):
        return jax.random.normal(self._next(), shape, dtype=jnp.bfloat16)

    def randint(self, lo, hi, shape):
        return jax.random.randint(self._next(), shape, lo, hi, dtype=jnp.int32)

    def uniform(self, shape, lo=0.0, hi=1.0):
        return jax.random.uniform(self._next(), shape, jnp.bfloat16, lo, hi)

    def permutation(self, n):
        return jax.random.permutation(self._next(), n)
kernel_name = 'interleave_layers__linear_kernel_hedgehog__memory_aug_recurrent_mem_tr__prompt'

def setup_inputs():
    _rng = _Rng(jax.random.key(int.from_bytes(__import__("os").urandom(4), "little")))
    _w = lambda a: (lambda t: t.astype(jnp.bfloat16) if jnp.issubdtype(t.dtype, jnp.floating) else t)(jnp.asarray(a))

    def _A_setup():
        B, S, D, H = (1, 2048, 640, 32)
        Dh = D // H
        return {'x': _w((lambda *s: _rng.normal(s) * 0.05)(B, S, D)), 'wqkv': _w((lambda *s: _rng.normal(s) * 0.05)(D, 3 * D)), 'w_phi': _w((lambda *s: _rng.normal(s) * 0.05)(H, Dh, Dh) * Dh ** (-0.5)), 'wo': _w((lambda *s: _rng.normal(s) * 0.05)(D, D))}
    _A_in = _A_setup()

    def _B_setup():
        B, S, Dm = (1, 2048, 640)
        H, Dh = (32, 192)
        M, seg = (8, 32)
        seg = min(seg, S)
        S = S // seg * seg
        return {'x': _w((lambda *s: _rng.normal(s) * 0.05)(B, S, Dm)), 'mem0': _w((lambda *s: _rng.normal(s) * 0.05)(B, M, Dm)), 'Wq': _w((lambda *s: _rng.normal(s) * 0.05)(Dm, H, Dh) * Dm ** (-0.5)), 'Wk': _w((lambda *s: _rng.normal(s) * 0.05)(Dm, H, Dh) * Dm ** (-0.5)), 'Wv': _w((lambda *s: _rng.normal(s) * 0.05)(Dm, H, Dh) * Dm ** (-0.5)), 'Wo': _w((lambda *s: _rng.normal(s) * 0.05)(H, Dh, Dm) * (H * Dh) ** (-0.5)), 'seg_len': seg}
    _B_in = _B_setup()
    return {'A_x': _A_in['x'], 'A_wqkv': _A_in['wqkv'], 'A_w_phi': _A_in['w_phi'], 'A_wo': _A_in['wo'], 'B_x': _B_in['x'], 'B_mem0': _B_in['mem0'], 'B_Wq': _B_in['Wq'], 'B_Wk': _B_in['Wk'], 'B_Wv': _B_in['Wv'], 'B_Wo': _B_in['Wo'], 'B_seg_len': _B_in['seg_len']}

def reference(A_x, A_wqkv, A_w_phi, A_wo, B_x, B_mem0, B_Wq, B_Wk, B_Wv, B_Wo, B_seg_len):

    def _A_ref(x, wqkv, w_phi, wo):
        B, S, D = x.shape
        H = 32
        Dh = D // H
        qkv = (lambda x, *d: x.transpose(*d))((x @ wqkv).reshape(B, S, 3, H, Dh), 2, 0, 3, 1, 4)
        q, k, v = (qkv[0], qkv[1], qkv[2])
        pq = jnp.einsum('bhsd,hdf->bhsf', q, w_phi)
        pk = jnp.einsum('bhsd,hdf->bhsf', k, w_phi)
        phi_q = jnp.concatenate([_softmax(pq, axis=-1), _softmax(-pq, axis=-1)], axis=-1)
        phi_k = jnp.concatenate([_softmax(pk, axis=-1), _softmax(-pk, axis=-1)], axis=-1)
        kv = jnp.einsum('bhsf,bhsd->bhfd', phi_k, v)
        z = jnp.einsum('bhsf->bhf', phi_k)
        num = jnp.einsum('bhqf,bhfd->bhqd', phi_q, kv)
        den = jnp.einsum('bhqf,bhf->bhq', phi_q, z)[..., None] + 1e-06
        o = num / den
        return (lambda x, *d: x.transpose(*d))(o, 0, 2, 1, 3).reshape(B, S, D) @ wo

    def _B_ref(x, mem0, Wq, Wk, Wv, Wo, seg_len):
        B, S, Dm = x.shape
        H, Dh = (Wq.shape[1], Wq.shape[2])
        M = mem0.shape[1]
        scale = Dh ** (-0.5)
        n_seg = S // seg_len
        L = M + seg_len
        idx = jnp.arange(L)
        mask = (idx[:, None] < M) | (idx[:, None] >= idx[None, :])
        mem = mem0
        outs = []
        for s in range(n_seg):
            xs = x[:, s * seg_len:(s + 1) * seg_len, :].copy()
            h = jnp.concatenate([mem, xs], axis=1)
            q = jnp.einsum('btd,dhe->bhte', h, Wq)
            k = jnp.einsum('btd,dhe->bhte', h, Wk)
            v = jnp.einsum('btd,dhe->bhte', h, Wv)
            scores = jnp.einsum('bhqe,bhke->bhqk', q, k) * scale
            scores = jnp.where(mask[None, None], scores, -1000000000.0)
            p = _softmax(scores, axis=-1)
            o = jnp.einsum('bhqk,bhke->bhqe', p, v)
            o = jnp.einsum('bhte,hed->btd', o, Wo)
            mem = o[:, :M, :].copy()
            outs.append(o[:, M:, :])
        return jnp.concatenate(outs, axis=1)
    x = A_x
    x = x + _A_ref(_layernorm(x, axis=-1), A_wqkv, A_w_phi, A_wo)
    x = x + _B_ref(_layernorm(x, axis=-1), B_mem0, B_Wq, B_Wk, B_Wv, B_Wo, B_seg_len)
    x = x + _A_ref(_layernorm(x, axis=-1), A_wqkv, A_w_phi, A_wo)
    x = x + _B_ref(_layernorm(x, axis=-1), B_mem0, B_Wq, B_Wk, B_Wv, B_Wo, B_seg_len)
    return x
```

```python
import functools

import jax
import jax.numpy as jnp
from jax import lax
import jax.experimental.pallas as pl
import jax.experimental.pallas.tpu as pltpu

F32 = jnp.float32
BF16 = jnp.bfloat16

S = 2048
D = 640
HA = 32
FA = 20
GA = 4
GR = 8 * FA
TN = 256
HB = 32
DH = 192
HD = HB * DH
M = 8
SEG = 32
L = M + SEG
PW = 2 * DH
NP = HB // 2

NT = (((1,), (1,)), ((), ()))


def _dot(a, b):
    return jnp.dot(a, b, preferred_element_type=F32)


def _dot_nt(a, b):
    return lax.dot_general(a, b, NT, preferred_element_type=F32)


def _layernorm(x):
    m = jnp.mean(x, axis=-1, keepdims=True)
    c = x - m
    v = jnp.mean(c * c, axis=-1, keepdims=True)
    return c * lax.rsqrt(v + 1e-5)


def _feature_map(p):
    t = p.shape[-1]
    p3 = p.reshape(FA, 8, t)
    mx = jnp.max(p3, axis=0, keepdims=True)
    mn = jnp.min(p3, axis=0, keepdims=True)
    ep = jnp.exp(p3 - mx)
    en = jnp.exp(mn - p3)
    rp = 1.0 / jnp.sum(ep, axis=0, keepdims=True)
    rn = 1.0 / jnp.sum(en, axis=0, keepdims=True)
    out = jnp.concatenate([(ep * rp).reshape(GR, t), (en * rn).reshape(GR, t)], axis=0)
    return out.astype(BF16)


def _block_diag_pair(a):
    lane = lax.broadcasted_iota(jnp.int32, (L, 128), 1)
    mid = a[:, 128:256]
    zero = jnp.zeros((L, 128), F32)
    lo = jnp.concatenate([a[:, 0:128], jnp.where(lane < 64, mid, 0.0), zero], axis=1)
    hi = jnp.concatenate([zero, jnp.where(lane < 64, 0.0, mid), a[:, 256:384]], axis=1)
    return jnp.concatenate([lo, hi], axis=0).astype(BF16)


def _attn_pair(y):
    q = y[:, 0:PW].astype(BF16)
    kbd = _block_diag_pair(y[:, PW:2 * PW])
    vbd = _block_diag_pair(y[:, 2 * PW:3 * PW])
    s = _dot_nt(q, kbd) * (DH ** -0.5)
    row = lax.broadcasted_iota(jnp.int32, (L, 2 * L), 0)
    col = lax.broadcasted_iota(jnp.int32, (L, 2 * L), 1)
    first = col < L
    key = jnp.where(first, col, col - L)
    valid = jnp.logical_or(row < M, row >= key)
    s = jnp.where(valid, s, -1e9)
    m0 = jnp.max(jnp.where(first, s, -jnp.inf), axis=-1, keepdims=True)
    m1 = jnp.max(jnp.where(first, -jnp.inf, s), axis=-1, keepdims=True)
    e = jnp.exp(s - jnp.where(first, m0, m1))
    s0 = jnp.sum(jnp.where(first, e, 0.0), axis=-1, keepdims=True)
    s1 = jnp.sum(jnp.where(first, 0.0, e), axis=-1, keepdims=True)
    p = e * jnp.where(first, 1.0 / s0, 1.0 / s1)
    return _dot(p.astype(BF16), vbd)


def _kernel(x_ref, wqkv_ref, cphi_ref, woa_ref, mem0_ref,
            wq_hbm, wk_hbm, wv_hbm, wo_hbm,
            out_ref,
            xres, xa, xb, wat, wot, phq, kvacc, wraw, wb, wob, ysave, sems):
    copies = [pltpu.make_async_copy(src, wraw.at[i], sems.at[i])
              for i, src in enumerate((wq_hbm, wk_hbm, wv_hbm))]
    copies.append(pltpu.make_async_copy(wo_hbm, wob, sems.at[3]))
    for c in copies:
        c.start()

    cphi = cphi_ref[...].astype(F32)
    cb = jnp.concatenate(
        [jnp.broadcast_to(cphi[f:f + 1, :], (8, D)) for f in range(FA)], axis=0)
    for g in range(GA):
        row = lax.broadcasted_iota(jnp.int32, (GR, 256), 0)
        col = lax.broadcasted_iota(jnp.int32, (GR, 256), 1) + 128 * g
        lo = (8 * g + (row & 7)) * FA
        bd = jnp.where(jnp.logical_and(col >= lo, col < lo + FA),
                       cb[:, 128 * g:128 * g + 256], 0.0).astype(BF16)
        perm = jnp.where(col == lo + (row >> 3), 1.0, 0.0).astype(BF16)
        for i, lhs in enumerate((bd, bd, perm)):
            w = wqkv_ref[:, i * D + 128 * g:i * D + 128 * g + 256]
            wat[i * D + g * GR:i * D + (g + 1) * GR, :] = _dot_nt(lhs, w).astype(BF16)
        wog = _dot(perm, woa_ref[128 * g:128 * g + 256, :])
        phq[g * GR:(g + 1) * GR, 0:D] = wog.astype(BF16)
    wot[...] = phq[0:D, 0:D].T

    def ln0(j, _):
        r = pl.ds(pl.multiple_of(j * TN, TN), TN)
        x = x_ref[r, :].astype(F32)
        xres[r, :] = x
        xa[r, :] = _layernorm(x).astype(BF16)
        return 0
    lax.fori_loop(0, S // TN, ln0, 0)

    def a1(j, _):
        off = pl.multiple_of(j * TN, TN)
        xn = xa[pl.ds(off, TN), :]
        ones = jnp.ones((16, TN), BF16)
        for g in range(GA):
            pq = _dot_nt(wat[g * GR:(g + 1) * GR, :], xn)
            phq[2 * g * GR:2 * (g + 1) * GR, pl.ds(off, TN)] = _feature_map(pq)
            pk = _dot_nt(wat[D + g * GR:D + (g + 1) * GR, :], xn)
            vt = _dot_nt(wat[2 * D + g * GR:2 * D + (g + 1) * GR, :], xn)
            vt = jnp.concatenate([vt.astype(BF16), ones], axis=0)
            kvacc[g] += _dot_nt(vt, _feature_map(pk))
        return 0

    def a2(j, kvs):
        off = pl.multiple_of(j * TN, TN)
        os_ = []
        for g in range(GA):
            nt = _dot(kvs[g], phq[2 * g * GR:2 * (g + 1) * GR, pl.ds(off, TN)])
            rden = 1.0 / (nt[GR:GR + 8, :] + 1e-6)
            o = nt[0:GR, :].reshape(FA, 8, TN) * rden[None]
            os_.append(o.reshape(GR, TN).astype(BF16))
        ot = _dot(wot[...], jnp.concatenate(os_, axis=0))
        r = pl.ds(off, TN)
        x = xres[r, :] + ot.T
        xres[r, :] = x
        xb[r, :] = _layernorm(x)
        return kvs

    def b_pair(i, mem):
        base = pl.multiple_of(i * 2 * SEG, 2 * SEG)
        h = jnp.concatenate([mem, xb[pl.ds(base, 40), :]], axis=0).astype(BF16)
        oa = []
        for p in range(NP):
            y = _dot(h, wb[:, p * 3 * PW:(p + 1) * 3 * PW])
            ysave[:, p * 3 * PW:(p + 1) * 3 * PW] = y[L:L + 8, :]
            oa.append(_attn_pair(y[0:L, :]))
        oa = jnp.concatenate(oa, axis=1)
        ra = _dot(oa[0:32, :].astype(BF16), wob[...])
        h = jnp.concatenate([ra[0:M, :], xb[pl.ds(base + 40, 24), :]], axis=0).astype(BF16)
        ob = []
        for p in range(NP):
            y = _dot(h, wb[:, p * 3 * PW:(p + 1) * 3 * PW])
            y = jnp.concatenate(
                [y[0:M, :], ysave[:, p * 3 * PW:(p + 1) * 3 * PW], y[M:, :]], axis=0)
            ob.append(_attn_pair(y))
        ob = jnp.concatenate(ob, axis=1)
        rb = _dot(jnp.concatenate([ob, oa[32:40, :]], axis=0).astype(BF16), wob[...])
        r = pl.ds(base, 2 * SEG)
        x = xres[r, :] + jnp.concatenate([ra[M:, :], rb[L:, :], rb[M:L, :]], axis=0)
        xres[r, :] = x
        xa[r, :] = _layernorm(x).astype(BF16)
        out_ref[r, :] = x.astype(out_ref.dtype)
        return rb[0:M, :]

    def layer(l, _):
        kvacc[...] = jnp.zeros(kvacc.shape, F32)
        lax.fori_loop(0, S // TN, a1, 0)
        row = lax.broadcasted_iota(jnp.int32, (GR + 16, 2 * GR), 0)
        col = lax.broadcasted_iota(jnp.int32, (GR + 16, 2 * GR), 1)
        same = (row & 7) == (col & 7)
        kvs = tuple(jnp.where(same, kvacc[g], 0.0).astype(BF16) for g in range(GA))
        lax.fori_loop(0, S // TN, a2, kvs)

        @pl.when(l == 0)
        def _():
            for c in copies:
                c.wait()

            def tr(p, _):
                for i in range(3):
                    src = wraw[i, pl.ds(pl.multiple_of(p * PW, PW), PW), :]
                    wb[:, pl.ds(pl.multiple_of((3 * p + i) * PW, PW), PW)] = src.T
                return 0
            lax.fori_loop(0, NP, tr, 0)

        lax.fori_loop(0, S // (2 * SEG), b_pair, mem0_ref[...].astype(F32))
        return 0

    lax.fori_loop(0, 2, layer, 0)


@functools.partial(jax.jit, static_argnames=("B_seg_len",))
def pallas_interleave_layers__linear_kernel_hedgehog__memory_aug_recurrent_mem_tr__prompt_kernel(
    A_x, A_wqkv, A_w_phi, A_wo, B_x, B_mem0, B_Wq, B_Wk, B_Wv, B_Wo, B_seg_len,
):
    del B_x
    assert B_seg_len == SEG
    x = A_x.reshape(S, D)
    cphi = A_w_phi.reshape(D, FA).T
    mem0 = B_mem0.reshape(M, D)
    wq, wk, wv = (w.transpose(1, 2, 0).reshape(HD, D) for w in (B_Wq, B_Wk, B_Wv))
    wo = B_Wo.reshape(HD, D)
    vmem = pl.BlockSpec(memory_space=pltpu.VMEM)
    hbm = pl.BlockSpec(memory_space=pl.ANY)
    out = pl.pallas_call(
        _kernel,
        out_shape=jax.ShapeDtypeStruct((S, D), A_x.dtype),
        in_specs=[vmem] * 5 + [hbm] * 4,
        out_specs=vmem,
        scratch_shapes=[
            pltpu.VMEM((S, D), F32),
            pltpu.VMEM((S, D), BF16),
            pltpu.VMEM((S, D), F32),
            pltpu.VMEM((3 * D, D), BF16),
            pltpu.VMEM((D, D), BF16),
            pltpu.VMEM((2 * D, S), BF16),
            pltpu.VMEM((GA, GR + 16, 2 * GR), F32),
            pltpu.VMEM((3, HD, D), BF16),
            pltpu.VMEM((D, 3 * HD), BF16),
            pltpu.VMEM((HD, D), BF16),
            pltpu.VMEM((8, 3 * HD), F32),
            pltpu.SemaphoreType.DMA((4,)),
        ],
        compiler_params=pltpu.CompilerParams(vmem_limit_bytes=120 * 1024 * 1024),
    )(x, A_wqkv, cphi, A_wo, mem0, wq, wk, wv, wo)
    return out.reshape(1, S, D)
```

```python
import functools

import jax
import jax.numpy as jnp
from jax import lax
import jax.experimental.pallas as pl
import jax.experimental.pallas.tpu as pltpu

F32 = jnp.float32
BF16 = jnp.bfloat16
U32 = jnp.uint32

S = 2048
D = 640
HA = 32
FA = 20
GA = 4
GR = 8 * FA
TN = 256
HB = 32
DH = 192
HD = HB * DH
M = 8
SEG = 32
L = M + SEG
PW = 2 * DH
NP = HB // 2

NT = (((1,), (1,)), ((), ()))


def _dot(a, b):
    return jnp.dot(a, b, preferred_element_type=F32)


def _dot_nt(a, b):
    return lax.dot_general(a, b, NT, preferred_element_type=F32)


def _pack(a):
    return pltpu.bitcast(a, U32)


def _unpack(a):
    return pltpu.bitcast(a, BF16)


def _recip(x):
    r = pl.reciprocal(x, approx=True)
    return r * (2.0 - x * r)


def _layernorm(x):
    m = jnp.mean(x, axis=-1, keepdims=True)
    c = x - m
    v = jnp.mean(c * c, axis=-1, keepdims=True)
    return c * lax.rsqrt(v + 1e-5)


def _feature_map(p):
    t = p.shape[-1]
    p3 = p.reshape(FA, 8, t)
    mx = jnp.max(p3, axis=0, keepdims=True)
    mn = jnp.min(p3, axis=0, keepdims=True)
    ep = jnp.exp(p3 - mx)
    en = jnp.exp(mn - p3)
    rp = _recip(jnp.sum(ep, axis=0, keepdims=True))
    rn = _recip(jnp.sum(en, axis=0, keepdims=True))
    out = jnp.concatenate([(ep * rp).reshape(GR, t), (en * rn).reshape(GR, t)], axis=0)
    return out.astype(BF16)


def _block_diag_pair(a):
    lane = lax.broadcasted_iota(jnp.int32, (L, 128), 1)
    mid = a[:, 128:256]
    zero = jnp.zeros((L, 128), F32)
    lo = jnp.concatenate([a[:, 0:128], jnp.where(lane < 64, mid, 0.0), zero], axis=1)
    hi = jnp.concatenate([zero, jnp.where(lane < 64, 0.0, mid), a[:, 256:384]], axis=1)
    return jnp.concatenate([lo, hi], axis=0).astype(BF16)


def _scores(y):
    q = y[:, 0:PW].astype(BF16)
    kbd = _block_diag_pair(y[:, PW:2 * PW])
    s = _dot_nt(q, kbd) * (DH ** -0.5)
    row = lax.broadcasted_iota(jnp.int32, (L, 2 * L), 0)
    col = lax.broadcasted_iota(jnp.int32, (L, 2 * L), 1)
    first = col < L
    key = jnp.where(first, col, col - L)
    valid = jnp.logical_or(row < M, row >= key)
    s = jnp.where(valid, s, -1e9)
    m0 = jnp.max(jnp.where(first, s, -jnp.inf), axis=-1, keepdims=True)
    m1 = jnp.max(jnp.where(first, -jnp.inf, s), axis=-1, keepdims=True)
    e = jnp.exp(s - jnp.where(first, m0, m1))
    s0 = jnp.sum(jnp.where(first, e, 0.0), axis=-1, keepdims=True)
    s1 = jnp.sum(jnp.where(first, 0.0, e), axis=-1, keepdims=True)
    p = e * _recip(jnp.where(first, s0, s1))
    return p.astype(BF16)


def _segment(h, wb, wob, fix_y, fix_o):
    ps, vs, os_ = {}, {}, {}
    ys = {}

    def proj(p):
        ys[p] = fix_y(p, _dot(h, _unpack(wb[:, p * 3 * PW:(p + 1) * 3 * PW])))

    def score(p):
        y = ys.pop(p)
        vs[p] = _block_diag_pair(y[:, 2 * PW:3 * PW])
        ps[p] = _scores(y)

    def pv(p):
        os_[p] = fix_o(p, _dot(ps.pop(p), vs.pop(p))).astype(BF16)

    def oproj(lo, hi):
        o = jnp.concatenate([os_.pop(p) for p in range(lo, hi)], axis=1)
        return _dot(o, _unpack(wob[lo * PW // 2:hi * PW // 2, :]))

    for p in range(NP):
        proj(p)
        if p >= 1:
            score(p - 1)
        if p >= 2:
            pv(p - 2)
    r = oproj(0, 4)
    score(NP - 1)
    pv(NP - 2)
    r = oproj(4, 9) + r
    pv(NP - 1)
    r = oproj(9, 14) + r
    r = oproj(14, 16) + r
    return r


def _kernel(x_ref, wqkv_ref, cphi_ref, woa_ref, mem0_ref,
            wq_hbm, wk_hbm, wv_hbm, wo_hbm,
            out_ref,
            xres, xa, xb, wat, wot, phq, kvacc, kvs, wraw, wb, wob,
            ysave, osave, rsave, sems):
    copies = [pltpu.make_async_copy(src, wraw.at[i], sems.at[i])
              for i, src in enumerate((wq_hbm, wk_hbm, wv_hbm, wo_hbm))]
    for c in copies:
        c.start()

    cphi = cphi_ref[...].astype(F32)
    cb = jnp.concatenate(
        [jnp.broadcast_to(cphi[f:f + 1, :], (8, D)) for f in range(FA)], axis=0)
    wog = []
    for g in range(GA):
        row = lax.broadcasted_iota(jnp.int32, (GR, 256), 0)
        col = lax.broadcasted_iota(jnp.int32, (GR, 256), 1) + 128 * g
        lo = (8 * g + (row & 7)) * FA
        bd = jnp.where(jnp.logical_and(col >= lo, col < lo + FA),
                       cb[:, 128 * g:128 * g + 256], 0.0).astype(BF16)
        perm = jnp.where(col == lo + (row >> 3), 1.0, 0.0).astype(BF16)
        for i, lhs in enumerate((bd, bd, perm)):
            w = wqkv_ref[:, i * D + 128 * g:i * D + 128 * g + 256]
            wat[i * GA + g] = _pack(_dot_nt(lhs, w).astype(BF16))
        wog.append(_dot(perm, woa_ref[128 * g:128 * g + 256, :]).astype(BF16))
    wot[...] = _pack(jnp.concatenate(wog, axis=0).T)

    def ln0(j, _):
        r = pl.ds(pl.multiple_of(j * TN, TN), TN)
        x = x_ref[r, :].astype(F32)
        xres[r, :] = x
        xa[pl.ds(pl.multiple_of(j * (TN // 2), TN // 2), TN // 2), :] = _pack(
            _layernorm(x).astype(BF16))
        return 0
    with jax.named_scope("ln0"):
        lax.fori_loop(0, S // TN, ln0, 0)

    def a1(j, _):
        off = pl.multiple_of(j * TN, TN)
        xn = _unpack(xa[pl.ds(pl.multiple_of(j * (TN // 2), TN // 2), TN // 2), :])
        ones = jnp.ones((16, TN), BF16)
        prev = None
        for g in range(GA):
            pk = _dot_nt(_unpack(wat[GA + g]), xn)
            vt = _dot_nt(_unpack(wat[2 * GA + g]), xn)
            if prev is not None:
                kvacc[g - 1] += _dot_nt(*prev)
            pq = _dot_nt(_unpack(wat[g]), xn)
            phq[g, :, pl.ds(off, TN)] = _pack(_feature_map(pq))
            prev = (jnp.concatenate([vt.astype(BF16), ones], axis=0), _feature_map(pk))
        kvacc[GA - 1] += _dot_nt(*prev)
        return 0

    def a2(j, _):
        off = pl.multiple_of(j * TN, TN)
        os_ = []
        for g in range(GA):
            nt = _dot(_unpack(kvs[g]), _unpack(phq[g, :, pl.ds(off, TN)]))
            rden = 1.0 / (nt[GR:GR + 8, :] + 1e-6)
            o = nt[0:GR, :].reshape(FA, 8, TN) * rden[None]
            os_.append(o.reshape(GR, TN).astype(BF16))
        ot = _dot(_unpack(wot[...]), jnp.concatenate(os_, axis=0))
        r = pl.ds(off, TN)
        x = xres[r, :] + ot.T
        xres[r, :] = x
        xb[r, :] = _layernorm(x)
        return 0

    def b_finish(base):
        r = pl.ds(base, 2 * SEG)
        x = xres[r, :] + rsave[...]
        xres[r, :] = x
        xa[pl.ds(base // 2 if isinstance(base, int) else pl.multiple_of(base // 2, SEG), SEG), :] = _pack(_layernorm(x).astype(BF16))
        out_ref[r, :] = x.astype(out_ref.dtype)

    def b_pair(i, mem):
        base = pl.multiple_of(i * 2 * SEG, 2 * SEG)
        b_finish(pl.multiple_of(jnp.maximum(i - 1, 0) * 2 * SEG, 2 * SEG))

        def fix_ya(p, y):
            ysave[:, p * 3 * PW:(p + 1) * 3 * PW] = y[L:L + 8, :]
            return y[0:L, :]

        def fix_oa(p, o):
            osave[:, p * PW:(p + 1) * PW] = o[32:L, :]
            return o[0:32, :]

        h = jnp.concatenate([mem, xb[pl.ds(base, 40), :]], axis=0).astype(BF16)
        ra = _segment(h, wb, wob, fix_ya, fix_oa)
        rsave[0:24, :] = ra[M:, :]

        def fix_yb(p, y):
            return jnp.concatenate(
                [y[0:M, :], ysave[:, p * 3 * PW:(p + 1) * 3 * PW], y[M:, :]], axis=0)

        def fix_ob(p, o):
            return jnp.concatenate([o, osave[:, p * PW:(p + 1) * PW]], axis=0)

        h = jnp.concatenate([ra[0:M, :], xb[pl.ds(base + 40, 24), :]], axis=0).astype(BF16)
        rb = _segment(h, wb, wob, fix_yb, fix_ob)
        rsave[24:32, :] = rb[L:, :]
        rsave[32:64, :] = rb[M:L, :]
        return rb[0:M, :]

    def layer(l, _):
        kvacc[...] = jnp.zeros(kvacc.shape, F32)
        with jax.named_scope("a1"):
            lax.fori_loop(0, S // TN, a1, 0)
        row = lax.broadcasted_iota(jnp.int32, (GR + 16, 2 * GR), 0)
        col = lax.broadcasted_iota(jnp.int32, (GR + 16, 2 * GR), 1)
        same = (row & 7) == (col & 7)
        for g in range(GA):
            kvs[g] = _pack(jnp.where(same, kvacc[g], 0.0).astype(BF16))
        with jax.named_scope("a2"):
            lax.fori_loop(0, S // TN, a2, 0)

        @pl.when(l == 0)
        def _():
            for c in copies:
                c.wait()

            def tr(p, _):
                rows = pl.ds(pl.multiple_of(p * PW, PW), PW)
                for i in range(3):
                    wb[:, pl.ds(pl.multiple_of((3 * p + i) * PW, PW), PW)] = _pack(
                        wraw[i, rows, :].T)
                wob[pl.ds(pl.multiple_of(p * DH, DH), DH), :] = _pack(wraw[3, rows, :])
                return 0
            with jax.named_scope("tr"):
                lax.fori_loop(0, NP, tr, 0)

        rsave[...] = jnp.zeros(rsave.shape, F32)
        with jax.named_scope("b"):
            lax.fori_loop(0, S // (2 * SEG), b_pair, mem0_ref[...].astype(F32))
        b_finish(S - 2 * SEG)
        return 0

    lax.fori_loop(0, 2, layer, 0)


@functools.partial(jax.jit, static_argnames=("B_seg_len",))
def pallas_interleave_layers__linear_kernel_hedgehog__memory_aug_recurrent_mem_tr__prompt_kernel(
    A_x, A_wqkv, A_w_phi, A_wo, B_x, B_mem0, B_Wq, B_Wk, B_Wv, B_Wo, B_seg_len,
):
    del B_x
    assert B_seg_len == SEG
    x = A_x.reshape(S, D)
    cphi = A_w_phi.reshape(D, FA).T
    mem0 = B_mem0.reshape(M, D)
    wq, wk, wv = (w.transpose(1, 2, 0).reshape(HD, D) for w in (B_Wq, B_Wk, B_Wv))
    wo = B_Wo.reshape(HD, D)
    vmem = pl.BlockSpec(memory_space=pltpu.VMEM)
    hbm = pl.BlockSpec(memory_space=pl.ANY)
    out = pl.pallas_call(
        _kernel,
        out_shape=jax.ShapeDtypeStruct((S, D), A_x.dtype),
        in_specs=[vmem] * 5 + [hbm] * 4,
        out_specs=vmem,
        scratch_shapes=[
            pltpu.VMEM((S, D), F32),
            pltpu.VMEM((S // 2, D), U32),
            pltpu.VMEM((S, D), F32),
            pltpu.VMEM((3 * GA, GR // 2, D), U32),
            pltpu.VMEM((D // 2, D), U32),
            pltpu.VMEM((GA, GR, S), U32),
            pltpu.VMEM((GA, GR + 16, 2 * GR), F32),
            pltpu.VMEM((GA, GR // 2 + 8, 2 * GR), U32),
            pltpu.VMEM((4, HD, D), BF16),
            pltpu.VMEM((D // 2, 3 * HD), U32),
            pltpu.VMEM((HD // 2, D), U32),
            pltpu.VMEM((8, 3 * HD), F32),
            pltpu.VMEM((8, HD), F32),
            pltpu.VMEM((2 * SEG, D), F32),
            pltpu.SemaphoreType.DMA((4,)),
        ],
        compiler_params=pltpu.CompilerParams(vmem_limit_bytes=120 * 1024 * 1024),
    )(x, A_wqkv, cphi, A_wo, mem0, wq, wk, wv, wo)
    return out.reshape(1, S, D)
```

```python
import functools

import jax
import jax.numpy as jnp
from jax import lax
import jax.experimental.pallas as pl
import jax.experimental.pallas.tpu as pltpu

F32 = jnp.float32
BF16 = jnp.bfloat16
U32 = jnp.uint32

S = 2048
D = 640
HA = 32
FA = 20
GA = 4
GR = 8 * FA
TN = 256
HB = 32
DH = 192
HD = HB * DH
M = 8
SEG = 32
L = M + SEG
PW = 2 * DH
NP = HB // 2

NT = (((1,), (1,)), ((), ()))


def _dot(a, b):
    return jnp.dot(a, b, preferred_element_type=F32)


def _dot_nt(a, b):
    return lax.dot_general(a, b, NT, preferred_element_type=F32)


def _pack(a):
    return pltpu.bitcast(a, U32)


def _unpack(a):
    return pltpu.bitcast(a, BF16)


def _recip(x):
    r = pl.reciprocal(x, approx=True)
    return r * (2.0 - x * r)


def _layernorm(x):
    m = jnp.mean(x, axis=-1, keepdims=True)
    c = x - m
    v = jnp.mean(c * c, axis=-1, keepdims=True)
    return c * lax.rsqrt(v + 1e-5)


def _feature_map(p):
    t = p.shape[-1]
    p3 = p.reshape(FA, 8, t)
    mx = jnp.max(p3, axis=0, keepdims=True)
    mn = jnp.min(p3, axis=0, keepdims=True)
    ep = jnp.exp(p3 - mx)
    en = jnp.exp(mn - p3)
    rp = _recip(jnp.sum(ep, axis=0, keepdims=True))
    rn = _recip(jnp.sum(en, axis=0, keepdims=True))
    out = jnp.concatenate([(ep * rp).reshape(GR, t), (en * rn).reshape(GR, t)], axis=0)
    return out.astype(BF16)


def _split_pair(a):
    lane = lax.broadcasted_iota(jnp.int32, (L, 128), 1)
    mid = a[:, 128:256]
    outer = jnp.concatenate([a[:, 0:128], a[:, 256:384]], axis=0)
    mid = jnp.concatenate(
        [jnp.where(lane < 64, mid, 0.0), jnp.where(lane < 64, 0.0, mid)], axis=0)
    return outer.astype(BF16), mid.astype(BF16)


def _scores(y):
    q_outer = jnp.concatenate([y[:, 0:128], y[:, 256:384]], axis=0).astype(BF16)
    q_mid = y[:, 128:256].astype(BF16)
    k_outer, k_mid = _split_pair(y[:, PW:2 * PW])
    s_outer = _dot_nt(q_outer, k_outer)
    s_mid = _dot_nt(q_mid, k_mid)
    row = lax.broadcasted_iota(jnp.int32, (L, 2 * L), 0)
    col = lax.broadcasted_iota(jnp.int32, (L, 2 * L), 1)
    first = col < L
    key = jnp.where(first, col, col - L)
    valid = jnp.logical_or(row < M, row >= key)
    s = (jnp.where(first, s_outer[0:L, :], s_outer[L:, :]) + s_mid) * (DH ** -0.5)
    s = jnp.where(valid, s, -1e9)
    m0 = jnp.max(jnp.where(first, s, -jnp.inf), axis=-1, keepdims=True)
    m1 = jnp.max(jnp.where(first, -jnp.inf, s), axis=-1, keepdims=True)
    e = jnp.exp(s - jnp.where(first, m0, m1))
    s0 = jnp.sum(jnp.where(first, e, 0.0), axis=-1, keepdims=True)
    s1 = jnp.sum(jnp.where(first, 0.0, e), axis=-1, keepdims=True)
    p = e * _recip(jnp.where(first, s0, s1))
    ps = jnp.concatenate([jnp.where(first, p, 0.0), jnp.where(first, 0.0, p)], axis=0)
    return p.astype(BF16), ps.astype(BF16)


def _pv(p, ps, v_outer, v_mid):
    o_outer = _dot(ps, v_outer)
    o_mid = _dot(p, v_mid)
    return jnp.concatenate([o_outer[0:L, :], o_mid, o_outer[L:, :]], axis=1)


def _segment(h, wb, wob, fix_y, fix_o):
    ps, vs, os_ = {}, {}, {}
    ys = {}

    def proj(p):
        ys[p] = fix_y(p, _dot(h, _unpack(wb[:, p * 3 * PW:(p + 1) * 3 * PW])))

    def score(p):
        y = ys.pop(p)
        vs[p] = _split_pair(y[:, 2 * PW:3 * PW])
        ps[p] = _scores(y)

    def pv(p):
        os_[p] = fix_o(p, _pv(*ps.pop(p), *vs.pop(p))).astype(BF16)

    def oproj(lo, hi):
        o = jnp.concatenate([os_.pop(p) for p in range(lo, hi)], axis=1)
        return _dot(o, _unpack(wob[lo * PW // 2:hi * PW // 2, :]))

    for p in range(NP):
        proj(p)
        if p >= 1:
            score(p - 1)
        if p >= 3:
            pv(p - 3)
    r = oproj(0, 3)
    score(NP - 1)
    pv(NP - 3)
    r = oproj(3, 6) + r
    pv(NP - 2)
    r = oproj(6, 10) + r
    pv(NP - 1)
    r = oproj(10, 14) + r
    r = oproj(14, 16) + r
    return r


def _kernel(x_ref, wqkv_ref, cphi_ref, woa_ref, mem0_ref,
            wq_hbm, wk_hbm, wv_hbm, wo_hbm,
            out_ref,
            xres, xa, xb, wat, wot, phq, kvacc, kvs, wraw, wb, wob,
            ysave, osave, rsave, sems):
    copies = [pltpu.make_async_copy(src, wraw.at[i], sems.at[i])
              for i, src in enumerate((wq_hbm, wk_hbm, wv_hbm, wo_hbm))]
    for c in copies:
        c.start()

    cphi = cphi_ref[...].astype(F32)
    cb = jnp.concatenate(
        [jnp.broadcast_to(cphi[f:f + 1, :], (8, D)) for f in range(FA)], axis=0)
    wog = []
    for g in range(GA):
        row = lax.broadcasted_iota(jnp.int32, (GR, 256), 0)
        col = lax.broadcasted_iota(jnp.int32, (GR, 256), 1) + 128 * g
        lo = (8 * g + (row & 7)) * FA
        bd = jnp.where(jnp.logical_and(col >= lo, col < lo + FA),
                       cb[:, 128 * g:128 * g + 256], 0.0).astype(BF16)
        perm = jnp.where(col == lo + (row >> 3), 1.0, 0.0).astype(BF16)
        for i, lhs in enumerate((bd, bd, perm)):
            w = wqkv_ref[:, i * D + 128 * g:i * D + 128 * g + 256]
            wat[i * GA + g] = _pack(_dot_nt(lhs, w).astype(BF16))
        wog.append(_dot(perm, woa_ref[128 * g:128 * g + 256, :]).astype(BF16))
    wot[...] = _pack(jnp.concatenate(wog, axis=0).T)

    def ln0(j, _):
        r = pl.ds(pl.multiple_of(j * TN, TN), TN)
        x = x_ref[r, :].astype(F32)
        xres[r, :] = x
        xa[pl.ds(pl.multiple_of(j * (TN // 2), TN // 2), TN // 2), :] = _pack(
            _layernorm(x).astype(BF16))
        return 0
    with jax.named_scope("ln0"):
        lax.fori_loop(0, S // TN, ln0, 0)

    def a1(j, _):
        off = pl.multiple_of(j * TN, TN)
        xn = _unpack(xa[pl.ds(pl.multiple_of(j * (TN // 2), TN // 2), TN // 2), :])
        ones = jnp.ones((16, TN), BF16)
        prev = None
        for g in range(GA):
            pk = _dot_nt(_unpack(wat[GA + g]), xn)
            vt = _dot_nt(_unpack(wat[2 * GA + g]), xn)
            if prev is not None:
                kvacc[g - 1] += _dot_nt(*prev)
            pq = _dot_nt(_unpack(wat[g]), xn)
            phq[g, :, pl.ds(off, TN)] = _pack(_feature_map(pq))
            prev = (jnp.concatenate([vt.astype(BF16), ones], axis=0), _feature_map(pk))
        kvacc[GA - 1] += _dot_nt(*prev)
        return 0

    def a2(j, _):
        off = pl.multiple_of(j * TN, TN)
        os_ = []
        for g in range(GA):
            nt = _dot(_unpack(kvs[g]), _unpack(phq[g, :, pl.ds(off, TN)]))
            rden = 1.0 / (nt[GR:GR + 8, :] + 1e-6)
            o = nt[0:GR, :].reshape(FA, 8, TN) * rden[None]
            os_.append(o.reshape(GR, TN).astype(BF16))
        ot = _dot(_unpack(wot[...]), jnp.concatenate(os_, axis=0))
        r = pl.ds(off, TN)
        x = xres[r, :] + ot.T
        xres[r, :] = x
        xb[r, :] = _layernorm(x)
        return 0

    def b_finish(base):
        r = pl.ds(base, 2 * SEG)
        x = xres[r, :] + rsave[...]
        xres[r, :] = x
        xa[pl.ds(base // 2 if isinstance(base, int) else pl.multiple_of(base // 2, SEG), SEG), :] = _pack(_layernorm(x).astype(BF16))
        out_ref[r, :] = x.astype(out_ref.dtype)

    def b_pair(i, mem):
        base = pl.multiple_of(i * 2 * SEG, 2 * SEG)
        b_finish(pl.multiple_of(jnp.maximum(i - 1, 0) * 2 * SEG, 2 * SEG))

        def fix_ya(p, y):
            ysave[:, p * 3 * PW:(p + 1) * 3 * PW] = y[L:L + 8, :]
            return y[0:L, :]

        def fix_oa(p, o):
            osave[:, p * PW:(p + 1) * PW] = o[32:L, :]
            return o[0:32, :]

        h = jnp.concatenate([mem, xb[pl.ds(base, 40), :]], axis=0).astype(BF16)
        ra = _segment(h, wb, wob, fix_ya, fix_oa)
        rsave[0:24, :] = ra[M:, :]

        def fix_yb(p, y):
            return jnp.concatenate(
                [y[0:M, :], ysave[:, p * 3 * PW:(p + 1) * 3 * PW], y[M:, :]], axis=0)

        def fix_ob(p, o):
            return jnp.concatenate([o, osave[:, p * PW:(p + 1) * PW]], axis=0)

        h = jnp.concatenate([ra[0:M, :], xb[pl.ds(base + 40, 24), :]], axis=0).astype(BF16)
        rb = _segment(h, wb, wob, fix_yb, fix_ob)
        rsave[24:32, :] = rb[L:, :]
        rsave[32:64, :] = rb[M:L, :]
        return rb[0:M, :]

    def layer(l, _):
        kvacc[...] = jnp.zeros(kvacc.shape, F32)
        with jax.named_scope("a1"):
            lax.fori_loop(0, S // TN, a1, 0)
        row = lax.broadcasted_iota(jnp.int32, (GR + 16, 2 * GR), 0)
        col = lax.broadcasted_iota(jnp.int32, (GR + 16, 2 * GR), 1)
        same = (row & 7) == (col & 7)
        for g in range(GA):
            kvs[g] = _pack(jnp.where(same, kvacc[g], 0.0).astype(BF16))
        with jax.named_scope("a2"):
            lax.fori_loop(0, S // TN, a2, 0)

        @pl.when(l == 0)
        def _():
            for c in copies:
                c.wait()

            def tr(p, _):
                rows = pl.ds(pl.multiple_of(p * PW, PW), PW)
                for i in range(3):
                    wb[:, pl.ds(pl.multiple_of((3 * p + i) * PW, PW), PW)] = _pack(
                        wraw[i, rows, :].T)
                wob[pl.ds(pl.multiple_of(p * DH, DH), DH), :] = _pack(wraw[3, rows, :])
                return 0
            with jax.named_scope("tr"):
                lax.fori_loop(0, NP, tr, 0)

        rsave[...] = jnp.zeros(rsave.shape, F32)
        with jax.named_scope("b"):
            lax.fori_loop(0, S // (2 * SEG), b_pair, mem0_ref[...].astype(F32))
        b_finish(S - 2 * SEG)
        return 0

    lax.fori_loop(0, 2, layer, 0)


@functools.partial(jax.jit, static_argnames=("B_seg_len",))
def pallas_interleave_layers__linear_kernel_hedgehog__memory_aug_recurrent_mem_tr__prompt_kernel(
    A_x, A_wqkv, A_w_phi, A_wo, B_x, B_mem0, B_Wq, B_Wk, B_Wv, B_Wo, B_seg_len,
):
    del B_x
    assert B_seg_len == SEG
    x = A_x.reshape(S, D)
    cphi = A_w_phi.reshape(D, FA).T
    mem0 = B_mem0.reshape(M, D)
    wq, wk, wv = (w.transpose(1, 2, 0).reshape(HD, D) for w in (B_Wq, B_Wk, B_Wv))
    wo = B_Wo.reshape(HD, D)
    vmem = pl.BlockSpec(memory_space=pltpu.VMEM)
    hbm = pl.BlockSpec(memory_space=pl.ANY)
    out = pl.pallas_call(
        _kernel,
        out_shape=jax.ShapeDtypeStruct((S, D), A_x.dtype),
        in_specs=[vmem] * 5 + [hbm] * 4,
        out_specs=vmem,
        scratch_shapes=[
            pltpu.VMEM((S, D), F32),
            pltpu.VMEM((S // 2, D), U32),
            pltpu.VMEM((S, D), F32),
            pltpu.VMEM((3 * GA, GR // 2, D), U32),
            pltpu.VMEM((D // 2, D), U32),
            pltpu.VMEM((GA, GR, S), U32),
            pltpu.VMEM((GA, GR + 16, 2 * GR), F32),
            pltpu.VMEM((GA, GR // 2 + 8, 2 * GR), U32),
            pltpu.VMEM((4, HD, D), BF16),
            pltpu.VMEM((D // 2, 3 * HD), U32),
            pltpu.VMEM((HD // 2, D), U32),
            pltpu.VMEM((8, 3 * HD), F32),
            pltpu.VMEM((8, HD), F32),
            pltpu.VMEM((2 * SEG, D), F32),
            pltpu.SemaphoreType.DMA((4,)),
        ],
        compiler_params=pltpu.CompilerParams(vmem_limit_bytes=120 * 1024 * 1024),
    )(x, A_wqkv, cphi, A_wo, mem0, wq, wk, wv, wo)
    return out.reshape(1, S, D)
```

```python
import functools

import jax
import jax.numpy as jnp
from jax import lax
import jax.experimental.pallas as pl
import jax.experimental.pallas.tpu as pltpu

F32 = jnp.float32
BF16 = jnp.bfloat16
U32 = jnp.uint32

S = 2048
D = 640
HA = 32
FA = 20
GA = 4
GR = 8 * FA
TN = 256
HB = 32
DH = 192
HD = HB * DH
M = 8
SEG = 32
L = M + SEG
PW = 2 * DH
NP = HB // 2

NT = (((1,), (1,)), ((), ()))


def _dot(a, b):
    return jnp.dot(a, b, preferred_element_type=F32)


def _dot_nt(a, b):
    return lax.dot_general(a, b, NT, preferred_element_type=F32)


def _pack(a):
    return pltpu.bitcast(a, U32)


def _unpack(a):
    return pltpu.bitcast(a, BF16)


def _recip(x):
    r = pl.reciprocal(x, approx=True)
    return r * (2.0 - x * r)


def _layernorm(x):
    m = jnp.mean(x, axis=-1, keepdims=True)
    c = x - m
    v = jnp.mean(c * c, axis=-1, keepdims=True)
    return c * lax.rsqrt(v + 1e-5)


def _feature_map(p):
    t = p.shape[-1]
    p3 = p.reshape(FA, 8, t)
    mx = jnp.max(p3, axis=0, keepdims=True)
    mn = jnp.min(p3, axis=0, keepdims=True)
    ep = jnp.exp(p3 - mx)
    en = jnp.exp(mn - p3)
    rp = _recip(jnp.sum(ep, axis=0, keepdims=True))
    rn = _recip(jnp.sum(en, axis=0, keepdims=True))
    out = jnp.concatenate([(ep * rp).reshape(GR, t), (en * rn).reshape(GR, t)], axis=0)
    return out.astype(BF16)


def _split_pair(a):
    lane = lax.broadcasted_iota(jnp.int32, (L, 128), 1)
    mid = a[:, 128:256]
    outer = jnp.concatenate([a[:, 0:128], a[:, 256:384]], axis=0)
    mid = jnp.concatenate(
        [jnp.where(lane < 64, mid, 0.0), jnp.where(lane < 64, 0.0, mid)], axis=0)
    return outer.astype(BF16), mid.astype(BF16)


def _scores(y):
    q_outer = jnp.concatenate([y[:, 0:128], y[:, 256:384]], axis=0).astype(BF16)
    q_mid = y[:, 128:256].astype(BF16)
    k_outer, k_mid = _split_pair(y[:, PW:2 * PW])
    s_outer = _dot_nt(q_outer, k_outer)
    s_mid = _dot_nt(q_mid, k_mid)
    row = lax.broadcasted_iota(jnp.int32, (L, 2 * L), 0)
    col = lax.broadcasted_iota(jnp.int32, (L, 2 * L), 1)
    first = col < L
    key = jnp.where(first, col, col - L)
    valid = jnp.logical_or(row < M, row >= key)
    s = (jnp.where(first, s_outer[0:L, :], s_outer[L:, :]) + s_mid) * (DH ** -0.5)
    s = jnp.where(valid, s, -1e9)
    m0 = jnp.max(jnp.where(first, s, -jnp.inf), axis=-1, keepdims=True)
    m1 = jnp.max(jnp.where(first, -jnp.inf, s), axis=-1, keepdims=True)
    e = jnp.exp(s - jnp.where(first, m0, m1))
    s0 = jnp.sum(jnp.where(first, e, 0.0), axis=-1, keepdims=True)
    s1 = jnp.sum(jnp.where(first, 0.0, e), axis=-1, keepdims=True)
    p = e * _recip(jnp.where(first, s0, s1))
    ps = jnp.concatenate([jnp.where(first, p, 0.0), jnp.where(first, 0.0, p)], axis=0)
    return p.astype(BF16), ps.astype(BF16)


def _pv(p, ps, v_outer, v_mid):
    o_outer = _dot(ps, v_outer)
    o_mid = _dot(p, v_mid)
    return jnp.concatenate([o_outer[0:L, :], o_mid, o_outer[L:, :]], axis=1)


def _segment(h, wb, wob, fix_y, fix_o):
    ps, vs, os_ = {}, {}, {}
    ys = {}

    def proj(p):
        ys[p] = fix_y(p, _dot(h, _unpack(wb[:, p * 3 * PW:(p + 1) * 3 * PW])))

    def score(p):
        y = ys.pop(p)
        vs[p] = _split_pair(y[:, 2 * PW:3 * PW])
        ps[p] = _scores(y)

    def pv(p):
        os_[p] = fix_o(p, _pv(*ps.pop(p), *vs.pop(p))).astype(BF16)

    def oproj(lo, hi):
        o = jnp.concatenate([os_.pop(p) for p in range(lo, hi)], axis=1)
        return _dot(o, _unpack(wob[lo * PW // 2:hi * PW // 2, :]))

    for p in range(NP):
        proj(p)
        if p >= 1:
            score(p - 1)
        if p >= 3:
            pv(p - 3)
    r = oproj(0, 3)
    score(NP - 1)
    pv(NP - 3)
    r = oproj(3, 6) + r
    pv(NP - 2)
    r = oproj(6, 10) + r
    pv(NP - 1)
    r = oproj(10, 14) + r
    r = oproj(14, 16) + r
    return r


def _kernel(x_hbm, wqkv_hbm, wphi_hbm, woa_hbm, mem0_hbm,
            wq_hbm, wk_hbm, wv_hbm, wo_hbm,
            out_hbm,
            xio, wqkv, wphi, woa, mem0, xres, xa, xb, wat, wop, phq, phk, vts, kvs, osc,
            wraw, wb, wob, ysave, osave, rsave, sem_in, sem_x, sem_w, sem_out):
    nt = S // TN
    half = TN // 2

    def rows(j, n):
        return pl.ds(j * n if isinstance(j, int) else pl.multiple_of(j * n, n), n)

    def x_copy(j):
        return pltpu.make_async_copy(x_hbm.at[rows(j, TN), :], xio.at[rows(j, TN), :],
                                     sem_x.at[j])

    def w_copies(p):
        return [pltpu.make_async_copy(src.at[rows(p, PW), :], wraw.at[i, rows(p, PW), :],
                                      sem_w.at[4 * p + i])
                for i, src in enumerate((wq_hbm, wk_hbm, wv_hbm, wo_hbm))]

    def out_copy(i):
        return pltpu.make_async_copy(xio.at[rows(i, 2 * SEG), :],
                                     out_hbm.at[rows(i, 2 * SEG), :], sem_out.at[0])

    small = [pltpu.make_async_copy(src, dst, sem_in.at[i]) for i, (src, dst) in enumerate(
        ((wphi_hbm, wphi), (wqkv_hbm, wqkv), (woa_hbm, woa), (mem0_hbm, mem0)))]
    small[0].start()
    small[1].start()
    x_copy(0).start()
    small[2].start()
    small[3].start()

    small[0].wait()
    cphi = jnp.zeros((FA, D), F32)
    hh = lax.broadcasted_iota(jnp.int32, (HA, D), 0) * FA
    jj = lax.broadcasted_iota(jnp.int32, (HA, D), 1)
    for d in range(FA):
        cphi = _dot(wphi[d], jnp.where(jj == hh + d, 1.0, 0.0).astype(BF16)) + cphi
    cb = jnp.concatenate(
        [jnp.broadcast_to(cphi[f:f + 1, :], (8, D)) for f in range(FA)], axis=0)
    bds, perms = [], []
    for g in range(GA):
        row = lax.broadcasted_iota(jnp.int32, (GR, 256), 0)
        col = lax.broadcasted_iota(jnp.int32, (GR, 256), 1) + 128 * g
        lo = (8 * g + (row & 7)) * FA
        bds.append(jnp.where(jnp.logical_and(col >= lo, col < lo + FA),
                             cb[:, 128 * g:128 * g + 256], 0.0).astype(BF16))
        perms.append(jnp.where(col == lo + (row >> 3), 1.0, 0.0).astype(BF16))
    vts[:, GR // 2:, :] = _pack(jnp.ones((GA, 16, S), BF16))
    small[1].wait()
    x_copy(0).wait()
    small[2].wait()
    small[3].wait()
    for j in range(1, nt):
        x_copy(j).start()
    for p in range(2):
        for c in w_copies(p):
            c.start()
    for g in range(GA):
        for i, lhs in enumerate((bds[g], bds[g], perms[g])):
            w = wqkv[:, i * D + 128 * g:i * D + 128 * g + 256]
            wat[i * GA + g] = _pack(_dot_nt(lhs, w).astype(BF16))
        wop[g * GR // 2:(g + 1) * GR // 2, :] = _pack(
            _dot(perms[g], woa[128 * g:128 * g + 256, :]).astype(BF16))
    xa[rows(0, half), :] = _pack(_layernorm(xio[rows(0, TN), :].astype(F32)).astype(BF16))

    def relayout_b_weights(p):
        for i in range(3):
            wb[:, rows(3 * p + i, PW)] = _pack(wraw[i, rows(p, PW), :].T)
        wob[rows(p, DH), :] = _pack(wraw[3, rows(p, PW), :])

    def block_a(first):
        def a1(j, _):
            if first:
                @pl.when(j + 1 < nt)
                def _():
                    x_copy(j + 1).wait()
                    for p in range(2):
                        for c in w_copies(2 * j + 2 + p):
                            c.start()
                for c in w_copies(j):
                    c.wait()
            xn = _unpack(xa[rows(j, half), :])
            for g in range(GA):
                phk[g, :, rows(j, TN)] = _pack(_feature_map(_dot_nt(_unpack(wat[GA + g]), xn)))
            for g in range(GA):
                phq[g, :, rows(j, TN)] = _pack(_feature_map(_dot_nt(_unpack(wat[g]), xn)))
            for g in range(GA):
                vts[g, 0:GR // 2, rows(j, TN)] = _pack(
                    _dot_nt(_unpack(wat[2 * GA + g]), xn).astype(BF16))
            if first:
                relayout_b_weights(j)
                jn = jnp.minimum(j + 1, nt - 1)
                xa[rows(jn, half), :] = _pack(
                    _layernorm(xio[rows(jn, TN), :].astype(F32)).astype(BF16))
            return 0

        def attend(j):
            os_ = []
            for g in range(GA):
                nd = _dot(_unpack(kvs[g]), _unpack(phq[g, :, rows(j, TN)]))
                rden = 1.0 / (nd[GR:GR + 8, :] + 1e-6)
                o = nd[0:GR, :].reshape(FA, 8, TN) * rden[None]
                os_.append(o.reshape(GR, TN).astype(BF16))
            return _pack(jnp.concatenate(os_, axis=0).T)

        def project(j, o):
            r = rows(j, TN)
            x = xio[r, :].astype(F32) if first else xres[r, :]
            xres[r, :] = _dot(_unpack(o), _unpack(wop[...])) + x

        def a2(j, _):
            if first:
                for c in w_copies(nt + j):
                    c.wait()
            o = osc[...]
            osc[...] = attend(j + 1)
            project(j, o)
            if first:
                relayout_b_weights(nt + j)
            return 0

        with jax.named_scope("a1"):
            lax.fori_loop(0, nt, a1, 0)
        with jax.named_scope("kv"):
            row = lax.broadcasted_iota(jnp.int32, (GR + 16, 2 * GR), 0)
            col = lax.broadcasted_iota(jnp.int32, (GR + 16, 2 * GR), 1)
            same = (row & 7) == (col & 7)
            for g in range(GA):
                kv = _dot_nt(_unpack(vts[g]), _unpack(phk[g]))
                kvs[g] = _pack(jnp.where(same, kv, 0.0).astype(BF16))
            osc[...] = attend(0)
        with jax.named_scope("a2"):
            lax.fori_loop(0, nt - 1, a2, 0)
        if first:
            for c in w_copies(2 * nt - 1):
                c.wait()
        xb[...] = _layernorm(xres[rows(0, 2 * SEG), :])
        rsave[...] = jnp.zeros(rsave.shape, F32)
        project(nt - 1, osc[...])
        if first:
            relayout_b_weights(2 * nt - 1)

    nb = S // (2 * SEG)

    def b_finish(i):
        r = rows(i, 2 * SEG)
        x = xres[r, :] + rsave[...]
        xres[r, :] = x
        xa[rows(i, SEG), :] = _pack(_layernorm(x).astype(BF16))
        xio[r, :] = x.astype(BF16)

    def layer(l, _):
        def b_pair(i, mem):
            @pl.when(jnp.logical_and(l == 1, i >= 2))
            def _():
                out_copy(i - 2).start()

            ha = jnp.concatenate([mem, xb[0:40, :]], axis=0).astype(BF16)
            xb_b = xb[40:64, :]
            b_finish(jnp.maximum(i - 1, 0))
            xb[...] = _layernorm(xres[rows(jnp.minimum(i + 1, nb - 1), 2 * SEG), :])

            def fix_ya(p, y):
                ysave[:, p * 3 * PW:(p + 1) * 3 * PW] = y[L:L + 8, :]
                return y[0:L, :]

            def fix_oa(p, o):
                osave[:, p * PW:(p + 1) * PW] = o[32:L, :]
                return o[0:32, :]

            ra = _segment(ha, wb, wob, fix_ya, fix_oa)
            rsave[0:24, :] = ra[M:, :]

            def fix_yb(p, y):
                return jnp.concatenate(
                    [y[0:M, :], ysave[:, p * 3 * PW:(p + 1) * 3 * PW], y[M:, :]], axis=0)

            def fix_ob(p, o):
                return jnp.concatenate([o, osave[:, p * PW:(p + 1) * PW]], axis=0)

            hb = jnp.concatenate([ra[0:M, :], xb_b], axis=0).astype(BF16)
            rb = _segment(hb, wb, wob, fix_yb, fix_ob)
            rsave[24:32, :] = rb[L:, :]
            rsave[32:64, :] = rb[M:L, :]
            return rb[0:M, :]

        with jax.named_scope("b"):
            lax.fori_loop(0, nb, b_pair, mem0[...].astype(F32))
        b_finish(nb - 1)

        @pl.when(l == 0)
        def _():
            block_a(False)
        return 0

    block_a(True)
    lax.fori_loop(0, 2, layer, 0)
    out_copy(nb - 2).start()
    out_copy(nb - 1).start()
    pltpu.make_async_copy(xio, out_hbm, sem_out.at[0]).wait()


@functools.partial(jax.jit, static_argnames=("B_seg_len",))
def pallas_interleave_layers__linear_kernel_hedgehog__memory_aug_recurrent_mem_tr__prompt_kernel(
    A_x, A_wqkv, A_w_phi, A_wo, B_x, B_mem0, B_Wq, B_Wk, B_Wv, B_Wo, B_seg_len,
):
    del B_x
    assert B_seg_len == SEG
    x = A_x.reshape(S, D)
    wphi = A_w_phi.transpose(1, 2, 0)
    mem0 = B_mem0.reshape(M, D)
    wq, wk, wv = (w.transpose(1, 2, 0).reshape(HD, D) for w in (B_Wq, B_Wk, B_Wv))
    wo = B_Wo.reshape(HD, D)
    hbm = pl.BlockSpec(memory_space=pl.ANY)
    out = pl.pallas_call(
        _kernel,
        out_shape=jax.ShapeDtypeStruct((S, D), A_x.dtype),
        in_specs=[hbm] * 9,
        out_specs=hbm,
        scratch_shapes=[
            pltpu.VMEM((S, D), BF16),
            pltpu.VMEM((D, 3 * D), BF16),
            pltpu.VMEM((FA, FA, HA), BF16),
            pltpu.VMEM((D, D), BF16),
            pltpu.VMEM((M, D), BF16),
            pltpu.VMEM((S, D), F32),
            pltpu.VMEM((S // 2, D), U32),
            pltpu.VMEM((2 * SEG, D), F32),
            pltpu.VMEM((3 * GA, GR // 2, D), U32),
            pltpu.VMEM((D // 2, D), U32),
            pltpu.VMEM((GA, GR, S), U32),
            pltpu.VMEM((GA, GR, S), U32),
            pltpu.VMEM((GA, GR // 2 + 8, S), U32),
            pltpu.VMEM((GA, GR // 2 + 8, 2 * GR), U32),
            pltpu.VMEM((TN // 2, D), U32),
            pltpu.VMEM((4, HD, D), BF16),
            pltpu.VMEM((D // 2, 3 * HD), U32),
            pltpu.VMEM((HD // 2, D), U32),
            pltpu.VMEM((8, 3 * HD), F32),
            pltpu.VMEM((8, HD), F32),
            pltpu.VMEM((2 * SEG, D), F32),
            pltpu.SemaphoreType.DMA((4,)),
            pltpu.SemaphoreType.DMA((S // TN,)),
            pltpu.SemaphoreType.DMA((4 * NP,)),
            pltpu.SemaphoreType.DMA((1,)),
        ],
        compiler_params=pltpu.CompilerParams(vmem_limit_bytes=120 * 1024 * 1024),
    )(x, A_wqkv, wphi, A_wo, mem0, wq, wk, wv, wo)
    return out.reshape(1, S, D)
```

```python
import functools

import jax
import jax.numpy as jnp
from jax import lax
import jax.experimental.pallas as pl
import jax.experimental.pallas.tpu as pltpu

F32 = jnp.float32
BF16 = jnp.bfloat16
U32 = jnp.uint32

S = 2048
D = 640
HA = 32
FA = 20
GA = 4
GR = 8 * FA
TN = 256
HB = 32
DH = 192
HD = HB * DH
M = 8
SEG = 32
L = M + SEG
PW = 2 * DH
NP = HB // 2

NT = (((1,), (1,)), ((), ()))
LOG2E = 1.4426950408889634


def _dot(a, b):
    return jnp.dot(a, b, preferred_element_type=F32)


def _dot_nt(a, b):
    return lax.dot_general(a, b, NT, preferred_element_type=F32)


def _pack(a):
    return pltpu.bitcast(a, U32)


def _unpack(a):
    return pltpu.bitcast(a, BF16)


def _interleave(a, b):
    return pltpu.pack_elementwise([a, b], packed_dtype=BF16).astype(U32)


def _recip(x):
    r = pl.reciprocal(x, approx=True)
    return r * (2.0 - x * r)


def _layernorm(x):
    m = jnp.mean(x, axis=-1, keepdims=True)
    c = x - m
    v = jnp.mean(c * c, axis=-1, keepdims=True)
    return c * lax.rsqrt(v + 1e-5)


def _feature_map(p):
    t = p.shape[-1]
    p3 = p.reshape(FA, 8, t)
    ep = jnp.exp2(p3 - jnp.max(p3, axis=0, keepdims=True))
    ep = ep * _recip(jnp.sum(ep, axis=0, keepdims=True))
    en = jnp.exp2(jnp.min(p3, axis=0, keepdims=True) - p3)
    en = en * _recip(jnp.sum(en, axis=0, keepdims=True))
    return _interleave(ep.reshape(GR, t), en.reshape(GR, t))


def _split_pair(a):
    lane = lax.broadcasted_iota(jnp.int32, (L, 128), 1)
    mid = a[:, 128:256]
    outer = jnp.concatenate([a[:, 0:128], a[:, 256:384]], axis=0)
    mid = jnp.concatenate(
        [jnp.where(lane < 64, mid, 0.0), jnp.where(lane < 64, 0.0, mid)], axis=0)
    return outer.astype(BF16), mid.astype(BF16)


def _scores(y):
    q_outer = jnp.concatenate([y[:, 0:128], y[:, 256:384]], axis=0).astype(BF16)
    q_mid = y[:, 128:256].astype(BF16)
    k_outer, k_mid = _split_pair(y[:, PW:2 * PW])
    s_outer = _dot_nt(q_outer, k_outer)
    s_mid = _dot_nt(q_mid, k_mid)
    row = lax.broadcasted_iota(jnp.int32, (L, 2 * L), 0)
    col = lax.broadcasted_iota(jnp.int32, (L, 2 * L), 1)
    first = col < L
    key = jnp.where(first, col, col - L)
    valid = jnp.logical_or(row < M, row >= key)
    s = (jnp.where(first, s_outer[0:L, :], s_outer[L:, :]) + s_mid) * (DH ** -0.5)
    s = jnp.where(valid, s, -1e9)
    m0 = jnp.max(jnp.where(first, s, -jnp.inf), axis=-1, keepdims=True)
    m1 = jnp.max(jnp.where(first, -jnp.inf, s), axis=-1, keepdims=True)
    e = jnp.exp(s - jnp.where(first, m0, m1))
    s0 = jnp.sum(jnp.where(first, e, 0.0), axis=-1, keepdims=True)
    s1 = jnp.sum(jnp.where(first, 0.0, e), axis=-1, keepdims=True)
    p = e * _recip(jnp.where(first, s0, s1))
    ps = jnp.concatenate([jnp.where(first, p, 0.0), jnp.where(first, 0.0, p)], axis=0)
    return p.astype(BF16), ps.astype(BF16)


def _pv(p, ps, v_outer, v_mid):
    o_outer = _dot(ps, v_outer)
    o_mid = _dot(p, v_mid)
    return jnp.concatenate([o_outer[0:L, :], o_mid, o_outer[L:, :]], axis=1)


def _segment(h, wb, wob, fix_y, fix_o):
    ps, vs, os_ = {}, {}, {}
    ys = {}

    def proj(p):
        ys[p] = fix_y(p, _dot(h, _unpack(wb[:, p * 3 * PW:(p + 1) * 3 * PW])))

    def score(p):
        y = ys.pop(p)
        vs[p] = _split_pair(y[:, 2 * PW:3 * PW])
        ps[p] = _scores(y)

    def pv(p):
        os_[p] = fix_o(p, _pv(*ps.pop(p), *vs.pop(p))).astype(BF16)

    def oproj(lo, hi):
        o = jnp.concatenate([os_.pop(p) for p in range(lo, hi)], axis=1)
        return _dot(o, _unpack(wob[lo * PW // 2:hi * PW // 2, :]))

    for p in range(NP):
        proj(p)
        if p >= 1:
            score(p - 1)
        if p >= 3:
            pv(p - 3)
    r = oproj(0, 3)
    score(NP - 1)
    pv(NP - 3)
    r = oproj(3, 6) + r
    pv(NP - 2)
    r = oproj(6, 10) + r
    pv(NP - 1)
    r = oproj(10, 14) + r
    r = oproj(14, 16) + r
    return r


def _kernel(x_hbm, wqkv_hbm, wphi_hbm, woa_hbm, mem0_hbm,
            wq_hbm, wk_hbm, wv_hbm, wo_hbm,
            out_hbm,
            xio, wqkv, wphi, woa, mem0, xres, xa, xb, wat, wop, phq, phk, vts, kvs, osc,
            wraw, wb, wob, ysave, osave, rsave, sem_in, sem_x, sem_w, sem_out):
    nt = S // TN
    half = TN // 2

    def rows(j, n):
        return pl.ds(j * n if isinstance(j, int) else pl.multiple_of(j * n, n), n)

    def x_copy(j):
        return pltpu.make_async_copy(x_hbm.at[rows(j, TN), :], xio.at[rows(j, TN), :],
                                     sem_x.at[j])

    def w_copies(p):
        return [pltpu.make_async_copy(src.at[rows(p, PW), :], wraw.at[i, rows(p, PW), :],
                                      sem_w.at[4 * p + i])
                for i, src in enumerate((wq_hbm, wk_hbm, wv_hbm, wo_hbm))]

    def out_copy(i):
        return pltpu.make_async_copy(xio.at[rows(i, 2 * SEG), :],
                                     out_hbm.at[rows(i, 2 * SEG), :], sem_out.at[0])

    small = [pltpu.make_async_copy(src, dst, sem_in.at[i]) for i, (src, dst) in enumerate(
        ((wphi_hbm, wphi), (wqkv_hbm, wqkv), (woa_hbm, woa), (mem0_hbm, mem0)))]
    small[0].start()
    small[1].start()
    x_copy(0).start()
    small[2].start()
    small[3].start()

    small[0].wait()
    cphi = jnp.zeros((FA, D), F32)
    hh = lax.broadcasted_iota(jnp.int32, (HA, D), 0) * FA
    jj = lax.broadcasted_iota(jnp.int32, (HA, D), 1)
    for d in range(FA):
        cphi = _dot(wphi[d], jnp.where(jj == hh + d, 1.0, 0.0).astype(BF16)) + cphi
    cb = jnp.concatenate(
        [jnp.broadcast_to(cphi[f:f + 1, :], (8, D)) for f in range(FA)], axis=0)
    bds, perms, vperms = [], [], []
    for g in range(GA):
        row = lax.broadcasted_iota(jnp.int32, (GR, 256), 0)
        col = lax.broadcasted_iota(jnp.int32, (GR, 256), 1) + 128 * g
        lo = (8 * g + (row & 7)) * FA
        bds.append(jnp.where(jnp.logical_and(col >= lo, col < lo + FA),
                             cb[:, 128 * g:128 * g + 256], 0.0).astype(BF16))
        perms.append(jnp.where(col == lo + (row >> 3), 1.0, 0.0).astype(BF16))
        vrow = jnp.where(row < GR // 2, 2 * row, 2 * row - (GR - 1))
        vperms.append(jnp.where(col == (8 * g + (vrow & 7)) * FA + (vrow >> 3),
                                1.0, 0.0).astype(BF16))
    vts[:, GR // 2:, :] = _pack(jnp.ones((GA, 16, S), BF16))
    small[1].wait()
    x_copy(0).wait()
    small[2].wait()
    small[3].wait()
    for j in range(1, nt):
        x_copy(j).start()
    for p in range(2):
        for c in w_copies(p):
            c.start()
    for g in range(GA):
        for i, lhs in enumerate((bds[g], bds[g], vperms[g])):
            w = wqkv[:, i * D + 128 * g:i * D + 128 * g + 256]
            w = _dot_nt(lhs, w)
            wat[i * GA + g] = _pack((w * LOG2E if i < 2 else w).astype(BF16))
        wop[g * GR // 2:(g + 1) * GR // 2, :] = _pack(
            _dot(perms[g], woa[128 * g:128 * g + 256, :]).astype(BF16))
    xa[rows(0, half), :] = _pack(_layernorm(xio[rows(0, TN), :].astype(F32)).astype(BF16))

    def relayout_b_weights(p):
        for i in range(3):
            wb[:, rows(3 * p + i, PW)] = _pack(wraw[i, rows(p, PW), :].T)
        wob[rows(p, DH), :] = _pack(wraw[3, rows(p, PW), :])

    def block_a(first):
        def a1(j, _):
            if first:
                @pl.when(j + 1 < nt)
                def _():
                    x_copy(j + 1).wait()
                    for p in range(2):
                        for c in w_copies(2 * j + 2 + p):
                            c.start()
                for c in w_copies(j):
                    c.wait()
            for u in range(TN // 128):
                t = rows(j * (TN // 128) + u, 128)
                xn = _unpack(xa[rows(j * (TN // 128) + u, 64), :])
                for g in range(GA):
                    phk[g, :, t] = _feature_map(_dot_nt(_unpack(wat[GA + g]), xn))
                    phq[g, :, t] = _feature_map(_dot_nt(_unpack(wat[g]), xn))
                    vt = _dot_nt(_unpack(wat[2 * GA + g]), xn)
                    vts[g, 0:GR // 2, t] = _interleave(vt[0:GR // 2, :], vt[GR // 2:, :])
            if first:
                relayout_b_weights(j)
                jn = jnp.minimum(j + 1, nt - 1)
                xa[rows(jn, half), :] = _pack(
                    _layernorm(xio[rows(jn, TN), :].astype(F32)).astype(BF16))
            return 0

        def attend(j):
            os_ = []
            for g in range(GA):
                nd = _dot(_unpack(kvs[g]), _unpack(phq[g, :, rows(j, TN)]))
                rden = 1.0 / (nd[GR:GR + 8, :] + 1e-6)
                o = nd[0:GR, :].reshape(FA, 8, TN) * rden[None]
                os_.append(o.reshape(GR, TN))
            return _pack(jnp.concatenate(os_, axis=0).astype(BF16).T)

        def project(j, o):
            r = rows(j, TN)
            x = xio[r, :].astype(F32) if first else xres[r, :]
            xres[r, :] = _dot(_unpack(o), _unpack(wop[...])) + x

        def a2(j, _):
            if first:
                for c in w_copies(nt + j):
                    c.wait()
            o = osc[...]
            osc[...] = attend(j + 1)
            project(j, o)
            if first:
                relayout_b_weights(nt + j)
            return 0

        with jax.named_scope("a1"):
            lax.fori_loop(0, nt, a1, 0)
        with jax.named_scope("kv"):
            row = lax.broadcasted_iota(jnp.int32, (GR + 16, 2 * GR), 0)
            col = lax.broadcasted_iota(jnp.int32, (GR + 16, 2 * GR), 1)
            same = (row & 7) == ((col >> 1) & 7)
            for g in range(GA):
                kv = _dot_nt(_unpack(vts[g]), _unpack(phk[g]))
                kvs[g] = _pack(jnp.where(same, kv, 0.0).astype(BF16))
            osc[...] = attend(0)
        with jax.named_scope("a2"):
            lax.fori_loop(0, nt - 1, a2, 0)
        if first:
            for c in w_copies(2 * nt - 1):
                c.wait()
        xb[...] = _layernorm(xres[rows(0, 2 * SEG), :])
        rsave[...] = jnp.zeros(rsave.shape, F32)
        project(nt - 1, osc[...])
        if first:
            relayout_b_weights(2 * nt - 1)

    nb = S // (2 * SEG)

    def b_finish(i):
        r = rows(i, 2 * SEG)
        x = xres[r, :] + rsave[...]
        xres[r, :] = x
        xa[rows(i, SEG), :] = _pack(_layernorm(x).astype(BF16))
        xio[r, :] = x.astype(BF16)

    def layer(l, _):
        def b_pair(i, mem):
            @pl.when(jnp.logical_and(l == 1, i >= 2))
            def _():
                out_copy(i - 2).start()

            ha = jnp.concatenate([mem, xb[0:40, :]], axis=0).astype(BF16)
            xb_b = xb[40:64, :]
            b_finish(jnp.maximum(i - 1, 0))
            xb[...] = _layernorm(xres[rows(jnp.minimum(i + 1, nb - 1), 2 * SEG), :])

            def fix_ya(p, y):
                ysave[:, p * 3 * PW:(p + 1) * 3 * PW] = y[L:L + 8, :]
                return y[0:L, :]

            def fix_oa(p, o):
                osave[:, p * PW:(p + 1) * PW] = o[32:L, :]
                return o[0:32, :]

            ra = _segment(ha, wb, wob, fix_ya, fix_oa)
            rsave[0:24, :] = ra[M:, :]

            def fix_yb(p, y):
                return jnp.concatenate(
                    [y[0:M, :], ysave[:, p * 3 * PW:(p + 1) * 3 * PW], y[M:, :]], axis=0)

            def fix_ob(p, o):
                return jnp.concatenate([o, osave[:, p * PW:(p + 1) * PW]], axis=0)

            hb = jnp.concatenate([ra[0:M, :], xb_b], axis=0).astype(BF16)
            rb = _segment(hb, wb, wob, fix_yb, fix_ob)
            rsave[24:32, :] = rb[L:, :]
            rsave[32:64, :] = rb[M:L, :]
            return rb[0:M, :]

        with jax.named_scope("b"):
            lax.fori_loop(0, nb, b_pair, mem0[...].astype(F32))
        b_finish(nb - 1)

        @pl.when(l == 0)
        def _():
            block_a(False)
        return 0

    block_a(True)
    lax.fori_loop(0, 2, layer, 0)
    out_copy(nb - 2).start()
    out_copy(nb - 1).start()
    pltpu.make_async_copy(xio, out_hbm, sem_out.at[0]).wait()


@functools.partial(jax.jit, static_argnames=("B_seg_len",))
def pallas_interleave_layers__linear_kernel_hedgehog__memory_aug_recurrent_mem_tr__prompt_kernel(
    A_x, A_wqkv, A_w_phi, A_wo, B_x, B_mem0, B_Wq, B_Wk, B_Wv, B_Wo, B_seg_len,
):
    del B_x
    assert B_seg_len == SEG
    x = A_x.reshape(S, D)
    wphi = A_w_phi.transpose(1, 2, 0)
    mem0 = B_mem0.reshape(M, D)
    wq, wk, wv = (w.transpose(1, 2, 0).reshape(HD, D) for w in (B_Wq, B_Wk, B_Wv))
    wo = B_Wo.reshape(HD, D)
    hbm = pl.BlockSpec(memory_space=pl.ANY)
    out = pl.pallas_call(
        _kernel,
        out_shape=jax.ShapeDtypeStruct((S, D), A_x.dtype),
        in_specs=[hbm] * 9,
        out_specs=hbm,
        scratch_shapes=[
            pltpu.VMEM((S, D), BF16),
            pltpu.VMEM((D, 3 * D), BF16),
            pltpu.VMEM((FA, FA, HA), BF16),
            pltpu.VMEM((D, D), BF16),
            pltpu.VMEM((M, D), BF16),
            pltpu.VMEM((S, D), F32),
            pltpu.VMEM((S // 2, D), U32),
            pltpu.VMEM((2 * SEG, D), F32),
            pltpu.VMEM((3 * GA, GR // 2, D), U32),
            pltpu.VMEM((D // 2, D), U32),
            pltpu.VMEM((GA, GR, S), U32),
            pltpu.VMEM((GA, GR, S), U32),
            pltpu.VMEM((GA, GR // 2 + 8, S), U32),
            pltpu.VMEM((GA, GR // 2 + 8, 2 * GR), U32),
            pltpu.VMEM((TN // 2, D), U32),
            pltpu.VMEM((4, HD, D), BF16),
            pltpu.VMEM((D // 2, 3 * HD), U32),
            pltpu.VMEM((HD // 2, D), U32),
            pltpu.VMEM((8, 3 * HD), F32),
            pltpu.VMEM((8, HD), F32),
            pltpu.VMEM((2 * SEG, D), F32),
            pltpu.SemaphoreType.DMA((4,)),
            pltpu.SemaphoreType.DMA((S // TN,)),
            pltpu.SemaphoreType.DMA((4 * NP,)),
            pltpu.SemaphoreType.DMA((1,)),
        ],
        compiler_params=pltpu.CompilerParams(vmem_limit_bytes=120 * 1024 * 1024,
                                             disable_bounds_checks=True),
    )(x, A_wqkv, wphi, A_wo, mem0, wq, wk, wv, wo)
    return out.reshape(1, S, D)
```

```python
import functools

import jax
import jax.numpy as jnp
from jax import lax
import jax.experimental.pallas as pl
import jax.experimental.pallas.tpu as pltpu

F32 = jnp.float32
BF16 = jnp.bfloat16
U32 = jnp.uint32

S = 2048
D = 640
HA = 32
FA = 20
GA = 4
GR = 8 * FA
VR = 24
PA = HA // 2
TN = 256
HB = 32
DH = 192
HD = HB * DH
M = 8
SEG = 32
L = M + SEG
PW = 2 * DH
NP = HB // 2

NT = (((1,), (1,)), ((), ()))
LOG2E = 1.4426950408889634


def _dot(a, b):
    return jnp.dot(a, b, preferred_element_type=F32)


def _dot_nt(a, b):
    return lax.dot_general(a, b, NT, preferred_element_type=F32)


def _pack(a):
    return pltpu.bitcast(a, U32)


def _unpack(a):
    return pltpu.bitcast(a, BF16)


def _interleave(a, b):
    return pltpu.pack_elementwise([a, b], packed_dtype=BF16).astype(U32)


def _recip(x):
    r = pl.reciprocal(x, approx=True)
    return r * (2.0 - x * r)


def _layernorm(x):
    m = jnp.mean(x, axis=-1, keepdims=True)
    c = x - m
    v = jnp.mean(c * c, axis=-1, keepdims=True)
    return c * lax.rsqrt(v + 1e-5)


def _feature_map(p):
    t = p.shape[-1]
    p3 = p.reshape(FA, 8, t)
    mx = jnp.max(p3, axis=0, keepdims=True)
    mn = jnp.min(p3, axis=0, keepdims=True)
    lp = mx + jnp.log2(jnp.sum(jnp.exp2(p3 - mx), axis=0, keepdims=True))
    ln = mn - jnp.log2(jnp.sum(jnp.exp2(mn - p3), axis=0, keepdims=True))
    ep = jnp.exp2(p3 - lp)
    en = jnp.exp2(ln - p3)
    return _interleave(ep.reshape(GR, t), en.reshape(GR, t))


def _split_pair(a):
    lane = lax.broadcasted_iota(jnp.int32, (L, 128), 1)
    mid = a[:, 128:256]
    outer = jnp.concatenate([a[:, 0:128], a[:, 256:384]], axis=0)
    mid = jnp.concatenate(
        [jnp.where(lane < 64, mid, 0.0), jnp.where(lane < 64, 0.0, mid)], axis=0)
    return outer.astype(BF16), mid.astype(BF16)


def _scores(y):
    q_outer = jnp.concatenate([y[:, 0:128], y[:, 256:384]], axis=0).astype(BF16)
    q_mid = y[:, 128:256].astype(BF16)
    k_outer, k_mid = _split_pair(y[:, PW:2 * PW])
    s_outer = _dot_nt(q_outer, k_outer)
    s_mid = _dot_nt(q_mid, k_mid)
    row = lax.broadcasted_iota(jnp.int32, (L, 2 * L), 0)
    col = lax.broadcasted_iota(jnp.int32, (L, 2 * L), 1)
    first = col < L
    key = jnp.where(first, col, col - L)
    valid = jnp.logical_or(row < M, row >= key)
    s = (jnp.where(first, s_outer[0:L, :], s_outer[L:, :]) + s_mid) * (DH ** -0.5)
    s = jnp.where(valid, s, -1e9)
    m0 = jnp.max(jnp.where(first, s, -jnp.inf), axis=-1, keepdims=True)
    m1 = jnp.max(jnp.where(first, -jnp.inf, s), axis=-1, keepdims=True)
    e = jnp.exp(s - jnp.where(first, m0, m1))
    s0 = jnp.sum(jnp.where(first, e, 0.0), axis=-1, keepdims=True)
    s1 = jnp.sum(jnp.where(first, 0.0, e), axis=-1, keepdims=True)
    p = e * _recip(jnp.where(first, s0, s1))
    ps = jnp.concatenate([jnp.where(first, p, 0.0), jnp.where(first, 0.0, p)], axis=0)
    return p.astype(BF16), ps.astype(BF16)


def _pv(p, ps, v_outer, v_mid):
    o_outer = _dot(ps, v_outer)
    o_mid = _dot(p, v_mid)
    return jnp.concatenate([o_outer[0:L, :], o_mid, o_outer[L:, :]], axis=1)


def _segment(h, wb, wob, fix_y, fix_o):
    ps, vs, os_ = {}, {}, {}
    ys = {}

    def proj(p):
        ys[p] = fix_y(p, _dot(h, _unpack(wb[:, p * 3 * PW:(p + 1) * 3 * PW])))

    def score(p):
        y = ys.pop(p)
        vs[p] = _split_pair(y[:, 2 * PW:3 * PW])
        ps[p] = _scores(y)

    def pv(p):
        os_[p] = fix_o(p, _pv(*ps.pop(p), *vs.pop(p))).astype(BF16)

    def oproj(lo, hi):
        o = jnp.concatenate([os_.pop(p) for p in range(lo, hi)], axis=1)
        return _dot(o, _unpack(wob[lo * PW // 2:hi * PW // 2, :]))

    for p in range(NP):
        proj(p)
        if p >= 1:
            score(p - 1)
        if p >= 3:
            pv(p - 3)
    r = oproj(0, 3)
    score(NP - 1)
    pv(NP - 3)
    r = oproj(3, 6) + r
    pv(NP - 2)
    r = oproj(6, 10) + r
    pv(NP - 1)
    r = oproj(10, 14) + r
    r = oproj(14, 16) + r
    return r


def _kernel(x_hbm, wqkv_hbm, wphi_hbm, woa_hbm, mem0_hbm,
            wq_hbm, wk_hbm, wv_hbm, wo_hbm,
            out_hbm,
            xio, wqkv, wphi, woa, mem0, xres, xa, xb, wat, wop, phq, phk, vts, kvs, osc,
            wraw, wb, wob, ysave, osave, rsave, sem_in, sem_x, sem_w, sem_out):
    nt = S // TN
    half = TN // 2

    def rows(j, n):
        return pl.ds(j * n if isinstance(j, int) else pl.multiple_of(j * n, n), n)

    def x_copy(j):
        return pltpu.make_async_copy(x_hbm.at[rows(j, TN), :], xio.at[rows(j, TN), :],
                                     sem_x.at[j])

    def w_copies(p):
        return [pltpu.make_async_copy(src.at[rows(p, PW), :], wraw.at[i, rows(p, PW), :],
                                      sem_w.at[4 * p + i])
                for i, src in enumerate((wq_hbm, wk_hbm, wv_hbm, wo_hbm))]

    def out_copy(i):
        return pltpu.make_async_copy(xio.at[rows(i, 2 * SEG), :],
                                     out_hbm.at[rows(i, 2 * SEG), :], sem_out.at[0])

    small = [pltpu.make_async_copy(src, dst, sem_in.at[i]) for i, (src, dst) in enumerate(
        ((wphi_hbm, wphi), (wqkv_hbm, wqkv), (woa_hbm, woa), (mem0_hbm, mem0)))]
    small[0].start()
    small[1].start()
    x_copy(0).start()
    small[2].start()
    small[3].start()

    small[0].wait()
    cphi = jnp.zeros((FA, D), F32)
    hh = lax.broadcasted_iota(jnp.int32, (HA, D), 0) * FA
    jj = lax.broadcasted_iota(jnp.int32, (HA, D), 1)
    for d in range(FA):
        cphi = _dot(wphi[d], jnp.where(jj == hh + d, 1.0, 0.0).astype(BF16)) + cphi
    cb = jnp.concatenate(
        [jnp.broadcast_to(cphi[f:f + 1, :], (8, D)) for f in range(FA)], axis=0)
    bds, operms, vperms = [], [], []
    for g in range(GA):
        row = lax.broadcasted_iota(jnp.int32, (GR, 256), 0)
        col = lax.broadcasted_iota(jnp.int32, (GR, 256), 1) + 128 * g
        lo = (8 * g + (row & 7)) * FA
        bds.append(jnp.where(jnp.logical_and(col >= lo, col < lo + FA),
                             cb[:, 128 * g:128 * g + 256], 0.0).astype(BF16))
        pair = lax.broadcasted_iota(jnp.int32, (4, 2 * FA, 256), 0).reshape(GR, 256)
        r = lax.broadcasted_iota(jnp.int32, (4, 2 * FA, 256), 1).reshape(GR, 256)
        base = (4 * g + pair) * 2 * FA
        operms.append(jnp.where(col == base + (r & 1) * FA + (r >> 1), 1.0, 0.0).astype(BF16))
        src = jnp.where(r < 16, r, jnp.where(r < 32, r + 4, jnp.where(r < 36, r - 16, r)))
        vperms.append(jnp.where(col == base + src, 1.0, 0.0).astype(BF16))
    small[1].wait()
    x_copy(0).wait()
    small[2].wait()
    small[3].wait()
    for j in range(1, nt):
        x_copy(j).start()
    for p in range(2):
        for c in w_copies(p):
            c.start()
    for g in range(GA):
        for i, lhs in enumerate((bds[g], bds[g], vperms[g])):
            w = wqkv[:, i * D + 128 * g:i * D + 128 * g + 256]
            w = _dot_nt(lhs, w)
            wat[i * GA + g] = _pack((w * LOG2E if i < 2 else w).astype(BF16))
        wop[g * GR // 2:(g + 1) * GR // 2, :] = _pack(
            _dot(operms[g], woa[128 * g:128 * g + 256, :]).astype(BF16))
    xa[rows(0, half), :] = _pack(_layernorm(xio[rows(0, TN), :].astype(F32)).astype(BF16))

    def relayout_b_weights(p):
        for i in range(3):
            wb[:, rows(3 * p + i, PW)] = _pack(wraw[i, rows(p, PW), :].T)
        wob[rows(p, DH), :] = _pack(wraw[3, rows(p, PW), :])

    def block_a(first):
        def a1(j, _):
            if first:
                @pl.when(j + 1 < nt)
                def _():
                    x_copy(j + 1).wait()
                    for p in range(2):
                        for c in w_copies(2 * j + 2 + p):
                            c.start()
                for c in w_copies(j):
                    c.wait()
            low = lax.broadcasted_iota(jnp.int32, (8, 128), 0) < 4
            for u in range(TN // 128):
                t = j * (TN // 128) + u
                xn = _unpack(xa[rows(t, 64), :])
                for g in range(GA):
                    for ph, w in ((phk, wat[GA + g]), (phq, wat[g])):
                        fm = _feature_map(_dot_nt(_unpack(w), xn))
                        for f in range(FA):
                            ph[t, pl.ds(GR * g + f, 8, stride=FA), :] = fm[8 * f:8 * f + 8, :]
                    vt = _dot_nt(_unpack(wat[2 * GA + g]), xn)
                    for q in range(4):
                        v = vt[40 * q:40 * q + 40, :]
                        va = jnp.concatenate([v[0:16, :], jnp.where(low, v[32:40, :], 1.0)], axis=0)
                        vb = jnp.concatenate([v[16:32, :], jnp.where(low, 1.0, v[32:40, :])], axis=0)
                        vts[4 * g + q, :, rows(t, 128)] = _interleave(va, vb)
            if first:
                relayout_b_weights(j)
                jn = jnp.minimum(j + 1, nt - 1)
                xa[rows(jn, half), :] = _pack(
                    _layernorm(xio[rows(jn, TN), :].astype(F32)).astype(BF16))
            return 0

        def pair_rows(ph, q, t0, n):
            return _unpack(jnp.concatenate(
                [ph[t0 + u, 2 * FA * q:2 * FA * (q + 1), :] for u in range(n)], axis=1))

        def attend(j):
            even = (lax.broadcasted_iota(jnp.int32, (8, TN), 0) & 1) == 0
            os_ = []
            for q in range(PA):
                nd = _dot(_unpack(kvs[q]), pair_rows(phq, q, j * (TN // 128), TN // 128))
                rden = 1.0 / (jnp.where(even, nd[40:48, :], nd[32:40, :]) + 1e-6)
                num = jnp.concatenate(
                    [nd[0:32, :], jnp.where(even, nd[32:40, :], nd[40:48, :])], axis=0)
                os_.append((num.reshape(5, 8, TN) * rden[None]).reshape(40, TN))
            return _pack(jnp.concatenate(os_, axis=0).astype(BF16).T)

        def project(j, o):
            r = rows(j, TN)
            x = xio[r, :].astype(F32) if first else xres[r, :]
            xres[r, :] = _dot(_unpack(o), _unpack(wop[...])) + x

        def a2(j, _):
            if first:
                for c in w_copies(nt + j):
                    c.wait()
            o = osc[...]
            osc[...] = attend(j + 1)
            project(j, o)
            if first:
                relayout_b_weights(nt + j)
            return 0

        with jax.named_scope("a1"):
            lax.fori_loop(0, nt, a1, 0)
        with jax.named_scope("kv"):
            row = lax.broadcasted_iota(jnp.int32, (2 * VR, 4 * FA), 0)
            col = lax.broadcasted_iota(jnp.int32, (2 * VR, 4 * FA), 1)
            same = ((row & 1) == 1) == (col >= 2 * FA)
            for q in range(PA):
                kv = _dot_nt(_unpack(vts[q]), pair_rows(phk, q, 0, S // 128))
                kvs[q] = _pack(jnp.where(same, kv, 0.0).astype(BF16))
            osc[...] = attend(0)
        with jax.named_scope("a2"):
            lax.fori_loop(0, nt - 1, a2, 0)
        if first:
            for c in w_copies(2 * nt - 1):
                c.wait()
        xb[...] = _layernorm(xres[rows(0, 2 * SEG), :])
        rsave[...] = jnp.zeros(rsave.shape, F32)
        project(nt - 1, osc[...])
        if first:
            relayout_b_weights(2 * nt - 1)

    nb = S // (2 * SEG)

    def b_finish(i):
        r = rows(i, 2 * SEG)
        x = xres[r, :] + rsave[...]
        xres[r, :] = x
        xa[rows(i, SEG), :] = _pack(_layernorm(x).astype(BF16))
        xio[r, :] = x.astype(BF16)

    def layer(l, _):
        def b_pair(i, mem):
            @pl.when(jnp.logical_and(l == 1, i >= 2))
            def _():
                out_copy(i - 2).start()

            ha = jnp.concatenate([mem, xb[0:40, :]], axis=0).astype(BF16)
            xb_b = xb[40:64, :]
            b_finish(jnp.maximum(i - 1, 0))
            xb[...] = _layernorm(xres[rows(jnp.minimum(i + 1, nb - 1), 2 * SEG), :])

            def fix_ya(p, y):
                ysave[:, p * 3 * PW:(p + 1) * 3 * PW] = y[L:L + 8, :]
                return y[0:L, :]

            def fix_oa(p, o):
                osave[:, p * PW:(p + 1) * PW] = o[32:L, :]
                return o[0:32, :]

            ra = _segment(ha, wb, wob, fix_ya, fix_oa)
            rsave[0:24, :] = ra[M:, :]

            def fix_yb(p, y):
                return jnp.concatenate(
                    [y[0:M, :], ysave[:, p * 3 * PW:(p + 1) * 3 * PW], y[M:, :]], axis=0)

            def fix_ob(p, o):
                return jnp.concatenate([o, osave[:, p * PW:(p + 1) * PW]], axis=0)

            hb = jnp.concatenate([ra[0:M, :], xb_b], axis=0).astype(BF16)
            rb = _segment(hb, wb, wob, fix_yb, fix_ob)
            rsave[24:32, :] = rb[L:, :]
            rsave[32:64, :] = rb[M:L, :]
            return rb[0:M, :]

        with jax.named_scope("b"):
            lax.fori_loop(0, nb, b_pair, mem0[...].astype(F32))
        b_finish(nb - 1)

        @pl.when(l == 0)
        def _():
            block_a(False)
        return 0

    block_a(True)
    lax.fori_loop(0, 2, layer, 0)
    out_copy(nb - 2).start()
    out_copy(nb - 1).start()
    pltpu.make_async_copy(xio, out_hbm, sem_out.at[0]).wait()


@functools.partial(jax.jit, static_argnames=("B_seg_len",))
def pallas_interleave_layers__linear_kernel_hedgehog__memory_aug_recurrent_mem_tr__prompt_kernel(
    A_x, A_wqkv, A_w_phi, A_wo, B_x, B_mem0, B_Wq, B_Wk, B_Wv, B_Wo, B_seg_len,
):
    del B_x
    assert B_seg_len == SEG
    x = A_x.reshape(S, D)
    wphi = A_w_phi.transpose(1, 2, 0)
    mem0 = B_mem0.reshape(M, D)
    wq, wk, wv = (w.transpose(1, 2, 0).reshape(HD, D) for w in (B_Wq, B_Wk, B_Wv))
    wo = B_Wo.reshape(HD, D)
    hbm = pl.BlockSpec(memory_space=pl.ANY)
    out = pl.pallas_call(
        _kernel,
        out_shape=jax.ShapeDtypeStruct((S, D), A_x.dtype),
        in_specs=[hbm] * 9,
        out_specs=hbm,
        scratch_shapes=[
            pltpu.VMEM((S, D), BF16),
            pltpu.VMEM((D, 3 * D), BF16),
            pltpu.VMEM((FA, FA, HA), BF16),
            pltpu.VMEM((D, D), BF16),
            pltpu.VMEM((M, D), BF16),
            pltpu.VMEM((S, D), F32),
            pltpu.VMEM((S // 2, D), U32),
            pltpu.VMEM((2 * SEG, D), F32),
            pltpu.VMEM((3 * GA, GR // 2, D), U32),
            pltpu.VMEM((D // 2, D), U32),
            pltpu.VMEM((S // 128, D, 128), U32),
            pltpu.VMEM((S // 128, D, 128), U32),
            pltpu.VMEM((PA, VR, S), U32),
            pltpu.VMEM((PA, VR, 4 * FA), U32),
            pltpu.VMEM((TN // 2, D), U32),
            pltpu.VMEM((4, HD, D), BF16),
            pltpu.VMEM((D // 2, 3 * HD), U32),
            pltpu.VMEM((HD // 2, D), U32),
            pltpu.VMEM((8, 3 * HD), F32),
            pltpu.VMEM((8, HD), F32),
            pltpu.VMEM((2 * SEG, D), F32),
            pltpu.SemaphoreType.DMA((4,)),
            pltpu.SemaphoreType.DMA((S // TN,)),
            pltpu.SemaphoreType.DMA((4 * NP,)),
            pltpu.SemaphoreType.DMA((1,)),
        ],
        compiler_params=pltpu.CompilerParams(vmem_limit_bytes=120 * 1024 * 1024,
                                             disable_bounds_checks=True),
    )(x, A_wqkv, wphi, A_wo, mem0, wq, wk, wv, wo)
    return out.reshape(1, S, D)
```

```python
import functools

import jax
import jax.numpy as jnp
from jax import lax
import jax.experimental.pallas as pl
import jax.experimental.pallas.tpu as pltpu

F32 = jnp.float32
BF16 = jnp.bfloat16
U32 = jnp.uint32

S = 2048
D = 640
HA = 32
FA = 20
GA = 4
GR = 8 * FA
VR = 24
PA = HA // 2
TN = 256
HB = 32
DH = 192
HD = HB * DH
M = 8
SEG = 32
L = M + SEG
PW = 2 * DH
NP = HB // 2
TB = 64

NT = (((1,), (1,)), ((), ()))
LOG2E = 1.4426950408889634


def _dot(a, b):
    return jnp.dot(a, b, preferred_element_type=F32)


def _dot_nt(a, b):
    return lax.dot_general(a, b, NT, preferred_element_type=F32)


def _pack(a):
    return pltpu.bitcast(a, U32)


def _unpack(a):
    return pltpu.bitcast(a, BF16)


def _interleave(a, b):
    return pltpu.pack_elementwise([a, b], packed_dtype=BF16).astype(U32)


def _recip(x):
    r = pl.reciprocal(x, approx=True)
    return r * (2.0 - x * r)


def _layernorm(x):
    m = jnp.mean(x, axis=-1, keepdims=True)
    c = x - m
    v = jnp.mean(c * c, axis=-1, keepdims=True)
    return c * lax.rsqrt(v + 1e-5)


def _feature_map(p):
    t = p.shape[-1]
    p3 = p.reshape(FA, 8, t)
    mx = jnp.max(p3, axis=0, keepdims=True)
    mn = jnp.min(p3, axis=0, keepdims=True)
    lp = mx + jnp.log2(jnp.sum(jnp.exp2(p3 - mx), axis=0, keepdims=True))
    ln = mn - jnp.log2(jnp.sum(jnp.exp2(mn - p3), axis=0, keepdims=True))
    ep = jnp.exp2(p3 - lp)
    en = jnp.exp2(ln - p3)
    return _interleave(ep.reshape(GR, t), en.reshape(GR, t))


def _split_pair(a):
    lane = lax.broadcasted_iota(jnp.int32, (L, 128), 1)
    mid = a[:, 128:256]
    outer = jnp.concatenate([a[:, 0:128], a[:, 256:384]], axis=0)
    mid = jnp.concatenate(
        [jnp.where(lane < 64, mid, 0.0), jnp.where(lane < 64, 0.0, mid)], axis=0)
    return outer.astype(BF16), mid.astype(BF16)


def _scores(y):
    q_outer = jnp.concatenate([y[:, 0:128], y[:, 256:384]], axis=0).astype(BF16)
    q_mid = y[:, 128:256].astype(BF16)
    k_outer, k_mid = _split_pair(y[:, PW:2 * PW])
    s_outer = _dot_nt(q_outer, k_outer)
    s_mid = _dot_nt(q_mid, k_mid)
    row = lax.broadcasted_iota(jnp.int32, (L, 2 * L), 0)
    col = lax.broadcasted_iota(jnp.int32, (L, 2 * L), 1)
    first = col < L
    key = jnp.where(first, col, col - L)
    valid = jnp.logical_or(row < M, row >= key)
    s = (jnp.where(first, s_outer[0:L, :], s_outer[L:, :]) + s_mid) * (DH ** -0.5)
    s = jnp.where(valid, s, -1e9)
    m0 = jnp.max(jnp.where(first, s, -jnp.inf), axis=-1, keepdims=True)
    m1 = jnp.max(jnp.where(first, -jnp.inf, s), axis=-1, keepdims=True)
    e = jnp.exp(s - jnp.where(first, m0, m1))
    s0 = jnp.sum(jnp.where(first, e, 0.0), axis=-1, keepdims=True)
    s1 = jnp.sum(jnp.where(first, 0.0, e), axis=-1, keepdims=True)
    p = e * _recip(jnp.where(first, s0, s1))
    ps = jnp.concatenate([jnp.where(first, p, 0.0), jnp.where(first, 0.0, p)], axis=0)
    return p.astype(BF16), ps.astype(BF16)


def _pv(p, ps, v_outer, v_mid):
    o_outer = _dot(ps, v_outer)
    o_mid = _dot(p, v_mid)
    return jnp.concatenate([o_outer[0:L, :], o_mid, o_outer[L:, :]], axis=1)


def _segment(h, wb, wob, fix_y, fix_o):
    ps, vs, os_ = {}, {}, {}
    ys = {}

    def proj(p):
        ys[p] = fix_y(p, _dot(h, _unpack(wb[:, p * 3 * PW:(p + 1) * 3 * PW])))

    def score(p):
        y = ys.pop(p)
        vs[p] = _split_pair(y[:, 2 * PW:3 * PW])
        ps[p] = _scores(y)

    def pv(p):
        os_[p] = fix_o(p, _pv(*ps.pop(p), *vs.pop(p))).astype(BF16)

    def oproj(lo, hi):
        o = jnp.concatenate([os_.pop(p) for p in range(lo, hi)], axis=1)
        return _dot(o, wob[lo * PW:hi * PW, :])

    for p in range(NP):
        proj(p)
        if p >= 1:
            score(p - 1)
        if p >= 3:
            pv(p - 3)
    r = oproj(0, 3)
    score(NP - 1)
    pv(NP - 3)
    r = oproj(3, 6) + r
    pv(NP - 2)
    r = oproj(6, 10) + r
    pv(NP - 1)
    r = oproj(10, 14) + r
    r = oproj(14, 16) + r
    return r


def _kernel(x_hbm, wqkv_hbm, wphi_hbm, woa_hbm, mem0_hbm,
            wq_hbm, wk_hbm, wv_hbm, wo_hbm,
            out_hbm,
            xio, wqkv, wphi, woa, mem0, xres, xa, xb, wat, phq, phk, vts, kvs, osc,
            wraw, wb, wob, ysave, osave, rsave, sem_in, sem_out):
    nt = S // TN
    nsub = TN // 128

    def rows(j, n):
        return pl.ds(j * n if isinstance(j, int) else pl.multiple_of(j * n, n), n)

    def x_copy(j):
        return pltpu.make_async_copy(x_hbm.at[rows(j, TN), :], xio.at[rows(j, TN), :],
                                     sem_in.at[7 + j])

    def w_copies(p):
        return [pltpu.make_async_copy(src.at[rows(p, PW), :], wraw.at[i, rows(p, PW), :],
                                      sem_in.at[7 + nt + 3 * p + i])
                for i, src in enumerate((wq_hbm, wk_hbm, wv_hbm))]

    def out_copy(i):
        return pltpu.make_async_copy(xio.at[rows(i, TB), :],
                                     out_hbm.at[rows(i, TB), :], sem_out.at[0])

    wa_copy = [pltpu.make_async_copy(wqkv_hbm.at[:, rows(i, D)], wqkv.at[i], sem_in.at[i])
               for i in range(3)]
    wphi_copy = pltpu.make_async_copy(wphi_hbm, wphi, sem_in.at[3])
    woa_copy = pltpu.make_async_copy(woa_hbm, woa, sem_in.at[4])
    mem0_copy = pltpu.make_async_copy(mem0_hbm, mem0, sem_in.at[5])
    wob_copy = pltpu.make_async_copy(wo_hbm, wob, sem_in.at[6])
    order = [wphi_copy, x_copy(0), wa_copy[1], wa_copy[0], wa_copy[2], x_copy(1)]
    for p in range(NP):
        order += w_copies(p)
        if p + 2 < nt:
            order.append(x_copy(p + 2))
        if p + 2 == nt:
            order += [woa_copy, mem0_copy]
    for c in order + [wob_copy]:
        c.start()

    def ln_in(t):
        return _pack(_layernorm(xio[rows(t, 128), :].astype(F32)).astype(BF16))

    def qk_features(which, t, xn, g):
        ph = (phq, phk)[which]
        fm = _feature_map(_dot_nt(_unpack(wat[which * GA + g]), xn))
        for f in range(FA):
            ph[t, pl.ds(GR * g + f, 8, stride=FA), :] = fm[8 * f:8 * f + 8, :]

    def values(t, xn, g):
        vt = _dot_nt(_unpack(wat[2 * GA + g]), xn)
        for q in range(4):
            v = jnp.concatenate([vt[40 * q:40 * q + 40, :], jnp.ones((8, 128), F32)], axis=0)
            vts[4 * g + q, :, rows(t, 128)] = _pack(v.astype(BF16))

    def relayout_b_weights(p):
        for i in range(3):
            wb[:, rows(3 * p + i, PW)] = _pack(wraw[i, rows(p, PW), :].T)

    wphi_copy.wait()
    x_copy(0).wait()
    cphi = jnp.zeros((FA, D), F32)
    hh = lax.broadcasted_iota(jnp.int32, (HA, D), 0) * FA
    jj = lax.broadcasted_iota(jnp.int32, (HA, D), 1)
    for d in range(FA):
        cphi = _dot(wphi[d], jnp.where(jj == hh + d, 1.0, 0.0).astype(BF16)) + cphi
    cb = jnp.concatenate(
        [jnp.broadcast_to(cphi[f:f + 1, :], (8, D)) for f in range(FA)], axis=0)
    bds = []
    for g in range(GA):
        row = lax.broadcasted_iota(jnp.int32, (GR, 256), 0)
        col = lax.broadcasted_iota(jnp.int32, (GR, 256), 1) + 128 * g
        lo = (8 * g + (row & 7)) * FA
        bds.append(jnp.where(jnp.logical_and(col >= lo, col < lo + FA),
                             cb[:, 128 * g:128 * g + 256], 0.0).astype(BF16))
    for u in range(nsub):
        xa[rows(u, 64), :] = ln_in(u)

    def fold(i):
        for g in range(GA):
            w = _dot_nt(bds[g], wqkv[i, :, 128 * g:128 * g + 256]) * LOG2E
            wat[i * GA + g] = _pack(w.astype(BF16))

    wa_copy[1].wait()
    fold(1)
    for u in range(nsub):
        for g in range(GA):
            qk_features(1, u, _unpack(xa[rows(u, 64), :]), g)
    wa_copy[0].wait()
    wa_copy[2].wait()
    x_copy(1).wait()
    fold(0)
    wvt = _pack(wqkv[2].T)
    for g in range(GA):
        wat[2 * GA + g] = wvt[g * GR // 2:(g + 1) * GR // 2, :]
    for u in range(nsub):
        xn = _unpack(xa[rows(u, 64), :])
        for g in range(GA):
            qk_features(0, u, xn, g)
            values(u, xn, g)
    xa[rows(nsub, 64), :] = ln_in(nsub)

    def block_a(first):
        def a1(j, _):
            if first:
                @pl.when(j + 1 < nt)
                def _():
                    x_copy(j + 1).wait()
                for c in w_copies(j - 1):
                    c.wait()
            for u in range(nsub):
                t = j * nsub + u
                xn = _unpack(ln_in(t) if first and u > 0 else xa[rows(t, 64), :])
                for g in range(GA):
                    qk_features(1, t, xn, g)
                    qk_features(0, t, xn, g)
                    values(t, xn, g)
            if first:
                relayout_b_weights(j - 1)
                tn = jnp.minimum(j + 1, nt - 1) * nsub
                xa[rows(tn, 64), :] = ln_in(tn)
            return 0

        def pair_rows(ph, q, t0, n):
            return _unpack(jnp.concatenate(
                [ph[t0 + u, 2 * FA * q:2 * FA * (q + 1), :] for u in range(n)], axis=1))

        def attend(j):
            low = lax.broadcasted_iota(jnp.int32, (8, TN), 0) < 4
            os_ = []
            for q in range(PA):
                nd = _dot(_unpack(kvs[q]), pair_rows(phq, q, j * nsub, nsub))
                rab = 1.0 / (nd[40:48, :] + 1e-6)
                rba = pltpu.roll(rab, 4, 0)
                ra = jnp.where(low, rab, rba)
                rb = jnp.where(low, rba, rab)
                os_.append(nd[0:40, :] * jnp.concatenate([ra, ra, rab, rb, rb], axis=0))
            return _pack(jnp.concatenate(os_, axis=0).astype(BF16).T)

        def project(j, o):
            r = rows(j, TN)
            x = xio[r, :].astype(F32) if first else xres[r, :]
            xres[r, :] = _dot(_unpack(o), woa[...]) + x

        def a2(j, _):
            if first:
                for c in w_copies(nt + 1 + j):
                    c.wait()
            o = osc[...]
            osc[...] = attend(j + 1)
            project(j, o)
            if first:
                relayout_b_weights(nt + 1 + j)
            return 0

        with jax.named_scope("a1"):
            lax.fori_loop(1 if first else 0, nt, a1, 0)
        with jax.named_scope("kv"):
            if first:
                for c in w_copies(nt - 1) + w_copies(nt) + [woa_copy, mem0_copy]:
                    c.wait()
            row = lax.broadcasted_iota(jnp.int32, (2 * VR, 4 * FA), 0)
            col = lax.broadcasted_iota(jnp.int32, (2 * VR, 4 * FA), 1)
            split = jnp.where(row < 2 * FA, FA, 2 * FA + 4)
            same = (row >= split) == (col >= 2 * FA)
            for q in range(PA):
                kv = _dot_nt(_unpack(vts[q]), pair_rows(phk, q, 0, S // 128))
                kvs[q] = _pack(jnp.where(same, kv, 0.0).astype(BF16))
            osc[...] = attend(0)
            if first:
                relayout_b_weights(nt - 1)
                relayout_b_weights(nt)
        with jax.named_scope("a2"):
            lax.fori_loop(0, nt - 1, a2, 0)
        xb[...] = _layernorm(xres[rows(0, TB), :])
        rsave[...] = jnp.zeros(rsave.shape, F32)
        project(nt - 1, osc[...])

    nb = S // TB

    def b_finish(i):
        r = rows(i, TB)
        x = xres[r, :] + rsave[...]
        xres[r, :] = x
        xa[rows(i, TB // 2), :] = _pack(_layernorm(x).astype(BF16))
        xio[r, :] = x.astype(BF16)

    def b_pair(mem, xn, base):
        def fix_ya(p, y):
            ysave[:, p * 3 * PW:(p + 1) * 3 * PW] = y[L:L + 8, :]
            return y[0:L, :]

        def fix_oa(p, o):
            osave[:, p * PW:(p + 1) * PW] = o[32:L, :]
            return o[0:32, :]

        ha = jnp.concatenate([mem, xn[0:40, :]], axis=0).astype(BF16)
        ra = _segment(ha, wb, wob, fix_ya, fix_oa)
        rsave[base:base + 24, :] = ra[M:, :]

        def fix_yb(p, y):
            return jnp.concatenate(
                [y[0:M, :], ysave[:, p * 3 * PW:(p + 1) * 3 * PW], y[M:, :]], axis=0)

        def fix_ob(p, o):
            return jnp.concatenate([o, osave[:, p * PW:(p + 1) * PW]], axis=0)

        hb = jnp.concatenate([ra[0:M, :], xn[40:64, :]], axis=0).astype(BF16)
        rb = _segment(hb, wb, wob, fix_yb, fix_ob)
        rsave[base + 24:base + 32, :] = rb[L:, :]
        rsave[base + 32:base + 64, :] = rb[M:L, :]
        return rb[0:M, :]

    def layer(l, _):
        def b_step(i, mem):
            @pl.when(jnp.logical_and(l == 1, i >= 2))
            def _():
                out_copy(i - 2).start()

            xn = xb[...]
            b_finish(jnp.maximum(i - 1, 0))
            xb[...] = _layernorm(xres[rows(jnp.minimum(i + 1, nb - 1), TB), :])
            for u in range(0, TB, 2 * SEG):
                mem = b_pair(mem, xn[u:u + 2 * SEG, :], u)
            return mem

        with jax.named_scope("b"):
            lax.fori_loop(0, nb, b_step, mem0[...].astype(F32))
        b_finish(nb - 1)

        @pl.when(l == 0)
        def _():
            block_a(False)
        return 0

    block_a(True)
    with jax.named_scope("wait_wo"):
        wob_copy.wait()
    lax.fori_loop(0, 2, layer, 0)
    out_copy(nb - 2).start()
    out_copy(nb - 1).start()
    pltpu.make_async_copy(xio, out_hbm, sem_out.at[0]).wait()


@functools.partial(jax.jit, static_argnames=("B_seg_len",))
def pallas_interleave_layers__linear_kernel_hedgehog__memory_aug_recurrent_mem_tr__prompt_kernel(
    A_x, A_wqkv, A_w_phi, A_wo, B_x, B_mem0, B_Wq, B_Wk, B_Wv, B_Wo, B_seg_len,
):
    del B_x
    assert B_seg_len == SEG
    x = A_x.reshape(S, D)
    wphi = A_w_phi.transpose(1, 2, 0)
    mem0 = B_mem0.reshape(M, D)
    wq, wk, wv = (w.transpose(1, 2, 0).reshape(HD, D) for w in (B_Wq, B_Wk, B_Wv))
    wo = B_Wo.reshape(HD, D)
    hbm = pl.BlockSpec(memory_space=pl.ANY)
    out = pl.pallas_call(
        _kernel,
        out_shape=jax.ShapeDtypeStruct((S, D), A_x.dtype),
        in_specs=[hbm] * 9,
        out_specs=hbm,
        scratch_shapes=[
            pltpu.VMEM((S, D), BF16),
            pltpu.VMEM((3, D, D), BF16),
            pltpu.VMEM((FA, FA, HA), BF16),
            pltpu.VMEM((D, D), BF16),
            pltpu.VMEM((M, D), BF16),
            pltpu.VMEM((S, D), F32),
            pltpu.VMEM((S // 2, D), U32),
            pltpu.VMEM((TB, D), F32),
            pltpu.VMEM((3 * GA, GR // 2, D), U32),
            pltpu.VMEM((S // 128, D, 128), U32),
            pltpu.VMEM((S // 128, D, 128), U32),
            pltpu.VMEM((PA, VR, S), U32),
            pltpu.VMEM((PA, VR, 4 * FA), U32),
            pltpu.VMEM((TN // 2, D), U32),
            pltpu.VMEM((3, HD, D), BF16),
            pltpu.VMEM((D // 2, 3 * HD), U32),
            pltpu.VMEM((HD, D), BF16),
            pltpu.VMEM((8, 3 * HD), F32),
            pltpu.VMEM((8, HD), F32),
            pltpu.VMEM((TB, D), F32),
            pltpu.SemaphoreType.DMA((7 + S // TN + 3 * NP,)),
            pltpu.SemaphoreType.DMA((1,)),
        ],
        compiler_params=pltpu.CompilerParams(vmem_limit_bytes=120 * 1024 * 1024,
                                             disable_bounds_checks=True),
    )(x, A_wqkv, wphi, A_wo, mem0, wq, wk, wv, wo)
    return out.reshape(1, S, D)
```

```python
import functools

import jax
import jax.numpy as jnp
from jax import lax
import jax.experimental.pallas as pl
import jax.experimental.pallas.tpu as pltpu

F32 = jnp.float32
BF16 = jnp.bfloat16
U32 = jnp.uint32

S = 2048
D = 640
HA = 32
FA = 20
GA = 4
GR = 8 * FA
VR = 24
PA = HA // 2
TN = 256
HB = 32
DH = 192
HD = HB * DH
M = 8
SEG = 32
L = M + SEG
PW = 2 * DH
NP = HB // 2
TB = 64

NT = (((1,), (1,)), ((), ()))
LOG2E = 1.4426950408889634


def _dot(a, b):
    return jnp.dot(a, b, preferred_element_type=F32)


def _dot_nt(a, b):
    return lax.dot_general(a, b, NT, preferred_element_type=F32)


def _pack(a):
    return pltpu.bitcast(a, U32)


def _unpack(a):
    return pltpu.bitcast(a, BF16)


def _interleave(a, b):
    return pltpu.pack_elementwise([a, b], packed_dtype=BF16).astype(U32)


def _recip(x):
    r = pl.reciprocal(x, approx=True)
    return r * (2.0 - x * r)


def _layernorm(x):
    m = jnp.mean(x, axis=-1, keepdims=True)
    c = x - m
    v = jnp.mean(c * c, axis=-1, keepdims=True)
    return c * lax.rsqrt(v + 1e-5)


def _feature_map(p):
    t = p.shape[-1]
    p3 = p.reshape(FA, 8, t)
    mx = jnp.max(p3, axis=0, keepdims=True)
    mn = jnp.min(p3, axis=0, keepdims=True)
    lp = mx + jnp.log2(jnp.sum(jnp.exp2(p3 - mx), axis=0, keepdims=True))
    ln = mn - jnp.log2(jnp.sum(jnp.exp2(mn - p3), axis=0, keepdims=True))
    ep = jnp.exp2(p3 - lp)
    en = jnp.exp2(ln - p3)
    return _interleave(ep.reshape(GR, t), en.reshape(GR, t))


def _tiles(a, odd):
    t0, t1, t2 = a[:, 0:128], a[:, 128:256], a[:, 256:384]
    return (t1, t2, t0) if odd else (t1, t0, t2)


def _weights(a2):
    lane = lax.broadcasted_iota(jnp.int32, (L, 128), 1)
    out, other = [], []
    for odd, a in enumerate(a2):
        mid, own, rest = _tiles(a, odd)
        out.append(jnp.concatenate(
            [jnp.where(lane < 64, mid, 0.0), jnp.where(lane < 64, 0.0, mid), own,
             jnp.zeros((128 - 3 * L, 128), F32)], axis=0).astype(BF16))
        other.append(rest)
    out.append(jnp.concatenate(
        [other[1], other[0], jnp.zeros((128 - 2 * L, 128), F32)], axis=0).astype(BF16))
    return out


def _scores(q2, k2):
    kw = _weights(k2)
    qt = [_tiles(q, odd) for odd, q in enumerate(q2)]
    s1 = [_dot_nt(jnp.concatenate(qt[e][0:2], axis=0).astype(BF16), kw[e]) for e in range(2)]
    s2 = _dot_nt(jnp.concatenate([qt[1][2], qt[0][2]], axis=0).astype(BF16), kw[2])
    row = lax.broadcasted_iota(jnp.int32, (L, 128), 0)
    col = lax.broadcasted_iota(jnp.int32, (L, 128), 1)
    first = col < L
    second = jnp.logical_and(col >= L, col < 2 * L)
    key = jnp.where(first, col, col - L)
    valid = jnp.logical_or(row < M, row >= key)
    out, other = [], []
    for odd in range(2):
        own = pltpu.roll(s1[odd][L:, :], 128 - L if odd else 128 - 2 * L, 1)
        s = jnp.where(first, s2[0:L, :], own) if odd else jnp.where(first, own, s2[L:, :])
        s = jnp.where(valid, (s + s1[odd][0:L, :]) * (DH ** -0.5), -1e9)
        m0 = jnp.max(jnp.where(first, s, -jnp.inf), axis=-1, keepdims=True)
        m1 = jnp.max(jnp.where(second, s, -jnp.inf), axis=-1, keepdims=True)
        e = jnp.exp(s - jnp.where(first, m0, m1))
        e0 = jnp.where(first, e, 0.0)
        e1 = jnp.where(second, e, 0.0)
        p0 = e0 * _recip(jnp.sum(e0, axis=-1, keepdims=True))
        p1 = e1 * _recip(jnp.sum(e1, axis=-1, keepdims=True))
        own = pltpu.roll(p1, L, 1) if odd else pltpu.roll(p0, 2 * L, 1)
        out.append(jnp.concatenate([p0 + p1, own], axis=0).astype(BF16))
        other.append(p0 if odd else p1)
    out.append(jnp.concatenate([other[1], other[0]], axis=0).astype(BF16))
    return out


def _pv(ps, vw):
    o0, o1, o2 = [_dot(p, v) for p, v in zip(ps, vw)]
    return (jnp.concatenate([o0[L:, :], o0[0:L, :], o2[L:, :]], axis=1),
            jnp.concatenate([o2[0:L, :], o1[0:L, :], o1[L:, :]], axis=1))


def _segment(h, wb, wob, fix_y, fix_o):
    ys, ps, vs, os_ = {}, {}, {}, {}

    def proj(p):
        ys[p] = fix_y(p, _dot(h, _unpack(wb[:, p * 3 * PW:(p + 1) * 3 * PW])))

    def score(c):
        y2 = [ys.pop(2 * c), ys.pop(2 * c + 1)]
        vs[c] = _weights([y[:, 2 * PW:3 * PW] for y in y2])
        ps[c] = _scores([y[:, 0:PW] for y in y2], [y[:, PW:2 * PW] for y in y2])

    def pv(c):
        for e, o in enumerate(_pv(ps.pop(c), vs.pop(c))):
            os_[2 * c + e] = fix_o(2 * c + e, o)

    def oproj(lo, hi):
        o = jnp.concatenate([os_.pop(p) for p in range(lo, hi)], axis=1).astype(BF16)
        return _dot(o, wob[lo * PW:hi * PW, :])

    nc = NP // 2
    for c in range(nc):
        proj(2 * c)
        if c >= 1:
            score(c - 1)
        if c >= 2:
            pv(c - 2)
        proj(2 * c + 1)
    r = oproj(0, 3)
    score(nc - 1)
    pv(nc - 2)
    r = oproj(3, 9) + r
    pv(nc - 1)
    r = oproj(9, 14) + r
    r = oproj(14, 16) + r
    return r


def _kernel(x_hbm, wqkv_hbm, wphi_hbm, woa_hbm, mem0_hbm,
            wq_hbm, wk_hbm, wv_hbm, wo_hbm,
            out_hbm,
            xio, wqkv, wphi, woa, mem0, xres, xa, xb, wat, phq, phk, vts, kvs, osc,
            wraw, wb, wob, ysave, osave, rsave, sem_in, sem_out):
    nt = S // TN
    nsub = TN // 128

    def rows(j, n):
        return pl.ds(j * n if isinstance(j, int) else pl.multiple_of(j * n, n), n)

    def x_copy(j):
        return pltpu.make_async_copy(x_hbm.at[rows(j, TN), :], xio.at[rows(j, TN), :],
                                     sem_in.at[7 + j])

    def w_copies(p):
        return [pltpu.make_async_copy(src.at[rows(p, PW), :], wraw.at[i, rows(p, PW), :],
                                      sem_in.at[7 + nt + 3 * p + i])
                for i, src in enumerate((wq_hbm, wk_hbm, wv_hbm))]

    def out_copy(i):
        return pltpu.make_async_copy(xio.at[rows(i, TB), :],
                                     out_hbm.at[rows(i, TB), :], sem_out.at[0])

    wa_copy = [pltpu.make_async_copy(wqkv_hbm.at[:, rows(i, D)], wqkv.at[i], sem_in.at[i])
               for i in range(3)]
    wphi_copy = pltpu.make_async_copy(wphi_hbm, wphi, sem_in.at[3])
    woa_copy = pltpu.make_async_copy(woa_hbm, woa, sem_in.at[4])
    mem0_copy = pltpu.make_async_copy(mem0_hbm, mem0, sem_in.at[5])
    wob_copy = pltpu.make_async_copy(wo_hbm, wob, sem_in.at[6])
    order = [wphi_copy, x_copy(0), wa_copy[1], wa_copy[0], wa_copy[2], x_copy(1)]
    for p in range(NP):
        order += w_copies(p)
        if p + 2 < nt:
            order.append(x_copy(p + 2))
        if p + 2 == nt:
            order += [woa_copy, mem0_copy]
    for c in order + [wob_copy]:
        c.start()

    def ln_in(t):
        return _pack(_layernorm(xio[rows(t, 128), :].astype(F32)).astype(BF16))

    def qk_features(which, t, xn, g):
        ph = (phq, phk)[which]
        fm = _feature_map(_dot_nt(_unpack(wat[which * GA + g]), xn))
        for f in range(FA):
            ph[t, pl.ds(GR * g + f, 8, stride=FA), :] = fm[8 * f:8 * f + 8, :]

    def values(t, xn, g):
        vt = _dot_nt(_unpack(wat[2 * GA + g]), xn)
        for q in range(4):
            v = jnp.concatenate([vt[40 * q:40 * q + 40, :], jnp.ones((8, 128), F32)], axis=0)
            vts[4 * g + q, :, rows(t, 128)] = _pack(v.astype(BF16))

    def relayout_b_weights(p):
        for i in range(3):
            wb[:, rows(3 * p + i, PW)] = _pack(wraw[i, rows(p, PW), :].T)

    wphi_copy.wait()
    x_copy(0).wait()
    cphi = jnp.zeros((FA, D), F32)
    hh = lax.broadcasted_iota(jnp.int32, (HA, D), 0) * FA
    jj = lax.broadcasted_iota(jnp.int32, (HA, D), 1)
    for d in range(FA):
        cphi = _dot(wphi[d], jnp.where(jj == hh + d, 1.0, 0.0).astype(BF16)) + cphi
    cb = jnp.concatenate(
        [jnp.broadcast_to(cphi[f:f + 1, :], (8, D)) for f in range(FA)], axis=0)
    bds = []
    for g in range(GA):
        row = lax.broadcasted_iota(jnp.int32, (GR, 256), 0)
        col = lax.broadcasted_iota(jnp.int32, (GR, 256), 1) + 128 * g
        lo = (8 * g + (row & 7)) * FA
        bds.append(jnp.where(jnp.logical_and(col >= lo, col < lo + FA),
                             cb[:, 128 * g:128 * g + 256], 0.0).astype(BF16))
    for u in range(nsub):
        xa[rows(u, 64), :] = ln_in(u)

    def fold(i):
        for g in range(GA):
            w = _dot_nt(bds[g], wqkv[i, :, 128 * g:128 * g + 256]) * LOG2E
            wat[i * GA + g] = _pack(w.astype(BF16))

    wa_copy[1].wait()
    fold(1)
    for u in range(nsub):
        for g in range(GA):
            qk_features(1, u, _unpack(xa[rows(u, 64), :]), g)
    wa_copy[0].wait()
    wa_copy[2].wait()
    x_copy(1).wait()
    fold(0)
    wvt = _pack(wqkv[2].T)
    for g in range(GA):
        wat[2 * GA + g] = wvt[g * GR // 2:(g + 1) * GR // 2, :]
    for u in range(nsub):
        xn = _unpack(xa[rows(u, 64), :])
        for g in range(GA):
            qk_features(0, u, xn, g)
            values(u, xn, g)
    xa[rows(nsub, 64), :] = ln_in(nsub)

    def block_a(first):
        def a1(j, _):
            if first:
                @pl.when(j + 1 < nt)
                def _():
                    x_copy(j + 1).wait()
                for c in w_copies(j - 1):
                    c.wait()
            for u in range(nsub):
                t = j * nsub + u
                xn = _unpack(ln_in(t) if first and u > 0 else xa[rows(t, 64), :])
                for g in range(GA):
                    qk_features(1, t, xn, g)
                    qk_features(0, t, xn, g)
                    values(t, xn, g)
            if first:
                relayout_b_weights(j - 1)
                tn = jnp.minimum(j + 1, nt - 1) * nsub
                xa[rows(tn, 64), :] = ln_in(tn)
            return 0

        def pair_rows(ph, q, t0, n):
            return _unpack(jnp.concatenate(
                [ph[t0 + u, 2 * FA * q:2 * FA * (q + 1), :] for u in range(n)], axis=1))

        def attend(j):
            low = lax.broadcasted_iota(jnp.int32, (8, TN), 0) < 4
            os_ = []
            for q in range(PA):
                nd = _dot(_unpack(kvs[q]), pair_rows(phq, q, j * nsub, nsub))
                rab = 1.0 / (nd[40:48, :] + 1e-6)
                rba = pltpu.roll(rab, 4, 0)
                ra = jnp.where(low, rab, rba)
                rb = jnp.where(low, rba, rab)
                os_.append(nd[0:40, :] * jnp.concatenate([ra, ra, rab, rb, rb], axis=0))
            return _pack(jnp.concatenate(os_, axis=0).astype(BF16).T)

        def project(j, o):
            r = rows(j, TN)
            x = xio[r, :].astype(F32) if first else xres[r, :]
            xres[r, :] = _dot(_unpack(o), woa[...]) + x

        def a2(j, _):
            if first:
                for c in w_copies(nt + 1 + j):
                    c.wait()
            o = osc[...]
            osc[...] = attend(j + 1)
            project(j, o)
            if first:
                relayout_b_weights(nt + 1 + j)
            return 0

        with jax.named_scope("a1"):
            lax.fori_loop(1 if first else 0, nt, a1, 0)
        with jax.named_scope("kv"):
            if first:
                for c in w_copies(nt - 1) + w_copies(nt) + [woa_copy, mem0_copy]:
                    c.wait()
            row = lax.broadcasted_iota(jnp.int32, (2 * VR, 4 * FA), 0)
            col = lax.broadcasted_iota(jnp.int32, (2 * VR, 4 * FA), 1)
            split = jnp.where(row < 2 * FA, FA, 2 * FA + 4)
            same = (row >= split) == (col >= 2 * FA)
            for q in range(PA):
                kv = _dot_nt(_unpack(vts[q]), pair_rows(phk, q, 0, S // 128))
                kvs[q] = _pack(jnp.where(same, kv, 0.0).astype(BF16))
            osc[...] = attend(0)
            if first:
                relayout_b_weights(nt - 1)
                relayout_b_weights(nt)
        with jax.named_scope("a2"):
            lax.fori_loop(0, nt - 1, a2, 0)
        xb[...] = _layernorm(xres[rows(0, TB), :])
        rsave[...] = jnp.zeros(rsave.shape, F32)
        project(nt - 1, osc[...])

    nb = S // TB

    def b_finish(i):
        r = rows(i, TB)
        x = xres[r, :] + rsave[...]
        xres[r, :] = x
        xa[rows(i, TB // 2), :] = _pack(_layernorm(x).astype(BF16))
        xio[r, :] = x.astype(BF16)

    def b_pair(mem, xn, base):
        def fix_ya(p, y):
            ysave[:, p * 3 * PW:(p + 1) * 3 * PW] = y[L:L + 8, :]
            return y[0:L, :]

        def fix_oa(p, o):
            osave[:, p * PW:(p + 1) * PW] = o[32:L, :]
            return o[0:32, :]

        ha = jnp.concatenate([mem, xn[0:40, :]], axis=0).astype(BF16)
        ra = _segment(ha, wb, wob, fix_ya, fix_oa)
        rsave[base:base + 24, :] = ra[M:, :]

        def fix_yb(p, y):
            return jnp.concatenate(
                [y[0:M, :], ysave[:, p * 3 * PW:(p + 1) * 3 * PW], y[M:, :]], axis=0)

        def fix_ob(p, o):
            return jnp.concatenate([o, osave[:, p * PW:(p + 1) * PW]], axis=0)

        hb = jnp.concatenate([ra[0:M, :], xn[40:64, :]], axis=0).astype(BF16)
        rb = _segment(hb, wb, wob, fix_yb, fix_ob)
        rsave[base + 24:base + 32, :] = rb[L:, :]
        rsave[base + 32:base + 64, :] = rb[M:L, :]
        return rb[0:M, :]

    def layer(l, _):
        def b_step(i, mem):
            @pl.when(jnp.logical_and(l == 1, i >= 2))
            def _():
                out_copy(i - 2).start()

            xn = xb[...]
            b_finish(jnp.maximum(i - 1, 0))
            xb[...] = _layernorm(xres[rows(jnp.minimum(i + 1, nb - 1), TB), :])
            for u in range(0, TB, 2 * SEG):
                mem = b_pair(mem, xn[u:u + 2 * SEG, :], u)
            return mem

        with jax.named_scope("b"):
            lax.fori_loop(0, nb, b_step, mem0[...].astype(F32))
        b_finish(nb - 1)

        @pl.when(l == 0)
        def _():
            block_a(False)
        return 0

    block_a(True)
    with jax.named_scope("wait_wo"):
        wob_copy.wait()
    lax.fori_loop(0, 2, layer, 0)
    out_copy(nb - 2).start()
    out_copy(nb - 1).start()
    pltpu.make_async_copy(xio, out_hbm, sem_out.at[0]).wait()


@functools.partial(jax.jit, static_argnames=("B_seg_len",))
def pallas_interleave_layers__linear_kernel_hedgehog__memory_aug_recurrent_mem_tr__prompt_kernel(
    A_x, A_wqkv, A_w_phi, A_wo, B_x, B_mem0, B_Wq, B_Wk, B_Wv, B_Wo, B_seg_len,
):
    del B_x
    assert B_seg_len == SEG
    x = A_x.reshape(S, D)
    wphi = A_w_phi.transpose(1, 2, 0)
    mem0 = B_mem0.reshape(M, D)
    wq, wk, wv = (w.transpose(1, 2, 0).reshape(HD, D) for w in (B_Wq, B_Wk, B_Wv))
    wo = B_Wo.reshape(HD, D)
    hbm = pl.BlockSpec(memory_space=pl.ANY)
    out = pl.pallas_call(
        _kernel,
        out_shape=jax.ShapeDtypeStruct((S, D), A_x.dtype),
        in_specs=[hbm] * 9,
        out_specs=hbm,
        scratch_shapes=[
            pltpu.VMEM((S, D), BF16),
            pltpu.VMEM((3, D, D), BF16),
            pltpu.VMEM((FA, FA, HA), BF16),
            pltpu.VMEM((D, D), BF16),
            pltpu.VMEM((M, D), BF16),
            pltpu.VMEM((S, D), F32),
            pltpu.VMEM((S // 2, D), U32),
            pltpu.VMEM((TB, D), F32),
            pltpu.VMEM((3 * GA, GR // 2, D), U32),
            pltpu.VMEM((S // 128, D, 128), U32),
            pltpu.VMEM((S // 128, D, 128), U32),
            pltpu.VMEM((PA, VR, S), U32),
            pltpu.VMEM((PA, VR, 4 * FA), U32),
            pltpu.VMEM((TN // 2, D), U32),
            pltpu.VMEM((3, HD, D), BF16),
            pltpu.VMEM((D // 2, 3 * HD), U32),
            pltpu.VMEM((HD, D), BF16),
            pltpu.VMEM((8, 3 * HD), F32),
            pltpu.VMEM((8, HD), F32),
            pltpu.VMEM((TB, D), F32),
            pltpu.SemaphoreType.DMA((7 + S // TN + 3 * NP,)),
            pltpu.SemaphoreType.DMA((1,)),
        ],
        compiler_params=pltpu.CompilerParams(vmem_limit_bytes=120 * 1024 * 1024,
                                             disable_bounds_checks=True),
    )(x, A_wqkv, wphi, A_wo, mem0, wq, wk, wv, wo)
    return out.reshape(1, S, D)
```

```python
import functools

import jax
import jax.numpy as jnp
from jax import lax
import jax.experimental.pallas as pl
import jax.experimental.pallas.tpu as pltpu

F32 = jnp.float32
BF16 = jnp.bfloat16
U32 = jnp.uint32

S = 2048
D = 640
HA = 32
FA = 20
GA = 4
GR = 8 * FA
VR = 24
PA = HA // 2
TN = 256
HB = 32
DH = 192
HD = HB * DH
M = 8
SEG = 32
L = M + SEG
PW = 2 * DH
NP = HB // 2
TB = 64
PRE = (7,)

NT = (((1,), (1,)), ((), ()))
LOG2E = 1.4426950408889634


def _dot(a, b):
    return jnp.dot(a, b, preferred_element_type=F32)


def _dot_nt(a, b):
    return lax.dot_general(a, b, NT, preferred_element_type=F32)


def _pack(a):
    return pltpu.bitcast(a, U32)


def _unpack(a):
    return pltpu.bitcast(a, BF16)


def _interleave(a, b):
    return pltpu.pack_elementwise([a, b], packed_dtype=BF16).astype(U32)


def _recip(x):
    r = pl.reciprocal(x, approx=True)
    return r * (2.0 - x * r)


def _layernorm(x):
    m = jnp.mean(x, axis=-1, keepdims=True)
    c = x - m
    v = jnp.mean(c * c, axis=-1, keepdims=True)
    return c * lax.rsqrt(v + 1e-5)


def _feature_map(p):
    t = p.shape[-1]
    p3 = p.reshape(FA, 8, t)
    mx = jnp.max(p3, axis=0, keepdims=True)
    mn = jnp.min(p3, axis=0, keepdims=True)
    lp = mx + jnp.log2(jnp.sum(jnp.exp2(p3 - mx), axis=0, keepdims=True))
    ln = mn - jnp.log2(jnp.sum(jnp.exp2(mn - p3), axis=0, keepdims=True))
    ep = jnp.exp2(p3 - lp)
    en = jnp.exp2(ln - p3)
    return _interleave(ep.reshape(GR, t), en.reshape(GR, t))


def _tiles(a, odd):
    t0, t1, t2 = a[:, 0:128], a[:, 128:256], a[:, 256:384]
    return (t1, t2, t0) if odd else (t1, t0, t2)


def _weights(a2):
    lane = lax.broadcasted_iota(jnp.int32, (L, 128), 1)
    out, other = [], []
    for odd, a in enumerate(a2):
        mid, own, rest = _tiles(a, odd)
        out.append(jnp.concatenate(
            [jnp.where(lane < 64, mid, 0.0), jnp.where(lane < 64, 0.0, mid), own,
             jnp.zeros((128 - 3 * L, 128), F32)], axis=0).astype(BF16))
        other.append(rest)
    out.append(jnp.concatenate(
        [other[1], other[0], jnp.zeros((128 - 2 * L, 128), F32)], axis=0).astype(BF16))
    return out


def _scores(q2, k2):
    kw = _weights(k2)
    qt = [_tiles(q, odd) for odd, q in enumerate(q2)]
    s1 = [_dot_nt(jnp.concatenate(qt[e][0:2], axis=0).astype(BF16), kw[e]) for e in range(2)]
    s2 = _dot_nt(jnp.concatenate([qt[1][2], qt[0][2]], axis=0).astype(BF16), kw[2])
    row = lax.broadcasted_iota(jnp.int32, (L, 128), 0)
    col = lax.broadcasted_iota(jnp.int32, (L, 128), 1)
    first = col < L
    second = jnp.logical_and(col >= L, col < 2 * L)
    key = jnp.where(first, col, col - L)
    valid = jnp.logical_or(row < M, row >= key)
    out, other = [], []
    for odd in range(2):
        own = pltpu.roll(s1[odd][L:, :], 128 - L if odd else 128 - 2 * L, 1)
        s = jnp.where(first, s2[0:L, :], own) if odd else jnp.where(first, own, s2[L:, :])
        s = jnp.where(valid, (s + s1[odd][0:L, :]) * (DH ** -0.5), -1e9)
        m0 = jnp.max(jnp.where(first, s, -jnp.inf), axis=-1, keepdims=True)
        m1 = jnp.max(jnp.where(second, s, -jnp.inf), axis=-1, keepdims=True)
        e = jnp.exp(s - jnp.where(first, m0, m1))
        e0 = jnp.where(first, e, 0.0)
        e1 = jnp.where(second, e, 0.0)
        p0 = e0 * _recip(jnp.sum(e0, axis=-1, keepdims=True))
        p1 = e1 * _recip(jnp.sum(e1, axis=-1, keepdims=True))
        own = pltpu.roll(p1, L, 1) if odd else pltpu.roll(p0, 2 * L, 1)
        out.append(jnp.concatenate([p0 + p1, own], axis=0).astype(BF16))
        other.append(p0 if odd else p1)
    out.append(jnp.concatenate([other[1], other[0]], axis=0).astype(BF16))
    return out


def _pv(ps, vw):
    o0, o1, o2 = [_dot(p, v) for p, v in zip(ps, vw)]
    return (jnp.concatenate([o0[L:, :], o0[0:L, :], o2[L:, :]], axis=1),
            jnp.concatenate([o2[0:L, :], o1[0:L, :], o1[L:, :]], axis=1))


def _pre_cols(p):
    k = PRE.index(p)
    return slice(k * 3 * PW, (k + 1) * 3 * PW)


def _segment(h, wb, wpre, wob, fix_y, fix_o):
    ys, ps, vs, os_ = {}, {}, {}, {}

    def proj(p):
        if p in PRE:
            y = _dot(h[0:32, :], _unpack(wpre[:, _pre_cols(p)]))
        else:
            y = _dot(h, _unpack(wb[:, p * 3 * PW:(p + 1) * 3 * PW]))
        ys[p] = fix_y(p, y)

    def score(c):
        y2 = [ys.pop(2 * c), ys.pop(2 * c + 1)]
        vs[c] = _weights([y[:, 2 * PW:3 * PW] for y in y2])
        ps[c] = _scores([y[:, 0:PW] for y in y2], [y[:, PW:2 * PW] for y in y2])

    def pv(c):
        for e, o in enumerate(_pv(ps.pop(c), vs.pop(c))):
            os_[2 * c + e] = fix_o(2 * c + e, o)

    def oproj(lo, hi):
        o = jnp.concatenate([os_.pop(p) for p in range(lo, hi)], axis=1).astype(BF16)
        return _dot(o, wob[lo * PW:hi * PW, :])

    nc = NP // 2
    for c in range(nc):
        proj(2 * c)
        if c >= 1:
            score(c - 1)
        if c >= 2:
            pv(c - 2)
        proj(2 * c + 1)
    r = oproj(0, 3)
    score(nc - 1)
    pv(nc - 2)
    r = oproj(3, 9) + r
    pv(nc - 1)
    r = oproj(9, 14) + r
    r = oproj(14, 16) + r
    return r


def _kernel(x_hbm, wqkv_hbm, wphi_hbm, woa_hbm, mem0_hbm,
            wq_hbm, wk_hbm, wv_hbm, wo_hbm,
            out_hbm,
            xio, wqkv, wphi, woa, mem0, xres, xa, xb, wat, phq, phk, vts, kvs, osc,
            wraw, wb, wpre, wob, ypre, ysave, osave, rsave, sem_in, sem_out):
    nt = S // TN
    nsub = TN // 128

    def rows(j, n):
        return pl.ds(j * n if isinstance(j, int) else pl.multiple_of(j * n, n), n)

    def x_copy(j):
        return pltpu.make_async_copy(x_hbm.at[rows(j, TN), :], xio.at[rows(j, TN), :],
                                     sem_in.at[7 + j])

    def w_copies(p):
        return [pltpu.make_async_copy(src.at[rows(p, PW), :], wraw.at[i, rows(p, PW), :],
                                      sem_in.at[7 + nt + 3 * p + i])
                for i, src in enumerate((wq_hbm, wk_hbm, wv_hbm))]

    def out_copy(i):
        return pltpu.make_async_copy(xio.at[rows(i, TB), :],
                                     out_hbm.at[rows(i, TB), :], sem_out.at[0])

    wa_copy = [pltpu.make_async_copy(wqkv_hbm.at[:, rows(i, D)], wqkv.at[i], sem_in.at[i])
               for i in range(3)]
    wphi_copy = pltpu.make_async_copy(wphi_hbm, wphi, sem_in.at[3])
    woa_copy = pltpu.make_async_copy(woa_hbm, woa, sem_in.at[4])
    mem0_copy = pltpu.make_async_copy(mem0_hbm, mem0, sem_in.at[5])
    wob_copy = pltpu.make_async_copy(wo_hbm, wob, sem_in.at[6])
    order = [wphi_copy, x_copy(0), wa_copy[1], wa_copy[0], wa_copy[2], x_copy(1)]
    for p in range(NP):
        order += w_copies(p)
        if p + 2 < nt:
            order.append(x_copy(p + 2))
        if p + 2 == nt:
            order += [woa_copy, mem0_copy]
    for c in order + [wob_copy]:
        c.start()

    def ln_in(t):
        return _pack(_layernorm(xio[rows(t, 128), :].astype(F32)).astype(BF16))

    def qk_features(which, t, xn, g):
        ph = (phq, phk)[which]
        fm = _feature_map(_dot_nt(_unpack(wat[which * GA + g]), xn))
        for f in range(FA):
            ph[t, pl.ds(GR * g + f, 8, stride=FA), :] = fm[8 * f:8 * f + 8, :]

    def values(t, xn, g):
        vt = _dot_nt(_unpack(wat[2 * GA + g]), xn)
        for q in range(4):
            v = jnp.concatenate([vt[40 * q:40 * q + 40, :], jnp.ones((8, 128), F32)], axis=0)
            vts[4 * g + q, :, rows(t, 128)] = _pack(v.astype(BF16))

    def relayout_b_weights(p):
        for i in range(3):
            w = _pack(wraw[i, rows(p, PW), :].T)
            if isinstance(p, int) and p in PRE:
                wpre[:, rows(3 * PRE.index(p) + i, PW)] = w
            else:
                wb[:, rows(3 * p + i, PW)] = w

    wphi_copy.wait()
    x_copy(0).wait()
    cphi = jnp.zeros((FA, D), F32)
    hh = lax.broadcasted_iota(jnp.int32, (HA, D), 0) * FA
    jj = lax.broadcasted_iota(jnp.int32, (HA, D), 1)
    for d in range(FA):
        cphi = _dot(wphi[d], jnp.where(jj == hh + d, 1.0, 0.0).astype(BF16)) + cphi
    cb = jnp.concatenate(
        [jnp.broadcast_to(cphi[f:f + 1, :], (8, D)) for f in range(FA)], axis=0)
    bds = []
    for g in range(GA):
        row = lax.broadcasted_iota(jnp.int32, (GR, 256), 0)
        col = lax.broadcasted_iota(jnp.int32, (GR, 256), 1) + 128 * g
        lo = (8 * g + (row & 7)) * FA
        bds.append(jnp.where(jnp.logical_and(col >= lo, col < lo + FA),
                             cb[:, 128 * g:128 * g + 256], 0.0).astype(BF16))
    for u in range(nsub):
        xa[rows(u, 64), :] = ln_in(u)

    def fold(i):
        for g in range(GA):
            w = _dot_nt(bds[g], wqkv[i, :, 128 * g:128 * g + 256]) * LOG2E
            wat[i * GA + g] = _pack(w.astype(BF16))

    wa_copy[1].wait()
    fold(1)
    for u in range(nsub):
        for g in range(GA):
            qk_features(1, u, _unpack(xa[rows(u, 64), :]), g)
    wa_copy[0].wait()
    wa_copy[2].wait()
    x_copy(1).wait()
    fold(0)
    wvt = _pack(wqkv[2].T)
    for g in range(GA):
        wat[2 * GA + g] = wvt[g * GR // 2:(g + 1) * GR // 2, :]
    for u in range(nsub):
        xn = _unpack(xa[rows(u, 64), :])
        for g in range(GA):
            qk_features(0, u, xn, g)
            values(u, xn, g)
    xa[rows(nsub, 64), :] = ln_in(nsub)

    def block_a(first):
        def a1(j, _):
            if first:
                @pl.when(j + 1 < nt)
                def _():
                    x_copy(j + 1).wait()
                for c in w_copies(j - 1):
                    c.wait()
            for u in range(nsub):
                t = j * nsub + u
                xn = _unpack(ln_in(t) if first and u > 0 else xa[rows(t, 64), :])
                for g in range(GA):
                    qk_features(1, t, xn, g)
                    qk_features(0, t, xn, g)
                    values(t, xn, g)
            if first:
                relayout_b_weights(j - 1)
                tn = jnp.minimum(j + 1, nt - 1) * nsub
                xa[rows(tn, 64), :] = ln_in(tn)
            return 0

        def pair_rows(ph, q, t0, n):
            return _unpack(jnp.concatenate(
                [ph[t0 + u, 2 * FA * q:2 * FA * (q + 1), :] for u in range(n)], axis=1))

        def attend(j):
            low = lax.broadcasted_iota(jnp.int32, (8, TN), 0) < 4
            os_ = []
            for q in range(PA):
                nd = _dot(_unpack(kvs[q]), pair_rows(phq, q, j * nsub, nsub))
                rab = 1.0 / (nd[40:48, :] + 1e-6)
                rba = pltpu.roll(rab, 4, 0)
                ra = jnp.where(low, rab, rba)
                rb = jnp.where(low, rba, rab)
                os_.append(nd[0:40, :] * jnp.concatenate([ra, ra, rab, rb, rb], axis=0))
            return _pack(jnp.concatenate(os_, axis=0).astype(BF16).T)

        def project(j, o):
            r = rows(j, TN)
            x = xio[r, :].astype(F32) if first else xres[r, :]
            xres[r, :] = _dot(_unpack(o), woa[...]) + x

        def pre_rows(j):
            x = jnp.concatenate(
                [xres[rows(j * (TN // 8) + b + 3, 8), :] for b0 in range(0, TN // 8, 8)
                 for b in (b0, b0 + 1)], axis=0)
            return _layernorm(x).astype(BF16)

        def b_pre(j, h):
            ypre[rows(j, TN // 4), :] = _dot(h, _unpack(wpre[...]))

        def a2(j, _):
            if first:
                for c in w_copies(nt + 1 + j):
                    c.wait()
            h = pre_rows(j - 1)
            o = osc[...]
            osc[...] = attend(j + 1)
            project(j, o)
            b_pre(j - 1, h)
            if first:
                relayout_b_weights(nt + 1 + j)
            return 0

        with jax.named_scope("a1"):
            lax.fori_loop(1 if first else 0, nt, a1, 0)
        with jax.named_scope("kv"):
            if first:
                for c in (w_copies(nt - 1) + w_copies(nt) + w_copies(nt + 1)
                          + [woa_copy, mem0_copy]):
                    c.wait()
            row = lax.broadcasted_iota(jnp.int32, (2 * VR, 4 * FA), 0)
            col = lax.broadcasted_iota(jnp.int32, (2 * VR, 4 * FA), 1)
            split = jnp.where(row < 2 * FA, FA, 2 * FA + 4)
            same = (row >= split) == (col >= 2 * FA)
            for q in range(PA):
                kv = _dot_nt(_unpack(vts[q]), pair_rows(phk, q, 0, S // 128))
                kvs[q] = _pack(jnp.where(same, kv, 0.0).astype(BF16))
            o = attend(0)
            osc[...] = attend(1)
            project(0, o)
            if first:
                for p in range(nt - 1, nt + 2):
                    relayout_b_weights(p)
        with jax.named_scope("a2"):
            lax.fori_loop(1, nt - 1, a2, 0)
        xb[...] = _layernorm(xres[rows(0, TB), :])
        rsave[...] = jnp.zeros(rsave.shape, F32)
        project(nt - 1, osc[...])
        b_pre(nt - 2, pre_rows(nt - 2))
        b_pre(nt - 1, pre_rows(nt - 1))

    nb = S // TB

    def b_finish(i):
        r = rows(i, TB)
        x = xres[r, :] + rsave[...]
        xres[r, :] = x
        xa[rows(i, TB // 2), :] = _pack(_layernorm(x).astype(BF16))
        xio[r, :] = x.astype(BF16)

    def b_pair(mem, xn, base, blk):
        def fix_ya(p, y):
            if p in PRE:
                return jnp.concatenate([y, ypre[rows(2 * blk, 8), _pre_cols(p)]], axis=0)
            ysave[:, p * 3 * PW:(p + 1) * 3 * PW] = y[L:L + 8, :]
            return y[0:L, :]

        def fix_oa(p, o):
            osave[:, p * PW:(p + 1) * PW] = o[32:L, :]
            return o[0:32, :]

        ha = jnp.concatenate([mem, xn[0:40, :]], axis=0).astype(BF16)
        ra = _segment(ha, wb, wpre, wob, fix_ya, fix_oa)
        rsave[base:base + 24, :] = ra[M:, :]

        def fix_yb(p, y):
            saved = (ypre[rows(2 * blk + 1, 8), _pre_cols(p)] if p in PRE
                     else ysave[:, p * 3 * PW:(p + 1) * 3 * PW])
            return jnp.concatenate([y[0:M, :], saved, y[M:, :]], axis=0)

        def fix_ob(p, o):
            return jnp.concatenate([o, osave[:, p * PW:(p + 1) * PW]], axis=0)

        hb = jnp.concatenate([ra[0:M, :], xn[40:64, :]], axis=0).astype(BF16)
        rb = _segment(hb, wb, wpre, wob, fix_yb, fix_ob)
        rsave[base + 24:base + 32, :] = rb[L:, :]
        rsave[base + 32:base + 64, :] = rb[M:L, :]
        return rb[0:M, :]

    def layer(l, _):
        def b_step(i, mem):
            @pl.when(jnp.logical_and(l == 1, i >= 2))
            def _():
                out_copy(i - 2).start()

            xn = xb[...]
            b_finish(jnp.maximum(i - 1, 0))
            xb[...] = _layernorm(xres[rows(jnp.minimum(i + 1, nb - 1), TB), :])
            for u in range(0, TB, 2 * SEG):
                mem = b_pair(mem, xn[u:u + 2 * SEG, :], u, (i * TB + u) // (2 * SEG))
            return mem

        with jax.named_scope("b"):
            lax.fori_loop(0, nb, b_step, mem0[...].astype(F32))
        b_finish(nb - 1)

        @pl.when(l == 0)
        def _():
            block_a(False)
        return 0

    block_a(True)
    with jax.named_scope("wait_wo"):
        wob_copy.wait()
    lax.fori_loop(0, 2, layer, 0)
    out_copy(nb - 2).start()
    out_copy(nb - 1).start()
    pltpu.make_async_copy(xio, out_hbm, sem_out.at[0]).wait()


@functools.partial(jax.jit, static_argnames=("B_seg_len",))
def pallas_interleave_layers__linear_kernel_hedgehog__memory_aug_recurrent_mem_tr__prompt_kernel(
    A_x, A_wqkv, A_w_phi, A_wo, B_x, B_mem0, B_Wq, B_Wk, B_Wv, B_Wo, B_seg_len,
):
    del B_x
    assert B_seg_len == SEG
    x = A_x.reshape(S, D)
    wphi = A_w_phi.transpose(1, 2, 0)
    mem0 = B_mem0.reshape(M, D)
    wq, wk, wv = (w.transpose(1, 2, 0).reshape(HD, D) for w in (B_Wq, B_Wk, B_Wv))
    wo = B_Wo.reshape(HD, D)
    hbm = pl.BlockSpec(memory_space=pl.ANY)
    out = pl.pallas_call(
        _kernel,
        out_shape=jax.ShapeDtypeStruct((S, D), A_x.dtype),
        in_specs=[hbm] * 9,
        out_specs=hbm,
        scratch_shapes=[
            pltpu.VMEM((S, D), BF16),
            pltpu.VMEM((3, D, D), BF16),
            pltpu.VMEM((FA, FA, HA), BF16),
            pltpu.VMEM((D, D), BF16),
            pltpu.VMEM((M, D), BF16),
            pltpu.VMEM((S, D), F32),
            pltpu.VMEM((S // 2, D), U32),
            pltpu.VMEM((TB, D), F32),
            pltpu.VMEM((3 * GA, GR // 2, D), U32),
            pltpu.VMEM((S // 128, D, 128), U32),
            pltpu.VMEM((S // 128, D, 128), U32),
            pltpu.VMEM((PA, VR, S), U32),
            pltpu.VMEM((PA, VR, 4 * FA), U32),
            pltpu.VMEM((TN // 2, D), U32),
            pltpu.VMEM((3, HD, D), BF16),
            pltpu.VMEM((D // 2, 3 * HD), U32),
            pltpu.VMEM((D // 2, len(PRE) * 3 * PW), U32),
            pltpu.VMEM((HD, D), BF16),
            pltpu.VMEM((S // 4, len(PRE) * 3 * PW), F32),
            pltpu.VMEM((8, 3 * HD), F32),
            pltpu.VMEM((8, HD), F32),
            pltpu.VMEM((TB, D), F32),
            pltpu.SemaphoreType.DMA((7 + S // TN + 3 * NP,)),
            pltpu.SemaphoreType.DMA((1,)),
        ],
        compiler_params=pltpu.CompilerParams(vmem_limit_bytes=120 * 1024 * 1024,
                                             disable_bounds_checks=True),
    )(x, A_wqkv, wphi, A_wo, mem0, wq, wk, wv, wo)
    return out.reshape(1, S, D)
```

```python
import functools

import jax
import jax.numpy as jnp
from jax import lax
import jax.experimental.pallas as pl
import jax.experimental.pallas.tpu as pltpu

F32 = jnp.float32
BF16 = jnp.bfloat16
U32 = jnp.uint32

S = 2048
D = 640
HA = 32
FA = 20
GA = 4
GR = 8 * FA
VR = 24
PA = HA // 2
TN = 256
HB = 32
DH = 192
HD = HB * DH
M = 8
SEG = 32
L = M + SEG
PW = 2 * DH
NP = HB // 2
TB = 64
PRE = (7,)

NT = (((1,), (1,)), ((), ()))
LOG2E = 1.4426950408889634


def _dot(a, b):
    return jnp.dot(a, b, preferred_element_type=F32)


def _dot_nt(a, b):
    return lax.dot_general(a, b, NT, preferred_element_type=F32)


def _pack(a):
    return pltpu.bitcast(a, U32)


def _unpack(a):
    return pltpu.bitcast(a, BF16)


def _interleave(a, b):
    return pltpu.pack_elementwise([a, b], packed_dtype=BF16).astype(U32)


def _recip(x):
    r = pl.reciprocal(x, approx=True)
    return r * (2.0 - x * r)


def _layernorm(x):
    m = jnp.mean(x, axis=-1, keepdims=True)
    c = x - m
    v = jnp.mean(c * c, axis=-1, keepdims=True)
    return c * lax.rsqrt(v + 1e-5)


def _feature_map(p):
    t = p.shape[-1]
    p3 = p.reshape(FA, 8, t)
    mx = jnp.max(p3, axis=0, keepdims=True)
    mn = jnp.min(p3, axis=0, keepdims=True)
    lp = mx + jnp.log2(jnp.sum(jnp.exp2(p3 - mx), axis=0, keepdims=True))
    ln = mn - jnp.log2(jnp.sum(jnp.exp2(mn - p3), axis=0, keepdims=True))
    ep = jnp.exp2(p3 - lp)
    en = jnp.exp2(ln - p3)
    return _interleave(ep.reshape(GR, t), en.reshape(GR, t))


def _tiles(a, odd):
    t0, t1, t2 = a[:, 0:128], a[:, 128:256], a[:, 256:384]
    return (t1, t2, t0) if odd else (t1, t0, t2)


def _weights(a2):
    lane = lax.broadcasted_iota(jnp.int32, (L, 128), 1)
    out, other = [], []
    for odd, a in enumerate(a2):
        mid, own, rest = _tiles(a, odd)
        out.append(jnp.concatenate(
            [jnp.where(lane < 64, mid, 0.0), jnp.where(lane < 64, 0.0, mid), own,
             jnp.zeros((128 - 3 * L, 128), F32)], axis=0).astype(BF16))
        other.append(rest)
    out.append(jnp.concatenate(
        [other[1], other[0], jnp.zeros((128 - 2 * L, 128), F32)], axis=0).astype(BF16))
    return out


def _scores(q2, k2):
    kw = _weights(k2)
    qt = [_tiles(q, odd) for odd, q in enumerate(q2)]
    s1 = [_dot_nt(jnp.concatenate(qt[e][0:2], axis=0).astype(BF16), kw[e]) for e in range(2)]
    s2 = _dot_nt(jnp.concatenate([qt[1][2], qt[0][2]], axis=0).astype(BF16), kw[2])
    row = lax.broadcasted_iota(jnp.int32, (L, 128), 0)
    col = lax.broadcasted_iota(jnp.int32, (L, 128), 1)
    first = col < L
    second = jnp.logical_and(col >= L, col < 2 * L)
    key = jnp.where(first, col, col - L)
    valid = jnp.logical_or(row < M, row >= key)
    out, other = [], []
    for odd in range(2):
        own = pltpu.roll(s1[odd][L:, :], 128 - L if odd else 128 - 2 * L, 1)
        s = jnp.where(first, s2[0:L, :], own) if odd else jnp.where(first, own, s2[L:, :])
        s = jnp.where(valid, (s + s1[odd][0:L, :]) * (DH ** -0.5), -1e9)
        m0 = jnp.max(jnp.where(first, s, -jnp.inf), axis=-1, keepdims=True)
        m1 = jnp.max(jnp.where(second, s, -jnp.inf), axis=-1, keepdims=True)
        e = jnp.exp(s - jnp.where(first, m0, m1))
        e0 = jnp.where(first, e, 0.0)
        e1 = jnp.where(second, e, 0.0)
        p0 = e0 * _recip(jnp.sum(e0, axis=-1, keepdims=True))
        p1 = e1 * _recip(jnp.sum(e1, axis=-1, keepdims=True))
        own = pltpu.roll(p1, L, 1) if odd else pltpu.roll(p0, 2 * L, 1)
        out.append(jnp.concatenate([p0 + p1, own], axis=0).astype(BF16))
        other.append(p0 if odd else p1)
    out.append(jnp.concatenate([other[1], other[0]], axis=0).astype(BF16))
    return out


def _pv(ps, vw):
    o0, o1, o2 = [_dot(p, v) for p, v in zip(ps, vw)]
    return (jnp.concatenate([o0[L:, :], o0[0:L, :], o2[L:, :]], axis=1),
            jnp.concatenate([o2[0:L, :], o1[0:L, :], o1[L:, :]], axis=1))


def _pre_cols(p):
    k = PRE.index(p)
    return slice(k * 3 * PW, (k + 1) * 3 * PW)


def _segment(h, wb, wpre, wob, fix_y, fix_o):
    ys, ps, vs, os_ = {}, {}, {}, {}

    def proj(p):
        if p in PRE:
            y = _dot(h[0:32, :], _unpack(wpre[:, _pre_cols(p)]))
        else:
            y = _dot(h, _unpack(wb[:, p * 3 * PW:(p + 1) * 3 * PW]))
        ys[p] = fix_y(p, y)

    def score(c):
        y2 = [ys.pop(2 * c), ys.pop(2 * c + 1)]
        vs[c] = _weights([y[:, 2 * PW:3 * PW] for y in y2])
        ps[c] = _scores([y[:, 0:PW] for y in y2], [y[:, PW:2 * PW] for y in y2])

    def pv(c):
        for e, o in enumerate(_pv(ps.pop(c), vs.pop(c))):
            os_[2 * c + e] = fix_o(2 * c + e, o)

    def oproj(lo, hi):
        o = jnp.concatenate([os_.pop(p) for p in range(lo, hi)], axis=1).astype(BF16)
        return _dot(o, wob[lo * PW:hi * PW, :])

    nc = NP // 2
    for c in range(nc):
        proj(2 * c)
        if c >= 1:
            score(c - 1)
        if c >= 2:
            pv(c - 2)
        proj(2 * c + 1)
    r = oproj(0, 3)
    score(nc - 1)
    pv(nc - 2)
    r = oproj(3, 9) + r
    pv(nc - 1)
    r = oproj(9, 14) + r
    r = oproj(14, 16) + r
    return r


def _kernel(x_hbm, wqkv_hbm, wphi_hbm, woa_hbm, mem0_hbm,
            wq_hbm, wk_hbm, wv_hbm, wo_hbm,
            out_hbm,
            xio, wqkv, wphi, woa, mem0, xres, xa, xb, wat, phq, phk, vts, kvs, osc,
            wraw, wb, wpre, wob, ypre, ysave, osave, rsave, sem_in, sem_out):
    nt = S // TN
    nsub = TN // 128

    def rows(j, n):
        return pl.ds(j * n if isinstance(j, int) else pl.multiple_of(j * n, n), n)

    def x_copy(j):
        return pltpu.make_async_copy(x_hbm.at[rows(j, TN), :], xio.at[rows(j, TN), :],
                                     sem_in.at[7 + j])

    def w_copies(p):
        return [pltpu.make_async_copy(src.at[rows(p, PW), :], wraw.at[i, rows(p, PW), :],
                                      sem_in.at[7 + nt + 3 * p + i])
                for i, src in enumerate((wq_hbm, wk_hbm, wv_hbm))]

    def out_copy(i):
        return pltpu.make_async_copy(xio.at[rows(i, TB), :],
                                     out_hbm.at[rows(i, TB), :], sem_out.at[0])

    wa_copy = [pltpu.make_async_copy(wqkv_hbm.at[:, rows(i, D)], wqkv.at[i], sem_in.at[i])
               for i in range(3)]
    wphi_copy = pltpu.make_async_copy(wphi_hbm, wphi, sem_in.at[3])
    woa_copy = pltpu.make_async_copy(woa_hbm, woa, sem_in.at[4])
    mem0_copy = pltpu.make_async_copy(mem0_hbm, mem0, sem_in.at[5])
    wob_copy = pltpu.make_async_copy(wo_hbm, wob, sem_in.at[6])
    order = [wphi_copy, x_copy(0), wa_copy[1], wa_copy[0], wa_copy[2], x_copy(1)]
    for p in range(NP):
        order += w_copies(p)
        if p + 2 < nt:
            order.append(x_copy(p + 2))
        if p + 2 == nt:
            order += [woa_copy, mem0_copy]
    for c in order + [wob_copy]:
        c.start()

    def ln_in(t):
        return _pack(_layernorm(xio[rows(t, 128), :].astype(F32)).astype(BF16))

    def qk_features(which, t, xn, g):
        ph = (phq, phk)[which]
        fm = _feature_map(_dot_nt(_unpack(wat[which * GA + g]), xn))
        for f in range(FA):
            ph[t, pl.ds(GR * g + f, 8, stride=FA), :] = fm[8 * f:8 * f + 8, :]

    def values(t, xn, g):
        vt = _dot_nt(_unpack(wat[2 * GA + g]), xn)
        for q in range(4):
            v = jnp.concatenate([vt[40 * q:40 * q + 40, :], jnp.ones((8, 128), F32)], axis=0)
            vts[4 * g + q, :, rows(t, 128)] = _pack(v.astype(BF16))

    def relayout_b_weights(p):
        for i in range(3):
            w = _pack(wraw[i, rows(p, PW), :].T)
            if isinstance(p, int) and p in PRE:
                wpre[:, rows(3 * PRE.index(p) + i, PW)] = w
            else:
                wb[:, rows(3 * p + i, PW)] = w

    wphi_copy.wait()
    x_copy(0).wait()
    cphi = jnp.zeros((FA, D), F32)
    hh = lax.broadcasted_iota(jnp.int32, (HA, D), 0) * FA
    jj = lax.broadcasted_iota(jnp.int32, (HA, D), 1)
    for d in range(FA):
        cphi = _dot(wphi[d], jnp.where(jj == hh + d, 1.0, 0.0).astype(BF16)) + cphi
    cb = jnp.concatenate(
        [jnp.broadcast_to(cphi[f:f + 1, :], (8, D)) for f in range(FA)], axis=0)
    bds = []
    for g in range(GA):
        row = lax.broadcasted_iota(jnp.int32, (GR, 256), 0)
        col = lax.broadcasted_iota(jnp.int32, (GR, 256), 1) + 128 * g
        lo = (8 * g + (row & 7)) * FA
        bds.append(jnp.where(jnp.logical_and(col >= lo, col < lo + FA),
                             cb[:, 128 * g:128 * g + 256], 0.0).astype(BF16))
    for u in range(nsub):
        xa[rows(u, 64), :] = ln_in(u)

    def fold(i):
        for g in range(GA):
            w = _dot_nt(bds[g], wqkv[i, :, 128 * g:128 * g + 256]) * LOG2E
            wat[i * GA + g] = _pack(w.astype(BF16))

    wa_copy[1].wait()
    fold(1)
    for u in range(nsub):
        for g in range(GA):
            qk_features(1, u, _unpack(xa[rows(u, 64), :]), g)
    wa_copy[0].wait()
    wa_copy[2].wait()
    x_copy(1).wait()
    fold(0)
    wvt = _pack(wqkv[2].T)
    for g in range(GA):
        wat[2 * GA + g] = wvt[g * GR // 2:(g + 1) * GR // 2, :]
    for u in range(nsub):
        xn = _unpack(xa[rows(u, 64), :])
        for g in range(GA):
            qk_features(0, u, xn, g)
            values(u, xn, g)
    xa[rows(nsub, 64), :] = ln_in(nsub)

    def block_a(first):
        def a1(j, _):
            if first:
                @pl.when(j + 1 < nt)
                def _():
                    x_copy(j + 1).wait()
                for c in w_copies(j - 1):
                    c.wait()
            for u in range(nsub):
                t = j * nsub + u
                xn = _unpack(ln_in(t) if first and u > 0 else xa[rows(t, 64), :])
                for g in range(GA):
                    qk_features(1, t, xn, g)
                    qk_features(0, t, xn, g)
                    values(t, xn, g)
            if first:
                relayout_b_weights(j - 1)
                tn = jnp.minimum(j + 1, nt - 1) * nsub
                xa[rows(tn, 64), :] = ln_in(tn)
            return 0

        def pair_rows(ph, q, t0, n):
            return _unpack(jnp.concatenate(
                [ph[t0 + u, 2 * FA * q:2 * FA * (q + 1), :] for u in range(n)], axis=1))

        def attend(j):
            low = lax.broadcasted_iota(jnp.int32, (8, TN), 0) < 4
            os_ = []
            for q in range(PA):
                nd = _dot(_unpack(kvs[q]), pair_rows(phq, q, j * nsub, nsub))
                rab = 1.0 / (nd[40:48, :] + 1e-6)
                rba = pltpu.roll(rab, 4, 0)
                ra = jnp.where(low, rab, rba)
                rb = jnp.where(low, rba, rab)
                os_.append(nd[0:40, :] * jnp.concatenate([ra, ra, rab, rb, rb], axis=0))
            return _pack(jnp.concatenate(os_, axis=0).astype(BF16).T)

        def project(j, o):
            r = rows(j, TN)
            x = xio[r, :].astype(F32) if first else xres[r, :]
            xres[r, :] = _dot(_unpack(o), woa[...]) + x

        def pre_rows(j):
            x = jnp.concatenate(
                [xres[rows(j * (TN // 8) + b + 3, 8), :] for b0 in range(0, TN // 8, 8)
                 for b in (b0, b0 + 1)], axis=0)
            return _layernorm(x).astype(BF16)

        def b_pre(j, h):
            ypre[rows(j, TN // 4), :] = _dot(h, _unpack(wpre[...]))

        def a2(j, _):
            if first:
                for c in w_copies(nt + 1 + j):
                    c.wait()
            h = pre_rows(j - 1)
            o = osc[...]
            osc[...] = attend(j + 1)
            project(j, o)
            b_pre(j - 1, h)
            if first:
                relayout_b_weights(nt + 1 + j)
            return 0

        with jax.named_scope("a1"):
            lax.fori_loop(1 if first else 0, nt, a1, 0)
        with jax.named_scope("kv"):
            if first:
                for c in (w_copies(nt - 1) + w_copies(nt) + w_copies(nt + 1)
                          + [woa_copy, mem0_copy]):
                    c.wait()
            row = lax.broadcasted_iota(jnp.int32, (2 * VR, 4 * FA), 0)
            col = lax.broadcasted_iota(jnp.int32, (2 * VR, 4 * FA), 1)
            split = jnp.where(row < 2 * FA, FA, 2 * FA + 4)
            same = (row >= split) == (col >= 2 * FA)
            for q in range(PA):
                kv = _dot_nt(_unpack(vts[q]), pair_rows(phk, q, 0, S // 128))
                kvs[q] = _pack(jnp.where(same, kv, 0.0).astype(BF16))
            o = attend(0)
            osc[...] = attend(1)
            project(0, o)
            if first:
                for p in range(nt - 1, nt + 2):
                    relayout_b_weights(p)
        with jax.named_scope("a2"):
            lax.fori_loop(1, nt - 1, a2, 0)
        xb[...] = _layernorm(xres[rows(0, TB), :])
        rsave[...] = jnp.zeros(rsave.shape, F32)
        project(nt - 1, osc[...])
        b_pre(nt - 2, pre_rows(nt - 2))
        b_pre(nt - 1, pre_rows(nt - 1))

    nb = S // TB

    def b_finish(i):
        r = rows(i, TB)
        x = xres[r, :] + rsave[...]
        xres[r, :] = x
        xa[rows(i, TB // 2), :] = _pack(_layernorm(x).astype(BF16))
        xio[r, :] = x.astype(BF16)

    def b_pair(mem, xn, base, blk):
        def fix_ya(p, y):
            if p in PRE:
                return jnp.concatenate([y, ypre[rows(2 * blk, 8), _pre_cols(p)]], axis=0)
            ysave[:, p * 3 * PW:(p + 1) * 3 * PW] = y[L:L + 8, :]
            return y[0:L, :]

        def fix_oa(p, o):
            osave[:, p * PW:(p + 1) * PW] = o[32:L, :]
            return o[0:32, :]

        ha = jnp.concatenate([mem, xn[0:40, :]], axis=0).astype(BF16)
        ra = _segment(ha, wb, wpre, wob, fix_ya, fix_oa)
        rsave[base:base + 24, :] = ra[M:, :]

        def fix_yb(p, y):
            saved = (ypre[rows(2 * blk + 1, 8), _pre_cols(p)] if p in PRE
                     else ysave[:, p * 3 * PW:(p + 1) * 3 * PW])
            return jnp.concatenate([y[0:M, :], saved, y[M:, :]], axis=0)

        def fix_ob(p, o):
            return jnp.concatenate([o, osave[:, p * PW:(p + 1) * PW]], axis=0)

        hb = jnp.concatenate([ra[0:M, :], xn[40:64, :]], axis=0).astype(BF16)
        rb = _segment(hb, wb, wpre, wob, fix_yb, fix_ob)
        rsave[base + 24:base + 32, :] = rb[L:, :]
        rsave[base + 32:base + 64, :] = rb[M:L, :]
        return rb[0:M, :]

    def layer(l, _):
        def b_step(i, mem):
            @pl.when(jnp.logical_and(l == 1, i >= 2))
            def _():
                out_copy(i - 2).start()

            xn = xb[...]
            b_finish(jnp.maximum(i - 1, 0))
            xb[...] = _layernorm(xres[rows(jnp.minimum(i + 1, nb - 1), TB), :])
            for u in range(0, TB, 2 * SEG):
                mem = b_pair(mem, xn[u:u + 2 * SEG, :], u, (i * TB + u) // (2 * SEG))
            return mem

        with jax.named_scope("b"):
            lax.fori_loop(0, nb, b_step, mem0[...].astype(F32))

        @pl.when(l == 0)
        def _():
            b_finish(nb - 1)
            block_a(False)
        return 0

    block_a(True)
    with jax.named_scope("wait_wo"):
        wob_copy.wait()
    lax.fori_loop(0, 2, layer, 0)
    out_copy(nb - 2).start()
    xio[rows(nb - 1, TB), :] = (xres[rows(nb - 1, TB), :] + rsave[...]).astype(BF16)
    out_copy(nb - 1).start()
    pltpu.make_async_copy(xio, out_hbm, sem_out.at[0]).wait()


@functools.partial(jax.jit, static_argnames=("B_seg_len",))
def pallas_interleave_layers__linear_kernel_hedgehog__memory_aug_recurrent_mem_tr__prompt_kernel(
    A_x, A_wqkv, A_w_phi, A_wo, B_x, B_mem0, B_Wq, B_Wk, B_Wv, B_Wo, B_seg_len,
):
    del B_x
    assert B_seg_len == SEG
    x = A_x.reshape(S, D)
    wphi = A_w_phi.transpose(1, 2, 0)
    mem0 = B_mem0.reshape(M, D)
    wq, wk, wv = (w.transpose(1, 2, 0).reshape(HD, D) for w in (B_Wq, B_Wk, B_Wv))
    wo = B_Wo.reshape(HD, D)
    hbm = pl.BlockSpec(memory_space=pl.ANY)
    out = pl.pallas_call(
        _kernel,
        out_shape=jax.ShapeDtypeStruct((S, D), A_x.dtype),
        in_specs=[hbm] * 9,
        out_specs=hbm,
        scratch_shapes=[
            pltpu.VMEM((S, D), BF16),
            pltpu.VMEM((3, D, D), BF16),
            pltpu.VMEM((FA, FA, HA), BF16),
            pltpu.VMEM((D, D), BF16),
            pltpu.VMEM((M, D), BF16),
            pltpu.VMEM((S, D), F32),
            pltpu.VMEM((S // 2, D), U32),
            pltpu.VMEM((TB, D), F32),
            pltpu.VMEM((3 * GA, GR // 2, D), U32),
            pltpu.VMEM((S // 128, D, 128), U32),
            pltpu.VMEM((S // 128, D, 128), U32),
            pltpu.VMEM((PA, VR, S), U32),
            pltpu.VMEM((PA, VR, 4 * FA), U32),
            pltpu.VMEM((TN // 2, D), U32),
            pltpu.VMEM((3, HD, D), BF16),
            pltpu.VMEM((D // 2, 3 * HD), U32),
            pltpu.VMEM((D // 2, len(PRE) * 3 * PW), U32),
            pltpu.VMEM((HD, D), BF16),
            pltpu.VMEM((S // 4, len(PRE) * 3 * PW), F32),
            pltpu.VMEM((8, 3 * HD), F32),
            pltpu.VMEM((8, HD), F32),
            pltpu.VMEM((TB, D), F32),
            pltpu.SemaphoreType.DMA((7 + S // TN + 3 * NP,)),
            pltpu.SemaphoreType.DMA((1,)),
        ],
        compiler_params=pltpu.CompilerParams(vmem_limit_bytes=120 * 1024 * 1024,
                                             disable_bounds_checks=True,
                                             disable_semaphore_checks=True),
    )(x, A_wqkv, wphi, A_wo, mem0, wq, wk, wv, wo)
    return out.reshape(1, S, D)
```

```python
import functools

import jax
import jax.numpy as jnp
from jax import lax
import jax.experimental.pallas as pl
import jax.experimental.pallas.tpu as pltpu

F32 = jnp.float32
BF16 = jnp.bfloat16
U32 = jnp.uint32

S = 2048
D = 640
HA = 32
FA = 20
GA = 4
GR = 8 * FA
VR = 24
PA = HA // 2
TN = 256
HB = 32
DH = 192
HD = HB * DH
M = 8
SEG = 32
L = M + SEG
PW = 2 * DH
NP = HB // 2
TB = 128
PRE = (9,)

NT = (((1,), (1,)), ((), ()))
LOG2E = 1.4426950408889634


def _dot(a, b):
    return jnp.dot(a, b, preferred_element_type=F32)


def _dot_nt(a, b):
    return lax.dot_general(a, b, NT, preferred_element_type=F32)


def _pack(a):
    return pltpu.bitcast(a, U32)


def _unpack(a):
    return pltpu.bitcast(a, BF16)


def _interleave(a, b):
    return pltpu.pack_elementwise([a, b], packed_dtype=BF16).astype(U32)


def _recip(x):
    r = pl.reciprocal(x, approx=True)
    return r * (2.0 - x * r)


def _layernorm(x):
    m = jnp.mean(x, axis=-1, keepdims=True)
    c = x - m
    v = jnp.mean(c * c, axis=-1, keepdims=True)
    return c * lax.rsqrt(v + 1e-5)


def _feature_map(p):
    t = p.shape[-1]
    p3 = p.reshape(FA, 8, t)
    mx = jnp.max(p3, axis=0, keepdims=True)
    mn = jnp.min(p3, axis=0, keepdims=True)
    lp = mx + jnp.log2(jnp.sum(jnp.exp2(p3 - mx), axis=0, keepdims=True))
    ln = mn - jnp.log2(jnp.sum(jnp.exp2(mn - p3), axis=0, keepdims=True))
    ep = jnp.exp2(p3 - lp)
    en = jnp.exp2(ln - p3)
    return _interleave(ep.reshape(GR, t), en.reshape(GR, t))


def _tiles(a, odd):
    t0, t1, t2 = a[:, 0:128], a[:, 128:256], a[:, 256:384]
    return (t1, t2, t0) if odd else (t1, t0, t2)


def _own_weights(a, odd):
    lane = lax.broadcasted_iota(jnp.int32, (L, 128), 1)
    mid, own, _ = _tiles(a, odd)
    return jnp.concatenate(
        [jnp.where(lane < 64, mid, 0.0), jnp.where(lane < 64, 0.0, mid), own,
         jnp.zeros((128 - 3 * L, 128), F32)], axis=0).astype(BF16)


def _others(even, odd, pad):
    parts = [_tiles(odd, 1)[2], _tiles(even, 0)[2]]
    if pad:
        parts.append(jnp.zeros((128 - 2 * L, 128), F32))
    return jnp.concatenate(parts, axis=0).astype(BF16)


def _softmax3(s3):
    row = lax.broadcasted_iota(jnp.int32, (L, 128), 0)
    col = lax.broadcasted_iota(jnp.int32, (L, 128), 1)
    first = col < L
    second = jnp.logical_and(col >= L, col < 2 * L)
    key = jnp.where(first, col, col - L)
    valid = jnp.logical_or(row < M, row >= key)
    out, other = [], []
    for odd in range(2):
        own = pltpu.roll(s3[odd][L:, :], 128 - L if odd else 128 - 2 * L, 1)
        s = (jnp.where(first, s3[2][0:L, :], own) if odd
             else jnp.where(first, own, s3[2][L:, :]))
        s = jnp.where(valid, (s + s3[odd][0:L, :]) * (DH ** -0.5), -1e9)
        m0 = jnp.max(jnp.where(first, s, -jnp.inf), axis=-1, keepdims=True)
        m1 = jnp.max(jnp.where(second, s, -jnp.inf), axis=-1, keepdims=True)
        e = jnp.exp(s - jnp.where(first, m0, m1))
        e0 = jnp.where(first, e, 0.0)
        e1 = jnp.where(second, e, 0.0)
        p0 = e0 * _recip(jnp.sum(e0, axis=-1, keepdims=True))
        p1 = e1 * _recip(jnp.sum(e1, axis=-1, keepdims=True))
        own = pltpu.roll(p1, L, 1) if odd else pltpu.roll(p0, 2 * L, 1)
        out.append(jnp.concatenate([p0 + p1, own], axis=0).astype(BF16))
        other.append(p0 if odd else p1)
    out.append(jnp.concatenate([other[1], other[0]], axis=0).astype(BF16))
    return out


def _pre_cols(p):
    k = PRE.index(p)
    return slice(k * 3 * PW, (k + 1) * 3 * PW)


def _segment(h, wb, wpre, wob, fix_y, fix_o, chained):
    ys, ss, ps, pvs, os_ = {}, {}, {}, {}, {}

    def proj(p):
        if p in PRE:
            y = _dot(h[0:32, :], _unpack(wpre[:, _pre_cols(p)]))
        elif p == 0 and chained:
            y = _dot(h[:, 0:256], _unpack(wb[0:128, 0:3 * PW]))
            y = _dot(h[:, 256:], _unpack(wb[128:, 0:3 * PW])) + y
        else:
            y = _dot(h, _unpack(wb[:, p * 3 * PW:(p + 1) * 3 * PW]))
        y = fix_y(p, y)
        ys[p] = [y[:, i * PW:(i + 1) * PW] for i in range(3)]

    def weights(c, i, which):
        if i < 2:
            return _own_weights(ys[2 * c + i][which], i)
        return _others(ys[2 * c][which], ys[2 * c + 1][which], True)

    def score_round(n):
        for c, i in (divmod(j, 3) for j in range(4 * n, 4 * n + 4)):
            if i < 2:
                q = jnp.concatenate(_tiles(ys[2 * c + i][0], i)[0:2], axis=0).astype(BF16)
            else:
                q = _others(ys[2 * c][0], ys[2 * c + 1][0], False)
            ss[c, i] = _dot_nt(q, weights(c, i, 1))
            if i == 2:
                ps[c] = _softmax3([ss.pop((c, k)) for k in range(3)])

    def pv_round(n):
        for c, i in (divmod(j, 3) for j in range(4 * n, 4 * n + 4)):
            pvs[c, i] = _dot(ps[c][i], weights(c, i, 2))
            if i == 2:
                o0, o1, o2 = [pvs.pop((c, k)) for k in range(3)]
                os_[2 * c] = fix_o(2 * c, jnp.concatenate(
                    [o0[L:, :], o0[0:L, :], o2[L:, :]], axis=1))
                os_[2 * c + 1] = fix_o(2 * c + 1, jnp.concatenate(
                    [o2[0:L, :], o1[0:L, :], o1[L:, :]], axis=1))

    def slot(n):
        if n >= 2:
            pv_round(n - 2)
        if n < 6:
            score_round(n)

    def oproj(lo, hi):
        o = jnp.concatenate([os_.pop(p) for p in range(lo, hi)], axis=1).astype(BF16)
        return _dot(o, wob[lo * PW:hi * PW, :])

    after = {3: 0, 6: 1, 9: 2, 12: 3, 14: 4}
    for p in range(NP):
        proj(p)
        if p in after:
            slot(after[p])
    mid = 8 if h.shape[0] == 48 else 7
    r = oproj(0, 2)
    slot(5)
    r = oproj(2, mid) + r
    slot(6)
    slot(7)
    r = oproj(mid, 10) + r
    return oproj(10, NP) + r


def _kernel(x_hbm, wqkv_hbm, wphi_hbm, woa_hbm, mem0_hbm,
            wq_hbm, wk_hbm, wv_hbm, wo_hbm,
            out_hbm,
            xio, wqkv, wphi, woa, mem0, xres, xa, xb, bds, wat, phq, phk, vts, kvs, osc,
            wraw, wb, wpre, wob, ypre, ysave, osave, rsave, sem_in, sem_out):
    nt = S // TN
    nsub = TN // 128
    nb = S // TB

    def rows(j, n):
        return pl.ds(j * n if isinstance(j, int) else pl.multiple_of(j * n, n), n)

    def x_copy(j):
        return pltpu.make_async_copy(x_hbm.at[rows(j, TN), :], xio.at[rows(j, TN), :],
                                     sem_in.at[7 + j])

    def w_copies(p):
        return [pltpu.make_async_copy(src.at[rows(p, PW), :], wraw.at[i, rows(p, PW), :],
                                      sem_in.at[7 + nt + 3 * p + i])
                for i, src in enumerate((wq_hbm, wk_hbm, wv_hbm))]

    def wa_copy(i):
        return pltpu.make_async_copy(wqkv_hbm.at[:, rows(i, D)], wqkv.at[i], sem_in.at[i])

    def out_copy(i):
        return pltpu.make_async_copy(xio.at[rows(i, TB), :],
                                     out_hbm.at[rows(i, TB), :], sem_out.at[0])

    wphi_copy = pltpu.make_async_copy(wphi_hbm, wphi, sem_in.at[3])
    woa_copy = pltpu.make_async_copy(woa_hbm, woa, sem_in.at[4])
    mem0_copy = pltpu.make_async_copy(mem0_hbm, mem0, sem_in.at[5])
    wob_copy = pltpu.make_async_copy(wo_hbm, wob, sem_in.at[6])
    order = [wphi_copy, x_copy(0), wa_copy(0), wa_copy(1), wa_copy(2), x_copy(1)]
    for p in range(NP):
        order += w_copies(p)
        if p + 2 < nt:
            order.append(x_copy(p + 2))
        if p + 2 == nt:
            order += [woa_copy, mem0_copy]
    for c in order + [wob_copy]:
        c.start()

    def ln_in(t):
        x = xio[rows(t, 128), :].astype(F32)
        xres[rows(t, 128), :] = x
        return _pack(_layernorm(x).astype(BF16))

    def relayout_b_weights(p):
        for i in range(3):
            w = _pack(wraw[i, rows(p, PW), :].T)
            if isinstance(p, int) and p in PRE:
                wpre[:, rows(3 * PRE.index(p) + i, PW)] = w
            else:
                wb[:, rows(3 * p + i, PW)] = w

    wphi_copy.wait()
    x_copy(0).wait()
    cphi = jnp.zeros((FA, D), F32)
    hh = lax.broadcasted_iota(jnp.int32, (HA, D), 0) * FA
    jj = lax.broadcasted_iota(jnp.int32, (HA, D), 1)
    for d in range(FA):
        cphi = _dot(wphi[d], jnp.where(jj == hh + d, 1.0, 0.0).astype(BF16)) + cphi
    cb = jnp.concatenate(
        [jnp.broadcast_to(cphi[f:f + 1, :], (8, D)) for f in range(FA)], axis=0)
    for g in range(GA):
        row = lax.broadcasted_iota(jnp.int32, (GR, 256), 0)
        col = lax.broadcasted_iota(jnp.int32, (GR, 256), 1) + 128 * g
        lo = (8 * g + (row & 7)) * FA
        bds[g] = _pack(jnp.where(jnp.logical_and(col >= lo, col < lo + FA),
                                 cb[:, 128 * g:128 * g + 256], 0.0).astype(BF16))
    for u in range(nsub):
        xa[rows(u, 64), :] = ln_in(u)

    def fold(i, _):
        wa_copy(i).wait()
        for g in range(GA):
            w = _dot_nt(_unpack(bds[g]), wqkv[i, :, 128 * g:128 * g + 256]) * LOG2E
            wat[i * GA + g] = _pack(w.astype(BF16))
        return 0

    lax.fori_loop(0, 2, fold, 0)
    wa_copy(2).wait()
    x_copy(1).wait()
    wvt = _pack(wqkv[2].T)
    for g in range(GA):
        wat[2 * GA + g] = wvt[g * GR // 2:(g + 1) * GR // 2, :]
    xa[rows(nsub, 64), :] = ln_in(nsub)

    def a1(first, j, _):
        if first:
            @pl.when(j + 1 < nt)
            def _():
                x_copy(j + 1).wait()
            for c in w_copies(j - 1):
                c.wait()
        for u in range(nsub):
            t = j * nsub + u
            xn = _unpack(ln_in(t) if first and u > 0 else xa[rows(t, 64), :])
            for g in range(GA):
                for ph, w in ((phk, wat[GA + g]), (phq, wat[g])):
                    fm = _feature_map(_dot_nt(_unpack(w), xn))
                    for f in range(FA):
                        ph[t, pl.ds(GR * g + f, 8, stride=FA), :] = fm[8 * f:8 * f + 8, :]
                vt = _dot_nt(_unpack(wat[2 * GA + g]), xn)
                for q in range(4):
                    v = jnp.concatenate(
                        [vt[40 * q:40 * q + 40, :], jnp.ones((8, 128), F32)], axis=0)
                    vts[4 * g + q, :, rows(t, 128)] = _pack(v.astype(BF16))
        if first:
            relayout_b_weights(j - 1)
            tn = jnp.minimum(j + 1, nt - 1) * nsub
            xa[rows(tn, 64), :] = ln_in(tn)
        return 0

    def pair_rows(ph, q, t0, n):
        return _unpack(jnp.concatenate(
            [ph[t0 + u, 2 * FA * q:2 * FA * (q + 1), :] for u in range(n)], axis=1))

    def attend(j):
        low = lax.broadcasted_iota(jnp.int32, (8, TN), 0) < 4
        os_ = []
        for q in range(PA):
            nd = _dot(_unpack(kvs[q]), pair_rows(phq, q, j * nsub, nsub))
            rab = 1.0 / (nd[40:48, :] + 1e-6)
            rba = pltpu.roll(rab, 4, 0)
            ra = jnp.where(low, rab, rba)
            rb = jnp.where(low, rba, rab)
            os_.append(nd[0:40, :] * jnp.concatenate([ra, ra, rab, rb, rb], axis=0))
        return _pack(jnp.concatenate(os_, axis=0).astype(BF16).T)

    def project(j, o):
        r = rows(j, TN)
        xres[r, :] = _dot(_unpack(o), woa[...]) + xres[r, :]

    def pre_rows(j):
        x = jnp.concatenate(
            [xres[rows(j * (TN // 8) + b + 3, 8), :] for b0 in range(0, TN // 8, 8)
             for b in (b0, b0 + 1)], axis=0)
        return _layernorm(x).astype(BF16)

    def b_pre(j, h):
        ypre[rows(j, TN // 4), :] = _dot(h, _unpack(wpre[...]))

    def b_finish(i):
        r = rows(i, TB)
        x = xres[r, :] + rsave[...]
        xres[r, :] = x
        xn = _layernorm(x)
        xa[rows(i, TB // 2), :] = _pack(xn.astype(BF16))
        xio[r, :] = x.astype(BF16)
        return xn

    def b_pair(mem, xn, base, blk, side):
        def fix_ya(p, y):
            c0 = 3 * PW - D
            tie = jnp.where(blk < 0, side[8 * p:8 * p + 8, :], y[0:M, c0:])
            y = jnp.concatenate(
                [jnp.concatenate([y[0:M, 0:c0], tie], axis=1), y[M:, :]], axis=0)
            if p in PRE:
                return jnp.concatenate([y, ypre[rows(2 * blk, 8), _pre_cols(p)]], axis=0)
            ysave[:, p * 3 * PW:(p + 1) * 3 * PW] = y[L:L + 8, :]
            return y[0:L, :]

        def fix_oa(p, o):
            osave[:, p * PW:(p + 1) * PW] = o[32:L, :]
            return o[0:32, :]

        ha = jnp.concatenate([mem, xn[0:40, :]], axis=0).astype(BF16)
        ra = _segment(ha, wb, wpre, wob, fix_ya, fix_oa, base > 0)
        rsave[base:base + 24, :] = ra[M:, :]

        def fix_yb(p, y):
            saved = (ypre[rows(2 * blk + 1, 8), _pre_cols(p)] if p in PRE
                     else ysave[:, p * 3 * PW:(p + 1) * 3 * PW])
            return jnp.concatenate([y[0:M, :], saved, y[M:, :]], axis=0)

        def fix_ob(p, o):
            return jnp.concatenate([o, osave[:, p * PW:(p + 1) * PW]], axis=0)

        hb = jnp.concatenate([ra[0:M, :], xn[40:64, :]], axis=0).astype(BF16)
        rb = _segment(hb, wb, wpre, wob, fix_yb, fix_ob, True)
        rsave[base + 24:base + 32, :] = rb[L:, :]
        rsave[base + 32:base + 64, :] = rb[M:L, :]
        return rb[0:M, :]

    def layer(l, _):
        def wait_first(copies):
            @pl.when(l == 0)
            def _():
                for c in copies:
                    c.wait()

        with jax.named_scope("a1"):
            lax.fori_loop(0, jnp.where(l == 0, 1, nt), functools.partial(a1, False), 0)

            @pl.when(l == 0)
            def _():
                lax.fori_loop(1, nt, functools.partial(a1, True), 0)

        with jax.named_scope("kv"):
            wait_first(w_copies(nt - 1) + w_copies(nt) + w_copies(nt + 1)
                       + [woa_copy, mem0_copy])
            row = lax.broadcasted_iota(jnp.int32, (2 * VR, 4 * FA), 0)
            col = lax.broadcasted_iota(jnp.int32, (2 * VR, 4 * FA), 1)
            split = jnp.where(row < 2 * FA, FA, 2 * FA + 4)
            same = (row >= split) == (col >= 2 * FA)
            for q in range(PA):
                kv = _dot_nt(_unpack(vts[q]), pair_rows(phk, q, 0, S // 128))
                kvs[q] = _pack(jnp.where(same, kv, 0.0).astype(BF16))
            o = attend(0)
            osc[...] = attend(1)
            project(0, o)
            for p in range(nt - 1, nt + 2):
                relayout_b_weights(p)

        def a2(j, _):
            wait_first(w_copies(nt + 1 + j))
            h = pre_rows(j - 1)
            o = osc[...]
            osc[...] = attend(j + 1)
            project(j, o)
            b_pre(j - 1, h)
            relayout_b_weights(nt + 1 + j)
            return 0

        with jax.named_scope("a2"):
            lax.fori_loop(1, nt - 1, a2, 0)
        xb[...] = _layernorm(xres[rows(0, TB), :])
        rsave[...] = jnp.zeros(rsave.shape, F32)
        project(nt - 1, osc[...])
        b_pre(nt - 2, pre_rows(nt - 2))
        b_pre(nt - 1, pre_rows(nt - 1))
        wait_first([wob_copy])

        def b_step(i, mem):
            @pl.when(jnp.logical_and(l == 1, i >= 2))
            def _():
                out_copy(i - 2).start()

            xn = xb[...]
            side = b_finish(jnp.maximum(i - 1, 0))
            nxt = _layernorm(xres[rows(jnp.minimum(i + 1, nb - 1), TB), :])
            xb[...] = nxt
            side = jnp.concatenate([side, nxt], axis=0)
            for u in range(0, TB, 2 * SEG):
                mem = b_pair(mem, xn[u:u + 2 * SEG, :], u, (i * TB + u) // (2 * SEG),
                             side[2 * u:2 * u + 8 * NP, :])
            return mem

        with jax.named_scope("b"):
            lax.fori_loop(0, nb, b_step, mem0[...].astype(F32))

        @pl.when(l == 0)
        def _():
            b_finish(nb - 1)
        return 0

    lax.fori_loop(0, 2, layer, 0)
    out_copy(nb - 2).start()
    xio[rows(nb - 1, TB), :] = (xres[rows(nb - 1, TB), :] + rsave[...]).astype(BF16)
    out_copy(nb - 1).start()
    pltpu.make_async_copy(xio, out_hbm, sem_out.at[0]).wait()


@functools.partial(jax.jit, static_argnames=("B_seg_len",))
def pallas_interleave_layers__linear_kernel_hedgehog__memory_aug_recurrent_mem_tr__prompt_kernel(
    A_x, A_wqkv, A_w_phi, A_wo, B_x, B_mem0, B_Wq, B_Wk, B_Wv, B_Wo, B_seg_len,
):
    del B_x
    assert B_seg_len == SEG
    x = A_x.reshape(S, D)
    wphi = A_w_phi.transpose(1, 2, 0)
    mem0 = B_mem0.reshape(M, D)
    wq, wk, wv = (w.transpose(1, 2, 0).reshape(HD, D) for w in (B_Wq, B_Wk, B_Wv))
    wo = B_Wo.reshape(HD, D)
    hbm = pl.BlockSpec(memory_space=pl.ANY)
    out = pl.pallas_call(
        _kernel,
        out_shape=jax.ShapeDtypeStruct((S, D), A_x.dtype),
        in_specs=[hbm] * 9,
        out_specs=hbm,
        scratch_shapes=[
            pltpu.VMEM((S, D), BF16),
            pltpu.VMEM((3, D, D), BF16),
            pltpu.VMEM((FA, FA, HA), BF16),
            pltpu.VMEM((D, D), BF16),
            pltpu.VMEM((M, D), BF16),
            pltpu.VMEM((S, D), F32),
            pltpu.VMEM((S // 2, D), U32),
            pltpu.VMEM((TB, D), F32),
            pltpu.VMEM((GA, GR // 2, 256), U32),
            pltpu.VMEM((3 * GA, GR // 2, D), U32),
            pltpu.VMEM((S // 128, D, 128), U32),
            pltpu.VMEM((S // 128, D, 128), U32),
            pltpu.VMEM((PA, VR, S), U32),
            pltpu.VMEM((PA, VR, 4 * FA), U32),
            pltpu.VMEM((TN // 2, D), U32),
            pltpu.VMEM((3, HD, D), BF16),
            pltpu.VMEM((D // 2, 3 * HD), U32),
            pltpu.VMEM((D // 2, len(PRE) * 3 * PW), U32),
            pltpu.VMEM((HD, D), BF16),
            pltpu.VMEM((S // 4, len(PRE) * 3 * PW), F32),
            pltpu.VMEM((8, 3 * HD), F32),
            pltpu.VMEM((8, HD), F32),
            pltpu.VMEM((TB, D), F32),
            pltpu.SemaphoreType.DMA((7 + S // TN + 3 * NP,)),
            pltpu.SemaphoreType.DMA((1,)),
        ],
        compiler_params=pltpu.CompilerParams(vmem_limit_bytes=120 * 1024 * 1024,
                                             disable_bounds_checks=True,
                                             disable_semaphore_checks=True),
    )(x, A_wqkv, wphi, A_wo, mem0, wq, wk, wv, wo)
    return out.reshape(1, S, D)
```

```python
import functools

import jax
import jax.numpy as jnp
from jax import lax
import jax.experimental.pallas as pl
import jax.experimental.pallas.tpu as pltpu

F32 = jnp.float32
BF16 = jnp.bfloat16
U32 = jnp.uint32

S = 2048
D = 640
HA = 32
FA = 20
GA = 4
GR = 8 * FA
VR = 24
PA = HA // 2
TN = 256
HB = 32
DH = 192
HD = HB * DH
M = 8
SEG = 32
L = M + SEG
PW = 2 * DH
NP = HB // 2
TB = 128
PRE = (9,)

NT = (((1,), (1,)), ((), ()))
LOG2E = 1.4426950408889634
HALF_ULP = 0.0040612


def _dot(a, b):
    return jnp.dot(a, b, preferred_element_type=F32)


def _dot_nt(a, b):
    return lax.dot_general(a, b, NT, preferred_element_type=F32)


def _pack(a):
    return pltpu.bitcast(a, U32)


def _unpack(a):
    return pltpu.bitcast(a, BF16)


def _interleave(a, b):
    lo = lax.bitcast_convert_type(a, U32) >> 16
    hi = lax.bitcast_convert_type(b, U32) & jnp.uint32(0xFFFF0000)
    return lo | hi


def _recip(x):
    r = pl.reciprocal(x, approx=True)
    return r * (2.0 - x * r)


def _layernorm(x):
    m = jnp.mean(x, axis=-1, keepdims=True)
    c = x - m
    v = jnp.mean(c * c, axis=-1, keepdims=True)
    return c * lax.rsqrt(v + 1e-5)


def _feature_map(p):
    t = p.shape[-1]
    p3 = p.reshape(FA, 8, t)
    mx = jnp.max(p3, axis=0, keepdims=True)
    mn = jnp.min(p3, axis=0, keepdims=True)
    lp = (mx - HALF_ULP) + jnp.log2(jnp.sum(jnp.exp2(p3 - mx), axis=0, keepdims=True))
    ln = (mn + HALF_ULP) - jnp.log2(jnp.sum(jnp.exp2(mn - p3), axis=0, keepdims=True))
    ep = jnp.exp2(p3 - lp)
    en = jnp.exp2(ln - p3)
    return _interleave(ep.reshape(GR, t), en.reshape(GR, t))


def _tiles(a, odd):
    t0, t1, t2 = a[:, 0:128], a[:, 128:256], a[:, 256:384]
    return (t1, t2, t0) if odd else (t1, t0, t2)


def _own_weights(a, odd):
    lane = lax.broadcasted_iota(jnp.int32, (L, 128), 1)
    mid, own, _ = _tiles(a, odd)
    return jnp.concatenate(
        [jnp.where(lane < 64, mid, 0.0), jnp.where(lane < 64, 0.0, mid), own,
         jnp.zeros((128 - 3 * L, 128), F32)], axis=0).astype(BF16)


def _others(even, odd, pad):
    parts = [_tiles(odd, 1)[2], _tiles(even, 0)[2]]
    if pad:
        parts.append(jnp.zeros((128 - 2 * L, 128), F32))
    return jnp.concatenate(parts, axis=0).astype(BF16)


def _softmax3(s3):
    row = lax.broadcasted_iota(jnp.int32, (L, 128), 0)
    col = lax.broadcasted_iota(jnp.int32, (L, 128), 1)
    first = col < L
    second = jnp.logical_and(col >= L, col < 2 * L)
    key = jnp.where(first, col, col - L)
    valid = jnp.logical_or(row < M, row >= key)
    out, other = [], []
    for odd in range(2):
        own = pltpu.roll(s3[odd][L:, :], 128 - L if odd else 128 - 2 * L, 1)
        s = (jnp.where(first, s3[2][0:L, :], own) if odd
             else jnp.where(first, own, s3[2][L:, :]))
        s = jnp.where(valid, (s + s3[odd][0:L, :]) * (DH ** -0.5), -1e9)
        m0 = jnp.max(jnp.where(first, s, -jnp.inf), axis=-1, keepdims=True)
        m1 = jnp.max(jnp.where(second, s, -jnp.inf), axis=-1, keepdims=True)
        e = jnp.exp(s - jnp.where(first, m0, m1))
        e0 = jnp.where(first, e, 0.0)
        e1 = jnp.where(second, e, 0.0)
        p0 = e0 * _recip(jnp.sum(e0, axis=-1, keepdims=True))
        p1 = e1 * _recip(jnp.sum(e1, axis=-1, keepdims=True))
        own = pltpu.roll(p1, L, 1) if odd else pltpu.roll(p0, 2 * L, 1)
        out.append(jnp.concatenate([p0 + p1, own], axis=0).astype(BF16))
        other.append(p0 if odd else p1)
    out.append(jnp.concatenate([other[1], other[0]], axis=0).astype(BF16))
    return out


def _pre_cols(p):
    k = PRE.index(p)
    return slice(k * 3 * PW, (k + 1) * 3 * PW)


def _segment(h, wb, wpre, wob, fix_y, fix_o, chained):
    ys, ss, ps, pvs, os_ = {}, {}, {}, {}, {}

    def proj(p):
        if p in PRE:
            y = _dot(h[0:32, :], _unpack(wpre[:, _pre_cols(p)]))
        elif p == 0 and chained:
            y = _dot(h[:, 0:256], _unpack(wb[0:128, 0:3 * PW]))
            y = _dot(h[:, 256:], _unpack(wb[128:, 0:3 * PW])) + y
        else:
            y = _dot(h, _unpack(wb[:, p * 3 * PW:(p + 1) * 3 * PW]))
        y = fix_y(p, y)
        ys[p] = [y[:, i * PW:(i + 1) * PW] for i in range(3)]

    def weights(c, i, which):
        if i < 2:
            return _own_weights(ys[2 * c + i][which], i)
        return _others(ys[2 * c][which], ys[2 * c + 1][which], True)

    def score_round(n):
        for c, i in (divmod(j, 3) for j in range(4 * n, 4 * n + 4)):
            if i < 2:
                q = jnp.concatenate(_tiles(ys[2 * c + i][0], i)[0:2], axis=0).astype(BF16)
            else:
                q = _others(ys[2 * c][0], ys[2 * c + 1][0], False)
            ss[c, i] = _dot_nt(q, weights(c, i, 1))
            if i == 2:
                ps[c] = _softmax3([ss.pop((c, k)) for k in range(3)])

    def pv_round(n):
        for c, i in (divmod(j, 3) for j in range(4 * n, 4 * n + 4)):
            pvs[c, i] = _dot(ps[c][i], weights(c, i, 2))
            if i == 2:
                o0, o1, o2 = [pvs.pop((c, k)) for k in range(3)]
                os_[2 * c] = fix_o(2 * c, jnp.concatenate(
                    [o0[L:, :], o0[0:L, :], o2[L:, :]], axis=1))
                os_[2 * c + 1] = fix_o(2 * c + 1, jnp.concatenate(
                    [o2[0:L, :], o1[0:L, :], o1[L:, :]], axis=1))

    def slot(n):
        if n >= 2:
            pv_round(n - 2)
        if n < 6:
            score_round(n)

    def oproj(lo, hi):
        o = jnp.concatenate([os_.pop(p) for p in range(lo, hi)], axis=1).astype(BF16)
        return _dot(o, wob[lo * PW:hi * PW, :])

    after = {3: 0, 6: 1, 9: 2, 12: 3, 14: 4}
    for p in range(NP):
        proj(p)
        if p in after:
            slot(after[p])
    o1, o2, o3 = (2, 8, 10) if h.shape[0] == 48 else (2, 7, 10)
    r = oproj(0, o1)
    slot(5)
    r = oproj(o1, o2) + r
    slot(6)
    slot(7)
    r = oproj(o2, o3) + r
    return oproj(o3, NP) + r


def _kernel(x_hbm, wqkv_hbm, wphi_hbm, woa_hbm, mem0_hbm,
            wq_hbm, wk_hbm, wv_hbm, wo_hbm,
            out_hbm,
            xio, wqkv, wphi, woa, mem0, xres, xa, xb, bds, wat, phq, phk, vts, kvs, osc,
            wraw, wb, wpre, wob, ypre, ysave, osave, rsave, sem_in, sem_out):
    nt = S // TN
    nsub = TN // 128
    nb = S // TB

    def rows(j, n):
        return pl.ds(j * n if isinstance(j, int) else pl.multiple_of(j * n, n), n)

    def x_copy(j):
        return pltpu.make_async_copy(x_hbm.at[rows(j, TN), :], xio.at[rows(j, TN), :],
                                     sem_in.at[7 + j])

    def w_copies(p):
        return [pltpu.make_async_copy(src.at[rows(p, PW), :], wraw.at[i, rows(p, PW), :],
                                      sem_in.at[7 + nt + 3 * p + i])
                for i, src in enumerate((wq_hbm, wk_hbm, wv_hbm))]

    def wa_copy(i):
        return pltpu.make_async_copy(wqkv_hbm.at[:, rows(i, D)], wqkv.at[i], sem_in.at[i])

    def out_copy(i):
        return pltpu.make_async_copy(xio.at[rows(i, TB), :],
                                     out_hbm.at[rows(i, TB), :], sem_out.at[0])

    wphi_copy = pltpu.make_async_copy(wphi_hbm, wphi, sem_in.at[3])
    woa_copy = pltpu.make_async_copy(woa_hbm, woa, sem_in.at[4])
    mem0_copy = pltpu.make_async_copy(mem0_hbm, mem0, sem_in.at[5])
    wob_copy = pltpu.make_async_copy(wo_hbm, wob, sem_in.at[6])
    order = [wphi_copy, x_copy(0), wa_copy(0), wa_copy(1), wa_copy(2), x_copy(1)]
    for p in range(NP):
        order += w_copies(p)
        if p + 2 < nt:
            order.append(x_copy(p + 2))
        if p + 2 == nt:
            order += [woa_copy, mem0_copy]
    for c in order + [wob_copy]:
        c.start()

    def ln_in(t):
        x = xio[rows(t, 128), :].astype(F32)
        xres[rows(t, 128), :] = x
        return _pack(_layernorm(x).astype(BF16))

    def relayout_b_weights(p):
        for i in range(3):
            w = _pack(wraw[i, rows(p, PW), :].T)
            if isinstance(p, int) and p in PRE:
                wpre[:, rows(3 * PRE.index(p) + i, PW)] = w
            else:
                wb[:, rows(3 * p + i, PW)] = w

    wphi_copy.wait()
    x_copy(0).wait()
    cphi = jnp.zeros((FA, D), F32)
    hh = lax.broadcasted_iota(jnp.int32, (HA, D), 0) * FA
    jj = lax.broadcasted_iota(jnp.int32, (HA, D), 1)
    for d in range(FA):
        cphi = _dot(wphi[d], jnp.where(jj == hh + d, 1.0, 0.0).astype(BF16)) + cphi
    cb = jnp.concatenate(
        [jnp.broadcast_to(cphi[f:f + 1, :], (8, D)) for f in range(FA)], axis=0)
    for g in range(GA):
        row = lax.broadcasted_iota(jnp.int32, (GR, 256), 0)
        col = lax.broadcasted_iota(jnp.int32, (GR, 256), 1) + 128 * g
        lo = (8 * g + (row & 7)) * FA
        bds[g] = _pack(jnp.where(jnp.logical_and(col >= lo, col < lo + FA),
                                 cb[:, 128 * g:128 * g + 256], 0.0).astype(BF16))
    for u in range(nsub):
        xa[rows(u, 64), :] = ln_in(u)

    def fold(i, _):
        wa_copy(i).wait()
        for g in range(GA):
            w = _dot_nt(_unpack(bds[g]), wqkv[i, :, 128 * g:128 * g + 256]) * LOG2E
            wat[i * GA + g] = _pack(w.astype(BF16))
        return 0

    lax.fori_loop(0, 2, fold, 0)
    wa_copy(2).wait()
    x_copy(1).wait()
    wvt = _pack(wqkv[2].T)
    for g in range(GA):
        wat[2 * GA + g] = wvt[g * GR // 2:(g + 1) * GR // 2, :]
    xa[rows(nsub, 64), :] = ln_in(nsub)

    def a1(first, j, _):
        if first:
            @pl.when(j + 1 < nt)
            def _():
                x_copy(j + 1).wait()
            for c in w_copies(j - 1):
                c.wait()
        for u in range(nsub):
            t = j * nsub + u
            xn = _unpack(ln_in(t) if first and u > 0 else xa[rows(t, 64), :])
            for g in range(GA):
                for ph, w in ((phk, wat[GA + g]), (phq, wat[g])):
                    fm = _feature_map(_dot_nt(_unpack(w), xn))
                    for f in range(FA):
                        ph[t, pl.ds(GR * g + f, 8, stride=FA), :] = fm[8 * f:8 * f + 8, :]
                vt = _dot_nt(_unpack(wat[2 * GA + g]), xn)
                for q in range(4):
                    v = jnp.concatenate(
                        [vt[40 * q:40 * q + 40, :], jnp.ones((8, 128), F32)], axis=0)
                    vts[4 * g + q, :, rows(t, 128)] = _pack(v.astype(BF16))
        if first:
            relayout_b_weights(j - 1)
            tn = jnp.minimum(j + 1, nt - 1) * nsub
            xa[rows(tn, 64), :] = ln_in(tn)
        return 0

    def pair_rows(ph, q, t0, n):
        return _unpack(jnp.concatenate(
            [ph[t0 + u, rows(q, 2 * FA), :] for u in range(n)], axis=1))

    def attend(j):
        low = lax.broadcasted_iota(jnp.int32, (8, TN), 0) < 4
        os_ = []
        for q in range(PA):
            nd = _dot(_unpack(kvs[q]), pair_rows(phq, q, j * nsub, nsub))
            rab = 1.0 / (nd[40:48, :] + 1e-6)
            rba = pltpu.roll(rab, 4, 0)
            ra = jnp.where(low, rab, rba)
            rb = jnp.where(low, rba, rab)
            os_.append(nd[0:40, :] * jnp.concatenate([ra, ra, rab, rb, rb], axis=0))
        return _pack(jnp.concatenate(os_, axis=0).astype(BF16).T)

    def project(j, o):
        r = rows(j, TN)
        xres[r, :] = _dot(_unpack(o), woa[...]) + xres[r, :]

    def pre_rows(j):
        x = jnp.concatenate(
            [xres[rows(j * (TN // 8) + b + 3, 8), :] for b0 in range(0, TN // 8, 8)
             for b in (b0, b0 + 1)], axis=0)
        return _layernorm(x).astype(BF16)

    def b_pre(j, h):
        ypre[rows(j, TN // 4), :] = _dot(h, _unpack(wpre[...]))

    def b_finish(i):
        r = rows(i, TB)
        x = xres[r, :] + rsave[...]
        xres[r, :] = x
        xn = _layernorm(x)
        xa[rows(i, TB // 2), :] = _pack(xn.astype(BF16))
        xio[r, :] = x.astype(BF16)
        return xn

    def b_pair(mem, xn, base, blk, side):
        def fix_ya(p, y):
            c0 = 3 * PW - D
            tie = jnp.where(blk < 0, side[8 * p:8 * p + 8, :], y[0:M, c0:])
            y = jnp.concatenate(
                [jnp.concatenate([y[0:M, 0:c0], tie], axis=1), y[M:, :]], axis=0)
            if p in PRE:
                return jnp.concatenate([y, ypre[rows(2 * blk, 8), _pre_cols(p)]], axis=0)
            ysave[:, p * 3 * PW:(p + 1) * 3 * PW] = y[L:L + 8, :]
            return y[0:L, :]

        def fix_oa(p, o):
            osave[:, p * PW:(p + 1) * PW] = o[32:L, :]
            return o[0:32, :]

        ha = jnp.concatenate([mem, xn[0:40, :]], axis=0).astype(BF16)
        ra = _segment(ha, wb, wpre, wob, fix_ya, fix_oa, base > 0)
        rsave[base:base + 24, :] = ra[M:, :]

        def fix_yb(p, y):
            saved = (ypre[rows(2 * blk + 1, 8), _pre_cols(p)] if p in PRE
                     else ysave[:, p * 3 * PW:(p + 1) * 3 * PW])
            return jnp.concatenate([y[0:M, :], saved, y[M:, :]], axis=0)

        def fix_ob(p, o):
            return jnp.concatenate([o, osave[:, p * PW:(p + 1) * PW]], axis=0)

        hb = jnp.concatenate([ra[0:M, :], xn[40:64, :]], axis=0).astype(BF16)
        rb = _segment(hb, wb, wpre, wob, fix_yb, fix_ob, True)
        rsave[base + 24:base + 32, :] = rb[L:, :]
        rsave[base + 32:base + 64, :] = rb[M:L, :]
        return rb[0:M, :]

    def layer(l, _):
        def wait_first(copies):
            @pl.when(l == 0)
            def _():
                for c in copies:
                    c.wait()

        with jax.named_scope("a1"):
            lax.fori_loop(0, jnp.where(l == 0, 1, nt), functools.partial(a1, False), 0)

            @pl.when(l == 0)
            def _():
                lax.fori_loop(1, nt, functools.partial(a1, True), 0)

        with jax.named_scope("kv"):
            wait_first(w_copies(nt - 1) + w_copies(nt) + w_copies(nt + 1)
                       + [woa_copy, mem0_copy])

            def kv_half(c, _):
                row = lax.broadcasted_iota(jnp.int32, (2 * VR, 4 * FA), 0)
                col = lax.broadcasted_iota(jnp.int32, (2 * VR, 4 * FA), 1)
                split = jnp.where(row < 2 * FA, FA, 2 * FA + 4)
                same = (row >= split) == (col >= 2 * FA)
                for q in range(PA // 2):
                    q = c * (PA // 2) + q
                    kv = _dot_nt(_unpack(vts[q]), pair_rows(phk, q, 0, S // 128))
                    kvs[q] = _pack(jnp.where(same, kv, 0.0).astype(BF16))
                relayout_b_weights(nt - 1 + c)
                return 0

            lax.fori_loop(0, 2, kv_half, 0)
            o = attend(0)
            osc[...] = attend(1)
            project(0, o)
            relayout_b_weights(nt + 1)

        def a2(j, _):
            wait_first(w_copies(nt + 1 + j))
            h = pre_rows(j - 1)
            o = osc[...]
            osc[...] = attend(j + 1)
            project(j, o)
            b_pre(j - 1, h)
            relayout_b_weights(nt + 1 + j)
            return 0

        with jax.named_scope("a2"):
            lax.fori_loop(1, nt - 1, a2, 0)
        xb[...] = _layernorm(xres[rows(0, TB), :])
        rsave[...] = jnp.zeros(rsave.shape, F32)
        project(nt - 1, osc[...])
        b_pre(nt - 2, pre_rows(nt - 2))
        b_pre(nt - 1, pre_rows(nt - 1))
        wait_first([wob_copy])

        def b_step(i, mem):
            @pl.when(jnp.logical_and(l == 1, i >= 2))
            def _():
                out_copy(i - 2).start()

            xn = xb[...]
            side = b_finish(jnp.maximum(i - 1, 0))
            nxt = _layernorm(xres[rows(jnp.minimum(i + 1, nb - 1), TB), :])
            xb[...] = nxt
            side = jnp.concatenate([side, nxt], axis=0)
            for u in range(0, TB, 2 * SEG):
                mem = b_pair(mem, xn[u:u + 2 * SEG, :], u, (i * TB + u) // (2 * SEG),
                             side[2 * u:2 * u + 8 * NP, :])
            return mem

        with jax.named_scope("b"):
            lax.fori_loop(0, nb, b_step, mem0[...].astype(F32))

        @pl.when(l == 0)
        def _():
            b_finish(nb - 1)
        return 0

    lax.fori_loop(0, 2, layer, 0)
    out_copy(nb - 2).start()
    xio[rows(nb - 1, TB), :] = (xres[rows(nb - 1, TB), :] + rsave[...]).astype(BF16)
    out_copy(nb - 1).start()
    pltpu.make_async_copy(xio, out_hbm, sem_out.at[0]).wait()


@functools.partial(jax.jit, static_argnames=("B_seg_len",))
def pallas_interleave_layers__linear_kernel_hedgehog__memory_aug_recurrent_mem_tr__prompt_kernel(
    A_x, A_wqkv, A_w_phi, A_wo, B_x, B_mem0, B_Wq, B_Wk, B_Wv, B_Wo, B_seg_len,
):
    del B_x
    assert B_seg_len == SEG
    x = A_x.reshape(S, D)
    wphi = A_w_phi.transpose(1, 2, 0)
    mem0 = B_mem0.reshape(M, D)
    wq, wk, wv = (w.transpose(1, 2, 0).reshape(HD, D) for w in (B_Wq, B_Wk, B_Wv))
    wo = B_Wo.reshape(HD, D)
    hbm = pl.BlockSpec(memory_space=pl.ANY)
    out = pl.pallas_call(
        _kernel,
        out_shape=jax.ShapeDtypeStruct((S, D), A_x.dtype),
        in_specs=[hbm] * 9,
        out_specs=hbm,
        scratch_shapes=[
            pltpu.VMEM((S, D), BF16),
            pltpu.VMEM((3, D, D), BF16),
            pltpu.VMEM((FA, FA, HA), BF16),
            pltpu.VMEM((D, D), BF16),
            pltpu.VMEM((M, D), BF16),
            pltpu.VMEM((S, D), F32),
            pltpu.VMEM((S // 2, D), U32),
            pltpu.VMEM((TB, D), F32),
            pltpu.VMEM((GA, GR // 2, 256), U32),
            pltpu.VMEM((3 * GA, GR // 2, D), U32),
            pltpu.VMEM((S // 128, D, 128), U32),
            pltpu.VMEM((S // 128, D, 128), U32),
            pltpu.VMEM((PA, VR, S), U32),
            pltpu.VMEM((PA, VR, 4 * FA), U32),
            pltpu.VMEM((TN // 2, D), U32),
            pltpu.VMEM((3, HD, D), BF16),
            pltpu.VMEM((D // 2, 3 * HD), U32),
            pltpu.VMEM((D // 2, len(PRE) * 3 * PW), U32),
            pltpu.VMEM((HD, D), BF16),
            pltpu.VMEM((S // 4, len(PRE) * 3 * PW), F32),
            pltpu.VMEM((8, 3 * HD), F32),
            pltpu.VMEM((8, HD), F32),
            pltpu.VMEM((TB, D), F32),
            pltpu.SemaphoreType.DMA((7 + S // TN + 3 * NP,)),
            pltpu.SemaphoreType.DMA((1,)),
        ],
        compiler_params=pltpu.CompilerParams(vmem_limit_bytes=120 * 1024 * 1024,
                                             disable_bounds_checks=True,
                                             disable_semaphore_checks=True),
    )(x, A_wqkv, wphi, A_wo, mem0, wq, wk, wv, wo)
    return out.reshape(1, S, D)
```

```python
import functools

import jax
import jax.numpy as jnp
from jax import lax
import jax.experimental.pallas as pl
import jax.experimental.pallas.tpu as pltpu

F32 = jnp.float32
BF16 = jnp.bfloat16
U32 = jnp.uint32

S = 2048
D = 640
HA = 32
FA = 20
GA = 4
GR = 8 * FA
VR = 24
PA = HA // 2
TN = 256
HB = 32
DH = 192
HD = HB * DH
M = 8
SEG = 32
L = M + SEG
PW = 2 * DH
NP = HB // 2
TB = 128
PRE = (9,)

NT = (((1,), (1,)), ((), ()))
LOG2E = 1.4426950408889634
HALF_ULP = 0.0040612


def _dot(a, b):
    return jnp.dot(a, b, preferred_element_type=F32)


def _dot_nt(a, b):
    return lax.dot_general(a, b, NT, preferred_element_type=F32)


def _pack(a):
    return pltpu.bitcast(a, U32)


def _unpack(a):
    return pltpu.bitcast(a, BF16)


def _interleave(a, b):
    lo = lax.bitcast_convert_type(a, U32) >> 16
    hi = lax.bitcast_convert_type(b, U32) & jnp.uint32(0xFFFF0000)
    return lo | hi


def _recip(x):
    r = pl.reciprocal(x, approx=True)
    return r * (2.0 - x * r)


def _layernorm(x):
    m = jnp.mean(x, axis=-1, keepdims=True)
    c = x - m
    v = jnp.mean(c * c, axis=-1, keepdims=True)
    return c * lax.rsqrt(v + 1e-5)


def _feature_map(p):
    t = p.shape[-1]
    p3 = jnp.concatenate([jnp.zeros((8, t), F32), p], axis=0).reshape(FA, 8, t)
    mx = jnp.max(p3, axis=0, keepdims=True)
    mn = jnp.min(p3, axis=0, keepdims=True)
    lp = (mx - HALF_ULP) + jnp.log2(jnp.sum(jnp.exp2(p3 - mx), axis=0, keepdims=True))
    ln = (mn + HALF_ULP) - jnp.log2(jnp.sum(jnp.exp2(mn - p3), axis=0, keepdims=True))
    ep = jnp.exp2(p3 - lp)
    en = jnp.exp2(ln - p3)
    return _interleave(ep.reshape(GR, t), en.reshape(GR, t))


def _tiles(a, odd):
    t0, t1, t2 = a[:, 0:128], a[:, 128:256], a[:, 256:384]
    return (t1, t2, t0) if odd else (t1, t0, t2)


def _own_weights(a, odd):
    lane = lax.broadcasted_iota(jnp.int32, (L, 128), 1)
    mid, own, _ = _tiles(a, odd)
    return jnp.concatenate(
        [jnp.where(lane < 64, mid, 0.0), jnp.where(lane < 64, 0.0, mid), own,
         jnp.zeros((128 - 3 * L, 128), F32)], axis=0).astype(BF16)


def _others(even, odd, pad):
    parts = [_tiles(odd, 1)[2], _tiles(even, 0)[2]]
    if pad:
        parts.append(jnp.zeros((128 - 2 * L, 128), F32))
    return jnp.concatenate(parts, axis=0).astype(BF16)


def _softmax3(s3):
    row = lax.broadcasted_iota(jnp.int32, (L, 128), 0)
    col = lax.broadcasted_iota(jnp.int32, (L, 128), 1)
    first = col < L
    second = jnp.logical_and(col >= L, col < 2 * L)
    key = jnp.where(first, col, col - L)
    valid = jnp.logical_or(row < M, row >= key)
    out, other = [], []
    for odd in range(2):
        own = pltpu.roll(s3[odd][L:, :], 128 - L if odd else 128 - 2 * L, 1)
        s = (jnp.where(first, s3[2][0:L, :], own) if odd
             else jnp.where(first, own, s3[2][L:, :]))
        s = jnp.where(valid, (s + s3[odd][0:L, :]) * (DH ** -0.5), -1e9)
        m0 = jnp.max(jnp.where(first, s, -jnp.inf), axis=-1, keepdims=True)
        m1 = jnp.max(jnp.where(second, s, -jnp.inf), axis=-1, keepdims=True)
        e = jnp.exp(s - jnp.where(first, m0, m1))
        e0 = jnp.where(first, e, 0.0)
        e1 = jnp.where(second, e, 0.0)
        p0 = e0 * _recip(jnp.sum(e0, axis=-1, keepdims=True))
        p1 = e1 * _recip(jnp.sum(e1, axis=-1, keepdims=True))
        own = pltpu.roll(p1, L, 1) if odd else pltpu.roll(p0, 2 * L, 1)
        out.append(jnp.concatenate([p0 + p1, own], axis=0).astype(BF16))
        other.append(p0 if odd else p1)
    out.append(jnp.concatenate([other[1], other[0]], axis=0).astype(BF16))
    return out


def _pre_cols(p):
    k = PRE.index(p)
    return slice(k * 3 * PW, (k + 1) * 3 * PW)


def _segment(h, wb, wpre, wob, fix_y, fix_o, chained):
    ys, ss, ps, pvs, os_ = {}, {}, {}, {}, {}

    def proj(p):
        if p in PRE:
            y = _dot(h[0:32, :], _unpack(wpre[:, _pre_cols(p)]))
        elif p == 0 and chained:
            y = _dot(h[:, 0:256], _unpack(wb[0:128, 0:3 * PW]))
            y = _dot(h[:, 256:], _unpack(wb[128:, 0:3 * PW])) + y
        else:
            y = _dot(h, _unpack(wb[:, p * 3 * PW:(p + 1) * 3 * PW]))
        y = fix_y(p, y)
        ys[p] = [y[:, i * PW:(i + 1) * PW] for i in range(3)]

    def weights(c, i, which):
        if i < 2:
            return _own_weights(ys[2 * c + i][which], i)
        return _others(ys[2 * c][which], ys[2 * c + 1][which], True)

    def score_round(n):
        for c, i in (divmod(j, 3) for j in range(4 * n, 4 * n + 4)):
            if i < 2:
                q = jnp.concatenate(_tiles(ys[2 * c + i][0], i)[0:2], axis=0).astype(BF16)
            else:
                q = _others(ys[2 * c][0], ys[2 * c + 1][0], False)
            ss[c, i] = _dot_nt(q, weights(c, i, 1))
            if i == 2:
                ps[c] = _softmax3([ss.pop((c, k)) for k in range(3)])

    def pv_round(n):
        for c, i in (divmod(j, 3) for j in range(4 * n, 4 * n + 4)):
            pvs[c, i] = _dot(ps[c][i], weights(c, i, 2))
            if i == 2:
                o0, o1, o2 = [pvs.pop((c, k)) for k in range(3)]
                os_[2 * c] = fix_o(2 * c, jnp.concatenate(
                    [o0[L:, :], o0[0:L, :], o2[L:, :]], axis=1))
                os_[2 * c + 1] = fix_o(2 * c + 1, jnp.concatenate(
                    [o2[0:L, :], o1[0:L, :], o1[L:, :]], axis=1))

    def slot(n):
        if n >= 2:
            pv_round(n - 2)
        if n < 6:
            score_round(n)

    def oproj(lo, hi):
        o = jnp.concatenate([os_.pop(p) for p in range(lo, hi)], axis=1).astype(BF16)
        return _dot(o, wob[lo * PW:hi * PW, :])

    after = {3: 0, 6: 1, 9: 2, 12: 3, 14: 4}
    for p in range(NP):
        proj(p)
        if p in after:
            slot(after[p])
    o1, o2, o3 = (2, 8, 10) if h.shape[0] == 48 else (2, 7, 10)
    r = oproj(0, o1)
    slot(5)
    r = oproj(o1, o2) + r
    slot(6)
    slot(7)
    r = oproj(o2, o3) + r
    return oproj(o3, NP) + r


def _kernel(x_hbm, wqkv_hbm, wphi_hbm, woa_hbm, mem0_hbm,
            wq_hbm, wk_hbm, wv_hbm, wo_hbm,
            out_hbm,
            xio, wqkv, wphi, woa, mem0, xres, xa, xb, bds, wat, phq, phk, vts, kvs, osc,
            wraw, wb, wpre, wob, ypre, ysave, osave, rsave, sem_in, sem_out):
    nt = S // TN
    nsub = TN // 128
    nb = S // TB

    def rows(j, n):
        return pl.ds(j * n if isinstance(j, int) else pl.multiple_of(j * n, n), n)

    def x_copy(j):
        if isinstance(j, int) and j == 0:
            r = pl.ds(0, TN + 128)
        elif isinstance(j, int) and j == nt - 1:
            r = pl.ds(S - TN + 128, TN - 128)
        else:
            r = pl.ds(j * TN + 128 if isinstance(j, int)
                      else pl.multiple_of(j * TN + 128, 128), TN)
        return pltpu.make_async_copy(x_hbm.at[r, :], xio.at[r, :], sem_in.at[9 + j])

    def w_copies(p):
        return [pltpu.make_async_copy(src.at[rows(p, PW), :], wraw.at[i, rows(p, PW), :],
                                      sem_in.at[9 + nt + 3 * p + i])
                for i, src in enumerate((wq_hbm, wk_hbm, wv_hbm))]

    def wa_copy(r):
        return pltpu.make_async_copy(wqkv_hbm.at[rows(r, 128), :], wqkv.at[rows(r, 128), :],
                                     sem_in.at[4 + r])

    def out_copy(i):
        return pltpu.make_async_copy(xio.at[rows(i, TB), :],
                                     out_hbm.at[rows(i, TB), :], sem_out.at[0])

    wphi_copy = pltpu.make_async_copy(wphi_hbm, wphi, sem_in.at[0])
    woa_copy = pltpu.make_async_copy(woa_hbm, woa, sem_in.at[1])
    mem0_copy = pltpu.make_async_copy(mem0_hbm, mem0, sem_in.at[2])
    wob_copy = pltpu.make_async_copy(wo_hbm, wob, sem_in.at[3])
    order = [wphi_copy, x_copy(0)] + [wa_copy(r) for r in range(D // 128)] + [x_copy(1)]
    for p in range(NP):
        order += w_copies(p)
        if p + 2 < nt:
            order.append(x_copy(p + 2))
        if p + 2 == nt:
            order += [woa_copy, mem0_copy]
    for c in order + [wob_copy]:
        c.start()

    def ln_in(t):
        x = xio[rows(t, 128), :].astype(F32)
        xres[rows(t, 128), :] = x
        return _pack(_layernorm(x).astype(BF16))

    def relayout_b_weights(p):
        for i in range(3):
            w = _pack(wraw[i, rows(p, PW), :].T)
            if isinstance(p, int) and p in PRE:
                wpre[:, rows(3 * PRE.index(p) + i, PW)] = w
            else:
                wb[:, rows(3 * p + i, PW)] = w

    wphi_copy.wait()
    x_copy(0).wait()
    cphi = jnp.zeros((FA, D), F32)
    hh = lax.broadcasted_iota(jnp.int32, (HA, D), 0) * FA
    jj = lax.broadcasted_iota(jnp.int32, (HA, D), 1)
    for d in range(FA):
        cphi = _dot(wphi[d], jnp.where(jj == hh + d, 1.0, 0.0).astype(BF16)) + cphi
    cb = jnp.concatenate(
        [jnp.broadcast_to(cphi[f:f + 1, :], (8, D)) for f in range(FA)], axis=0)
    for g in range(GA):
        row = lax.broadcasted_iota(jnp.int32, (GR, 256), 0)
        col = lax.broadcasted_iota(jnp.int32, (GR, 256), 1) + 128 * g
        lo = (8 * g + (row & 7)) * FA
        bds[g] = _pack(jnp.where(jnp.logical_and(col >= lo, col < lo + FA),
                                 cb[:, 128 * g:128 * g + 256], 0.0).astype(BF16))
    for u in range(nsub + 1):
        xa[rows(u, 64), :] = ln_in(u)

    def fold(r, _):
        wa_copy(r).wait()
        rr = rows(r, 128)
        for g in range(GA):
            ws = []
            for i in range(2):
                c0 = i * D + 128 * g
                w = _dot_nt(_unpack(bds[g]), wqkv[rr, c0:c0 + 256]).reshape(FA, 8, 128)
                ws.append(((w[1:] - w[0:1]) * LOG2E).reshape(GR - 8, 128))
            wat[GA + g, :, rr] = _pack(
                jnp.concatenate([ws[1], ws[0][GR - 16:, :]], axis=0).astype(BF16))
            wat[g, 0:GR // 2 - 8, rr] = _pack(ws[0][0:GR - 16, :].astype(BF16))
        wvt = _pack(wqkv[rr, 2 * D:3 * D].T)
        for g in range(GA):
            wat[2 * GA + g, :, rr] = wvt[g * GR // 2:(g + 1) * GR // 2, :]
        return 0

    lax.fori_loop(0, D // 128, fold, 0)

    def a1(first, j, _):
        if first:
            @pl.when(j < nt - 1)
            def _():
                x_copy(j).wait()

            @pl.when(j == nt - 1)
            def _():
                x_copy(nt - 1).wait()
            for c in w_copies(j - 1):
                c.wait()
        for u in range(nsub):
            t = j * nsub + u
            xn = _unpack(ln_in(t) if first and u > 0 else xa[rows(t, 64), :])
            seq = 'k0q0k1q1k2q2k3q3v0v1v2v3'
            for kind, g in zip(seq[0::2], map(int, seq[1::2])):
                if kind == 'q':
                    y = _dot_nt(_unpack(wat[g, 0:GR // 2 - 8, :]), xn)
                    y = jnp.concatenate([y, qrest], axis=0)
                else:
                    y = _dot_nt(_unpack(wat['qkv'.index(kind) * GA + g]), xn)
                if kind == 'k':
                    y, qrest = y[0:GR - 8, :], y[GR - 8:, :]
                if kind == 'v':
                    for q in range(4):
                        v = jnp.concatenate(
                            [y[40 * q:40 * q + 40, :], jnp.ones((8, 128), F32)], axis=0)
                        vts[4 * g + q, :, rows(t, 128)] = _pack(v.astype(BF16))
                else:
                    ph = phq if kind == 'q' else phk
                    fm = _feature_map(y)
                    for f in range(FA):
                        ph[t, pl.ds(GR * g + f, 8, stride=FA), :] = fm[8 * f:8 * f + 8, :]
        if first:
            relayout_b_weights(j - 1)
            tn = jnp.minimum(j + 1, nt - 1) * nsub
            xa[rows(tn, 64), :] = ln_in(tn)
        return 0

    def pair_rows(ph, q, t0, n):
        return _unpack(jnp.concatenate(
            [ph[t0 + u, rows(q, 2 * FA), :] for u in range(n)], axis=1))

    def attend(j):
        low = lax.broadcasted_iota(jnp.int32, (8, TN), 0) < 4
        os_ = []
        for q in range(PA):
            nd = _dot(_unpack(kvs[q]), pair_rows(phq, q, j * nsub, nsub))
            rab = 1.0 / (nd[40:48, :] + 1e-6)
            rba = pltpu.roll(rab, 4, 0)
            ra = jnp.where(low, rab, rba)
            rb = jnp.where(low, rba, rab)
            os_.append(nd[0:40, :] * jnp.concatenate([ra, ra, rab, rb, rb], axis=0))
        return _pack(jnp.concatenate(os_, axis=0).astype(BF16).T)

    def project(j, o):
        r = rows(j, TN)
        xres[r, :] = _dot(_unpack(o), woa[...]) + xres[r, :]

    def pre_rows(j):
        x = jnp.concatenate(
            [xres[rows(j * (TN // 8) + b + 3, 8), :] for b0 in range(0, TN // 8, 8)
             for b in (b0, b0 + 1)], axis=0)
        return _layernorm(x).astype(BF16)

    def b_pre(j, h):
        ypre[rows(j, TN // 4), :] = _dot(h, _unpack(wpre[...]))

    def b_finish(i):
        r = rows(i, TB)
        x = xres[r, :] + rsave[...]
        xres[r, :] = x
        xn = _layernorm(x)
        xa[rows(i, TB // 2), :] = _pack(xn.astype(BF16))
        xio[r, :] = x.astype(BF16)
        return xn

    def b_pair(mem, xn, base, blk, side):
        def fix_ya(p, y):
            c0 = 3 * PW - D
            tie = jnp.where(blk < 0, side[8 * p:8 * p + 8, :], y[0:M, c0:])
            y = jnp.concatenate(
                [jnp.concatenate([y[0:M, 0:c0], tie], axis=1), y[M:, :]], axis=0)
            if p in PRE:
                return jnp.concatenate([y, ypre[rows(2 * blk, 8), _pre_cols(p)]], axis=0)
            ysave[:, p * 3 * PW:(p + 1) * 3 * PW] = y[L:L + 8, :]
            return y[0:L, :]

        def fix_oa(p, o):
            osave[:, p * PW:(p + 1) * PW] = o[32:L, :]
            return o[0:32, :]

        ha = jnp.concatenate([mem, xn[0:40, :]], axis=0).astype(BF16)
        ra = _segment(ha, wb, wpre, wob, fix_ya, fix_oa, base > 0)
        rsave[base:base + 24, :] = ra[M:, :]

        def fix_yb(p, y):
            saved = (ypre[rows(2 * blk + 1, 8), _pre_cols(p)] if p in PRE
                     else ysave[:, p * 3 * PW:(p + 1) * 3 * PW])
            return jnp.concatenate([y[0:M, :], saved, y[M:, :]], axis=0)

        def fix_ob(p, o):
            return jnp.concatenate([o, osave[:, p * PW:(p + 1) * PW]], axis=0)

        hb = jnp.concatenate([ra[0:M, :], xn[40:64, :]], axis=0).astype(BF16)
        rb = _segment(hb, wb, wpre, wob, fix_yb, fix_ob, True)
        rsave[base + 24:base + 32, :] = rb[L:, :]
        rsave[base + 32:base + 64, :] = rb[M:L, :]
        return rb[0:M, :]

    def layer(l, _):
        def wait_first(copies):
            @pl.when(l == 0)
            def _():
                for c in copies:
                    c.wait()

        with jax.named_scope("a1"):
            lax.fori_loop(0, jnp.where(l == 0, 1, nt), functools.partial(a1, False), 0)

            @pl.when(l == 0)
            def _():
                lax.fori_loop(1, nt, functools.partial(a1, True), 0)

        with jax.named_scope("kv"):
            wait_first(w_copies(nt - 1) + w_copies(nt) + w_copies(nt + 1)
                       + [woa_copy, mem0_copy])

            def kv_half(c, _):
                row = lax.broadcasted_iota(jnp.int32, (2 * VR, 4 * FA), 0)
                col = lax.broadcasted_iota(jnp.int32, (2 * VR, 4 * FA), 1)
                split = jnp.where(row < 2 * FA, FA, 2 * FA + 4)
                same = (row >= split) == (col >= 2 * FA)
                for q in range(PA // 2):
                    q = c * (PA // 2) + q
                    kv = _dot_nt(_unpack(vts[q]), pair_rows(phk, q, 0, S // 128))
                    kvs[q] = _pack(jnp.where(same, kv, 0.0).astype(BF16))
                relayout_b_weights(nt - 1 + c)
                return 0

            kv_half(0, 0)
            kv_half(1, 0)
            o = attend(0)
            osc[...] = attend(1)
            project(0, o)
            relayout_b_weights(nt + 1)

        def a2(j, _):
            wait_first(w_copies(nt + 1 + j))
            h = pre_rows(j - 1)
            o = osc[...]
            osc[...] = attend(j + 1)
            project(j, o)
            b_pre(j - 1, h)
            relayout_b_weights(nt + 1 + j)
            return 0

        with jax.named_scope("a2"):
            lax.fori_loop(1, nt - 1, a2, 0)
        xb[...] = _layernorm(xres[rows(0, TB), :])
        rsave[...] = jnp.zeros(rsave.shape, F32)
        project(nt - 1, osc[...])
        b_pre(nt - 2, pre_rows(nt - 2))
        b_pre(nt - 1, pre_rows(nt - 1))
        wait_first([wob_copy])

        def b_step(i, mem):
            xn = xb[...]
            side = b_finish(jnp.maximum(i - 1, 0))
            nxt = _layernorm(xres[rows(jnp.minimum(i + 1, nb - 1), TB), :])
            xb[...] = nxt
            side = jnp.concatenate([side, nxt], axis=0)
            for u in range(0, TB, 2 * SEG):
                mem = b_pair(mem, xn[u:u + 2 * SEG, :], u, (i * TB + u) // (2 * SEG),
                             side[2 * u:2 * u + 8 * NP, :])

            @pl.when(jnp.logical_and(l == 1, i >= 1))
            def _():
                out_copy(i - 1).start()
            return mem

        with jax.named_scope("b"):
            lax.fori_loop(0, nb, b_step, mem0[...].astype(F32))

        @pl.when(l == 0)
        def _():
            b_finish(nb - 1)
        return 0

    lax.fori_loop(0, 2, layer, 0)
    xio[rows(nb - 1, TB), :] = (xres[rows(nb - 1, TB), :] + rsave[...]).astype(BF16)
    out_copy(nb - 1).start()
    pltpu.make_async_copy(xio, out_hbm, sem_out.at[0]).wait()


@functools.partial(jax.jit, static_argnames=("B_seg_len",))
def pallas_interleave_layers__linear_kernel_hedgehog__memory_aug_recurrent_mem_tr__prompt_kernel(
    A_x, A_wqkv, A_w_phi, A_wo, B_x, B_mem0, B_Wq, B_Wk, B_Wv, B_Wo, B_seg_len,
):
    del B_x
    assert B_seg_len == SEG
    x = A_x.reshape(S, D)
    wphi = A_w_phi.transpose(1, 2, 0)
    mem0 = B_mem0.reshape(M, D)
    wq, wk, wv = (w.transpose(1, 2, 0).reshape(HD, D) for w in (B_Wq, B_Wk, B_Wv))
    wo = B_Wo.reshape(HD, D)
    hbm = pl.BlockSpec(memory_space=pl.ANY)
    out = pl.pallas_call(
        _kernel,
        out_shape=jax.ShapeDtypeStruct((S, D), A_x.dtype),
        in_specs=[hbm] * 9,
        out_specs=hbm,
        scratch_shapes=[
            pltpu.VMEM((S, D), BF16),
            pltpu.VMEM((D, 3 * D), BF16),
            pltpu.VMEM((FA, FA, HA), BF16),
            pltpu.VMEM((D, D), BF16),
            pltpu.VMEM((M, D), BF16),
            pltpu.VMEM((S, D), F32),
            pltpu.VMEM((S // 2, D), U32),
            pltpu.VMEM((TB, D), F32),
            pltpu.VMEM((GA, GR // 2, 256), U32),
            pltpu.VMEM((3 * GA, GR // 2, D), U32),
            pltpu.VMEM((S // 128, D, 128), U32),
            pltpu.VMEM((S // 128, D, 128), U32),
            pltpu.VMEM((PA, VR, S), U32),
            pltpu.VMEM((PA, VR, 4 * FA), U32),
            pltpu.VMEM((TN // 2, D), U32),
            pltpu.VMEM((3, HD, D), BF16),
            pltpu.VMEM((D // 2, 3 * HD), U32),
            pltpu.VMEM((D // 2, len(PRE) * 3 * PW), U32),
            pltpu.VMEM((HD, D), BF16),
            pltpu.VMEM((S // 4, len(PRE) * 3 * PW), F32),
            pltpu.VMEM((8, 3 * HD), F32),
            pltpu.VMEM((8, HD), F32),
            pltpu.VMEM((TB, D), F32),
            pltpu.SemaphoreType.DMA((9 + S // TN + 3 * NP,)),
            pltpu.SemaphoreType.DMA((1,)),
        ],
        compiler_params=pltpu.CompilerParams(vmem_limit_bytes=120 * 1024 * 1024,
                                             disable_bounds_checks=True,
                                             disable_semaphore_checks=True),
    )(x, A_wqkv, wphi, A_wo, mem0, wq, wk, wv, wo)
    return out.reshape(1, S, D)
```

```python
import functools

import jax
import jax.numpy as jnp
from jax import lax
import jax.experimental.pallas as pl
import jax.experimental.pallas.tpu as pltpu

F32 = jnp.float32
BF16 = jnp.bfloat16
U32 = jnp.uint32

S = 2048
D = 640
HA = 32
FA = 20
GA = 4
GR = 8 * FA
VR = 24
PA = HA // 2
TN = 256
HB = 32
DH = 192
HD = HB * DH
M = 8
SEG = 32
L = M + SEG
PW = 2 * DH
NP = HB // 2
TB = 128
KE = 7

NT = (((1,), (1,)), ((), ()))
LOG2E = 1.4426950408889634
HALF_ULP = 0.0040612


def _dot(a, b):
    return jnp.dot(a, b, preferred_element_type=F32)


def _dot_nt(a, b):
    return lax.dot_general(a, b, NT, preferred_element_type=F32)


def _pack(a):
    return pltpu.bitcast(a, U32)


def _unpack(a):
    return pltpu.bitcast(a, BF16)


def _interleave(a, b):
    lo = lax.bitcast_convert_type(a, U32) >> 16
    hi = lax.bitcast_convert_type(b, U32) & jnp.uint32(0xFFFF0000)
    return lo | hi


def _recip(x):
    r = pl.reciprocal(x, approx=True)
    return r * (2.0 - x * r)


def _layernorm(x):
    m = jnp.mean(x, axis=-1, keepdims=True)
    c = x - m
    v = jnp.mean(c * c, axis=-1, keepdims=True)
    return c * lax.rsqrt(v + 1e-5)


def _feature_map(p):
    t = p.shape[-1]
    p3 = jnp.concatenate([jnp.zeros((8, t), F32), p], axis=0).reshape(FA, 8, t)
    mx = jnp.max(p3, axis=0)
    mn = jnp.min(p3, axis=0)
    sp, sn = jnp.exp2(p3[0] - mx), jnp.exp2(mn - p3[0])
    for f in range(1, FA):
        sp, sn = sp + jnp.exp2(p3[f] - mx), sn + jnp.exp2(mn - p3[f])
    lp = (mx - HALF_ULP) + jnp.log2(sp)
    ln = (mn + HALF_ULP) - jnp.log2(sn)
    return [_interleave(jnp.exp2(p3[f] - lp), jnp.exp2(ln - p3[f])) for f in range(FA)]


def _tiles(a, odd):
    t0, t1, t2 = a[:, 0:128], a[:, 128:256], a[:, 256:384]
    return (t1, t2, t0) if odd else (t1, t0, t2)


def _own_weights(a, odd):
    lane = lax.broadcasted_iota(jnp.int32, (L, 128), 1)
    mid, own, _ = _tiles(a, odd)
    return jnp.concatenate(
        [jnp.where(lane < 64, mid, 0.0), jnp.where(lane < 64, 0.0, mid), own,
         jnp.zeros((128 - 3 * L, 128), F32)], axis=0).astype(BF16)


def _others(even, odd, pad):
    parts = [_tiles(odd, 1)[2], _tiles(even, 0)[2]]
    if pad:
        parts.append(jnp.zeros((128 - 2 * L, 128), F32))
    return jnp.concatenate(parts, axis=0).astype(BF16)


def _softmax3(s3):
    row = lax.broadcasted_iota(jnp.int32, (L, 128), 0)
    col = lax.broadcasted_iota(jnp.int32, (L, 128), 1)
    first = col < L
    second = jnp.logical_and(col >= L, col < 2 * L)
    key = jnp.where(first, col, col - L)
    valid = jnp.logical_or(row < M, row >= key)
    out, other = [], []
    for odd in range(2):
        own = pltpu.roll(s3[odd][L:, :], 128 - L if odd else 128 - 2 * L, 1)
        s = (jnp.where(first, s3[2][0:L, :], own) if odd
             else jnp.where(first, own, s3[2][L:, :]))
        s = jnp.where(valid, (s + s3[odd][0:L, :]) * (DH ** -0.5), -1e9)
        m0 = jnp.max(jnp.where(first, s, -jnp.inf), axis=-1, keepdims=True)
        m1 = jnp.max(jnp.where(second, s, -jnp.inf), axis=-1, keepdims=True)
        e = jnp.exp(s - jnp.where(first, m0, m1))
        e0 = jnp.where(first, e, 0.0)
        e1 = jnp.where(second, e, 0.0)
        p0 = e0 * _recip(jnp.sum(e0, axis=-1, keepdims=True))
        p1 = e1 * _recip(jnp.sum(e1, axis=-1, keepdims=True))
        own = pltpu.roll(p1, L, 1) if odd else pltpu.roll(p0, 2 * L, 1)
        out.append(jnp.concatenate([p0 + p1, own], axis=0).astype(BF16))
        other.append(p0 if odd else p1)
    out.append(jnp.concatenate([other[1], other[0]], axis=0).astype(BF16))
    return out


def _segment(h, hk, wqv, wk, wob, fix_qv, fix_k, fix_o, chained):
    ys, ks, ss, ps, pvs, os_ = {}, {}, {}, {}, {}, {}
    kg = 2

    def proj(p):
        cols = slice(p * 2 * PW, (p + 1) * 2 * PW)
        if p == 0 and chained:
            ksp = 512
            y = _dot(h[:, 0:ksp], _unpack(wqv[0:ksp // 2, cols]))
            y = _dot(h[:, ksp:], _unpack(wqv[ksp // 2:, cols])) + y
        else:
            y = _dot(h, _unpack(wqv[:, cols]))
        y = fix_qv(p, y)
        if p % kg == 0:
            k = _dot(hk, _unpack(wk[:, p * PW:(p + kg) * PW]))
            for e in range(kg):
                ks[p + e] = fix_k(p + e, k[:, e * PW:(e + 1) * PW])
        ys[p] = [y[:, 0:PW], ks.pop(p), y[:, PW:]]

    def weights(c, i, which):
        if i < 2:
            return _own_weights(ys[2 * c + i][which], i)
        return _others(ys[2 * c][which], ys[2 * c + 1][which], True)

    def score_round(n):
        for c, i in (divmod(j, 3) for j in range(4 * n, 4 * n + 4)):
            if i < 2:
                q = jnp.concatenate(_tiles(ys[2 * c + i][0], i)[0:2], axis=0).astype(BF16)
            else:
                q = _others(ys[2 * c][0], ys[2 * c + 1][0], False)
            ss[c, i] = _dot_nt(q, weights(c, i, 1))
            if i == 2:
                ps[c] = _softmax3([ss.pop((c, k)) for k in range(3)])

    def pv_round(n):
        for c, i in (divmod(j, 3) for j in range(4 * n, 4 * n + 4)):
            pvs[c, i] = _dot(ps[c][i], weights(c, i, 2))
            if i == 2:
                o0, o1, o2 = [pvs.pop((c, k)) for k in range(3)]
                os_[2 * c] = fix_o(2 * c, jnp.concatenate(
                    [o0[L:, :], o0[0:L, :], o2[L:, :]], axis=1))
                os_[2 * c + 1] = fix_o(2 * c + 1, jnp.concatenate(
                    [o2[0:L, :], o1[0:L, :], o1[L:, :]], axis=1))

    def slot(n):
        if n >= 2:
            pv_round(n - 2)
        if n < 6:
            score_round(n)

    def oproj(lo, hi):
        o = jnp.concatenate([os_.pop(p) for p in range(lo, hi)], axis=1).astype(BF16)
        return _dot(o, _unpack(wob[lo * DH:hi * DH, :]))

    after = {3: 0, 6: 1, 9: 2, 11: 3, 14: 4}
    for p in range(NP):
        proj(p)
        if p in after:
            slot(after[p])
    o1, o2, o3 = (2, 8, 10) if h.shape[0] == 48 else (2, 7, 10)
    r = oproj(0, o1)
    slot(5)
    r = oproj(o1, o2) + r
    slot(6)
    slot(7)
    r = oproj(o2, o3) + r
    return oproj(o3, NP) + r


def _kernel(x_hbm, wqkv_hbm, wphi_hbm, woa_hbm, mem0_hbm,
            wq_hbm, wk_hbm, wv_hbm, wo_hbm,
            out_hbm,
            xio, wqkv, wphi, woa, mem0, xres, xa, xb, bds, wat, phq, phk, vts, kvs, osc,
            wraw, wqv, wk, wob, xe, ke, ysave, osave, rsave, sem_in, sem_out):
    nt = S // TN
    nsub = TN // 128
    nb = S // TB
    nw = NP // 2

    def rows(j, n):
        return pl.ds(j * n if isinstance(j, int) else pl.multiple_of(j * n, n), n)

    def x_copy(j):
        if isinstance(j, int) and j < 0:
            r = pl.ds(0, 128)
        elif isinstance(j, int) and j == nt - 1:
            r = pl.ds(S - TN + 128, TN - 128)
        else:
            r = pl.ds(j * TN + 128 if isinstance(j, int)
                      else pl.multiple_of(j * TN + 128, 128), TN)
        return pltpu.make_async_copy(x_hbm.at[r, :], xio.at[r, :], sem_in.at[9 + j])

    def w_copies(c):
        r = rows(c, 2 * PW)
        return [pltpu.make_async_copy(src.at[r, :], wraw.at[i, r, :],
                                      sem_in.at[10 + nt + 3 * c + i])
                for i, src in enumerate((wq_hbm, wv_hbm, wo_hbm))]

    def wa_copy(r):
        return pltpu.make_async_copy(wqkv_hbm.at[rows(r, 128), :], wqkv.at[rows(r, 128), :],
                                     sem_in.at[3 + r])

    def out_copy(i):
        return pltpu.make_async_copy(xio.at[rows(i, TB), :],
                                     out_hbm.at[rows(i, TB), :], sem_out.at[0])

    wphi_copy = pltpu.make_async_copy(wphi_hbm, wphi, sem_in.at[0])
    woa_copy = pltpu.make_async_copy(woa_hbm, woa, sem_in.at[1])
    mem0_copy = pltpu.make_async_copy(mem0_hbm, mem0, sem_in.at[2])
    order = [wphi_copy, x_copy(-1)] + [wa_copy(r) for r in range(D // 128)]
    wk_copy = pltpu.make_async_copy(wk_hbm, wraw.at[3], sem_in.at[9 + nt])
    order += [x_copy(j) for j in range(nt)] + [woa_copy, mem0_copy, wk_copy]
    for c in range(nw):
        order += w_copies(c)
    for c in order:
        c.start()

    def ln_in(t, first):
        x = xio[rows(t, 128), :].astype(F32)
        if first is not True:
            x = jnp.where(first, x, xres[rows(t, 128), :])
        xres[rows(t, 128), :] = x
        return _pack(_layernorm(x).astype(BF16))

    wphi_copy.wait()
    x_copy(-1).wait()
    cphi = jnp.zeros((FA, D), F32)
    hh = lax.broadcasted_iota(jnp.int32, (HA, D), 0) * FA
    jj = lax.broadcasted_iota(jnp.int32, (HA, D), 1)
    for d in range(FA):
        cphi = _dot(wphi[d], jnp.where(jj == hh + d, 1.0, 0.0).astype(BF16)) + cphi
    cb = jnp.concatenate(
        [jnp.broadcast_to(cphi[f:f + 1, :], (8, D)) for f in range(FA)], axis=0)
    for g in range(GA):
        row = lax.broadcasted_iota(jnp.int32, (GR, 256), 0)
        col = lax.broadcasted_iota(jnp.int32, (GR, 256), 1) + 128 * g
        lo = (8 * g + (row & 7)) * FA
        bds[g] = _pack(jnp.where(jnp.logical_and(col >= lo, col < lo + FA),
                                 cb[:, 128 * g:128 * g + 256], 0.0).astype(BF16))
    xa[rows(0, 64), :] = ln_in(0, True)

    def fold(r, _):
        wa_copy(r).wait()
        rr = rows(r, 128)
        for g in range(GA):
            ws = []
            for i in range(2):
                c0 = i * D + 128 * g
                w = _dot_nt(_unpack(bds[g]), wqkv[rr, c0:c0 + 256]).reshape(FA, 8, 128)
                ws.append(((w[1:] - w[0:1]) * LOG2E).reshape(GR - 8, 128))
            wat[GA + g, :, rr] = _pack(
                jnp.concatenate([ws[1], ws[0][GR - 16:, :]], axis=0).astype(BF16))
            wat[g, 0:GR // 2 - 8, rr] = _pack(ws[0][0:GR - 16, :].astype(BF16))
        wvt = _pack(wqkv[rr, 2 * D:3 * D].T)
        for g in range(GA):
            wat[2 * GA + g, :, rr] = wvt[g * GR // 2:(g + 1) * GR // 2, :]
        return 0

    lax.fori_loop(0, D // 128, fold, 0)

    def a1(first, j, _):
        @pl.when(jnp.logical_and(first, j < nt - 1))
        def _():
            x_copy(j).wait()

        @pl.when(jnp.logical_and(first, j == nt - 1))
        def _():
            x_copy(nt - 1).wait()

        def features(ph, t, g, y):
            for f, w in enumerate(_feature_map(y)):
                ph[t, pl.ds(GR * g + f, 8, stride=FA), :] = w

        for u in range(nsub):
            t = j * nsub + u
            xn = _unpack(ln_in(t, first) if u > 0 else xa[rows(t, 64), :])
            for g in range(GA):
                y = _dot_nt(_unpack(wat[GA + g]), xn)
                features(phk, t, g, y[0:GR - 8, :])
                yq = _dot_nt(_unpack(wat[g, 0:GR // 2 - 8, :]), xn)
                features(phq, t, g, jnp.concatenate([yq, y[GR - 8:, :]], axis=0))
            for g in range(GA):
                y = _dot_nt(_unpack(wat[2 * GA + g]), xn)
                for q in range(4):
                    v = jnp.concatenate(
                        [y[40 * q:40 * q + 40, :], jnp.ones((8, 128), F32)], axis=0)
                    vts[4 * g + q, :, rows(t, 128)] = _pack(v.astype(BF16))
        tn = jnp.minimum(j + 1, nt - 1) * nsub
        xa[rows(tn, 64), :] = ln_in(tn, first)
        return 0

    def pair_rows(ph, q, t0, n):
        return _unpack(jnp.concatenate(
            [ph[t0 + u, rows(q, 2 * FA), :] for u in range(n)], axis=1))

    def attend(j):
        low = lax.broadcasted_iota(jnp.int32, (8, TN), 0) < 4
        os_ = []
        for q in range(PA):
            nd = _dot(_unpack(kvs[q]), pair_rows(phq, q, j * nsub, nsub))
            rab = 1.0 / (nd[40:48, :] + 1e-6)
            rba = pltpu.roll(rab, 4, 0)
            ra = jnp.where(low, rab, rba)
            rb = jnp.where(low, rba, rab)
            os_.append(nd[0:40, :] * jnp.concatenate([ra, ra, rab, rb, rb], axis=0))
        return _pack(jnp.concatenate(os_, axis=0).astype(BF16).T)

    def project(j, o):
        r = rows(j, TN)
        xres[r, :] = _dot(_unpack(o), woa[...]) + xres[r, :]

    def extra_rows(j):
        ns = TN // SEG
        x = jnp.concatenate(
            [xres[rows(j * (TN // 8) + (s // 2) * 8 + 3 + s % 2, 8), :] for s in range(ns)],
            axis=0)
        x = _layernorm(x).reshape(ns, 8, D)
        x = x - x[:, KE:KE + 1, :]
        for s in range(ns):
            for c in range(D // 128):
                xe[c, pl.ds((j * ns + s) * KE, 8), :] = x[s, :, 128 * c:128 * (c + 1)]

    def extra_keys(seg, p):
        k = jnp.concatenate(
            [ke[3 * p + c, pl.ds(seg * KE, 8), :] for c in range(3)], axis=1)
        return jnp.where(lax.broadcasted_iota(jnp.int32, (8, PW), 0) < KE, k, 0.0)

    def relayout_wk(j):
        r = rows(j, HD // nt)
        wk[:, r] = _pack(wraw[3, r, :].T)

    def b_finish(i):
        r = rows(i, TB)
        x = xres[r, :] + rsave[...]
        xres[r, :] = x
        xn = _layernorm(x)
        xa[rows(i, TB // 2), :] = _pack(xn.astype(BF16))
        xio[r, :] = x.astype(BF16)
        return xn

    def b_pair(mem, xn, base, blk, side):
        def fix_qva(p, y):
            c0 = 2 * PW - D
            tie = jnp.where(blk < 0, side[8 * p:8 * p + 8, :], y[0:M, c0:])
            ysave[:, p * 2 * PW:(p + 1) * 2 * PW] = y[L:L + 8, :]
            return jnp.concatenate(
                [jnp.concatenate([y[0:M, 0:c0], tie], axis=1), y[M:L, :]], axis=0)

        def fix_ka(p, k):
            return jnp.concatenate([k, extra_keys(2 * blk, p)], axis=0)

        def fix_oa(p, o):
            osave[:, p * PW:(p + 1) * PW] = o[32:L, :]
            return o[0:32, :]

        h = jnp.concatenate([mem, xn[0:40, :]], axis=0)
        ra = _segment(h.astype(BF16), (h[0:32, :] - xn[31:32, :]).astype(BF16),
                      wqv, wk, wob, fix_qva, fix_ka, fix_oa, base > 0)
        rsave[base:base + 24, :] = ra[M:, :]

        def fix_qvb(p, y):
            return jnp.concatenate(
                [y[0:M, :], ysave[:, p * 2 * PW:(p + 1) * 2 * PW], y[M:, :]], axis=0)

        def fix_kb(p, k):
            return jnp.concatenate([k[0:M, :], extra_keys(2 * blk + 1, p), k[M:, :]], axis=0)

        def fix_ob(p, o):
            return jnp.concatenate([o, osave[:, p * PW:(p + 1) * PW]], axis=0)

        h = jnp.concatenate([ra[0:M, :], xn[40:64, :]], axis=0)
        rb = _segment(h.astype(BF16), (h - xn[39:40, :]).astype(BF16),
                      wqv, wk, wob, fix_qvb, fix_kb, fix_ob, True)
        rsave[base + 24:base + 32, :] = rb[L:, :]
        rsave[base + 32:base + 64, :] = rb[M:L, :]
        return rb[0:M, :]

    def layer(l, _):
        def wait_first(copies):
            @pl.when(l == 0)
            def _():
                for c in copies:
                    c.wait()

        with jax.named_scope("a1"):
            lax.fori_loop(0, nt, functools.partial(a1, l == 0), 0)

        with jax.named_scope("kv"):
            wait_first([woa_copy, mem0_copy, wk_copy])
            row = lax.broadcasted_iota(jnp.int32, (2 * VR, 4 * FA), 0)
            col = lax.broadcasted_iota(jnp.int32, (2 * VR, 4 * FA), 1)
            split = jnp.where(row < 2 * FA, FA, 2 * FA + 4)
            same = (row >= split) == (col >= 2 * FA)
            for q in range(PA):
                kv = _dot_nt(_unpack(vts[q]), pair_rows(phk, q, 0, S // 128))
                kvs[q] = _pack(jnp.where(same, kv, 0.0).astype(BF16))
            o = attend(0)
            osc[...] = attend(1)
            project(0, o)
            relayout_wk(0)

        def a2(j, _):
            extra_rows(j - 1)
            o = osc[...]
            osc[...] = attend(j + 1)
            project(j, o)
            relayout_wk(j)
            return 0

        with jax.named_scope("a2"):
            lax.fori_loop(1, nt - 1, a2, 0, unroll=2)
        xb[...] = _layernorm(xres[rows(0, TB), :])
        rsave[...] = jnp.zeros(rsave.shape, F32)
        extra_rows(nt - 2)
        relayout_wk(nt - 1)
        for part in ((1, 2), (0, 3)):
            grp = [b + k for b in range(0, TN // 16, 4) for k in part]
            o = jnp.concatenate([osc[8 * g:8 * g + 8, :] for g in grp], axis=0)
            y = _dot(_unpack(o), woa[...])
            for n, g in enumerate(grp):
                r = pl.ds(S - TN + 16 * g, 16)
                xres[r, :] = y[16 * n:16 * n + 16, :] + xres[r, :]
            if part == (1, 2):
                extra_rows(nt - 1)

        pc = 2

        def b_pre(n, _):
            wait_first([cp for e in range(pc) for cp in w_copies(pc * n + e)])
            mr = 16 * KE
            for c in range(pc):
                c = pc * n + c
                for m in range(S // SEG * KE // mr):
                    x = jnp.concatenate(
                        [xe[t, m * mr:(m + 1) * mr, :] for t in range(D // 128)], axis=1)
                    k = _dot(x.astype(BF16), _unpack(wk[:, rows(c, 2 * PW)]))
                    for t in range(2 * PW // 128):
                        ke[6 * c + t, m * mr:(m + 1) * mr, :] = k[:, 128 * t:128 * (t + 1)]
                        e = (c * 4 + m) * 6 + t
                        tie = pltpu.bitcast(k[0:16, 128 * t:128 * (t + 1)], U32)
                        wob[rows(e, 16), :] = jnp.where(
                            n < 0, jnp.concatenate([tie] * (D // 128), axis=1),
                            _pack(wraw[2, rows(e, 32), :]))
                for e in range(2):
                    p = 2 * c + e
                    wqv[:, rows(2 * p, PW)] = _pack(wraw[0, rows(p, PW), :].T)
                    wqv[:, rows(2 * p + 1, PW)] = _pack(wraw[1, rows(p, PW), :].T)
            return 0

        with jax.named_scope("pre"):
            lax.fori_loop(0, nw // pc, b_pre, 0)

        def b_step(i, mem):
            xn = xb[...]
            side = b_finish(jnp.maximum(i - 1, 0))
            nxt = _layernorm(xres[rows(jnp.minimum(i + 1, nb - 1), TB), :])
            xb[...] = nxt
            side = jnp.concatenate([side, nxt], axis=0)
            for u in range(0, TB, 2 * SEG):
                mem = b_pair(mem, xn[u:u + 2 * SEG, :], u, (i * TB + u) // (2 * SEG),
                             side[2 * u:2 * u + 8 * NP, :])

            @pl.when(jnp.logical_and(l == 1, i >= 1))
            def _():
                out_copy(i - 1).start()
            return mem

        with jax.named_scope("b"):
            lax.fori_loop(0, nb, b_step, mem0[...].astype(F32))

        x = xres[rows(nb - 1, TB), :] + rsave[...]
        xres[rows(nb - 1, TB), :] = x
        xio[rows(nb - 1, TB), :] = x.astype(BF16)
        return 0

    lax.fori_loop(0, 2, layer, 0)
    out_copy(nb - 1).start()
    pltpu.make_async_copy(xio, out_hbm, sem_out.at[0]).wait()


@functools.partial(jax.jit, static_argnames=("B_seg_len",))
def pallas_interleave_layers__linear_kernel_hedgehog__memory_aug_recurrent_mem_tr__prompt_kernel(
    A_x, A_wqkv, A_w_phi, A_wo, B_x, B_mem0, B_Wq, B_Wk, B_Wv, B_Wo, B_seg_len,
):
    del B_x
    assert B_seg_len == SEG
    x = A_x.reshape(S, D)
    wphi = A_w_phi.transpose(1, 2, 0)
    mem0 = B_mem0.reshape(M, D)
    wq, wk, wv = (w.transpose(1, 2, 0).reshape(HD, D) for w in (B_Wq, B_Wk, B_Wv))
    wo = B_Wo.reshape(HD, D)
    hbm = pl.BlockSpec(memory_space=pl.ANY)
    out = pl.pallas_call(
        _kernel,
        out_shape=jax.ShapeDtypeStruct((S, D), A_x.dtype),
        in_specs=[hbm] * 9,
        out_specs=hbm,
        scratch_shapes=[
            pltpu.VMEM((S, D), BF16),
            pltpu.VMEM((D, 3 * D), BF16),
            pltpu.VMEM((FA, FA, HA), BF16),
            pltpu.VMEM((D, D), BF16),
            pltpu.VMEM((M, D), BF16),
            pltpu.VMEM((S, D), F32),
            pltpu.VMEM((S // 2, D), U32),
            pltpu.VMEM((TB, D), F32),
            pltpu.VMEM((GA, GR // 2, 256), U32),
            pltpu.VMEM((3 * GA, GR // 2, D), U32),
            pltpu.VMEM((S // 128, D, 128), U32),
            pltpu.VMEM((S // 128, D, 128), U32),
            pltpu.VMEM((PA, VR, S), U32),
            pltpu.VMEM((PA, VR, 4 * FA), U32),
            pltpu.VMEM((TN // 2, D), U32),
            pltpu.VMEM((4, HD, D), BF16),
            pltpu.VMEM((D // 2, 2 * HD), U32),
            pltpu.VMEM((D // 2, HD), U32),
            pltpu.VMEM((HD // 2, D), U32),
            pltpu.VMEM((D // 128, S // SEG * KE + 8, 128), F32),
            pltpu.VMEM((HD // 128, S // SEG * KE + 8, 128), F32),
            pltpu.VMEM((8, 2 * HD), F32),
            pltpu.VMEM((8, HD), F32),
            pltpu.VMEM((TB, D), F32),
            pltpu.SemaphoreType.DMA((10 + S // TN + 3 * NP // 2,)),
            pltpu.SemaphoreType.DMA((1,)),
        ],
        compiler_params=pltpu.CompilerParams(vmem_limit_bytes=120 * 1024 * 1024,
                                             disable_bounds_checks=True,
                                             disable_semaphore_checks=True),
    )(x, A_wqkv, wphi, A_wo, mem0, wq, wk, wv, wo)
    return out.reshape(1, S, D)
```

```python
import functools

import jax
import jax.numpy as jnp
from jax import lax
import jax.experimental.pallas as pl
import jax.experimental.pallas.tpu as pltpu

F32 = jnp.float32
BF16 = jnp.bfloat16
U32 = jnp.uint32

S = 2048
D = 640
HA = 32
FA = 20
GA = 4
GR = 8 * FA
VR = 24
PA = HA // 2
TN = 256
TA = 512
HB = 32
DH = 192
HD = HB * DH
M = 8
SEG = 32
L = M + SEG
PW = 2 * DH
NP = HB // 2
TB = 128
KE = 7

NT = (((1,), (1,)), ((), ()))
LOG2E = 1.4426950408889634
HALF_ULP = 0.0040612


def _dot(a, b):
    return jnp.dot(a, b, preferred_element_type=F32)


def _dot_nt(a, b):
    return lax.dot_general(a, b, NT, preferred_element_type=F32)


def _pack(a):
    return pltpu.bitcast(a, U32)


def _unpack(a):
    return pltpu.bitcast(a, BF16)


def _interleave(a, b):
    lo = lax.bitcast_convert_type(a, U32) >> 16
    hi = lax.bitcast_convert_type(b, U32) & jnp.uint32(0xFFFF0000)
    return lo | hi


def _recip(x):
    r = pl.reciprocal(x, approx=True)
    return r * (2.0 - x * r)


def _layernorm(x):
    m = jnp.mean(x, axis=-1, keepdims=True)
    c = x - m
    v = jnp.mean(c * c, axis=-1, keepdims=True)
    return c * lax.rsqrt(v + 1e-5)


def _feature_map(p):
    t = p.shape[-1]
    p3 = jnp.concatenate([jnp.zeros((8, t), F32), p], axis=0).reshape(FA, 8, t)
    mx = jnp.max(p3, axis=0)
    mn = jnp.min(p3, axis=0)
    sp, sn = jnp.exp2(p3[0] - mx), jnp.exp2(mn - p3[0])
    for f in range(1, FA):
        sp, sn = sp + jnp.exp2(p3[f] - mx), sn + jnp.exp2(mn - p3[f])
    lp = (mx - HALF_ULP) + jnp.log2(sp)
    ln = (mn + HALF_ULP) - jnp.log2(sn)
    return [_interleave(jnp.exp2(p3[f] - lp), jnp.exp2(ln - p3[f])) for f in range(FA)]


def _tiles(a, odd):
    t0, t1, t2 = a[:, 0:128], a[:, 128:256], a[:, 256:384]
    return (t1, t2, t0) if odd else (t1, t0, t2)


def _own_weights(a, odd):
    lane = lax.broadcasted_iota(jnp.int32, (L, 128), 1)
    mid, own, _ = _tiles(a, odd)
    return jnp.concatenate(
        [jnp.where(lane < 64, mid, 0.0), jnp.where(lane < 64, 0.0, mid), own,
         jnp.zeros((128 - 3 * L, 128), F32)], axis=0).astype(BF16)


def _others(even, odd, pad):
    parts = [_tiles(odd, 1)[2], _tiles(even, 0)[2]]
    if pad:
        parts.append(jnp.zeros((128 - 2 * L, 128), F32))
    return jnp.concatenate(parts, axis=0).astype(BF16)


def _softmax3(s3):
    row = lax.broadcasted_iota(jnp.int32, (L, 128), 0)
    col = lax.broadcasted_iota(jnp.int32, (L, 128), 1)
    first = col < L
    second = jnp.logical_and(col >= L, col < 2 * L)
    key = jnp.where(first, col, col - L)
    valid = jnp.logical_or(row < M, row >= key)
    out, other = [], []
    for odd in range(2):
        own = pltpu.roll(s3[odd][L:, :], 128 - L if odd else 128 - 2 * L, 1)
        s = (jnp.where(first, s3[2][0:L, :], own) if odd
             else jnp.where(first, own, s3[2][L:, :]))
        s = jnp.where(valid, (s + s3[odd][0:L, :]) * (DH ** -0.5), -1e9)
        m0 = jnp.max(jnp.where(first, s, -jnp.inf), axis=-1, keepdims=True)
        m1 = jnp.max(jnp.where(second, s, -jnp.inf), axis=-1, keepdims=True)
        e = jnp.exp(s - jnp.where(first, m0, m1))
        e0 = jnp.where(first, e, 0.0)
        e1 = jnp.where(second, e, 0.0)
        p0 = e0 * _recip(jnp.sum(e0, axis=-1, keepdims=True))
        p1 = e1 * _recip(jnp.sum(e1, axis=-1, keepdims=True))
        own = pltpu.roll(p1, L, 1) if odd else pltpu.roll(p0, 2 * L, 1)
        out.append(jnp.concatenate([p0 + p1, own], axis=0).astype(BF16))
        other.append(p0 if odd else p1)
    out.append(jnp.concatenate([other[1], other[0]], axis=0).astype(BF16))
    return out


def _segment(h, hk, wqv, wk, wob, fix_qv, fix_k, fix_o, chained):
    ys, ks, ss, ps, pvs, os_ = {}, {}, {}, {}, {}, {}
    kg = 2

    def proj(p):
        cols = slice(p * 2 * PW, (p + 1) * 2 * PW)
        if p == 0 and chained:
            ksp = 512
            y = _dot(h[:, 0:ksp], _unpack(wqv[0:ksp // 2, cols]))
            y = _dot(h[:, ksp:], _unpack(wqv[ksp // 2:, cols])) + y
        else:
            y = _dot(h, _unpack(wqv[:, cols]))
        y = fix_qv(p, y)
        if p % kg == 0:
            k = _dot(hk, _unpack(wk[:, p * PW:(p + kg) * PW]))
            for e in range(kg):
                ks[p + e] = fix_k(p + e, k[:, e * PW:(e + 1) * PW])
        ys[p] = [y[:, 0:PW], ks.pop(p), y[:, PW:]]

    def weights(c, i, which):
        if i < 2:
            return _own_weights(ys[2 * c + i][which], i)
        return _others(ys[2 * c][which], ys[2 * c + 1][which], True)

    def score_round(n):
        for c, i in (divmod(j, 3) for j in range(4 * n, 4 * n + 4)):
            if i < 2:
                q = jnp.concatenate(_tiles(ys[2 * c + i][0], i)[0:2], axis=0).astype(BF16)
            else:
                q = _others(ys[2 * c][0], ys[2 * c + 1][0], False)
            ss[c, i] = _dot_nt(q, weights(c, i, 1))
            if i == 2:
                ps[c] = _softmax3([ss.pop((c, k)) for k in range(3)])

    def pv_round(n):
        for c, i in (divmod(j, 3) for j in range(4 * n, 4 * n + 4)):
            pvs[c, i] = _dot(ps[c][i], weights(c, i, 2))
            if i == 2:
                o0, o1, o2 = [pvs.pop((c, k)) for k in range(3)]
                os_[2 * c] = fix_o(2 * c, jnp.concatenate(
                    [o0[L:, :], o0[0:L, :], o2[L:, :]], axis=1))
                os_[2 * c + 1] = fix_o(2 * c + 1, jnp.concatenate(
                    [o2[0:L, :], o1[0:L, :], o1[L:, :]], axis=1))

    def slot(n):
        if n >= 2:
            pv_round(n - 2)
        if n < 6:
            score_round(n)

    def oproj(lo, hi):
        o = jnp.concatenate([os_.pop(p) for p in range(lo, hi)], axis=1).astype(BF16)
        return _dot(o, _unpack(wob[lo * DH:hi * DH, :]))

    after = {3: 0, 6: 1, 9: 2, 11: 3, 14: 4}
    for p in range(NP):
        proj(p)
        if p in after:
            slot(after[p])
    o1, o2, o3 = (2, 8, 10) if h.shape[0] == 48 else (2, 7, 10)
    r = oproj(0, o1)
    slot(5)
    r = oproj(o1, o2) + r
    slot(6)
    slot(7)
    r = oproj(o2, o3) + r
    return oproj(o3, NP) + r


def _kernel(x_hbm, wqkv_hbm, wphi_hbm, woa_hbm, mem0_hbm,
            wq_hbm, wk_hbm, wv_hbm, wo_hbm,
            out_hbm,
            xio, wqkv, wphi, woa, mem0, xres, xa, xb, bds, wat, phq, phk, kvacc, kvs, osc,
            wraw, wqv, wk, wob, xe, ke, ysave, osave, rsave, sem_in, sem_out):
    nt = S // TN
    nsub = TN // 128
    na = S // TA
    asub = TA // 128
    nb = S // TB
    nw = NP // 2

    def rows(j, n):
        return pl.ds(j * n if isinstance(j, int) else pl.multiple_of(j * n, n), n)

    def x_copy(j):
        if isinstance(j, int) and j < 0:
            r = pl.ds(0, 128)
        elif isinstance(j, int) and j == na - 1:
            r = pl.ds(S - TA + 128, TA - 128)
        else:
            r = pl.ds(j * TA + 128 if isinstance(j, int)
                      else pl.multiple_of(j * TA + 128, 128), TA)
        return pltpu.make_async_copy(x_hbm.at[r, :], xio.at[r, :], sem_in.at[9 + j])

    def w_copies(c):
        r = rows(c, 2 * PW)
        return [pltpu.make_async_copy(src.at[r, :], wraw.at[i, r, :],
                                      sem_in.at[10 + nt + 3 * c + i])
                for i, src in enumerate((wq_hbm, wv_hbm, wo_hbm))]

    def wa_copy(r):
        return pltpu.make_async_copy(wqkv_hbm.at[rows(r, 128), :], wqkv.at[rows(r, 128), :],
                                     sem_in.at[3 + r])

    def out_copy(i):
        return pltpu.make_async_copy(xio.at[rows(i, TB), :],
                                     out_hbm.at[rows(i, TB), :], sem_out.at[0])

    wphi_copy = pltpu.make_async_copy(wphi_hbm, wphi, sem_in.at[0])
    woa_copy = pltpu.make_async_copy(woa_hbm, woa, sem_in.at[1])
    mem0_copy = pltpu.make_async_copy(mem0_hbm, mem0, sem_in.at[2])
    order = [wphi_copy, x_copy(-1)] + [wa_copy(r) for r in range(D // 128)]
    wk_copy = pltpu.make_async_copy(wk_hbm, wraw.at[3], sem_in.at[9 + nt])
    order += [x_copy(j) for j in range(na)] + [woa_copy, mem0_copy, wk_copy]
    for c in range(nw):
        order += w_copies(c)
    for c in order:
        c.start()

    def ln_in(t, first):
        x = xio[rows(t, 128), :].astype(F32)
        if first is not True:
            x = jnp.where(first, x, xres[rows(t, 128), :])
        xres[rows(t, 128), :] = x
        return _pack(_layernorm(x).astype(BF16))

    wphi_copy.wait()
    x_copy(-1).wait()
    cphi = jnp.zeros((FA, D), F32)
    hh = lax.broadcasted_iota(jnp.int32, (HA, D), 0) * FA
    jj = lax.broadcasted_iota(jnp.int32, (HA, D), 1)
    for d in range(FA):
        cphi = _dot(wphi[d], jnp.where(jj == hh + d, 1.0, 0.0).astype(BF16)) + cphi
    cb = jnp.concatenate(
        [jnp.broadcast_to(cphi[f:f + 1, :], (8, D)) for f in range(FA)], axis=0)
    for g in range(GA):
        row = lax.broadcasted_iota(jnp.int32, (GR, 256), 0)
        col = lax.broadcasted_iota(jnp.int32, (GR, 256), 1) + 128 * g
        lo = (8 * g + (row & 7)) * FA
        bds[g] = _pack(jnp.where(jnp.logical_and(col >= lo, col < lo + FA),
                                 cb[:, 128 * g:128 * g + 256], 0.0).astype(BF16))
    xa[rows(0, 64), :] = ln_in(0, True)

    def fold(r, _):
        wa_copy(r).wait()
        rr = rows(r, 128)
        for g in range(GA):
            ws = []
            for i in range(2):
                c0 = i * D + 128 * g
                w = _dot_nt(_unpack(bds[g]), wqkv[rr, c0:c0 + 256]).reshape(FA, 8, 128)
                ws.append(((w[1:] - w[0:1]) * LOG2E).reshape(GR - 8, 128))
            wat[GA + g, :, rr] = _pack(
                jnp.concatenate([ws[1], ws[0][GR - 16:, :]], axis=0).astype(BF16))
            wat[g, 0:GR // 2 - 8, rr] = _pack(ws[0][0:GR - 16, :].astype(BF16))
        wvt = _pack(wqkv[rr, 2 * D:3 * D].T)
        for g in range(GA):
            wat[2 * GA + g, :, rr] = wvt[g * GR // 2:(g + 1) * GR // 2, :]
        return 0

    lax.fori_loop(0, D // 128, fold, 0)

    def pair_rows(ph, q, t0, n):
        return _unpack(jnp.concatenate(
            [ph[t0 + u, rows(q, 2 * FA), :] for u in range(n)], axis=1))

    def a1(first, j, _):
        @pl.when(jnp.logical_and(first, j < na - 1))
        def _():
            x_copy(j).wait()

        @pl.when(jnp.logical_and(first, j == na - 1))
        def _():
            x_copy(na - 1).wait()

        def features(ph, t, g, y):
            for f, w in enumerate(_feature_map(y)):
                ph[t, pl.ds(GR * g + f, 8, stride=FA), :] = w

        vs = {}
        for u in range(asub):
            t = j * asub + u
            xn = _unpack(ln_in(t, first) if u > 0 else xa[rows(t, 64), :])
            for g in range(GA):
                y = _dot_nt(_unpack(wat[GA + g]), xn)
                features(phk, u, g, y[0:GR - 8, :])
                yq = _dot_nt(_unpack(wat[g, 0:GR // 2 - 8, :]), xn)
                features(phq, t, g, jnp.concatenate([yq, y[GR - 8:, :]], axis=0))
            for g in range(GA):
                y = _dot_nt(_unpack(wat[2 * GA + g]), xn)
                for q in range(4):
                    vs[4 * g + q, u] = y[40 * q:40 * q + 40, :]
        for q in range(PA):
            v = jnp.concatenate([vs[q, u] for u in range(asub)], axis=1)
            v = jnp.concatenate([v, jnp.ones((8, TA), F32)], axis=0)
            kv = _dot_nt(v.astype(BF16), pair_rows(phk, q, 0, asub))
            kvacc[q] = kv + jnp.where(j == 0, 0.0, kvacc[q])
        tn = jnp.minimum(j + 1, na - 1) * asub
        xa[rows(tn, 64), :] = ln_in(tn, first)
        return 0

    def attend(j):
        low = lax.broadcasted_iota(jnp.int32, (8, TN), 0) < 4
        os_ = []
        for q in range(PA):
            nd = _dot(_unpack(kvs[q]), pair_rows(phq, q, j * nsub, nsub))
            rab = 1.0 / (nd[40:48, :] + 1e-6)
            rba = pltpu.roll(rab, 4, 0)
            ra = jnp.where(low, rab, rba)
            rb = jnp.where(low, rba, rab)
            os_.append(nd[0:40, :] * jnp.concatenate([ra, ra, rab, rb, rb], axis=0))
        return _pack(jnp.concatenate(os_, axis=0).astype(BF16).T)

    def project(j, o):
        r = rows(j, TN)
        xres[r, :] = _dot(_unpack(o), woa[...]) + xres[r, :]

    def extra_rows(j):
        ns = TN // SEG
        x = jnp.concatenate(
            [xres[rows(j * (TN // 8) + (s // 2) * 8 + 3 + s % 2, 8), :] for s in range(ns)],
            axis=0)
        x = _layernorm(x).reshape(ns, 8, D)
        x = x - x[:, KE:KE + 1, :]
        for s in range(ns):
            for c in range(D // 128):
                xe[c, pl.ds((j * ns + s) * KE, 8), :] = x[s, :, 128 * c:128 * (c + 1)]

    def extra_keys(seg, p):
        k = jnp.concatenate(
            [ke[3 * p + c, pl.ds(seg * KE, 8), :] for c in range(3)], axis=1)
        return jnp.where(lax.broadcasted_iota(jnp.int32, (8, PW), 0) < KE, k, 0.0)

    def relayout_wk(j):
        r = rows(j, HD // nt)
        wk[:, r] = _pack(wraw[3, r, :].T)

    def b_finish(i):
        r = rows(i, TB)
        x = xres[r, :] + rsave[...]
        xres[r, :] = x
        xn = _layernorm(x)
        xa[rows(i, TB // 2), :] = _pack(xn.astype(BF16))
        xio[r, :] = x.astype(BF16)
        return xn

    def b_pair(mem, xn, base, blk, side):
        def fix_qva(p, y):
            c0 = 2 * PW - D
            tie = jnp.where(blk < 0, side[8 * p:8 * p + 8, :], y[0:M, c0:])
            ysave[:, p * 2 * PW:(p + 1) * 2 * PW] = y[L:L + 8, :]
            return jnp.concatenate(
                [jnp.concatenate([y[0:M, 0:c0], tie], axis=1), y[M:L, :]], axis=0)

        def fix_ka(p, k):
            return jnp.concatenate([k, extra_keys(2 * blk, p)], axis=0)

        def fix_oa(p, o):
            osave[:, p * PW:(p + 1) * PW] = o[32:L, :]
            return o[0:32, :]

        h = jnp.concatenate([mem, xn[0:40, :]], axis=0)
        ra = _segment(h.astype(BF16), (h[0:32, :] - xn[31:32, :]).astype(BF16),
                      wqv, wk, wob, fix_qva, fix_ka, fix_oa, base > 0)
        rsave[base:base + 24, :] = ra[M:, :]

        def fix_qvb(p, y):
            return jnp.concatenate(
                [y[0:M, :], ysave[:, p * 2 * PW:(p + 1) * 2 * PW], y[M:, :]], axis=0)

        def fix_kb(p, k):
            return jnp.concatenate([k[0:M, :], extra_keys(2 * blk + 1, p), k[M:, :]], axis=0)

        def fix_ob(p, o):
            return jnp.concatenate([o, osave[:, p * PW:(p + 1) * PW]], axis=0)

        h = jnp.concatenate([ra[0:M, :], xn[40:64, :]], axis=0)
        rb = _segment(h.astype(BF16), (h - xn[39:40, :]).astype(BF16),
                      wqv, wk, wob, fix_qvb, fix_kb, fix_ob, True)
        rsave[base + 24:base + 32, :] = rb[L:, :]
        rsave[base + 32:base + 64, :] = rb[M:L, :]
        return rb[0:M, :]

    def layer(l, _):
        def wait_first(copies):
            @pl.when(l == 0)
            def _():
                for c in copies:
                    c.wait()

        with jax.named_scope("a1"):
            lax.fori_loop(0, na, functools.partial(a1, l == 0), 0)

        with jax.named_scope("kv"):
            wait_first([woa_copy, mem0_copy, wk_copy])
            row = lax.broadcasted_iota(jnp.int32, (2 * VR, 4 * FA), 0)
            col = lax.broadcasted_iota(jnp.int32, (2 * VR, 4 * FA), 1)
            split = jnp.where(row < 2 * FA, FA, 2 * FA + 4)
            same = (row >= split) == (col >= 2 * FA)
            for q in range(PA):
                kvs[q] = _pack(jnp.where(same, kvacc[q], 0.0).astype(BF16))
            o = attend(0)
            osc[...] = attend(1)
            project(0, o)
            relayout_wk(0)

        def a2(j, _):
            extra_rows(j - 1)
            o = osc[...]
            osc[...] = attend(j + 1)
            project(j, o)
            relayout_wk(j)
            return 0

        with jax.named_scope("a2"):
            lax.fori_loop(1, nt - 1, a2, 0, unroll=1)
        xb[...] = _layernorm(xres[rows(0, TB), :])
        rsave[...] = jnp.zeros(rsave.shape, F32)
        extra_rows(nt - 2)
        relayout_wk(nt - 1)
        for part in ((1, 2), (0, 3)):
            grp = [b + k for b in range(0, TN // 16, 4) for k in part]
            o = jnp.concatenate([osc[8 * g:8 * g + 8, :] for g in grp], axis=0)
            y = _dot(_unpack(o), woa[...])
            for n, g in enumerate(grp):
                r = pl.ds(S - TN + 16 * g, 16)
                xres[r, :] = y[16 * n:16 * n + 16, :] + xres[r, :]
            if part == (1, 2):
                extra_rows(nt - 1)

        pc = 2

        def b_pre(n, _):
            wait_first([cp for e in range(pc) for cp in w_copies(pc * n + e)])
            mr = 16 * KE
            for c in range(pc):
                c = pc * n + c
                for m in range(S // SEG * KE // mr):
                    x = jnp.concatenate(
                        [xe[t, m * mr:(m + 1) * mr, :] for t in range(D // 128)], axis=1)
                    k = _dot(x.astype(BF16), _unpack(wk[:, rows(c, 2 * PW)]))
                    for t in range(2 * PW // 128):
                        ke[6 * c + t, m * mr:(m + 1) * mr, :] = k[:, 128 * t:128 * (t + 1)]
                        e = (c * 4 + m) * 6 + t
                        tie = pltpu.bitcast(k[0:16, 128 * t:128 * (t + 1)], U32)
                        wob[rows(e, 16), :] = jnp.where(
                            n < 0, jnp.concatenate([tie] * (D // 128), axis=1),
                            _pack(wraw[2, rows(e, 32), :]))
                for e in range(2):
                    p = 2 * c + e
                    wqv[:, rows(2 * p, PW)] = _pack(wraw[0, rows(p, PW), :].T)
                    wqv[:, rows(2 * p + 1, PW)] = _pack(wraw[1, rows(p, PW), :].T)
            return 0

        with jax.named_scope("pre"):
            lax.fori_loop(0, nw // pc, b_pre, 0)

        def b_step(i, mem):
            xn = xb[...]
            side = b_finish(jnp.maximum(i - 1, 0))
            nxt = _layernorm(xres[rows(jnp.minimum(i + 1, nb - 1), TB), :])
            xb[...] = nxt
            side = jnp.concatenate([side, nxt], axis=0)
            for u in range(0, TB, 2 * SEG):
                mem = b_pair(mem, xn[u:u + 2 * SEG, :], u, (i * TB + u) // (2 * SEG),
                             side[2 * u:2 * u + 8 * NP, :])

            @pl.when(jnp.logical_and(l == 1, i >= 1))
            def _():
                out_copy(i - 1).start()
            return mem

        with jax.named_scope("b"):
            lax.fori_loop(0, nb, b_step, mem0[...].astype(F32))

        x = xres[rows(nb - 1, TB), :] + rsave[...]
        xres[rows(nb - 1, TB), :] = x
        xio[rows(nb - 1, TB), :] = x.astype(BF16)
        return 0

    lax.fori_loop(0, 2, layer, 0)
    out_copy(nb - 1).start()
    pltpu.make_async_copy(xio, out_hbm, sem_out.at[0]).wait()


@functools.partial(jax.jit, static_argnames=("B_seg_len",))
def pallas_interleave_layers__linear_kernel_hedgehog__memory_aug_recurrent_mem_tr__prompt_kernel(
    A_x, A_wqkv, A_w_phi, A_wo, B_x, B_mem0, B_Wq, B_Wk, B_Wv, B_Wo, B_seg_len,
):
    del B_x
    assert B_seg_len == SEG
    x = A_x.reshape(S, D)
    wphi = A_w_phi.transpose(1, 2, 0)
    mem0 = B_mem0.reshape(M, D)
    wq, wk, wv = (w.transpose(1, 2, 0).reshape(HD, D) for w in (B_Wq, B_Wk, B_Wv))
    wo = B_Wo.reshape(HD, D)
    hbm = pl.BlockSpec(memory_space=pl.ANY)
    out = pl.pallas_call(
        _kernel,
        out_shape=jax.ShapeDtypeStruct((S, D), A_x.dtype),
        in_specs=[hbm] * 9,
        out_specs=hbm,
        scratch_shapes=[
            pltpu.VMEM((S, D), BF16),
            pltpu.VMEM((D, 3 * D), BF16),
            pltpu.VMEM((FA, FA, HA), BF16),
            pltpu.VMEM((D, D), BF16),
            pltpu.VMEM((M, D), BF16),
            pltpu.VMEM((S, D), F32),
            pltpu.VMEM((S // 2, D), U32),
            pltpu.VMEM((TB, D), F32),
            pltpu.VMEM((GA, GR // 2, 256), U32),
            pltpu.VMEM((3 * GA, GR // 2, D), U32),
            pltpu.VMEM((S // 128, D, 128), U32),
            pltpu.VMEM((TA // 128, D, 128), U32),
            pltpu.VMEM((PA, 2 * VR, 4 * FA), F32),
            pltpu.VMEM((PA, VR, 4 * FA), U32),
            pltpu.VMEM((TN // 2, D), U32),
            pltpu.VMEM((4, HD, D), BF16),
            pltpu.VMEM((D // 2, 2 * HD), U32),
            pltpu.VMEM((D // 2, HD), U32),
            pltpu.VMEM((HD // 2, D), U32),
            pltpu.VMEM((D // 128, S // SEG * KE + 8, 128), F32),
            pltpu.VMEM((HD // 128, S // SEG * KE + 8, 128), F32),
            pltpu.VMEM((8, 2 * HD), F32),
            pltpu.VMEM((8, HD), F32),
            pltpu.VMEM((TB, D), F32),
            pltpu.SemaphoreType.DMA((10 + S // TN + 3 * NP // 2,)),
            pltpu.SemaphoreType.DMA((1,)),
        ],
        compiler_params=pltpu.CompilerParams(vmem_limit_bytes=120 * 1024 * 1024,
                                             disable_bounds_checks=True,
                                             disable_semaphore_checks=True),
    )(x, A_wqkv, wphi, A_wo, mem0, wq, wk, wv, wo)
    return out.reshape(1, S, D)
```

```python
import functools

import jax
import jax.numpy as jnp
from jax import lax
import jax.experimental.pallas as pl
import jax.experimental.pallas.tpu as pltpu

F32 = jnp.float32
BF16 = jnp.bfloat16
U32 = jnp.uint32

S = 2048
D = 640
HA = 32
FA = 20
GA = 4
GR = 8 * FA
VR = 24
PA = HA // 2
TN = 256
TA = 512
HB = 32
DH = 192
HD = HB * DH
M = 8
SEG = 32
L = M + SEG
PW = 2 * DH
NP = HB // 2
TB = 128
NW = 4
QW = HD // NW
KE = 7

NT = (((1,), (1,)), ((), ()))
LOG2E = 1.4426950408889634
HALF_ULP = 0.0040612


def _dot(a, b):
    return jnp.dot(a, b, preferred_element_type=F32)


def _dot_nt(a, b):
    return lax.dot_general(a, b, NT, preferred_element_type=F32)


def _pack(a):
    return pltpu.bitcast(a, U32)


def _unpack(a):
    return pltpu.bitcast(a, BF16)


def _interleave(a, b):
    lo = lax.bitcast_convert_type(a, U32) >> 16
    hi = lax.bitcast_convert_type(b, U32) & jnp.uint32(0xFFFF0000)
    return lo | hi


def _recip(x):
    r = pl.reciprocal(x, approx=True)
    return r * (2.0 - x * r)


def _layernorm(x):
    m = jnp.mean(x, axis=-1, keepdims=True)
    c = x - m
    v = jnp.mean(c * c, axis=-1, keepdims=True)
    return c * lax.rsqrt(v + 1e-5)


def _feature_map(p):
    t = p.shape[-1]
    p3 = jnp.concatenate([jnp.zeros((8, t), F32), p], axis=0).reshape(FA, 8, t)
    mx = jnp.max(p3, axis=0)
    mn = jnp.min(p3, axis=0)
    sp, sn = jnp.exp2(p3[0] - mx), jnp.exp2(mn - p3[0])
    for f in range(1, FA):
        sp, sn = sp + jnp.exp2(p3[f] - mx), sn + jnp.exp2(mn - p3[f])
    lp = (mx - HALF_ULP) + jnp.log2(sp)
    ln = (mn + HALF_ULP) - jnp.log2(sn)
    return [_interleave(jnp.exp2(p3[f] - lp), jnp.exp2(ln - p3[f])) for f in range(FA)]


def _tiles(a, odd):
    t0, t1, t2 = a[:, 0:128], a[:, 128:256], a[:, 256:384]
    return (t1, t2, t0) if odd else (t1, t0, t2)


def _own_weights(a, odd):
    lane = lax.broadcasted_iota(jnp.int32, (L, 128), 1)
    mid, own, _ = _tiles(a, odd)
    return jnp.concatenate(
        [jnp.where(lane < 64, mid, 0.0), jnp.where(lane < 64, 0.0, mid), own,
         jnp.zeros((128 - 3 * L, 128), F32)], axis=0).astype(BF16)


def _others(even, odd, pad):
    parts = [_tiles(odd, 1)[2], _tiles(even, 0)[2]]
    if pad:
        parts.append(jnp.zeros((128 - 2 * L, 128), F32))
    return jnp.concatenate(parts, axis=0).astype(BF16)


def _softmax3(s3):
    row = lax.broadcasted_iota(jnp.int32, (L, 128), 0)
    col = lax.broadcasted_iota(jnp.int32, (L, 128), 1)
    first = col < L
    second = jnp.logical_and(col >= L, col < 2 * L)
    key = jnp.where(first, col, col - L)
    valid = jnp.logical_or(row < M, row >= key)
    out, other = [], []
    for odd in range(2):
        own = pltpu.roll(s3[odd][L:, :], 128 - L if odd else 128 - 2 * L, 1)
        s = (jnp.where(first, s3[2][0:L, :], own) if odd
             else jnp.where(first, own, s3[2][L:, :]))
        s = jnp.where(valid, (s + s3[odd][0:L, :]) * (DH ** -0.5), -1e9)
        m0 = jnp.max(jnp.where(first, s, -jnp.inf), axis=-1, keepdims=True)
        m1 = jnp.max(jnp.where(second, s, -jnp.inf), axis=-1, keepdims=True)
        e = jnp.exp(s - jnp.where(first, m0, m1))
        e0 = jnp.where(first, e, 0.0)
        e1 = jnp.where(second, e, 0.0)
        p0 = e0 * _recip(jnp.sum(e0, axis=-1, keepdims=True))
        p1 = e1 * _recip(jnp.sum(e1, axis=-1, keepdims=True))
        own = pltpu.roll(p1, L, 1) if odd else pltpu.roll(p0, 2 * L, 1)
        out.append(jnp.concatenate([p0 + p1, own], axis=0).astype(BF16))
        other.append(p0 if odd else p1)
    out.append(jnp.concatenate([other[1], other[0]], axis=0).astype(BF16))
    return out


def _segment(h, hk, wqv, wk, wob, fix_qv, fix_k, fix_o, chained):
    ys, ks, ss, ps, pvs, os_ = {}, {}, {}, {}, {}, {}
    kg = 2

    def proj(p):
        n, e = divmod(p, NP // NW)
        cols = slice(e * 2 * PW, (e + 1) * 2 * PW)
        if p == 0 and chained:
            ksp = 512
            y = _dot(h[:, 0:ksp], _unpack(wqv[n, 0:ksp // 2, cols]))
            y = _dot(h[:, ksp:], _unpack(wqv[n, ksp // 2:, cols])) + y
        else:
            y = _dot(h, _unpack(wqv[n, :, cols]))
        y = fix_qv(p, y)
        if p % kg == 0:
            k = _dot(hk, _unpack(wk[n, :, e * PW:(e + kg) * PW]))
            for i in range(kg):
                ks[p + i] = fix_k(p + i, k[:, i * PW:(i + 1) * PW])
        ys[p] = [y[:, 0:PW], ks.pop(p), y[:, PW:]]

    def weights(c, i, which):
        if i < 2:
            return _own_weights(ys[2 * c + i][which], i)
        return _others(ys[2 * c][which], ys[2 * c + 1][which], True)

    def score_round(n):
        for c, i in (divmod(j, 3) for j in range(4 * n, 4 * n + 4)):
            if i < 2:
                q = jnp.concatenate(_tiles(ys[2 * c + i][0], i)[0:2], axis=0).astype(BF16)
            else:
                q = _others(ys[2 * c][0], ys[2 * c + 1][0], False)
            ss[c, i] = _dot_nt(q, weights(c, i, 1))
            if i == 2:
                ps[c] = _softmax3([ss.pop((c, k)) for k in range(3)])

    def pv_round(n):
        for c, i in (divmod(j, 3) for j in range(4 * n, 4 * n + 4)):
            pvs[c, i] = _dot(ps[c][i], weights(c, i, 2))
            if i == 2:
                o0, o1, o2 = [pvs.pop((c, k)) for k in range(3)]
                os_[2 * c] = fix_o(2 * c, jnp.concatenate(
                    [o0[L:, :], o0[0:L, :], o2[L:, :]], axis=1))
                os_[2 * c + 1] = fix_o(2 * c + 1, jnp.concatenate(
                    [o2[0:L, :], o1[0:L, :], o1[L:, :]], axis=1))

    def slot(n):
        if n >= 2:
            pv_round(n - 2)
        if n < 6:
            score_round(n)

    def rows_of(e):
        return slice(e * DH, (e + 1) * DH)

    def oproj(lo, hi):
        o = jnp.concatenate([os_.pop(p) for p in range(lo, hi)], axis=1).astype(BF16)
        w = [wob[p // (NP // NW), rows_of(p % (NP // NW)), :] for p in range(lo, hi)]
        return _dot(o, _unpack(jnp.concatenate(w, axis=0)))

    after = {3: 0, 6: 1, 9: 2, 11: 3, 14: 4}
    for p in range(NP):
        proj(p)
        if p in after:
            slot(after[p])
    o1, o2, o3 = (2, 8, 10) if h.shape[0] == 48 else (2, 7, 10)
    r = oproj(0, o1)
    slot(5)
    r = oproj(o1, o2) + r
    slot(6)
    slot(7)
    r = oproj(o2, o3) + r
    return oproj(o3, NP) + r


def _kernel(x_hbm, wqkv_hbm, wphi_hbm, woa_hbm, mem0_hbm,
            wq_hbm, wk_hbm, wv_hbm, wo_hbm,
            out_hbm,
            xio, wqkv, wphi, woa, mem0, xres, xa, xb, bds, wat, phq, phk, kvacc, kvs,
            wraw, wqv, wk, wob, xe, ke, ysave, osave, rsave, sem_in, sem_out):
    nt = S // TN
    nsub = TN // 128
    na = S // TA
    asub = TA // 128
    nb = S // TB

    def rows(j, n):
        return pl.ds(j * n if isinstance(j, int) else pl.multiple_of(j * n, n), n)

    def x_copy(j):
        if isinstance(j, int) and j < 0:
            r = pl.ds(0, 128)
        elif isinstance(j, int) and j == na - 1:
            r = pl.ds(S - TA + 128, TA - 128)
        else:
            r = pl.ds(j * TA + 128 if isinstance(j, int)
                      else pl.multiple_of(j * TA + 128, 128), TA)
        return pltpu.make_async_copy(x_hbm.at[r, :], xio.at[r, :], sem_in.at[9 + j])

    def w_copies(c):
        return [pltpu.make_async_copy(src.at[c], wraw.at[i, c],
                                      sem_in.at[10 + nt + 3 * c + i])
                for i, src in enumerate((wq_hbm, wv_hbm, wo_hbm))]

    def wa_copy(r):
        return pltpu.make_async_copy(wqkv_hbm.at[rows(r, 128), :], wqkv.at[rows(r, 128), :],
                                     sem_in.at[3 + r])

    def out_copy(i):
        return pltpu.make_async_copy(xio.at[rows(i, TB), :],
                                     out_hbm.at[rows(i, TB), :], sem_out.at[0])

    wphi_copy = pltpu.make_async_copy(wphi_hbm, wphi, sem_in.at[0])
    woa_copy = pltpu.make_async_copy(woa_hbm, woa, sem_in.at[1])
    mem0_copy = pltpu.make_async_copy(mem0_hbm, mem0, sem_in.at[2])
    order = [wphi_copy, x_copy(-1)] + [wa_copy(r) for r in range(D // 128)]
    wk_copy = pltpu.make_async_copy(wk_hbm, wraw.at[3], sem_in.at[9 + nt])
    order += [x_copy(j) for j in range(na)] + [woa_copy, mem0_copy, wk_copy]
    for c in range(NW):
        order += w_copies(c)
    for c in order:
        c.start()

    def ln_in(t, first):
        x = xio[rows(t, 128), :].astype(F32)
        if first is not True:
            x = jnp.where(first, x, xres[rows(t, 128), :])
        xres[rows(t, 128), :] = x
        return _pack(_layernorm(x).astype(BF16))

    wphi_copy.wait()
    x_copy(-1).wait()
    cphi = jnp.zeros((FA, D), F32)
    hh = lax.broadcasted_iota(jnp.int32, (HA, D), 0) * FA
    jj = lax.broadcasted_iota(jnp.int32, (HA, D), 1)
    for d in range(FA):
        cphi = _dot(wphi[d], jnp.where(jj == hh + d, 1.0, 0.0).astype(BF16)) + cphi
    cb = jnp.concatenate(
        [jnp.broadcast_to(cphi[f:f + 1, :], (8, D)) for f in range(FA)], axis=0)
    for g in range(GA):
        row = lax.broadcasted_iota(jnp.int32, (GR, 256), 0)
        col = lax.broadcasted_iota(jnp.int32, (GR, 256), 1) + 128 * g
        lo = (8 * g + (row & 7)) * FA
        bds[g] = _pack(jnp.where(jnp.logical_and(col >= lo, col < lo + FA),
                                 cb[:, 128 * g:128 * g + 256], 0.0).astype(BF16))
    xa[rows(0, 64), :] = ln_in(0, True)

    def fold(r, _):
        wa_copy(r).wait()
        rr = rows(r, 128)
        for g in range(GA):
            ws = []
            for i in range(2):
                c0 = i * D + 128 * g
                w = _dot_nt(_unpack(bds[g]), wqkv[rr, c0:c0 + 256]).reshape(FA, 8, 128)
                ws.append(((w[1:] - w[0:1]) * LOG2E).reshape(GR - 8, 128))
            wat[GA + g, :, rr] = _pack(
                jnp.concatenate([ws[1], ws[0][GR - 16:, :]], axis=0).astype(BF16))
            wat[g, 0:GR // 2 - 8, rr] = _pack(ws[0][0:GR - 16, :].astype(BF16))
        wvt = _pack(wqkv[rr, 2 * D:3 * D].T)
        for g in range(GA):
            wat[2 * GA + g, :, rr] = wvt[g * GR // 2:(g + 1) * GR // 2, :]
        return 0

    lax.fori_loop(0, D // 128, fold, 0)

    def pair_rows(ph, q, t0, n):
        return _unpack(jnp.concatenate(
            [ph[t0 + u, rows(q, 2 * FA), :] for u in range(n)], axis=1))

    def a1(first, j, _):
        @pl.when(jnp.logical_and(first, j < na - 1))
        def _():
            x_copy(j).wait()

        @pl.when(jnp.logical_and(first, j == na - 1))
        def _():
            x_copy(na - 1).wait()

        def features(ph, t, g, y):
            for f, w in enumerate(_feature_map(y)):
                ph[t, pl.ds(GR * g + f, 8, stride=FA), :] = w

        vs = {}
        for u in range(asub):
            t = j * asub + u
            xn = _unpack(ln_in(t, first) if u > 0 else xa[rows(t, 64), :])
            for g in range(GA):
                y = _dot_nt(_unpack(wat[GA + g]), xn)
                features(phk, u, g, y[0:GR - 8, :])
                yq = _dot_nt(_unpack(wat[g, 0:GR // 2 - 8, :]), xn)
                features(phq, t, g, jnp.concatenate([yq, y[GR - 8:, :]], axis=0))
            for g in range(GA):
                y = _dot_nt(_unpack(wat[2 * GA + g]), xn)
                for q in range(4):
                    vs[4 * g + q, u] = y[40 * q:40 * q + 40, :]
        row = lax.broadcasted_iota(jnp.int32, (2 * VR, 4 * FA), 0)
        col = lax.broadcasted_iota(jnp.int32, (2 * VR, 4 * FA), 1)
        split = jnp.where(row < 2 * FA, FA, 2 * FA + 4)
        same = (row >= split) == (col >= 2 * FA)
        for q in range(PA):
            v = jnp.concatenate([vs[q, u] for u in range(asub)], axis=1)
            v = jnp.concatenate([v, jnp.ones((8, TA), F32)], axis=0)
            kv = _dot_nt(v.astype(BF16), pair_rows(phk, q, 0, asub))
            kv = kv + jnp.where(j == 0, 0.0, kvacc[q])
            kvacc[q] = kv
            kvs[q] = _pack(jnp.where(same, kv, 0.0).astype(BF16))
        tn = jnp.minimum(j + 1, na - 1) * asub
        xa[rows(tn, 64), :] = ln_in(tn, first)
        return 0

    def attend(j):
        low = lax.broadcasted_iota(jnp.int32, (8, TN), 0) < 4
        os_ = []
        for q in range(PA):
            nd = _dot(_unpack(kvs[q]), pair_rows(phq, q, j * nsub, nsub))
            rab = 1.0 / (nd[40:48, :] + 1e-6)
            rba = pltpu.roll(rab, 4, 0)
            ra = jnp.where(low, rab, rba)
            rb = jnp.where(low, rba, rab)
            os_.append(nd[0:40, :] * jnp.concatenate([ra, ra, rab, rb, rb], axis=0))
        return _pack(jnp.concatenate(os_, axis=0).astype(BF16).T)

    def project(j, o, slot):
        ns = TN // SEG
        xs = []
        r = rows(j, TN)
        old, new = xres[r, :], {}
        for part in ((1, 2), (0, 3)):
            grp = [b + k for b in range(0, TN // 16, 4) for k in part]
            oo = jnp.concatenate([o[8 * g:8 * g + 8, :] for g in grp], axis=0)
            x = _dot(_unpack(oo), woa[...]) + jnp.concatenate(
                [old[16 * g:16 * g + 16, :] for g in grp], axis=0)
            for n, g in enumerate(grp):
                new[g] = x[16 * n:16 * n + 16, :]
            xs.append(x)
        xres[r, :] = jnp.concatenate([new[g] for g in range(TN // 16)], axis=0)
        for s in range(ns):
            x = xs[0][16 * s + 8 - 8 * (s % 2):16 * s + 16 - 8 * (s % 2), :]
            x = _layernorm(x)
            x = x - x[KE:KE + 1, :]
            for c in range(D // 128):
                xe[c, pl.ds((slot * ns + s) * KE, 8), :] = x[:, 128 * c:128 * (c + 1)]

    def extra_keys(seg, p):
        k = jnp.concatenate(
            [ke[seg // 16, 3 * p + c, pl.ds((seg % 16) * KE, 8), :] for c in range(3)], axis=1)
        return jnp.where(lax.broadcasted_iota(jnp.int32, (8, PW), 0) < KE, k, 0.0)

    def b_finish(i):
        r = rows(i, TB)
        x = xres[r, :] + rsave[...]
        xres[r, :] = x
        xn = _layernorm(x)
        xa[rows(i, TB // 2), :] = _pack(xn.astype(BF16))
        xio[r, :] = x.astype(BF16)
        return xn

    def b_pair(mem, xn, base, blk, side):
        def fix_qva(p, y):
            c0 = 2 * PW - D
            tie = jnp.where(blk < 0, side[8 * p:8 * p + 8, :], y[0:M, c0:])
            ysave[:, p * 2 * PW:(p + 1) * 2 * PW] = y[L:L + 8, :]
            return jnp.concatenate(
                [jnp.concatenate([y[0:M, 0:c0], tie], axis=1), y[M:L, :]], axis=0)

        def fix_ka(p, k):
            return jnp.concatenate([k, extra_keys(2 * blk, p)], axis=0)

        def fix_oa(p, o):
            osave[:, p * PW:(p + 1) * PW] = o[32:L, :]
            return o[0:32, :]

        h = jnp.concatenate([mem, xn[0:40, :]], axis=0)
        ra = _segment(h.astype(BF16), (h[0:32, :] - xn[31:32, :]).astype(BF16),
                      wqv, wk, wob, fix_qva, fix_ka, fix_oa, base > 0)
        rsave[base:base + 24, :] = ra[M:, :]

        def fix_qvb(p, y):
            return jnp.concatenate(
                [y[0:M, :], ysave[:, p * 2 * PW:(p + 1) * 2 * PW], y[M:, :]], axis=0)

        def fix_kb(p, k):
            return jnp.concatenate([k[0:M, :], extra_keys(2 * blk + 1, p), k[M:, :]], axis=0)

        def fix_ob(p, o):
            return jnp.concatenate([o, osave[:, p * PW:(p + 1) * PW]], axis=0)

        h = jnp.concatenate([ra[0:M, :], xn[40:64, :]], axis=0)
        rb = _segment(h.astype(BF16), (h - xn[39:40, :]).astype(BF16),
                      wqv, wk, wob, fix_qvb, fix_kb, fix_ob, True)
        rsave[base + 24:base + 32, :] = rb[L:, :]
        rsave[base + 32:base + 64, :] = rb[M:L, :]
        return rb[0:M, :]

    def layer(l, _):
        def wait_first(copies):
            @pl.when(l == 0)
            def _():
                for c in copies:
                    c.wait()

        with jax.named_scope("a1"):
            lax.fori_loop(0, na, functools.partial(a1, l == 0), 0)

        def a2(n, _):
            wait_first(w_copies(n))
            o0 = attend(2 * n)
            o1 = attend(2 * n + 1)
            wk[n] = _pack(wraw[3, n].T)
            project(2 * n, o0, 0)
            project(2 * n + 1, o1, 1)
            r = rows(n, TB // NW)
            xb[r, :] = _layernorm(xres[r, :])
            rsave[r, :] = jnp.zeros((TB // NW, D), F32)
            mr = 16 * KE
            x = jnp.concatenate([xe[t, 0:mr, :] for t in range(D // 128)], axis=1).astype(BF16)
            for c in range(NW):
                k = _dot_nt(x, wraw[3, c])
                for t in range(QW // 128):
                    e = c * (QW // 128) + t
                    ke[n, e, 0:mr, :] = k[:, 128 * t:128 * (t + 1)]
                    tie = pltpu.bitcast(k[0:16, 128 * t:128 * (t + 1)], U32)
                    wob[n, rows(e, 16), :] = jnp.where(
                        n < 0, jnp.concatenate([tie] * (D // 128), axis=1),
                        _pack(wraw[2, n, rows(e, 32), :]))
            for p in range(NP // NW):
                wqv[n, :, rows(2 * p, PW)] = _pack(wraw[0, n, rows(p, PW), :].T)
                wqv[n, :, rows(2 * p + 1, PW)] = _pack(wraw[1, n, rows(p, PW), :].T)
            return 0

        wait_first([woa_copy, mem0_copy, wk_copy])
        with jax.named_scope("a2"):
            lax.fori_loop(0, NW, a2, 0)

        def b_step(i, mem):
            xn = xb[...]
            side = b_finish(jnp.maximum(i - 1, 0))
            nxt = _layernorm(xres[rows(jnp.minimum(i + 1, nb - 1), TB), :])
            xb[...] = nxt
            side = jnp.concatenate([side, nxt], axis=0)
            for u in range(0, TB, 2 * SEG):
                mem = b_pair(mem, xn[u:u + 2 * SEG, :], u, (i * TB + u) // (2 * SEG),
                             side[2 * u:2 * u + 8 * NP, :])

            @pl.when(jnp.logical_and(l == 1, i >= 1))
            def _():
                out_copy(i - 1).start()
            return mem

        with jax.named_scope("b"):
            lax.fori_loop(0, nb, b_step, mem0[...].astype(F32))

        x = xres[rows(nb - 1, TB), :] + rsave[...]
        xres[rows(nb - 1, TB), :] = x
        xio[rows(nb - 1, TB), :] = x.astype(BF16)
        return 0

    lax.fori_loop(0, 2, layer, 0)
    out_copy(nb - 1).start()
    pltpu.make_async_copy(xio, out_hbm, sem_out.at[0]).wait()


@functools.partial(jax.jit, static_argnames=("B_seg_len",))
def pallas_interleave_layers__linear_kernel_hedgehog__memory_aug_recurrent_mem_tr__prompt_kernel(
    A_x, A_wqkv, A_w_phi, A_wo, B_x, B_mem0, B_Wq, B_Wk, B_Wv, B_Wo, B_seg_len,
):
    del B_x
    assert B_seg_len == SEG
    x = A_x.reshape(S, D)
    wphi = A_w_phi.transpose(1, 2, 0)
    mem0 = B_mem0.reshape(M, D)
    wq, wk, wv = (w.transpose(1, 2, 0).reshape(NW, QW, D) for w in (B_Wq, B_Wk, B_Wv))
    wo = B_Wo.reshape(NW, QW, D)
    hbm = pl.BlockSpec(memory_space=pl.ANY)
    out = pl.pallas_call(
        _kernel,
        out_shape=jax.ShapeDtypeStruct((S, D), A_x.dtype),
        in_specs=[hbm] * 9,
        out_specs=hbm,
        scratch_shapes=[
            pltpu.VMEM((S, D), BF16),
            pltpu.VMEM((D, 3 * D), BF16),
            pltpu.VMEM((FA, FA, HA), BF16),
            pltpu.VMEM((D, D), BF16),
            pltpu.VMEM((M, D), BF16),
            pltpu.VMEM((S, D), F32),
            pltpu.VMEM((S // 2, D), U32),
            pltpu.VMEM((TB, D), F32),
            pltpu.VMEM((GA, GR // 2, 256), U32),
            pltpu.VMEM((3 * GA, GR // 2, D), U32),
            pltpu.VMEM((S // 128, D, 128), U32),
            pltpu.VMEM((TA // 128, D, 128), U32),
            pltpu.VMEM((PA, 2 * VR, 4 * FA), F32),
            pltpu.VMEM((PA, VR, 4 * FA), U32),
            pltpu.VMEM((4, NW, QW, D), BF16),
            pltpu.VMEM((NW, D // 2, 2 * QW), U32),
            pltpu.VMEM((NW, D // 2, QW), U32),
            pltpu.VMEM((NW, QW // 2, D), U32),
            pltpu.VMEM((D // 128, 16 * KE + 8, 128), F32),
            pltpu.VMEM((NW, HD // 128, 16 * KE + 8, 128), F32),
            pltpu.VMEM((8, 2 * HD), F32),
            pltpu.VMEM((8, HD), F32),
            pltpu.VMEM((TB, D), F32),
            pltpu.SemaphoreType.DMA((10 + S // TN + 3 * NP // 2,)),
            pltpu.SemaphoreType.DMA((1,)),
        ],
        compiler_params=pltpu.CompilerParams(vmem_limit_bytes=120 * 1024 * 1024,
                                             disable_bounds_checks=True,
                                             disable_semaphore_checks=True),
    )(x, A_wqkv, wphi, A_wo, mem0, wq, wk, wv, wo)
    return out.reshape(1, S, D)
```

```python
import functools

import jax
import jax.numpy as jnp
from jax import lax
import jax.experimental.pallas as pl
import jax.experimental.pallas.tpu as pltpu

F32 = jnp.float32
BF16 = jnp.bfloat16
U32 = jnp.uint32

S = 2048
D = 640
HA = 32
FA = 20
GA = 4
GR = 8 * FA
VR = 24
PA = HA // 2
TN = 256
TA = 512
HB = 32
DH = 192
HD = HB * DH
M = 8
SEG = 32
L = M + SEG
PW = 2 * DH
NP = HB // 2
TB = 128
NW = 4
QW = HD // NW
KE = 7

NT = (((1,), (1,)), ((), ()))
LOG2E = 1.4426950408889634
HALF_ULP = 0.0040612


def _dot(a, b):
    return jnp.dot(a, b, preferred_element_type=F32)


def _dot_nt(a, b):
    return lax.dot_general(a, b, NT, preferred_element_type=F32)


def _pack(a):
    return pltpu.bitcast(a, U32)


def _unpack(a):
    return pltpu.bitcast(a, BF16)


def _interleave(a, b):
    lo = lax.bitcast_convert_type(a, U32) >> 16
    hi = lax.bitcast_convert_type(b, U32) & jnp.uint32(0xFFFF0000)
    return lo | hi


def _recip(x):
    r = pl.reciprocal(x, approx=True)
    return r * (2.0 - x * r)


def _layernorm(x):
    m = jnp.mean(x, axis=-1, keepdims=True)
    c = x - m
    v = jnp.mean(c * c, axis=-1, keepdims=True)
    return c * lax.rsqrt(v + 1e-5)


def _feature_map(p):
    t = p.shape[-1]
    p3 = jnp.concatenate([jnp.zeros((8, t), F32), p], axis=0).reshape(FA, 8, t)
    mx = jnp.max(p3, axis=0)
    mn = jnp.min(p3, axis=0)
    sp, sn = jnp.exp2(p3[0] - mx), jnp.exp2(mn - p3[0])
    for f in range(1, FA):
        sp, sn = sp + jnp.exp2(p3[f] - mx), sn + jnp.exp2(mn - p3[f])
    lp = (mx - HALF_ULP) + jnp.log2(sp)
    ln = (mn + HALF_ULP) - jnp.log2(sn)
    return [_interleave(jnp.exp2(p3[f] - lp), jnp.exp2(ln - p3[f])) for f in range(FA)]


def _tiles(a, odd):
    t0, t1, t2 = a[:, 0:128], a[:, 128:256], a[:, 256:384]
    return (t1, t2, t0) if odd else (t1, t0, t2)


def _own_weights(a, odd):
    lane = lax.broadcasted_iota(jnp.int32, (L, 128), 1)
    mid, own, _ = _tiles(a, odd)
    return jnp.concatenate(
        [jnp.where(lane < 64, mid, 0.0), jnp.where(lane < 64, 0.0, mid), own,
         jnp.zeros((128 - 3 * L, 128), F32)], axis=0).astype(BF16)


def _others(even, odd, pad):
    parts = [_tiles(odd, 1)[2], _tiles(even, 0)[2]]
    if pad:
        parts.append(jnp.zeros((128 - 2 * L, 128), F32))
    return jnp.concatenate(parts, axis=0).astype(BF16)


def _softmax3(s3):
    row = lax.broadcasted_iota(jnp.int32, (L, 128), 0)
    col = lax.broadcasted_iota(jnp.int32, (L, 128), 1)
    first = col < L
    second = jnp.logical_and(col >= L, col < 2 * L)
    key = jnp.where(first, col, col - L)
    valid = jnp.logical_or(row < M, row >= key)
    out, other = [], []
    for odd in range(2):
        own = pltpu.roll(s3[odd][L:, :], 128 - L if odd else 128 - 2 * L, 1)
        s = (jnp.where(first, s3[2][0:L, :], own) if odd
             else jnp.where(first, own, s3[2][L:, :]))
        s = jnp.where(valid, (s + s3[odd][0:L, :]) * (DH ** -0.5), -1e9)
        m0 = jnp.max(jnp.where(first, s, -jnp.inf), axis=-1, keepdims=True)
        m1 = jnp.max(jnp.where(second, s, -jnp.inf), axis=-1, keepdims=True)
        e = jnp.exp(s - jnp.where(first, m0, m1))
        e0 = jnp.where(first, e, 0.0)
        e1 = jnp.where(second, e, 0.0)
        p0 = e0 * _recip(jnp.sum(e0, axis=-1, keepdims=True))
        p1 = e1 * _recip(jnp.sum(e1, axis=-1, keepdims=True))
        own = pltpu.roll(p1, L, 1) if odd else pltpu.roll(p0, 2 * L, 1)
        out.append(jnp.concatenate([p0 + p1, own], axis=0).astype(BF16))
        other.append(p0 if odd else p1)
    out.append(jnp.concatenate([other[1], other[0]], axis=0).astype(BF16))
    return out


def _segment(h, hk, wqv, wk, wob, fix_qv, fix_k, fix_o, chained):
    ys, ks, ss, ps, pvs, os_ = {}, {}, {}, {}, {}, {}
    kg = 4

    def proj(p):
        n, e = divmod(p, NP // NW)
        cols = slice(e * 2 * PW, (e + 1) * 2 * PW)
        if p == 0 and chained:
            ksp = 512
            y = _dot(h[:, 0:ksp], _unpack(wqv[n, 0:ksp // 2, cols]))
            y = _dot(h[:, ksp:], _unpack(wqv[n, ksp // 2:, cols])) + y
        else:
            y = _dot(h, _unpack(wqv[n, :, cols]))
        y = fix_qv(p, y)
        if p % kg == 0:
            k = _dot(hk, _unpack(wk[n, :, e * PW:(e + kg) * PW]))
            for i in range(kg):
                ks[p + i] = fix_k(p + i, k[:, i * PW:(i + 1) * PW])
        ys[p] = [y[:, 0:PW], ks.pop(p), y[:, PW:]]

    def weights(c, i, which):
        if i < 2:
            return _own_weights(ys[2 * c + i][which], i)
        return _others(ys[2 * c][which], ys[2 * c + 1][which], True)

    def score_round(n):
        for c, i in (divmod(j, 3) for j in range(4 * n, 4 * n + 4)):
            if i < 2:
                q = jnp.concatenate(_tiles(ys[2 * c + i][0], i)[0:2], axis=0).astype(BF16)
            else:
                q = _others(ys[2 * c][0], ys[2 * c + 1][0], False)
            ss[c, i] = _dot_nt(q, weights(c, i, 1))
            if i == 2:
                ps[c] = _softmax3([ss.pop((c, k)) for k in range(3)])

    def pv_round(n):
        for c, i in (divmod(j, 3) for j in range(4 * n, 4 * n + 4)):
            pvs[c, i] = _dot(ps[c][i], weights(c, i, 2))
            if i == 2:
                o0, o1, o2 = [pvs.pop((c, k)) for k in range(3)]
                os_[2 * c] = fix_o(2 * c, jnp.concatenate(
                    [o0[L:, :], o0[0:L, :], o2[L:, :]], axis=1))
                os_[2 * c + 1] = fix_o(2 * c + 1, jnp.concatenate(
                    [o2[0:L, :], o1[0:L, :], o1[L:, :]], axis=1))

    def slot(n):
        if n >= 2:
            pv_round(n - 2)
        if n < 6:
            score_round(n)

    def rows_of(e):
        return slice(e * DH, (e + 1) * DH)

    def oproj(lo, hi):
        o = jnp.concatenate([os_.pop(p) for p in range(lo, hi)], axis=1).astype(BF16)
        w = [wob[p // (NP // NW), rows_of(p % (NP // NW)), :] for p in range(lo, hi)]
        return _dot(o, _unpack(jnp.concatenate(w, axis=0)))

    after = {3: 0, 6: 1, 9: 2, 11: 3, 14: 4}
    for p in range(NP):
        proj(p)
        if p in after:
            slot(after[p])
    o1, o2, o3 = (2, 8, 10) if h.shape[0] == 48 else (2, 7, 10)
    r = oproj(0, o1)
    slot(5)
    r = oproj(o1, o2) + r
    slot(6)
    slot(7)
    r = oproj(o2, o3) + r
    return oproj(o3, NP) + r


def _kernel(x_hbm, wqkv_hbm, wphi_hbm, woa_hbm, mem0_hbm,
            wq_hbm, wk_hbm, wv_hbm, wo_hbm,
            out_hbm,
            xio, wqkv, wphi, woa, mem0, xres, xa, xb, bds, wat, phq, phk, kvacc, kvs,
            wraw, wqv, wk, wob, xe, ke, ysave, osave, rsave, sem_in, sem_out):
    nsub = TN // 128
    na = S // TA
    asub = TA // 128
    nb = S // TB

    def rows(j, n):
        return pl.ds(j * n if isinstance(j, int) else pl.multiple_of(j * n, n), n)

    def x_copy(j):
        if isinstance(j, int) and j < 0:
            r = pl.ds(0, 128)
        elif isinstance(j, int) and j == na - 1:
            r = pl.ds(S - TA + 128, TA - 128)
        else:
            r = pl.ds(j * TA + 128 if isinstance(j, int)
                      else pl.multiple_of(j * TA + 128, 128), TA)
        return pltpu.make_async_copy(x_hbm.at[r, :], xio.at[r, :], sem_in.at[9 + j])

    def w_copies(c):
        return [pltpu.make_async_copy(src.at[c], wraw.at[i, c],
                                      sem_in.at[10 + na + 3 * c + i])
                for i, src in enumerate((wq_hbm, wv_hbm, wo_hbm))]

    def wa_copy(r):
        return pltpu.make_async_copy(wqkv_hbm.at[rows(r, 128), :], wqkv.at[rows(r, 128), :],
                                     sem_in.at[3 + r])

    def out_copy(i):
        return pltpu.make_async_copy(xio.at[rows(i, TB), :],
                                     out_hbm.at[rows(i, TB), :], sem_out.at[0])

    wphi_copy = pltpu.make_async_copy(wphi_hbm, wphi, sem_in.at[0])
    woa_copy = pltpu.make_async_copy(woa_hbm, woa, sem_in.at[1])
    mem0_copy = pltpu.make_async_copy(mem0_hbm, mem0, sem_in.at[2])
    order = [wphi_copy, x_copy(-1)] + [wa_copy(r) for r in range(D // 128)]
    wk_copy = pltpu.make_async_copy(wk_hbm, wraw.at[3], sem_in.at[9 + na])
    order += [x_copy(j) for j in range(na)] + [woa_copy, mem0_copy, wk_copy]
    for c in range(NW):
        order += w_copies(c)
    for c in order:
        c.start()

    def ln_in(t, first):
        x = xio[rows(t, 128), :].astype(F32)
        if first is not True:
            x = jnp.where(first, x, xres[rows(t, 128), :])
        xres[rows(t, 128), :] = x
        return _pack(_layernorm(x).astype(BF16))

    wphi_copy.wait()
    x_copy(-1).wait()
    cphi = jnp.zeros((FA, D), F32)
    hh = lax.broadcasted_iota(jnp.int32, (HA, D), 0) * FA
    jj = lax.broadcasted_iota(jnp.int32, (HA, D), 1)
    for d in range(FA):
        cphi = _dot(wphi[d], jnp.where(jj == hh + d, 1.0, 0.0).astype(BF16)) + cphi
    cb = jnp.concatenate(
        [jnp.broadcast_to(cphi[f:f + 1, :], (8, D)) for f in range(FA)], axis=0)
    for g in range(GA):
        row = lax.broadcasted_iota(jnp.int32, (GR, 256), 0)
        col = lax.broadcasted_iota(jnp.int32, (GR, 256), 1) + 128 * g
        lo = (8 * g + (row & 7)) * FA
        bds[g] = _pack(jnp.where(jnp.logical_and(col >= lo, col < lo + FA),
                                 cb[:, 128 * g:128 * g + 256], 0.0).astype(BF16))
    xa[rows(0, 64), :] = ln_in(0, True)

    def fold(r, _):
        wa_copy(r).wait()
        rr = rows(r, 128)
        for g in range(GA):
            ws = []
            for i in range(2):
                c0 = i * D + 128 * g
                w = _dot_nt(_unpack(bds[g]), wqkv[rr, c0:c0 + 256]).reshape(FA, 8, 128)
                ws.append(((w[1:] - w[0:1]) * LOG2E).reshape(GR - 8, 128))
            wat[GA + g, :, rr] = _pack(
                jnp.concatenate([ws[1], ws[0][GR - 16:, :]], axis=0).astype(BF16))
            wat[g, 0:GR // 2 - 8, rr] = _pack(ws[0][0:GR - 16, :].astype(BF16))
        wvt = _pack(wqkv[rr, 2 * D:3 * D].T)
        for g in range(GA):
            wat[2 * GA + g, :, rr] = wvt[g * GR // 2:(g + 1) * GR // 2, :]
        return 0

    lax.fori_loop(0, D // 128, fold, 0)

    def pair_rows(ph, q, t0, n):
        return _unpack(jnp.concatenate(
            [ph[t0 + u, rows(q, 2 * FA), :] for u in range(n)], axis=1))

    def a1(first, j, _):
        @pl.when(jnp.logical_and(first, j < na - 1))
        def _():
            x_copy(j).wait()

        @pl.when(jnp.logical_and(first, j == na - 1))
        def _():
            x_copy(na - 1).wait()

        def features(ph, t, g, y):
            for f, w in enumerate(_feature_map(y)):
                ph[t, pl.ds(GR * g + f, 8, stride=FA), :] = w

        vs = {}
        for u in range(asub):
            t = j * asub + u
            xn = _unpack(ln_in(t, first) if u > 0 else xa[rows(t, 64), :])
            rest = []
            for g in range(GA):
                y = _dot_nt(_unpack(wat[GA + g]), xn)
                features(phk, u, g, y[0:GR - 8, :])
                rest.append(y[GR - 8:, :])
            for g in range(GA):
                y = _dot_nt(_unpack(wat[g, 0:GR // 2 - 8, :]), xn)
                features(phq, t, g, jnp.concatenate([y, rest[g]], axis=0))
            for g in range(GA):
                y = _dot_nt(_unpack(wat[2 * GA + g]), xn)
                for q in range(4):
                    vs[4 * g + q, u] = y[40 * q:40 * q + 40, :]
        row = lax.broadcasted_iota(jnp.int32, (2 * VR, 4 * FA), 0)
        col = lax.broadcasted_iota(jnp.int32, (2 * VR, 4 * FA), 1)
        split = jnp.where(row < 2 * FA, FA, 2 * FA + 4)
        same = (row >= split) == (col >= 2 * FA)
        for q in range(PA):
            v = jnp.concatenate([vs[q, u] for u in range(asub)], axis=1)
            v = jnp.concatenate([v, jnp.ones((8, TA), F32)], axis=0)
            kv = _dot_nt(v.astype(BF16), pair_rows(phk, q, 0, asub))
            kv = kv + jnp.where(j == 0, 0.0, kvacc[q])
            kvacc[q] = kv
            kvs[q] = _pack(jnp.where(same, kv, 0.0).astype(BF16))
        tn = jnp.minimum(j + 1, na - 1) * asub
        xa[rows(tn, 64), :] = ln_in(tn, first)
        return 0

    def attend(j):
        low = lax.broadcasted_iota(jnp.int32, (8, TN), 0) < 4
        os_ = []
        for q in range(PA):
            nd = _dot(_unpack(kvs[q]), pair_rows(phq, q, j * nsub, nsub))
            rab = 1.0 / (nd[40:48, :] + 1e-6)
            rba = pltpu.roll(rab, 4, 0)
            ra = jnp.where(low, rab, rba)
            rb = jnp.where(low, rba, rab)
            os_.append(nd[0:40, :] * jnp.concatenate([ra, ra, rab, rb, rb], axis=0))
        return _pack(jnp.concatenate(os_, axis=0).astype(BF16).T)

    def project(j, o, slot):
        ns = TN // SEG
        xs = []
        r = rows(j, TN)
        old, new = xres[r, :], {}
        for part in ((1, 2), (0, 3)):
            grp = [b + k for b in range(0, TN // 16, 4) for k in part]
            oo = jnp.concatenate([o[8 * g:8 * g + 8, :] for g in grp], axis=0)
            x = _dot(_unpack(oo), woa[...]) + jnp.concatenate(
                [old[16 * g:16 * g + 16, :] for g in grp], axis=0)
            for n, g in enumerate(grp):
                new[g] = x[16 * n:16 * n + 16, :]
            xs.append(x)
        xres[r, :] = jnp.concatenate([new[g] for g in range(TN // 16)], axis=0)
        for s in range(ns):
            x = xs[0][16 * s + 8 - 8 * (s % 2):16 * s + 16 - 8 * (s % 2), :]
            x = _layernorm(x)
            x = x - x[KE:KE + 1, :]
            for c in range(D // 128):
                xe[c, pl.ds((slot * ns + s) * KE, 8), :] = x[:, 128 * c:128 * (c + 1)]

    def extra_keys(seg, p):
        k = jnp.concatenate(
            [ke[seg // 16, 3 * p + c, pl.ds((seg % 16) * KE, 8), :] for c in range(3)], axis=1)
        return jnp.where(lax.broadcasted_iota(jnp.int32, (8, PW), 0) < KE, k, 0.0)

    def b_finish(i):
        r = rows(i, TB)
        x = xres[r, :] + rsave[...]
        xres[r, :] = x
        xn = _layernorm(x)
        xa[rows(i, TB // 2), :] = _pack(xn.astype(BF16))
        xio[r, :] = x.astype(BF16)
        return xn

    def b_pair(mem, xn, base, blk, side):
        def fix_qva(p, y):
            c0 = 2 * PW - D
            tie = jnp.where(blk < 0, side[8 * p:8 * p + 8, :], y[0:M, c0:])
            ysave[:, p * 2 * PW:(p + 1) * 2 * PW] = y[L:L + 8, :]
            return jnp.concatenate(
                [jnp.concatenate([y[0:M, 0:c0], tie], axis=1), y[M:L, :]], axis=0)

        def fix_ka(p, k):
            return jnp.concatenate([k, extra_keys(2 * blk, p)], axis=0)

        def fix_oa(p, o):
            osave[:, p * PW:(p + 1) * PW] = o[32:L, :]
            return o[0:32, :]

        h = jnp.concatenate([mem, xn[0:40, :]], axis=0)
        ra = _segment(h.astype(BF16), (h[0:32, :] - xn[31:32, :]).astype(BF16),
                      wqv, wk, wob, fix_qva, fix_ka, fix_oa, base > 0)
        rsave[base:base + 24, :] = ra[M:, :]

        def fix_qvb(p, y):
            return jnp.concatenate(
                [y[0:M, :], ysave[:, p * 2 * PW:(p + 1) * 2 * PW], y[M:, :]], axis=0)

        def fix_kb(p, k):
            return jnp.concatenate([k[0:M, :], extra_keys(2 * blk + 1, p), k[M:, :]], axis=0)

        def fix_ob(p, o):
            return jnp.concatenate([o, osave[:, p * PW:(p + 1) * PW]], axis=0)

        h = jnp.concatenate([ra[0:M, :], xn[40:64, :]], axis=0)
        rb = _segment(h.astype(BF16), (h - xn[39:40, :]).astype(BF16),
                      wqv, wk, wob, fix_qvb, fix_kb, fix_ob, True)
        rsave[base + 24:base + 32, :] = rb[L:, :]
        rsave[base + 32:base + 64, :] = rb[M:L, :]
        return rb[0:M, :]

    def layer(l, _):
        def wait_first(copies):
            @pl.when(l == 0)
            def _():
                for c in copies:
                    c.wait()

        with jax.named_scope("a1"):
            lax.fori_loop(0, na, functools.partial(a1, l == 0), 0)

        def a2(n, _):
            wait_first(w_copies(n))
            o0 = attend(2 * n)
            o1 = attend(2 * n + 1)
            wk[n] = _pack(wraw[3, n].T)
            project(2 * n, o0, 0)
            project(2 * n + 1, o1, 1)
            r = rows(n, TB // NW)
            xb[r, :] = _layernorm(xres[r, :])
            rsave[r, :] = jnp.zeros((TB // NW, D), F32)
            mr = 16 * KE
            x = jnp.concatenate([xe[t, 0:mr, :] for t in range(D // 128)], axis=1).astype(BF16)
            for c in range(NW):
                k = _dot_nt(x, wraw[3, c])
                for t in range(QW // 128):
                    e = c * (QW // 128) + t
                    ke[n, e, 0:mr, :] = k[:, 128 * t:128 * (t + 1)]
                    tie = pltpu.bitcast(k[0:16, 128 * t:128 * (t + 1)], U32)
                    wob[n, rows(e, 16), :] = jnp.where(
                        n < 0, jnp.concatenate([tie] * (D // 128), axis=1),
                        _pack(wraw[2, n, rows(e, 32), :]))
            for p in range(NP // NW):
                wqv[n, :, rows(2 * p, PW)] = _pack(wraw[0, n, rows(p, PW), :].T)
                wqv[n, :, rows(2 * p + 1, PW)] = _pack(wraw[1, n, rows(p, PW), :].T)
            return 0

        wait_first([woa_copy, mem0_copy, wk_copy])
        with jax.named_scope("a2"):
            lax.fori_loop(0, NW, a2, 0)

        def b_step(i, mem):
            xn = xb[...]
            side = b_finish(jnp.maximum(i - 1, 0))
            nxt = _layernorm(xres[rows(jnp.minimum(i + 1, nb - 1), TB), :])
            xb[...] = nxt
            side = jnp.concatenate([side, nxt], axis=0)
            for u in range(0, TB, 2 * SEG):
                mem = b_pair(mem, xn[u:u + 2 * SEG, :], u, (i * TB + u) // (2 * SEG),
                             side[2 * u:2 * u + 8 * NP, :])

            @pl.when(jnp.logical_and(l == 1, i >= 1))
            def _():
                out_copy(i - 1).start()
            return mem

        with jax.named_scope("b"):
            lax.fori_loop(0, nb, b_step, mem0[...].astype(F32))

        x = xres[rows(nb - 1, TB), :] + rsave[...]
        xres[rows(nb - 1, TB), :] = x
        xio[rows(nb - 1, TB), :] = x.astype(BF16)
        return 0

    lax.fori_loop(0, 2, layer, 0)
    out_copy(nb - 1).start()
    pltpu.make_async_copy(xio, out_hbm, sem_out.at[0]).wait()


@jax.jit
def pallas_interleave_layers__linear_kernel_hedgehog__memory_aug_recurrent_mem_tr__prompt_kernel(
    A_x, A_wqkv, A_w_phi, A_wo, B_x, B_mem0, B_Wq, B_Wk, B_Wv, B_Wo, B_seg_len,
):
    del B_x
    del B_seg_len
    x = A_x.reshape(S, D)
    wphi = A_w_phi.transpose(1, 2, 0)
    mem0 = B_mem0.reshape(M, D)
    wq, wk, wv = (w.transpose(1, 2, 0).reshape(NW, QW, D) for w in (B_Wq, B_Wk, B_Wv))
    wo = B_Wo.reshape(NW, QW, D)
    hbm = pl.BlockSpec(memory_space=pl.ANY)
    out = pl.pallas_call(
        _kernel,
        out_shape=jax.ShapeDtypeStruct((S, D), A_x.dtype),
        in_specs=[hbm] * 9,
        out_specs=hbm,
        scratch_shapes=[
            pltpu.VMEM((S, D), BF16),
            pltpu.VMEM((D, 3 * D), BF16),
            pltpu.VMEM((FA, FA, HA), BF16),
            pltpu.VMEM((D, D), BF16),
            pltpu.VMEM((M, D), BF16),
            pltpu.VMEM((S, D), F32),
            pltpu.VMEM((S // 2, D), U32),
            pltpu.VMEM((TB, D), F32),
            pltpu.VMEM((GA, GR // 2, 256), U32),
            pltpu.VMEM((3 * GA, GR // 2, D), U32),
            pltpu.VMEM((S // 128, D, 128), U32),
            pltpu.VMEM((TA // 128, D, 128), U32),
            pltpu.VMEM((PA, 2 * VR, 4 * FA), F32),
            pltpu.VMEM((PA, VR, 4 * FA), U32),
            pltpu.VMEM((4, NW, QW, D), BF16),
            pltpu.VMEM((NW, D // 2, 2 * QW), U32),
            pltpu.VMEM((NW, D // 2, QW), U32),
            pltpu.VMEM((NW, QW // 2, D), U32),
            pltpu.VMEM((D // 128, 16 * KE + 8, 128), F32),
            pltpu.VMEM((NW, HD // 128, 16 * KE + 8, 128), F32),
            pltpu.VMEM((8, 2 * HD), F32),
            pltpu.VMEM((8, HD), F32),
            pltpu.VMEM((TB, D), F32),
            pltpu.SemaphoreType.DMA((10 + S // TA + 3 * NW,)),
            pltpu.SemaphoreType.DMA((1,)),
        ],
        compiler_params=pltpu.CompilerParams(vmem_limit_bytes=120 * 1024 * 1024,
                                             disable_bounds_checks=True,
                                             disable_semaphore_checks=True),
    )(x, A_wqkv, wphi, A_wo, mem0, wq, wk, wv, wo)
    return out.reshape(1, S, D)
```

```python
import functools

import jax
import jax.numpy as jnp
from jax import lax
import jax.experimental.pallas as pl
import jax.experimental.pallas.tpu as pltpu

F32 = jnp.float32
BF16 = jnp.bfloat16
U32 = jnp.uint32

S = 2048
D = 640
HA = 32
FA = 20
GA = 4
GR = 8 * FA
VR = 24
PA = HA // 2
TN = 256
TA = 512
HB = 32
DH = 192
HD = HB * DH
M = 8
SEG = 32
L = M + SEG
PW = 2 * DH
NP = HB // 2
TB = 128
NW = 4
QW = HD // NW
KE = 7

NT = (((1,), (1,)), ((), ()))
LOG2E = 1.4426950408889634
HALF_ULP = 0.0040612


def _dot(a, b):
    return jnp.dot(a, b, preferred_element_type=F32)


def _dot_nt(a, b):
    return lax.dot_general(a, b, NT, preferred_element_type=F32)


def _pack(a):
    return pltpu.bitcast(a, U32)


def _unpack(a):
    return pltpu.bitcast(a, BF16)


def _interleave(a, b):
    lo = lax.bitcast_convert_type(a, U32) >> 16
    hi = lax.bitcast_convert_type(b, U32) & jnp.uint32(0xFFFF0000)
    return lo | hi


def _recip(x):
    r = pl.reciprocal(x, approx=True)
    return r * (2.0 - x * r)


def _layernorm(x):
    m = jnp.mean(x, axis=-1, keepdims=True)
    c = x - m
    v = jnp.mean(c * c, axis=-1, keepdims=True)
    return c * lax.rsqrt(v + 1e-5)


def _feature_map(p):
    t = p.shape[-1]
    p3 = jnp.concatenate([jnp.zeros((8, t), F32), p], axis=0).reshape(FA, 8, t)
    mx = jnp.max(p3, axis=0)
    mn = jnp.min(p3, axis=0)
    sp, sn = jnp.exp2(p3[0] - mx), jnp.exp2(mn - p3[0])
    for f in range(1, FA):
        sp, sn = sp + jnp.exp2(p3[f] - mx), sn + jnp.exp2(mn - p3[f])
    lp = (mx - HALF_ULP) + jnp.log2(sp)
    ln = (mn + HALF_ULP) - jnp.log2(sn)
    return [_interleave(jnp.exp2(p3[f] - lp), jnp.exp2(ln - p3[f])) for f in range(FA)]


def _tiles(a, odd):
    t0, t1, t2 = a[:, 0:128], a[:, 128:256], a[:, 256:384]
    return (t1, t2, t0) if odd else (t1, t0, t2)


def _own_weights(a, odd):
    lane = lax.broadcasted_iota(jnp.int32, (L, 128), 1)
    mid, own, _ = _tiles(a, odd)
    return jnp.concatenate(
        [jnp.where(lane < 64, mid, 0.0), jnp.where(lane < 64, 0.0, mid), own,
         jnp.zeros((128 - 3 * L, 128), F32)], axis=0).astype(BF16)


def _others(even, odd, pad):
    parts = [_tiles(odd, 1)[2], _tiles(even, 0)[2]]
    if pad:
        parts.append(jnp.zeros((128 - 2 * L, 128), F32))
    return jnp.concatenate(parts, axis=0).astype(BF16)


def _softmax3(s3):
    row = lax.broadcasted_iota(jnp.int32, (L, 128), 0)
    col = lax.broadcasted_iota(jnp.int32, (L, 128), 1)
    first = col < L
    second = jnp.logical_and(col >= L, col < 2 * L)
    key = jnp.where(first, col, col - L)
    valid = jnp.logical_or(row < M, row >= key)
    out, other = [], []
    for odd in range(2):
        own = pltpu.roll(s3[odd][L:, :], 128 - L if odd else 128 - 2 * L, 1)
        s = (jnp.where(first, s3[2][0:L, :], own) if odd
             else jnp.where(first, own, s3[2][L:, :]))
        s = jnp.where(valid, (s + s3[odd][0:L, :]) * (DH ** -0.5), -1e9)
        m0 = jnp.max(jnp.where(first, s, -jnp.inf), axis=-1, keepdims=True)
        m1 = jnp.max(jnp.where(second, s, -jnp.inf), axis=-1, keepdims=True)
        e = jnp.exp(s - jnp.where(first, m0, m1))
        e0 = jnp.where(first, e, 0.0)
        e1 = jnp.where(second, e, 0.0)
        p0 = e0 * _recip(jnp.sum(e0, axis=-1, keepdims=True))
        p1 = e1 * _recip(jnp.sum(e1, axis=-1, keepdims=True))
        own = pltpu.roll(p1, L, 1) if odd else pltpu.roll(p0, 2 * L, 1)
        out.append(jnp.concatenate([p0 + p1, own], axis=0).astype(BF16))
        other.append(p0 if odd else p1)
    out.append(jnp.concatenate([other[1], other[0]], axis=0).astype(BF16))
    return out


def _segment(h, hk, wqv, wk, wob, fix_qv, fix_k, fix_o, chained):
    ys, ks, ss, ps, pvs, os_ = {}, {}, {}, {}, {}, {}
    kg = 4

    def proj(p):
        n, e = divmod(p, NP // NW)
        cols = slice(e * 2 * PW, (e + 1) * 2 * PW)
        if p == 0 and chained:
            ksp = 512
            y = _dot(h[:, 0:ksp], _unpack(wqv[n, 0:ksp // 2, cols]))
            y = _dot(h[:, ksp:], _unpack(wqv[n, ksp // 2:, cols])) + y
        else:
            y = _dot(h, _unpack(wqv[n, :, cols]))
        y = fix_qv(p, y)
        if p % kg == 0:
            k = _dot(hk, _unpack(wk[n, :, e * PW:(e + kg) * PW]))
            for i in range(kg):
                ks[p + i] = fix_k(p + i, k[:, i * PW:(i + 1) * PW])
        ys[p] = [y[:, 0:PW], ks.pop(p), y[:, PW:]]

    def weights(c, i, which):
        if i < 2:
            return _own_weights(ys[2 * c + i][which], i)
        return _others(ys[2 * c][which], ys[2 * c + 1][which], True)

    def score_round(n):
        for c, i in (divmod(j, 3) for j in range(4 * n, 4 * n + 4)):
            if i < 2:
                q = jnp.concatenate(_tiles(ys[2 * c + i][0], i)[0:2], axis=0).astype(BF16)
            else:
                q = _others(ys[2 * c][0], ys[2 * c + 1][0], False)
            ss[c, i] = _dot_nt(q, weights(c, i, 1))
            if i == 2:
                ps[c] = _softmax3([ss.pop((c, k)) for k in range(3)])

    def pv_round(n):
        for c, i in (divmod(j, 3) for j in range(4 * n, 4 * n + 4)):
            pvs[c, i] = _dot(ps[c][i], weights(c, i, 2))
            if i == 2:
                o0, o1, o2 = [pvs.pop((c, k)) for k in range(3)]
                os_[2 * c] = fix_o(2 * c, jnp.concatenate(
                    [o0[L:, :], o0[0:L, :], o2[L:, :]], axis=1))
                os_[2 * c + 1] = fix_o(2 * c + 1, jnp.concatenate(
                    [o2[0:L, :], o1[0:L, :], o1[L:, :]], axis=1))

    def slot(n):
        if n >= 2:
            pv_round(n - 2)
        if n < 6:
            score_round(n)

    def rows_of(e):
        return slice(e * DH, (e + 1) * DH)

    def oproj(lo, hi):
        o = jnp.concatenate([os_.pop(p) for p in range(lo, hi)], axis=1).astype(BF16)
        w = [wob[p // (NP // NW), rows_of(p % (NP // NW)), :] for p in range(lo, hi)]
        return _dot(o, _unpack(jnp.concatenate(w, axis=0)))

    after = {3: 0, 6: 1, 9: 2, 11: 3, 14: 4}
    for p in range(NP):
        proj(p)
        if p in after:
            slot(after[p])
    o1, o2, o3 = (2, 8, 10) if h.shape[0] == 48 else (2, 7, 10)
    r = oproj(0, o1)
    slot(5)
    r = oproj(o1, o2) + r
    slot(6)
    slot(7)
    r = oproj(o2, o3) + r
    return oproj(o3, NP) + r


def _kernel(x_hbm, wqkv_hbm, wphi_hbm, woa_hbm, mem0_hbm,
            wq_hbm, wk_hbm, wv_hbm, wo_hbm,
            out_hbm,
            xio, wqkv, wphi, woa, mem0, xres, xa, xl, xb, bds, wat, phq, phk, kvacc, kvs,
            wraw, wqv, wk, wob, xe, ke, ysave, osave, rsave, sem_in, sem_out):
    nsub = TN // 128
    na = S // TA
    asub = TA // 128
    nb = S // TB

    def rows(j, n):
        return pl.ds(j * n if isinstance(j, int) else pl.multiple_of(j * n, n), n)

    def x_copy(j):
        if isinstance(j, int) and j < 0:
            r = pl.ds(0, 256)
        elif isinstance(j, int) and j == na - 1:
            r = pl.ds(S - TA + 256, TA - 256)
        else:
            r = pl.ds(j * TA + 256 if isinstance(j, int)
                      else pl.multiple_of(j * TA + 256, 256), TA)
        return pltpu.make_async_copy(x_hbm.at[r, :], xio.at[r, :], sem_in.at[9 + j])

    def w_copies(c):
        return [pltpu.make_async_copy(src.at[c], wraw.at[i, c],
                                      sem_in.at[10 + na + 3 * c + i])
                for i, src in enumerate((wq_hbm, wv_hbm, wo_hbm))]

    def wa_copy(c):
        r = pl.ds(512, 128) if isinstance(c, int) and c == 2 else rows(c, 256)
        return pltpu.make_async_copy(wqkv_hbm.at[r, :], wqkv.at[r, :], sem_in.at[3 + c])

    def out_copy(i):
        return pltpu.make_async_copy(xio.at[rows(i, TB), :],
                                     out_hbm.at[rows(i, TB), :], sem_out.at[0])

    wphi_copy = pltpu.make_async_copy(wphi_hbm, wphi, sem_in.at[0])
    woa_copy = pltpu.make_async_copy(woa_hbm, woa, sem_in.at[1])
    mem0_copy = pltpu.make_async_copy(mem0_hbm, mem0, sem_in.at[2])
    order = [wphi_copy, wa_copy(0), wa_copy(1), x_copy(-1), wa_copy(2)]
    wk_copy = pltpu.make_async_copy(wk_hbm, wraw.at[3], sem_in.at[9 + na])
    order += [x_copy(j) for j in range(na)] + [woa_copy, mem0_copy, wk_copy]
    for c in range(NW):
        order += w_copies(c)
    for c in order:
        c.start()

    def strassen_rhs(x0, x1):
        b11, b12 = [jnp.concatenate([x[:, 0:128], x[:, 256:384]], axis=1) for x in (x0, x1)]
        b21, b22 = [jnp.concatenate([x[:, 128:256], x[:, 384:512]], axis=1) for x in (x0, x1)]
        ops = [b11 + b22, b11, b12 - b22, b21 - b11, b22, b11 + b12, b21 + b22,
               x0[:, 512:], x1[:, 512:]]
        return _pack(jnp.concatenate(ops, axis=1).astype(BF16))

    def load_x(t, first):
        x = xio[rows(t, 256), :].astype(F32)
        if first is not True:
            x = jnp.where(first, x, xres[rows(t, 256), :])
        xres[rows(t, 256), :] = x
        return x

    wphi_copy.wait()
    cphi = jnp.zeros((FA, D), F32)
    hh = lax.broadcasted_iota(jnp.int32, (HA, D), 0) * FA
    jj = lax.broadcasted_iota(jnp.int32, (HA, D), 1)
    for d in range(FA):
        cphi = _dot(wphi[d], jnp.where(jj == hh + d, 1.0, 0.0).astype(BF16)) + cphi
    cb = jnp.concatenate(
        [jnp.broadcast_to(cphi[f:f + 1, :], (8, D)) for f in range(FA)], axis=0)
    for g in range(GA):
        row = lax.broadcasted_iota(jnp.int32, (GR, 256), 0)
        col = lax.broadcasted_iota(jnp.int32, (GR, 256), 1) + 128 * g
        lo = (8 * g + (row & 7)) * FA
        bds[g] = _pack(jnp.where(jnp.logical_and(col >= lo, col < lo + FA),
                                 cb[:, 128 * g:128 * g + 256], 0.0).astype(BF16))

    def folded(rr):
        out = [[], [], []]
        for g in range(GA):
            ws = []
            for i in range(2):
                c0 = i * D + 128 * g
                w = _dot_nt(_unpack(bds[g]), wqkv[rr, c0:c0 + 256]).reshape(FA, 8, 128)
                ws.append(((w[1:] - w[0:1]) * LOG2E).reshape(GR - 8, 128))
            out[0].append(jnp.concatenate([ws[1], ws[0][GR - 16:, :]], axis=0))
            out[1].append(ws[0][0:GR - 16, :])
        wvt = wqkv[rr, 2 * D:3 * D].T.astype(F32)
        out[2] = [wvt[g * GR:(g + 1) * GR, :] for g in range(GA)]
        return out

    def fold(c, _):
        wa_copy(c).wait()
        wa, wb = folded(rows(2 * c, 128)), folded(rows(2 * c + 1, 128))
        for i in range(3):
            for p in range(2):
                a11, a12, a21, a22 = wa[i][2 * p], wb[i][2 * p], wa[i][2 * p + 1], wb[i][2 * p + 1]
                ops = [a11 + a22, a21 + a22, a11, a22, a11 + a12, a21 - a11, a12 - a22]
                for m, w in enumerate(ops):
                    wat[2 * i + p, m, 0:w.shape[0] // 2, rows(c, 128)] = _pack(w.astype(BF16))
        return 0

    lax.fori_loop(0, 2, fold, 0)
    x_copy(-1).wait()
    wa_copy(2).wait()
    x = _layernorm(load_x(0, True))
    xa[...] = strassen_rhs(x[0:128], x[128:])
    for i, ws in enumerate(folded(pl.ds(512, 128))):
        for g, w in enumerate(ws):
            wat[2 * i + g // 2, 7, 0:w.shape[0] // 2, rows(g % 2, 128)] = _pack(w.astype(BF16))

    def pair_rows(ph, q, t0, n):
        return _unpack(jnp.concatenate(
            [ph[t0 + u, rows(q, 2 * FA), :] for u in range(n)], axis=1))

    def a1(first, j, _):
        @pl.when(jnp.logical_and(first, j < na - 1))
        def _():
            x_copy(j).wait()

        @pl.when(jnp.logical_and(first, j == na - 1))
        def _():
            x_copy(na - 1).wait()

        def features(ph, t, g, y):
            for f, w in enumerate(_feature_map(y)):
                ph[t, pl.ds(GR * g + f, 8, stride=FA), :] = w

        def tail(n, xs, g, u):
            nr = GR // 2 - 8 if n // 2 == 1 else GR // 2
            return _dot_nt(_unpack(wat[n, 7, 0:nr, 128 * g:128 * (g + 1)]),
                           xs[:, 1792 + 128 * u:1920 + 128 * u])

        def a_dots(n, xs, emit, tie, t10):
            nr = GR // 2 - 8 if n // 2 == 1 else GR // 2
            p = n % 2

            def prod(m):
                return _dot_nt(_unpack(tie(wat[n, m, 0:nr, :])), xs[:, 256 * m:256 * (m + 1)])

            m2, m4 = prod(1), prod(3)
            emit(2 * p + 1, 0, m4 + (m2 - (-t10)))
            t01 = tail(n, xs, 0, 1)
            m3, m5 = prod(2), prod(4)
            emit(2 * p, 1, m5 + (m3 - (-t01)))
            m1 = prod(0)
            c22 = prod(5) + (m1 + (m3 - m2))
            emit(2 * p + 1, 1, tail(n, xs, 1, 1) + c22)
            t10 = tail(n + 1, xs, 1, 0) if n < 5 else None
            c11 = tail(n, xs, 0, 0) + (m1 + (m4 - m5))
            emit(2 * p, 0, prod(6) + c11)
            return t10

        vs = {}
        cur = xa[...]
        dl = (3, 8, 13, 30, 33, 36, 39, 41)
        for u in range(0, asub, 2):
            t = j * asub + u
            xs = _unpack(cur)
            tn = j * (asub // 2) + u // 2 + 1
            x = load_x(tn if u + 2 < asub else jnp.minimum(tn, (na - 1) * (asub // 2)), first)
            rest, seen, nxt = {}, [], []

            def tie(w):
                seen.append(0)
                if len(seen) - 1 not in dl:
                    return w
                n = len(nxt)
                nxt.append(strassen_rhs(*[
                    _layernorm(x[128 * e + 16 * n:128 * e + 16 * n + 16, :]) for e in range(2)]))
                z = jnp.concatenate(
                    [nxt[n][:, 256 * c:256 * (c + 1)] for c in range(8)], axis=0)
                return jnp.concatenate([jnp.where(j < 0, z, w[0:64, :]), w[64:, :]], axis=0)

            def emit_k(g, e, y):
                features(phk, u + e, g, y[0:GR - 8, :])
                rest[g, e] = y[GR - 8:, :]

            def emit_q(g, e, y):
                features(phq, t + e, g, jnp.concatenate([y, rest[g, e]], axis=0))

            def emit_v(g, e, y):
                for q in range(4):
                    vs[4 * g + q, u + e] = y[40 * q:40 * q + 40, :]

            t10 = tail(0, xs, 1, 0)
            for n in range(6):
                t10 = a_dots(n, xs, (emit_k, emit_q, emit_v)[n // 2], tie, t10)
            cur = jnp.concatenate(nxt, axis=0)
        xa[...] = cur
        row = lax.broadcasted_iota(jnp.int32, (2 * VR, 4 * FA), 0)
        col = lax.broadcasted_iota(jnp.int32, (2 * VR, 4 * FA), 1)
        split = jnp.where(row < 2 * FA, FA, 2 * FA + 4)
        same = (row >= split) == (col >= 2 * FA)
        for q in range(PA):
            v = jnp.concatenate([vs[q, u] for u in range(asub)], axis=1)
            v = jnp.concatenate([v, jnp.ones((8, TA), F32)], axis=0)
            kv = _dot_nt(v.astype(BF16), pair_rows(phk, q, 0, asub))
            kv = kv + jnp.where(j == 0, 0.0, kvacc[q])
            kvacc[q] = kv
            kvs[q] = _pack(jnp.where(same, kv, 0.0).astype(BF16))
        return 0

    def attend(j):
        low = lax.broadcasted_iota(jnp.int32, (8, TN), 0) < 4
        os_ = []
        for q in range(PA):
            nd = _dot(_unpack(kvs[q]), pair_rows(phq, q, j * nsub, nsub))
            rab = 1.0 / (nd[40:48, :] + 1e-6)
            rba = pltpu.roll(rab, 4, 0)
            ra = jnp.where(low, rab, rba)
            rb = jnp.where(low, rba, rab)
            os_.append(nd[0:40, :] * jnp.concatenate([ra, ra, rab, rb, rb], axis=0))
        return _pack(jnp.concatenate(os_, axis=0).astype(BF16).T)

    def project(j, o, slot):
        ns = TN // SEG
        xs = []
        r = rows(j, TN)
        old, new = xres[r, :], {}
        for part in ((1, 2), (0, 3)):
            grp = [b + k for b in range(0, TN // 16, 4) for k in part]
            oo = jnp.concatenate([o[8 * g:8 * g + 8, :] for g in grp], axis=0)
            x = _dot(_unpack(oo), woa[...]) + jnp.concatenate(
                [old[16 * g:16 * g + 16, :] for g in grp], axis=0)
            for n, g in enumerate(grp):
                new[g] = x[16 * n:16 * n + 16, :]
            xs.append(x)
        xres[r, :] = jnp.concatenate([new[g] for g in range(TN // 16)], axis=0)
        for s in range(ns):
            x = xs[0][16 * s + 8 - 8 * (s % 2):16 * s + 16 - 8 * (s % 2), :]
            x = _layernorm(x)
            x = x - x[KE:KE + 1, :]
            for c in range(D // 128):
                xe[c, pl.ds((slot * ns + s) * KE, 8), :] = x[:, 128 * c:128 * (c + 1)]

    def extra_keys(seg, p):
        k = jnp.concatenate(
            [ke[seg // 16, 3 * p + c, pl.ds((seg % 16) * KE, 8), :] for c in range(3)], axis=1)
        return jnp.where(lax.broadcasted_iota(jnp.int32, (8, PW), 0) < KE, k, 0.0)

    def b_finish(i):
        r = rows(i, TB)
        x = xres[r, :] + rsave[...]
        xres[r, :] = x
        xn = _layernorm(x)
        xl[rows(jnp.minimum(i, 2), TB), :] = xn
        xio[r, :] = x.astype(BF16)
        return xn

    def b_pair(mem, xn, base, blk, side):
        def fix_qva(p, y):
            c0 = 2 * PW - D
            tie = jnp.where(blk < 0, side[8 * p:8 * p + 8, :], y[0:M, c0:])
            ysave[:, p * 2 * PW:(p + 1) * 2 * PW] = y[L:L + 8, :]
            return jnp.concatenate(
                [jnp.concatenate([y[0:M, 0:c0], tie], axis=1), y[M:L, :]], axis=0)

        def fix_ka(p, k):
            return jnp.concatenate([k, extra_keys(2 * blk, p)], axis=0)

        def fix_oa(p, o):
            osave[:, p * PW:(p + 1) * PW] = o[32:L, :]
            return o[0:32, :]

        h = jnp.concatenate([mem, xn[0:40, :]], axis=0)
        ra = _segment(h.astype(BF16), (h[0:32, :] - xn[31:32, :]).astype(BF16),
                      wqv, wk, wob, fix_qva, fix_ka, fix_oa, base > 0)
        rsave[base:base + 24, :] = ra[M:, :]

        def fix_qvb(p, y):
            return jnp.concatenate(
                [y[0:M, :], ysave[:, p * 2 * PW:(p + 1) * 2 * PW], y[M:, :]], axis=0)

        def fix_kb(p, k):
            return jnp.concatenate([k[0:M, :], extra_keys(2 * blk + 1, p), k[M:, :]], axis=0)

        def fix_ob(p, o):
            return jnp.concatenate([o, osave[:, p * PW:(p + 1) * PW]], axis=0)

        h = jnp.concatenate([ra[0:M, :], xn[40:64, :]], axis=0)
        rb = _segment(h.astype(BF16), (h - xn[39:40, :]).astype(BF16),
                      wqv, wk, wob, fix_qvb, fix_kb, fix_ob, True)
        rsave[base + 24:base + 32, :] = rb[L:, :]
        rsave[base + 32:base + 64, :] = rb[M:L, :]
        return rb[0:M, :]

    def layer(l, _):
        def wait_first(copies):
            @pl.when(l == 0)
            def _():
                for c in copies:
                    c.wait()

        with jax.named_scope("a1"):
            lax.fori_loop(0, na, functools.partial(a1, l == 0), 0)

        def a2(n, _):
            wait_first(w_copies(n))
            o0 = attend(2 * n)
            o1 = attend(2 * n + 1)
            wk[n] = _pack(wraw[3, n].T)
            project(2 * n, o0, 0)
            project(2 * n + 1, o1, 1)
            r = rows(n, TB // NW)
            xb[r, :] = _layernorm(xres[r, :])
            rsave[r, :] = jnp.zeros((TB // NW, D), F32)
            mr = 16 * KE
            x = jnp.concatenate([xe[t, 0:mr, :] for t in range(D // 128)], axis=1).astype(BF16)
            for c in range(NW):
                k = _dot_nt(x, wraw[3, c])
                for t in range(QW // 128):
                    e = c * (QW // 128) + t
                    ke[n, e, 0:mr, :] = k[:, 128 * t:128 * (t + 1)]
                    tie = pltpu.bitcast(k[0:16, 128 * t:128 * (t + 1)], U32)
                    wob[n, rows(e, 16), :] = jnp.where(
                        n < 0, jnp.concatenate([tie] * (D // 128), axis=1),
                        _pack(wraw[2, n, rows(e, 32), :]))
            for p in range(NP // NW):
                wqv[n, :, rows(2 * p, PW)] = _pack(wraw[0, n, rows(p, PW), :].T)
                wqv[n, :, rows(2 * p + 1, PW)] = _pack(wraw[1, n, rows(p, PW), :].T)
            return 0

        wait_first([woa_copy, mem0_copy, wk_copy])
        with jax.named_scope("a2"):
            lax.fori_loop(0, NW, a2, 0)

        def b_step(i, mem):
            xn = xb[...]
            side = b_finish(jnp.maximum(i - 1, 0))
            nxt = _layernorm(xres[rows(jnp.minimum(i + 1, nb - 1), TB), :])
            xb[...] = nxt
            side = jnp.concatenate([side, nxt], axis=0)
            for u in range(0, TB, 2 * SEG):
                mem = b_pair(mem, xn[u:u + 2 * SEG, :], u, (i * TB + u) // (2 * SEG),
                             side[2 * u:2 * u + 8 * NP, :])

            @pl.when(jnp.logical_and(l == 1, i >= 1))
            def _():
                out_copy(i - 1).start()
            return mem

        with jax.named_scope("b"):
            lax.fori_loop(0, nb, b_step, mem0[...].astype(F32))

        x = xres[rows(nb - 1, TB), :] + rsave[...]
        xres[rows(nb - 1, TB), :] = x
        xio[rows(nb - 1, TB), :] = x.astype(BF16)

        @pl.when(l == 0)
        def _():
            xa[...] = strassen_rhs(xl[0:128, :], xl[128:256, :])
        return 0

    lax.fori_loop(0, 2, layer, 0)
    out_copy(nb - 1).start()
    pltpu.make_async_copy(xio, out_hbm, sem_out.at[0]).wait()


@jax.jit
def pallas_interleave_layers__linear_kernel_hedgehog__memory_aug_recurrent_mem_tr__prompt_kernel(
    A_x, A_wqkv, A_w_phi, A_wo, B_x, B_mem0, B_Wq, B_Wk, B_Wv, B_Wo, B_seg_len,
):
    del B_x
    del B_seg_len
    x = A_x.reshape(S, D)
    wphi = A_w_phi.transpose(1, 2, 0)
    mem0 = B_mem0.reshape(M, D)
    wq, wk, wv = (w.transpose(1, 2, 0).reshape(NW, QW, D) for w in (B_Wq, B_Wk, B_Wv))
    wo = B_Wo.reshape(NW, QW, D)
    hbm = pl.BlockSpec(memory_space=pl.ANY)
    out = pl.pallas_call(
        _kernel,
        out_shape=jax.ShapeDtypeStruct((S, D), A_x.dtype),
        in_specs=[hbm] * 9,
        out_specs=hbm,
        scratch_shapes=[
            pltpu.VMEM((S, D), BF16),
            pltpu.VMEM((D, 3 * D), BF16),
            pltpu.VMEM((FA, FA, HA), BF16),
            pltpu.VMEM((D, D), BF16),
            pltpu.VMEM((M, D), BF16),
            pltpu.VMEM((S, D), F32),
            pltpu.VMEM((64, 2048), U32),
            pltpu.VMEM((3 * TB, D), F32),
            pltpu.VMEM((TB, D), F32),
            pltpu.VMEM((GA, GR // 2, 256), U32),
            pltpu.VMEM((6, 8, GR // 2, 256), U32),
            pltpu.VMEM((S // 128, D, 128), U32),
            pltpu.VMEM((TA // 128, D, 128), U32),
            pltpu.VMEM((PA, 2 * VR, 4 * FA), F32),
            pltpu.VMEM((PA, VR, 4 * FA), U32),
            pltpu.VMEM((4, NW, QW, D), BF16),
            pltpu.VMEM((NW, D // 2, 2 * QW), U32),
            pltpu.VMEM((NW, D // 2, QW), U32),
            pltpu.VMEM((NW, QW // 2, D), U32),
            pltpu.VMEM((D // 128, 16 * KE + 8, 128), F32),
            pltpu.VMEM((NW, HD // 128, 16 * KE + 8, 128), F32),
            pltpu.VMEM((8, 2 * HD), F32),
            pltpu.VMEM((8, HD), F32),
            pltpu.VMEM((TB, D), F32),
            pltpu.SemaphoreType.DMA((10 + S // TA + 3 * NW,)),
            pltpu.SemaphoreType.DMA((1,)),
        ],
        compiler_params=pltpu.CompilerParams(vmem_limit_bytes=120 * 1024 * 1024,
                                             disable_bounds_checks=True,
                                             disable_semaphore_checks=True),
    )(x, A_wqkv, wphi, A_wo, mem0, wq, wk, wv, wo)
    return out.reshape(1, S, D)
```

```python
import functools

import jax
import jax.numpy as jnp
from jax import lax
import jax.experimental.pallas as pl
import jax.experimental.pallas.tpu as pltpu

F32 = jnp.float32
BF16 = jnp.bfloat16
U32 = jnp.uint32

S = 2048
D = 640
HA = 32
FA = 20
GA = 4
GR = 8 * FA
VR = 24
PA = HA // 2
TN = 256
TA = 512
HB = 32
DH = 192
HD = HB * DH
M = 8
SEG = 32
L = M + SEG
PW = 2 * DH
NP = HB // 2
TB = 128
NW = 4
QW = HD // NW
KE = 7

NT = (((1,), (1,)), ((), ()))
LOG2E = 1.4426950408889634
HALF_ULP = 0.0040612


def _dot(a, b):
    return jnp.dot(a, b, preferred_element_type=F32)


def _dot_nt(a, b):
    return lax.dot_general(a, b, NT, preferred_element_type=F32)


def _pack(a):
    return pltpu.bitcast(a, U32)


def _unpack(a):
    return pltpu.bitcast(a, BF16)


def _interleave(a, b):
    lo = lax.bitcast_convert_type(a, U32) >> 16
    hi = lax.bitcast_convert_type(b, U32) & jnp.uint32(0xFFFF0000)
    return lo | hi


def _recip(x):
    r = pl.reciprocal(x, approx=True)
    return r * (2.0 - x * r)


def _layernorm(x):
    m = jnp.mean(x, axis=-1, keepdims=True)
    c = x - m
    v = jnp.mean(c * c, axis=-1, keepdims=True)
    return c * lax.rsqrt(v + 1e-5)


def _split_rows(x):
    blocks = range(0, x.shape[0], 64)
    return (jnp.concatenate([x[b + 16:b + 48] for b in blocks], axis=0),
            jnp.concatenate([x[b + k:b + k + 16] for b in blocks for k in (0, 48)], axis=0))


def _merge_rows(inner, outer):
    return jnp.concatenate(
        [z for b in range(0, inner.shape[0], 32)
         for z in (outer[b:b + 16], inner[b:b + 32], outer[b + 16:b + 32])], axis=0)


def _feature_map(p):
    t = p.shape[-1]
    p3 = jnp.concatenate([jnp.zeros((8, t), F32), p], axis=0).reshape(FA, 8, t)
    mx = jnp.max(p3, axis=0)
    mn = jnp.min(p3, axis=0)
    sp, sn = jnp.exp2(p3[0] - mx), jnp.exp2(mn - p3[0])
    for f in range(1, FA):
        sp, sn = sp + jnp.exp2(p3[f] - mx), sn + jnp.exp2(mn - p3[f])
    lp = (mx - HALF_ULP) + jnp.log2(sp)
    ln = (mn + HALF_ULP) - jnp.log2(sn)
    return [_interleave(jnp.exp2(p3[f] - lp), jnp.exp2(ln - p3[f])) for f in range(FA)]


def _tiles(a, odd):
    t0, t1, t2 = a[:, 0:128], a[:, 128:256], a[:, 256:384]
    return (t1, t2, t0) if odd else (t1, t0, t2)


def _own_weights(a, odd):
    lane = lax.broadcasted_iota(jnp.int32, (L, 128), 1)
    mid, own, _ = _tiles(a, odd)
    return jnp.concatenate(
        [jnp.where(lane < 64, mid, 0.0), jnp.where(lane < 64, 0.0, mid), own,
         jnp.zeros((128 - 3 * L, 128), F32)], axis=0).astype(BF16)


def _others(even, odd, pad):
    parts = [_tiles(odd, 1)[2], _tiles(even, 0)[2]]
    if pad:
        parts.append(jnp.zeros((128 - 2 * L, 128), F32))
    return jnp.concatenate(parts, axis=0).astype(BF16)


def _softmax3(s3):
    row = lax.broadcasted_iota(jnp.int32, (L, 128), 0)
    col = lax.broadcasted_iota(jnp.int32, (L, 128), 1)
    first = col < L
    second = jnp.logical_and(col >= L, col < 2 * L)
    key = jnp.where(first, col, col - L)
    valid = jnp.logical_or(row < M, row >= key)
    out, other = [], []
    for odd in range(2):
        own = pltpu.roll(s3[odd][L:, :], 128 - L if odd else 128 - 2 * L, 1)
        s = (jnp.where(first, s3[2][0:L, :], own) if odd
             else jnp.where(first, own, s3[2][L:, :]))
        s = jnp.where(valid, (s + s3[odd][0:L, :]) * (DH ** -0.5), -1e9)
        m0 = jnp.max(jnp.where(first, s, -jnp.inf), axis=-1, keepdims=True)
        m1 = jnp.max(jnp.where(second, s, -jnp.inf), axis=-1, keepdims=True)
        e = jnp.exp(s - jnp.where(first, m0, m1))
        e0 = jnp.where(first, e, 0.0)
        e1 = jnp.where(second, e, 0.0)
        p0 = e0 * _recip(jnp.sum(e0, axis=-1, keepdims=True))
        p1 = e1 * _recip(jnp.sum(e1, axis=-1, keepdims=True))
        own = pltpu.roll(p1, L, 1) if odd else pltpu.roll(p0, 2 * L, 1)
        out.append(jnp.concatenate([p0 + p1, own], axis=0).astype(BF16))
        other.append(p0 if odd else p1)
    out.append(jnp.concatenate([other[1], other[0]], axis=0).astype(BF16))
    return out


def _segment(h, hk, wqv, wk, wob, fix_qv, fix_k, fix_o, chained):
    ys, ks, ss, ps, pvs, os_ = {}, {}, {}, {}, {}, {}
    kg = 4

    def proj(p):
        n, e = divmod(p, NP // NW)
        cols = slice(e * 2 * PW, (e + 1) * 2 * PW)
        if p == 0 and chained:
            ksp = 512
            y = _dot(h[:, 0:ksp], _unpack(wqv[n, 0:ksp // 2, cols]))
            y = _dot(h[:, ksp:], _unpack(wqv[n, ksp // 2:, cols])) + y
        else:
            y = _dot(h, _unpack(wqv[n, :, cols]))
        y = fix_qv(p, y)
        if p % kg == 0:
            k = _dot(hk, _unpack(wk[n, :, e * PW:(e + kg) * PW]))
            for i in range(kg):
                ks[p + i] = fix_k(p + i, k[:, i * PW:(i + 1) * PW])
        ys[p] = [y[:, 0:PW], ks.pop(p), y[:, PW:]]

    def weights(c, i, which):
        if i < 2:
            return _own_weights(ys[2 * c + i][which], i)
        return _others(ys[2 * c][which], ys[2 * c + 1][which], True)

    def score_round(n):
        for c, i in (divmod(j, 3) for j in range(4 * n, 4 * n + 4)):
            if i < 2:
                q = jnp.concatenate(_tiles(ys[2 * c + i][0], i)[0:2], axis=0).astype(BF16)
            else:
                q = _others(ys[2 * c][0], ys[2 * c + 1][0], False)
            ss[c, i] = _dot_nt(q, weights(c, i, 1))
            if i == 2:
                ps[c] = _softmax3([ss.pop((c, k)) for k in range(3)])

    def pv_round(n):
        for c, i in (divmod(j, 3) for j in range(4 * n, 4 * n + 4)):
            pvs[c, i] = _dot(ps[c][i], weights(c, i, 2))
            if i == 2:
                o0, o1, o2 = [pvs.pop((c, k)) for k in range(3)]
                os_[2 * c] = fix_o(2 * c, jnp.concatenate(
                    [o0[L:, :], o0[0:L, :], o2[L:, :]], axis=1))
                os_[2 * c + 1] = fix_o(2 * c + 1, jnp.concatenate(
                    [o2[0:L, :], o1[0:L, :], o1[L:, :]], axis=1))

    def slot(n):
        if n >= 2:
            pv_round(n - 2)
        if n < 6:
            score_round(n)

    def rows_of(e):
        return slice(e * DH, (e + 1) * DH)

    def oproj(lo, hi):
        o = jnp.concatenate([os_.pop(p) for p in range(lo, hi)], axis=1).astype(BF16)
        w = [wob[p // (NP // NW), rows_of(p % (NP // NW)), :] for p in range(lo, hi)]
        return _dot(o, _unpack(jnp.concatenate(w, axis=0)))

    after = {3: 0, 6: 1, 9: 2, 11: 3, 14: 4}
    for p in range(NP):
        proj(p)
        if p in after:
            slot(after[p])
    o1, o2, o3 = (2, 8, 10) if h.shape[0] == 48 else (2, 7, 10)
    r = oproj(0, o1)
    slot(5)
    r = oproj(o1, o2) + r
    slot(6)
    slot(7)
    r = oproj(o2, o3) + r
    return oproj(o3, NP) + r


def _kernel(x_hbm, wqkv_hbm, wphi_hbm, woa_hbm, mem0_hbm,
            wq_hbm, wk_hbm, wv_hbm, wo_hbm,
            out_hbm,
            xio, wqkv, wphi, woa, mem0, xres, xa, xl, xb, bds, wat, phq, phk, kvacc, kvs,
            wraw, wqv, wk, wob, xe, ke, ysave, osave, rsave, sem_in, sem_out):
    nsub = TN // 128
    na = S // TA
    asub = TA // 128
    nb = S // TB

    def rows(j, n):
        return pl.ds(j * n if isinstance(j, int) else pl.multiple_of(j * n, n), n)

    def x_copy(j):
        if isinstance(j, int) and j < 0:
            r = pl.ds(0, 256)
        elif isinstance(j, int) and j == na - 1:
            r = pl.ds(S - TA + 256, TA - 256)
        else:
            r = pl.ds(j * TA + 256 if isinstance(j, int)
                      else pl.multiple_of(j * TA + 256, 256), TA)
        return pltpu.make_async_copy(x_hbm.at[r, :], xio.at[r, :], sem_in.at[9 + j])

    def w_copies(c):
        return [pltpu.make_async_copy(src.at[c], wraw.at[i, c],
                                      sem_in.at[10 + na + 3 * c + i])
                for i, src in enumerate((wq_hbm, wv_hbm, wo_hbm))]

    def wa_copy(c):
        r = pl.ds(512, 128) if isinstance(c, int) and c == 2 else rows(c, 256)
        return pltpu.make_async_copy(wqkv_hbm.at[r, :], wqkv.at[r, :], sem_in.at[3 + c])

    def out_copy(i):
        return pltpu.make_async_copy(xio.at[rows(i, TB), :],
                                     out_hbm.at[rows(i, TB), :], sem_out.at[0])

    wphi_copy = pltpu.make_async_copy(wphi_hbm, wphi, sem_in.at[0])
    woa_copy = pltpu.make_async_copy(woa_hbm, woa, sem_in.at[1])
    mem0_copy = pltpu.make_async_copy(mem0_hbm, mem0, sem_in.at[2])
    order = [wphi_copy, wa_copy(0), wa_copy(1), x_copy(-1), wa_copy(2)]
    wk_copy = pltpu.make_async_copy(wk_hbm, wraw.at[3], sem_in.at[9 + na])
    order += [x_copy(j) for j in range(na)] + [woa_copy, mem0_copy, wk_copy]
    for c in range(NW):
        order += w_copies(c)
    for c in order:
        c.start()

    def strassen_rhs(x0, x1):
        b11, b12 = [jnp.concatenate([x[:, 0:128], x[:, 256:384]], axis=1) for x in (x0, x1)]
        b21, b22 = [jnp.concatenate([x[:, 128:256], x[:, 384:512]], axis=1) for x in (x0, x1)]
        ops = [b11 + b22, b11, b12 - b22, b21 - b11, b22, b11 + b12, b21 + b22,
               x0[:, 512:], x1[:, 512:]]
        return _pack(jnp.concatenate(ops, axis=1).astype(BF16))

    def load_x(t, first):
        xs = _split_rows(xio[rows(t, 256), :].astype(F32))
        if first is not True:
            xs = [jnp.where(first, x, xres[e, rows(t, 128), :]) for e, x in enumerate(xs)]
        for e, x in enumerate(xs):
            xres[e, rows(t, 128), :] = x
        return jnp.concatenate(xs, axis=0)

    wphi_copy.wait()
    cphi = jnp.zeros((FA, D), F32)
    hh = lax.broadcasted_iota(jnp.int32, (HA, D), 0) * FA
    jj = lax.broadcasted_iota(jnp.int32, (HA, D), 1)
    for d in range(FA):
        cphi = _dot(wphi[d], jnp.where(jj == hh + d, 1.0, 0.0).astype(BF16)) + cphi
    cb = jnp.concatenate(
        [jnp.broadcast_to(cphi[f:f + 1, :], (8, D)) for f in range(FA)], axis=0)
    for g in range(GA):
        row = lax.broadcasted_iota(jnp.int32, (GR, 256), 0)
        col = lax.broadcasted_iota(jnp.int32, (GR, 256), 1) + 128 * g
        lo = (8 * g + (row & 7)) * FA
        bds[g] = _pack(jnp.where(jnp.logical_and(col >= lo, col < lo + FA),
                                 cb[:, 128 * g:128 * g + 256], 0.0).astype(BF16))

    def folded(rr):
        out = [[], [], []]
        for g in range(GA):
            ws = []
            for i in range(2):
                c0 = i * D + 128 * g
                w = _dot_nt(_unpack(bds[g]), wqkv[rr, c0:c0 + 256]).reshape(FA, 8, 128)
                ws.append(((w[1:] - w[0:1]) * LOG2E).reshape(GR - 8, 128))
            out[0].append(jnp.concatenate([ws[1], ws[0][GR - 16:, :]], axis=0))
            out[1].append(ws[0][0:GR - 16, :])
        wvt = wqkv[rr, 2 * D:3 * D].T.astype(F32)
        out[2] = [wvt[g * GR:(g + 1) * GR, :] for g in range(GA)]
        return out

    def fold(c, _):
        wa_copy(c).wait()
        wa, wb = folded(rows(2 * c, 128)), folded(rows(2 * c + 1, 128))
        for i in range(3):
            for p in range(2):
                a11, a12, a21, a22 = wa[i][2 * p], wb[i][2 * p], wa[i][2 * p + 1], wb[i][2 * p + 1]
                ops = [a11 + a22, a21 + a22, a11, a22, a11 + a12, a21 - a11, a12 - a22]
                for m, w in enumerate(ops):
                    wat[2 * i + p, m, 0:w.shape[0] // 2, rows(c, 128)] = _pack(w.astype(BF16))
        return 0

    lax.fori_loop(0, 2, fold, 0)
    x_copy(-1).wait()
    wa_copy(2).wait()
    x = _layernorm(load_x(0, True))
    xa[...] = strassen_rhs(x[0:128], x[128:])
    for i, ws in enumerate(folded(pl.ds(512, 128))):
        for g, w in enumerate(ws):
            wat[2 * i + g // 2, 7, 0:w.shape[0] // 2, rows(g % 2, 128)] = _pack(w.astype(BF16))

    def pair_rows(ph, q, t0, n):
        return _unpack(jnp.concatenate(
            [ph[t0 + u, rows(q, 2 * FA), :] for u in range(n)], axis=1))

    def a1(first, j, _):
        @pl.when(jnp.logical_and(first, j < na - 1))
        def _():
            x_copy(j).wait()

        @pl.when(jnp.logical_and(first, j == na - 1))
        def _():
            x_copy(na - 1).wait()

        def features(ph, t, g, y):
            for f, w in enumerate(_feature_map(y)):
                ph[t, pl.ds(GR * g + f, 8, stride=FA), :] = w

        def tail(n, xs, g, u):
            nr = GR // 2 - 8 if n // 2 == 1 else GR // 2
            return _dot_nt(_unpack(wat[n, 7, 0:nr, 128 * g:128 * (g + 1)]),
                           xs[:, 1792 + 128 * u:1920 + 128 * u])

        def a_dots(n, xs, emit, tie, t10):
            nr = GR // 2 - 8 if n // 2 == 1 else GR // 2
            p = n % 2

            def prod(m):
                return _dot_nt(_unpack(tie(wat[n, m, 0:nr, :])), xs[:, 256 * m:256 * (m + 1)])

            m2, m4 = prod(1), prod(3)
            emit(2 * p + 1, 0, m4 + (m2 - (-t10)))
            t01 = tail(n, xs, 0, 1)
            m3, m5 = prod(2), prod(4)
            emit(2 * p, 1, m5 + (m3 - (-t01)))
            m1 = prod(0)
            c22 = prod(5) + (m1 + (m3 - m2))
            emit(2 * p + 1, 1, tail(n, xs, 1, 1) + c22)
            t10 = tail(n + 1, xs, 1, 0) if n < 5 else None
            c11 = tail(n, xs, 0, 0) + (m1 + (m4 - m5))
            emit(2 * p, 0, prod(6) + c11)
            return t10

        vs = {}
        cur = xa[...]
        dl = (3, 8, 13, 30, 33, 36, 39, 41)
        for u in range(0, asub, 2):
            t = j * (asub // 2) + u // 2
            xs = _unpack(cur)
            tn = t + 1
            x = load_x(tn if u + 2 < asub else jnp.minimum(tn, (na - 1) * (asub // 2)), first)
            rest, seen, nxt = {}, [], []

            def tie(w):
                seen.append(0)
                if len(seen) - 1 not in dl:
                    return w
                n = len(nxt)
                nxt.append(strassen_rhs(*[
                    _layernorm(x[128 * e + 16 * n:128 * e + 16 * n + 16, :]) for e in range(2)]))
                z = jnp.concatenate(
                    [nxt[n][:, 256 * c:256 * (c + 1)] for c in range(8)], axis=0)
                return jnp.concatenate([jnp.where(j < 0, z, w[0:64, :]), w[64:, :]], axis=0)

            def emit_k(g, e, y):
                features(phk, u + e, g, y[0:GR - 8, :])
                rest[g, e] = y[GR - 8:, :]

            def emit_q(g, e, y):
                features(phq, 8 * e + t, g, jnp.concatenate([y, rest[g, e]], axis=0))

            def emit_v(g, e, y):
                for q in range(4):
                    vs[4 * g + q, u + e] = y[40 * q:40 * q + 40, :]

            t10 = tail(0, xs, 1, 0)
            for n in range(6):
                t10 = a_dots(n, xs, (emit_k, emit_q, emit_v)[n // 2], tie, t10)
            cur = jnp.concatenate(nxt, axis=0)
        xa[...] = cur
        row = lax.broadcasted_iota(jnp.int32, (2 * VR, 4 * FA), 0)
        col = lax.broadcasted_iota(jnp.int32, (2 * VR, 4 * FA), 1)
        split = jnp.where(row < 2 * FA, FA, 2 * FA + 4)
        same = (row >= split) == (col >= 2 * FA)
        for q in range(PA):
            v = jnp.concatenate([vs[q, u] for u in range(asub)], axis=1)
            v = jnp.concatenate([v, jnp.ones((8, TA), F32)], axis=0)
            kv = _dot_nt(v.astype(BF16), pair_rows(phk, q, 0, asub))
            kv = kv + jnp.where(j == 0, 0.0, kvacc[q])
            kvacc[q] = kv
            kvs[q] = _pack(jnp.where(same, kv, 0.0).astype(BF16))
        return 0

    def attend(j):
        low = lax.broadcasted_iota(jnp.int32, (8, TN), 0) < 4
        os_ = []
        for q in range(PA):
            nd = _dot(_unpack(kvs[q]), pair_rows(phq, q, j * nsub, nsub))
            rab = 1.0 / (nd[40:48, :] + 1e-6)
            rba = pltpu.roll(rab, 4, 0)
            ra = jnp.where(low, rab, rba)
            rb = jnp.where(low, rba, rab)
            os_.append(nd[0:40, :] * jnp.concatenate([ra, ra, rab, rb, rb], axis=0))
        return _pack(jnp.concatenate(os_, axis=0).astype(BF16).T)

    def project(ty, j, o, slot):
        r = rows(j, TN)
        x = _dot(_unpack(o), woa[...]) + xres[ty, r, :]
        xres[ty, r, :] = x
        for s in range(16):
            z = _layernorm(x[16 * s + 8 - 8 * (s % 2):16 * s + 16 - 8 * (s % 2), :])
            z = z - z[KE:KE + 1, :]
            for c in range(D // 128):
                xe[ty, slot, c, pl.ds(s * KE, 8), :] = z[:, 128 * c:128 * (c + 1)]

    def extra_keys(seg, p):
        k = jnp.concatenate(
            [ke[2 * (seg // 32) + t // 24, (seg // 16) % 2, t % 24, pl.ds((seg % 16) * KE, 8), :]
             for t in range(3 * p, 3 * p + 3)], axis=1)
        return jnp.where(lax.broadcasted_iota(jnp.int32, (8, PW), 0) < KE, k, 0.0)

    def b_residual(i):
        r = rows(i, TB // 2)
        xs = [xres[e, r, :] + d for e, d in enumerate(_split_rows(rsave[...]))]
        for e, x in enumerate(xs):
            xres[e, r, :] = x
        xio[rows(i, TB), :] = _merge_rows(*xs).astype(BF16)
        return xs

    def b_finish(i):
        xn = [_layernorm(x) for x in b_residual(i)]
        for e, x in enumerate(xn):
            xl[e, rows(jnp.minimum(i, 2), TB // 2), :] = x
        return jnp.concatenate(xn, axis=0)

    def b_pair(mem, xn, base, blk, side):
        def fix_qva(p, y):
            c0 = 2 * PW - D
            tie = jnp.where(blk < 0, side[8 * p:8 * p + 8, :], y[0:M, c0:])
            ysave[:, p * 2 * PW:(p + 1) * 2 * PW] = y[L:L + 8, :]
            return jnp.concatenate(
                [jnp.concatenate([y[0:M, 0:c0], tie], axis=1), y[M:L, :]], axis=0)

        def fix_ka(p, k):
            return jnp.concatenate([k, extra_keys(2 * blk, p)], axis=0)

        def fix_oa(p, o):
            osave[:, p * PW:(p + 1) * PW] = o[32:L, :]
            return o[0:32, :]

        h = jnp.concatenate([mem, xn[0:40, :]], axis=0)
        ra = _segment(h.astype(BF16), (h[0:32, :] - xn[31:32, :]).astype(BF16),
                      wqv, wk, wob, fix_qva, fix_ka, fix_oa, base > 0)
        rsave[base:base + 24, :] = ra[M:, :]

        def fix_qvb(p, y):
            return jnp.concatenate(
                [y[0:M, :], ysave[:, p * 2 * PW:(p + 1) * 2 * PW], y[M:, :]], axis=0)

        def fix_kb(p, k):
            return jnp.concatenate([k[0:M, :], extra_keys(2 * blk + 1, p), k[M:, :]], axis=0)

        def fix_ob(p, o):
            return jnp.concatenate([o, osave[:, p * PW:(p + 1) * PW]], axis=0)

        h = jnp.concatenate([ra[0:M, :], xn[40:64, :]], axis=0)
        rb = _segment(h.astype(BF16), (h - xn[39:40, :]).astype(BF16),
                      wqv, wk, wob, fix_qvb, fix_kb, fix_ob, True)
        rsave[base + 24:base + 32, :] = rb[L:, :]
        rsave[base + 32:base + 64, :] = rb[M:L, :]
        return rb[0:M, :]

    def layer(l, _):
        def wait_first(copies):
            @pl.when(l == 0)
            def _():
                for c in copies:
                    c.wait()

        with jax.named_scope("a1"):
            lax.fori_loop(0, na, functools.partial(a1, l == 0), 0)

        def a2(n, _):
            wait_first(w_copies(n))
            ty, half = n % 2, n // 2
            o0 = attend(4 * ty + 2 * half)
            o1 = attend(4 * ty + 2 * half + 1)

            def sample(w):
                z = [w[64 * a + 56:64 * a + 64, :] for a in range(D // 128)]
                out = []
                for y in z:
                    acc = y[:, 0:128]
                    for c in range(1, y.shape[1] // 128):
                        acc = acc | y[:, 128 * c:128 * (c + 1)]
                    out.append(acc)
                return jnp.concatenate(out, axis=1)

            wt = _pack(wraw[3, n].T)
            wk[n] = wt
            o1 = jnp.concatenate([jnp.where(n < 0, sample(wt), o1[0:8, :]), o1[8:, :]], axis=0)
            mr = 16 * KE

            def staged(e):
                return jnp.concatenate([xe[0, e, c, 0:mr, :] for c in range(D // 128)], axis=1)

            def relayout(lo, hi):
                acc = None
                for p in range(lo, hi):
                    for i in range(2):
                        wt = _pack(wraw[i, n, rows(p, PW), :].T)
                        wqv[n, :, rows(2 * p + i, PW)] = wt
                        acc = sample(wt) if acc is None else acc | sample(wt)
                return acc

            early = 2
            project(ty, 2 * half, o0, 0)
            x0 = staged(0)
            tie = pltpu.bitcast(relayout(0, early), F32)
            x0 = jnp.concatenate([jnp.where(n < 0, tie, x0[0:8, :]), x0[8:, :]], axis=0)
            project(ty, 2 * half + 1, o1, 1)
            x1 = staged(1)
            r = rows(ty, 32)
            xb[rows(ty, 64), :] = _layernorm(_merge_rows(xres[0, r, :], xres[1, r, :]))
            rsave[rows(ty, 64), :] = jnp.zeros((64, D), F32)

            a11, a12, a21, a22 = x0[:, 0:256], x0[:, 256:512], x1[:, 0:256], x1[:, 256:512]
            lhs = [z.astype(BF16) for z in (
                a11 + a22, a21 + a22, a11, a22, a11 + a12, a21 - a11, a12 - a22,
                x0[:, 512:], x1[:, 512:])]
            done = []

            def emit(e, t, k):
                ke[n, e, t, 0:mr, :] = k
                q = len(done)
                done.append(q)
                tie = pltpu.bitcast(k[0:16, :], U32)
                wob[n, rows(q, 16), :] = jnp.where(
                    n < 0, jnp.concatenate([tie] * (D // 128), axis=1),
                    _pack(wraw[2, n, rows(q, 32), :]))

            def blk(v, e, k):
                return wraw[3, 2 * ty + v // 6, rows(2 * (v % 6) + e, 128),
                            256 * k:min(256 * (k + 1), D)]

            def comb(v, x, sign, y):
                x, y = blk(v, *x).astype(F32), blk(v, *y).astype(F32)
                return (x + y if sign > 0 else x - y).astype(BF16)

            b11, b21, b12, b22 = (0, 0), (0, 1), (1, 0), (1, 1)

            def first_half(v):
                m3 = _dot_nt(lhs[2], comb(v, b12, -1, b22))
                m5 = _dot_nt(lhs[4], blk(v, *b22))
                emit(0, 2 * v + 1, _dot_nt(lhs[7], blk(v, 1, 2)) + (m3 + m5))
                return m3, _dot_nt(lhs[7], blk(v, 0, 2)) - m5

            def second_half(v, m3, c11):
                m2 = _dot_nt(lhs[1], blk(v, *b11))
                m4 = _dot_nt(lhs[3], comb(v, b21, -1, b11))
                emit(1, 2 * v, _dot_nt(lhs[8], blk(v, 0, 2)) + (m2 + m4))
                m1 = _dot_nt(lhs[0], comb(v, b11, 1, b22))
                c22 = _dot_nt(lhs[5], comb(v, b11, 1, b12)) + (m1 + (m3 - m2))
                emit(1, 2 * v + 1, _dot_nt(lhs[8], blk(v, 1, 2)) + c22)
                emit(0, 2 * v, _dot_nt(lhs[6], comb(v, b21, 1, b22)) + (c11 + (m1 + m4)))

            lead = 8
            st = [first_half(v) for v in range(lead)]
            for v in range(12):
                second_half(v, *(st[v] if v < lead else first_half(v)))
            relayout(early, NP // NW)
            return 0

        wait_first([woa_copy, mem0_copy, wk_copy])
        with jax.named_scope("a2"):
            lax.fori_loop(0, NW, a2, 0)

        def b_step(i, mem):
            xn = xb[...]
            side = b_finish(jnp.maximum(i - 1, 0))
            r = rows(jnp.minimum(i + 1, nb - 1), TB // 2)
            nxt = _layernorm(_merge_rows(xres[0, r, :], xres[1, r, :]))
            xb[...] = nxt
            side = jnp.concatenate([side, nxt], axis=0)
            for u in range(0, TB, 2 * SEG):
                mem = b_pair(mem, xn[u:u + 2 * SEG, :], u, (i * TB + u) // (2 * SEG),
                             side[2 * u:2 * u + 8 * NP, :])

            @pl.when(jnp.logical_and(l == 1, i >= 1))
            def _():
                out_copy(i - 1).start()
            return mem

        with jax.named_scope("b"):
            lax.fori_loop(0, nb, b_step, mem0[...].astype(F32))

        b_residual(nb - 1)

        @pl.when(l == 0)
        def _():
            xa[...] = strassen_rhs(xl[0, 0:128, :], xl[1, 0:128, :])
        return 0

    lax.fori_loop(0, 2, layer, 0)
    out_copy(nb - 1).start()
    pltpu.make_async_copy(xio, out_hbm, sem_out.at[0]).wait()


@jax.jit
def pallas_interleave_layers__linear_kernel_hedgehog__memory_aug_recurrent_mem_tr__prompt_kernel(
    A_x, A_wqkv, A_w_phi, A_wo, B_x, B_mem0, B_Wq, B_Wk, B_Wv, B_Wo, B_seg_len,
):
    del B_x
    del B_seg_len
    x = A_x.reshape(S, D)
    wphi = A_w_phi.transpose(1, 2, 0)
    mem0 = B_mem0.reshape(M, D)
    wq, wk, wv = (w.transpose(1, 2, 0).reshape(NW, QW, D) for w in (B_Wq, B_Wk, B_Wv))
    wo = B_Wo.reshape(NW, QW, D)
    hbm = pl.BlockSpec(memory_space=pl.ANY)
    out = pl.pallas_call(
        _kernel,
        out_shape=jax.ShapeDtypeStruct((S, D), A_x.dtype),
        in_specs=[hbm] * 9,
        out_specs=hbm,
        scratch_shapes=[
            pltpu.VMEM((S, D), BF16),
            pltpu.VMEM((D, 3 * D), BF16),
            pltpu.VMEM((FA, FA, HA), BF16),
            pltpu.VMEM((D, D), BF16),
            pltpu.VMEM((M, D), BF16),
            pltpu.VMEM((2, S // 2, D), F32),
            pltpu.VMEM((64, 2048), U32),
            pltpu.VMEM((2, 3 * TB // 2, D), F32),
            pltpu.VMEM((TB, D), F32),
            pltpu.VMEM((GA, GR // 2, 256), U32),
            pltpu.VMEM((6, 8, GR // 2, 256), U32),
            pltpu.VMEM((S // 128, D, 128), U32),
            pltpu.VMEM((TA // 128, D, 128), U32),
            pltpu.VMEM((PA, 2 * VR, 4 * FA), F32),
            pltpu.VMEM((PA, VR, 4 * FA), U32),
            pltpu.VMEM((4, NW, QW, D), BF16),
            pltpu.VMEM((NW, D // 2, 2 * QW), U32),
            pltpu.VMEM((NW, D // 2, QW), U32),
            pltpu.VMEM((NW, QW // 2, D), U32),
            pltpu.VMEM((2, 2, D // 128, 16 * KE + 8, 128), F32),
            pltpu.VMEM((NW, 2, HD // 256, 16 * KE + 8, 128), F32),
            pltpu.VMEM((8, 2 * HD), F32),
            pltpu.VMEM((8, HD), F32),
            pltpu.VMEM((TB, D), F32),
            pltpu.SemaphoreType.DMA((10 + S // TA + 3 * NW,)),
            pltpu.SemaphoreType.DMA((1,)),
        ],
        compiler_params=pltpu.CompilerParams(vmem_limit_bytes=120 * 1024 * 1024,
                                             disable_bounds_checks=True,
                                             disable_semaphore_checks=True),
    )(x, A_wqkv, wphi, A_wo, mem0, wq, wk, wv, wo)
    return out.reshape(1, S, D)
```

```python
import functools

import jax
import jax.numpy as jnp
from jax import lax
import jax.experimental.pallas as pl
import jax.experimental.pallas.tpu as pltpu

F32 = jnp.float32
BF16 = jnp.bfloat16
U32 = jnp.uint32

S = 2048
D = 640
HA = 32
FA = 20
GA = 4
GR = 8 * FA
VR = 24
PA = HA // 2
TN = 256
TA = 512
HB = 32
DH = 192
HD = HB * DH
M = 8
SEG = 32
L = M + SEG
PW = 2 * DH
NP = HB // 2
TB = 128
NW = 4
QW = HD // NW
KE = 7

NT = (((1,), (1,)), ((), ()))
LOG2E = 1.4426950408889634
HALF_ULP = 0.0040612


def _dot(a, b):
    return jnp.dot(a, b, preferred_element_type=F32)


def _dot_nt(a, b):
    return lax.dot_general(a, b, NT, preferred_element_type=F32)


def _pack(a):
    return pltpu.bitcast(a, U32)


def _unpack(a):
    return pltpu.bitcast(a, BF16)


def _interleave(a, b):
    lo = lax.bitcast_convert_type(a, U32) >> 16
    hi = lax.bitcast_convert_type(b, U32) & jnp.uint32(0xFFFF0000)
    return lo | hi


def _recip(x):
    r = pl.reciprocal(x, approx=True)
    return r * (2.0 - x * r)


def _layernorm(x):
    m = jnp.mean(x, axis=-1, keepdims=True)
    c = x - m
    v = jnp.mean(c * c, axis=-1, keepdims=True)
    return c * lax.rsqrt(v + 1e-5)


def _split_rows(x):
    blocks = range(0, x.shape[0], 64)
    return (jnp.concatenate([x[b + 16:b + 48] for b in blocks], axis=0),
            jnp.concatenate([x[b + k:b + k + 16] for b in blocks for k in (0, 48)], axis=0))


def _merge_rows(inner, outer):
    return jnp.concatenate(
        [z for b in range(0, inner.shape[0], 32)
         for z in (outer[b:b + 16], inner[b:b + 32], outer[b + 16:b + 32])], axis=0)


def _feature_map(p):
    t = p.shape[-1]
    p3 = jnp.concatenate([jnp.zeros((8, t), F32), p], axis=0).reshape(FA, 8, t)
    mx = jnp.max(p3, axis=0)
    mn = jnp.min(p3, axis=0)
    sp, sn = jnp.exp2(p3[0] - mx), jnp.exp2(mn - p3[0])
    for f in range(1, FA):
        sp, sn = sp + jnp.exp2(p3[f] - mx), sn + jnp.exp2(mn - p3[f])
    lp = (mx - HALF_ULP) + jnp.log2(sp)
    ln = (mn + HALF_ULP) - jnp.log2(sn)
    return [_interleave(jnp.exp2(p3[f] - lp), jnp.exp2(ln - p3[f])) for f in range(FA)]


def _tiles(a, odd):
    t0, t1, t2 = a[:, 0:128], a[:, 128:256], a[:, 256:384]
    return (t1, t2, t0) if odd else (t1, t0, t2)


def _own_weights(a, odd):
    lane = lax.broadcasted_iota(jnp.int32, (L, 128), 1)
    mid, own, _ = _tiles(a, odd)
    return jnp.concatenate(
        [jnp.where(lane < 64, mid, 0.0), jnp.where(lane < 64, 0.0, mid), own,
         jnp.zeros((128 - 3 * L, 128), F32)], axis=0).astype(BF16)


def _others(even, odd, pad):
    parts = [_tiles(odd, 1)[2], _tiles(even, 0)[2]]
    if pad:
        parts.append(jnp.zeros((128 - 2 * L, 128), F32))
    return jnp.concatenate(parts, axis=0).astype(BF16)


def _softmax3(s3):
    row = lax.broadcasted_iota(jnp.int32, (L, 128), 0)
    col = lax.broadcasted_iota(jnp.int32, (L, 128), 1)
    first = col < L
    second = jnp.logical_and(col >= L, col < 2 * L)
    key = jnp.where(first, col, col - L)
    valid = jnp.logical_or(row < M, row >= key)
    out, other = [], []
    for odd in range(2):
        own = pltpu.roll(s3[odd][L:, :], 128 - L if odd else 128 - 2 * L, 1)
        s = (jnp.where(first, s3[2][0:L, :], own) if odd
             else jnp.where(first, own, s3[2][L:, :]))
        s = jnp.where(valid, (s + s3[odd][0:L, :]) * (DH ** -0.5), -1e9)
        m0 = jnp.max(jnp.where(first, s, -jnp.inf), axis=-1, keepdims=True)
        m1 = jnp.max(jnp.where(second, s, -jnp.inf), axis=-1, keepdims=True)
        e = jnp.exp(s - jnp.where(first, m0, m1))
        e0 = jnp.where(first, e, 0.0)
        e1 = jnp.where(second, e, 0.0)
        p0 = e0 * _recip(jnp.sum(e0, axis=-1, keepdims=True))
        p1 = e1 * _recip(jnp.sum(e1, axis=-1, keepdims=True))
        own = pltpu.roll(p1, L, 1) if odd else pltpu.roll(p0, 2 * L, 1)
        out.append(jnp.concatenate([p0 + p1, own], axis=0).astype(BF16))
        other.append(p0 if odd else p1)
    out.append(jnp.concatenate([other[1], other[0]], axis=0).astype(BF16))
    return out


def _strassen_lhs(a11, a12, a21, a22):
    return [z.astype(BF16) for z in (
        a11 + a22, a21 + a22, a11, a22, a11 + a12, a21 - a11, a12 - a22)]


def _strassen_sums(b11, b12, b21, b22):
    return [b11 + b22, b12 - b22, b21 - b11, b11 + b12, b21 + b22]


def _strassen(lhs, b11, b22, sums, c11, c12, c21, c22):
    m2 = _dot(lhs[1], b11)
    m4 = _dot(lhs[3], sums[2])
    m3 = _dot(lhs[2], sums[1])
    m5 = _dot(lhs[4], b22)
    m1 = _dot(lhs[0], sums[0])
    c22 = _dot(lhs[5], sums[3]) + (m1 + ((m3 - m2) - (-c22)))
    c11 = _dot(lhs[6], sums[4]) + (m1 + ((m4 - m5) - (-c11)))
    return c11, m5 + (m3 - (-c12)), m4 + (m2 - (-c21)), c22


def _segment(h, hk, wqv, sqv, wk, wob, sob, fix_qv, fix_k, fix_o, wide_o):
    ys, ks, ss, ps, pvs, os_, wide = {}, {}, {}, {}, {}, {}, {}
    kg = 4
    hb = h.astype(BF16)
    if h.shape[0] == 64:
        lhs = _strassen_lhs(h[0:32, 0:256], h[0:32, 256:512], h[32:, 0:256], h[32:, 256:512])

    def wide_proj(p):
        n, e = divmod(p, NP // NW)
        out = [[], []]
        for c in range(0, 2 * PW, 256):
            c0, c1 = e * 2 * PW + c, (e + 1) * 2 * PW + c
            t0 = _dot(hb[:, 512:], _unpack(wqv[n, 256:, c0:c0 + 256]))
            t1 = _dot(hb[:, 512:], _unpack(wqv[n, 256:, c1:c1 + 256]))
            cs = 5 * (e * PW + c)
            c11, c12, c21, c22 = _strassen(
                lhs, _unpack(wqv[n, 0:128, c0:c0 + 256]), _unpack(wqv[n, 128:256, c1:c1 + 256]),
                [_unpack(sqv[128 * n:128 * (n + 1), cs + 256 * m:cs + 256 * (m + 1)])
                 for m in range(5)],
                t0[0:32], t1[0:32], t0[32:], t1[32:])
            out[0].append(jnp.concatenate([c11, c21], axis=0))
            out[1].append(jnp.concatenate([c12, c22], axis=0))
            unit = 3 * (p // 2) + c // 256
            if unit in after:
                slot(after.index(unit))
        wide[p], wide[p + 1] = [jnp.concatenate(o, axis=1) for o in out]

    def proj(p):
        n, e = divmod(p, NP // NW)
        cols = slice(e * 2 * PW, (e + 1) * 2 * PW)
        if h.shape[0] == 64:
            if p % 2 == 0:
                wide_proj(p)
            y = wide.pop(p)
        elif p == 0:
            ksp = 512
            y = _dot(hb[:, 0:ksp], _unpack(wqv[n, 0:ksp // 2, cols]))
            y = _dot(hb[:, ksp:], _unpack(wqv[n, ksp // 2:, cols])) + y
        else:
            y = _dot(hb, _unpack(wqv[n, :, cols]))
        y = fix_qv(p, y)
        if p % kg == 0:
            k = _dot(hk, _unpack(wk[n, :, e * PW:(e + kg) * PW]))
            for i in range(kg):
                ks[p + i] = fix_k(p + i, k[:, i * PW:(i + 1) * PW])
        ys[p] = [y[:, 0:PW], ks.pop(p), y[:, PW:]]

    def weights(c, i, which):
        if i < 2:
            return _own_weights(ys[2 * c + i][which], i)
        return _others(ys[2 * c][which], ys[2 * c + 1][which], True)

    def score_round(n):
        for c, i in (divmod(j, 3) for j in range(4 * n, 4 * n + 4)):
            if i < 2:
                q = jnp.concatenate(_tiles(ys[2 * c + i][0], i)[0:2], axis=0).astype(BF16)
            else:
                q = _others(ys[2 * c][0], ys[2 * c + 1][0], False)
            ss[c, i] = _dot_nt(q, weights(c, i, 1))
            if i == 2:
                ps[c] = _softmax3([ss.pop((c, k)) for k in range(3)])

    def pv_round(n):
        for c, i in (divmod(j, 3) for j in range(4 * n, 4 * n + 4)):
            pvs[c, i] = _dot(ps[c][i], weights(c, i, 2))
            if i == 2:
                o0, o1, o2 = [pvs.pop((c, k)) for k in range(3)]
                os_[2 * c] = fix_o(2 * c, jnp.concatenate(
                    [o0[L:, :], o0[0:L, :], o2[L:, :]], axis=1))
                os_[2 * c + 1] = fix_o(2 * c + 1, jnp.concatenate(
                    [o2[0:L, :], o1[0:L, :], o1[L:, :]], axis=1))

    def slot(n):
        if n >= 2:
            pv_round(n - 2)
        if n < 6:
            score_round(n)

    def rows_of(e):
        return slice(e * DH, (e + 1) * DH)

    def wo_rows(ps_, cols):
        return _unpack(jnp.concatenate(
            [wob[rows_of(p), cols] for p in ps_], axis=0))

    def oproj(lo, hi, r):
        o = [os_.pop(p) for p in range(lo, hi)]
        ob = jnp.concatenate(o, axis=1).astype(BF16)
        if not wide_o:
            y = _dot(ob, wo_rows(range(lo, hi), slice(None)))
            return y if r is None else y + r
        t = _dot(ob, wo_rows(range(lo, hi), slice(512, D)))
        if r is None:
            r = jnp.zeros((64, D), F32)
        else:
            t = t + r[:, 512:]
        k1, k2 = jnp.concatenate(o[0::2], axis=1), jnp.concatenate(o[1::2], axis=1)
        sums = [_unpack(jnp.concatenate(
            [sob[rows_of(p // 2), 256 * m:256 * (m + 1)] for p in range(lo, hi, 2)],
            axis=0)) for m in range(5)]
        c11, c12, c21, c22 = _strassen(
            _strassen_lhs(k1[0:32], k2[0:32], k1[32:], k2[32:]),
            wo_rows(range(lo, hi, 2), slice(0, 256)), wo_rows(range(lo + 1, hi, 2), slice(256, 512)),
            sums, r[0:32, 0:256], r[0:32, 256:512], r[32:, 0:256], r[32:, 256:512])
        return jnp.concatenate([jnp.concatenate([c11, c21], axis=0),
                                jnp.concatenate([c12, c22], axis=0), t], axis=1)

    after = (6, 9, 12, 18, 21) if h.shape[0] == 64 else (3, 6, 9, 12, 14)
    for p in range(NP):
        proj(p)
        if h.shape[0] == 32 and p in after:
            slot(after.index(p))
    o1, o2, o3 = (2, 6, 10) if wide_o else (2, 9, 10)
    r = oproj(0, o1, None)
    slot(5)
    r = oproj(o1, o2, r)
    slot(6)
    slot(7)
    if o3 > o2:
        r = oproj(o2, o3, r)
    return oproj(o3, NP, r)


def _kernel(x_hbm, wqkv_hbm, wphi_hbm, woa_hbm, mem0_hbm,
            wq_hbm, wk_hbm, wv_hbm, wo_hbm,
            out_hbm,
            xio, wqkv, wphi, woa, mem0, xres, xa, xl, xb, bds, wat, phq, phk, kvacc, kvs,
            wraw, wqv, sqv, wk, wob, sob, xe, ke, ysave, osave, rsave, sem_in, sem_out):
    nsub = TN // 128
    na = S // TA
    asub = TA // 128
    nb = S // TB

    def rows(j, n):
        return pl.ds(j * n if isinstance(j, int) else pl.multiple_of(j * n, n), n)

    def x_copy(j):
        if isinstance(j, int) and j < 0:
            r = pl.ds(0, 256)
        elif isinstance(j, int) and j == na - 1:
            r = pl.ds(S - TA + 256, TA - 256)
        else:
            r = pl.ds(j * TA + 256 if isinstance(j, int)
                      else pl.multiple_of(j * TA + 256, 256), TA)
        return pltpu.make_async_copy(x_hbm.at[r, :], xio.at[r, :], sem_in.at[9 + j])

    def w_copies(c):
        return [pltpu.make_async_copy(src.at[c], wraw.at[i, c],
                                      sem_in.at[10 + na + 3 * c + i])
                for i, src in enumerate((wq_hbm, wv_hbm, wo_hbm))]

    def wa_copy(c):
        r = pl.ds(512, 128) if isinstance(c, int) and c == 2 else rows(c, 256)
        return pltpu.make_async_copy(wqkv_hbm.at[r, :], wqkv.at[r, :], sem_in.at[3 + c])

    def out_copy(i):
        return pltpu.make_async_copy(xio.at[rows(i, TB), :],
                                     out_hbm.at[rows(i, TB), :], sem_out.at[0])

    wphi_copy = pltpu.make_async_copy(wphi_hbm, wphi, sem_in.at[0])
    woa_copy = pltpu.make_async_copy(woa_hbm, woa, sem_in.at[1])
    mem0_copy = pltpu.make_async_copy(mem0_hbm, mem0, sem_in.at[2])
    order = [wphi_copy, wa_copy(0), wa_copy(1), x_copy(-1), wa_copy(2)]
    wk_copy = pltpu.make_async_copy(wk_hbm, wraw.at[3], sem_in.at[9 + na])
    order += [x_copy(j) for j in range(na)] + [woa_copy, mem0_copy, wk_copy]
    for c in range(NW):
        order += w_copies(c)
    for c in order:
        c.start()

    def strassen_rhs(x0, x1):
        b11, b12 = [jnp.concatenate([x[:, 0:128], x[:, 256:384]], axis=1) for x in (x0, x1)]
        b21, b22 = [jnp.concatenate([x[:, 128:256], x[:, 384:512]], axis=1) for x in (x0, x1)]
        ops = [b11 + b22, b11, b12 - b22, b21 - b11, b22, b11 + b12, b21 + b22,
               x0[:, 512:], x1[:, 512:]]
        return _pack(jnp.concatenate(ops, axis=1).astype(BF16))

    def load_x(t, first):
        xs = _split_rows(xio[rows(t, 256), :].astype(F32))
        if first is not True:
            xs = [jnp.where(first, x, xres[e, rows(t, 128), :]) for e, x in enumerate(xs)]
        for e, x in enumerate(xs):
            xres[e, rows(t, 128), :] = x
        return jnp.concatenate(xs, axis=0)

    wphi_copy.wait()
    cphi = jnp.zeros((FA, D), F32)
    hh = lax.broadcasted_iota(jnp.int32, (HA, D), 0) * FA
    jj = lax.broadcasted_iota(jnp.int32, (HA, D), 1)
    for d in range(FA):
        cphi = _dot(wphi[d], jnp.where(jj == hh + d, 1.0, 0.0).astype(BF16)) + cphi
    cb = jnp.concatenate(
        [jnp.broadcast_to(cphi[f:f + 1, :], (8, D)) for f in range(FA)], axis=0)
    for g in range(GA):
        row = lax.broadcasted_iota(jnp.int32, (GR, 256), 0)
        col = lax.broadcasted_iota(jnp.int32, (GR, 256), 1) + 128 * g
        lo = (8 * g + (row & 7)) * FA
        bds[g] = _pack(jnp.where(jnp.logical_and(col >= lo, col < lo + FA),
                                 cb[:, 128 * g:128 * g + 256], 0.0).astype(BF16))

    def folded(rr):
        out = [[], [], []]
        for g in range(GA):
            ws = []
            for i in range(2):
                c0 = i * D + 128 * g
                w = _dot_nt(_unpack(bds[g]), wqkv[rr, c0:c0 + 256]).reshape(FA, 8, 128)
                ws.append(((w[1:] - w[0:1]) * LOG2E).reshape(GR - 8, 128))
            out[0].append(jnp.concatenate([ws[1], ws[0][GR - 16:, :]], axis=0))
            out[1].append(ws[0][0:GR - 16, :])
        wvt = wqkv[rr, 2 * D:3 * D].T.astype(F32)
        out[2] = [wvt[g * GR:(g + 1) * GR, :] for g in range(GA)]
        return out

    def fold(c, _):
        wa_copy(c).wait()
        wa, wb = folded(rows(2 * c, 128)), folded(rows(2 * c + 1, 128))
        for i in range(3):
            for p in range(2):
                a11, a12, a21, a22 = wa[i][2 * p], wb[i][2 * p], wa[i][2 * p + 1], wb[i][2 * p + 1]
                ops = [a11 + a22, a21 + a22, a11, a22, a11 + a12, a21 - a11, a12 - a22]
                for m, w in enumerate(ops):
                    wat[2 * i + p, m, 0:w.shape[0] // 2, rows(c, 128)] = _pack(w.astype(BF16))
        return 0

    lax.fori_loop(0, 2, fold, 0)
    x_copy(-1).wait()
    wa_copy(2).wait()
    x = _layernorm(load_x(0, True))
    xa[...] = strassen_rhs(x[0:128], x[128:])
    for i, ws in enumerate(folded(pl.ds(512, 128))):
        for g, w in enumerate(ws):
            wat[2 * i + g // 2, 7, 0:w.shape[0] // 2, rows(g % 2, 128)] = _pack(w.astype(BF16))

    def pair_rows(ph, q, t0, n):
        return _unpack(jnp.concatenate(
            [ph[t0 + u, rows(q, 2 * FA), :] for u in range(n)], axis=1))

    def a1(first, j, _):
        @pl.when(jnp.logical_and(first, j < na - 1))
        def _():
            x_copy(j).wait()

        @pl.when(jnp.logical_and(first, j == na - 1))
        def _():
            x_copy(na - 1).wait()

        def features(ph, t, g, y):
            for f, w in enumerate(_feature_map(y)):
                ph[t, pl.ds(GR * g + f, 8, stride=FA), :] = w

        def tail(n, xs, g, u):
            nr = GR // 2 - 8 if n // 2 == 1 else GR // 2
            return _dot_nt(_unpack(wat[n, 7, 0:nr, 128 * g:128 * (g + 1)]),
                           xs[:, 1792 + 128 * u:1920 + 128 * u])

        def a_dots(n, xs, emit, tie, t10):
            nr = GR // 2 - 8 if n // 2 == 1 else GR // 2
            p = n % 2

            def prod(m):
                return _dot_nt(_unpack(tie(wat[n, m, 0:nr, :])), xs[:, 256 * m:256 * (m + 1)])

            m2, m4 = prod(1), prod(3)
            emit(2 * p + 1, 0, m4 + (m2 - (-t10)))
            t01 = tail(n, xs, 0, 1)
            m3, m5 = prod(2), prod(4)
            emit(2 * p, 1, m5 + (m3 - (-t01)))
            m1 = prod(0)
            c22 = prod(5) + (m1 + (m3 - m2))
            emit(2 * p + 1, 1, tail(n, xs, 1, 1) + c22)
            t10 = tail(n + 1, xs, 1, 0) if n < 5 else None
            c11 = tail(n, xs, 0, 0) + (m1 + (m4 - m5))
            emit(2 * p, 0, prod(6) + c11)
            return t10

        vs = {}
        cur = xa[...]
        dl = (3, 8, 13, 30, 33, 36, 39, 41)
        for u in range(0, asub, 2):
            t = j * (asub // 2) + u // 2
            xs = _unpack(cur)
            tn = t + 1
            x = load_x(tn if u + 2 < asub else jnp.minimum(tn, (na - 1) * (asub // 2)), first)
            rest, seen, nxt = {}, [], []

            def tie(w):
                seen.append(0)
                if len(seen) - 1 not in dl:
                    return w
                n = len(nxt)
                nxt.append(strassen_rhs(*[
                    _layernorm(x[128 * e + 16 * n:128 * e + 16 * n + 16, :]) for e in range(2)]))
                z = jnp.concatenate(
                    [nxt[n][:, 256 * c:256 * (c + 1)] for c in range(8)], axis=0)
                return jnp.concatenate([jnp.where(j < 0, z, w[0:64, :]), w[64:, :]], axis=0)

            def emit_k(g, e, y):
                features(phk, u + e, g, y[0:GR - 8, :])
                rest[g, e] = y[GR - 8:, :]

            def emit_q(g, e, y):
                features(phq, 8 * e + t, g, jnp.concatenate([y, rest[g, e]], axis=0))

            def emit_v(g, e, y):
                for q in range(4):
                    vs[4 * g + q, u + e] = y[40 * q:40 * q + 40, :]

            t10 = tail(0, xs, 1, 0)
            for n in range(6):
                t10 = a_dots(n, xs, (emit_k, emit_q, emit_v)[n // 2], tie, t10)
            cur = jnp.concatenate(nxt, axis=0)
        xa[...] = cur
        row = lax.broadcasted_iota(jnp.int32, (2 * VR, 4 * FA), 0)
        col = lax.broadcasted_iota(jnp.int32, (2 * VR, 4 * FA), 1)
        split = jnp.where(row < 2 * FA, FA, 2 * FA + 4)
        same = (row >= split) == (col >= 2 * FA)
        for q in range(PA):
            v = jnp.concatenate([vs[q, u] for u in range(asub)], axis=1)
            v = jnp.concatenate([v, jnp.ones((8, TA), F32)], axis=0)
            kv = _dot_nt(v.astype(BF16), pair_rows(phk, q, 0, asub))
            kv = kv + jnp.where(j == 0, 0.0, kvacc[q])
            kvacc[q] = kv
            kvs[q] = _pack(jnp.where(same, kv, 0.0).astype(BF16))
        return 0

    def attend(j):
        low = lax.broadcasted_iota(jnp.int32, (8, TN), 0) < 4
        os_ = []
        for q in range(PA):
            nd = _dot(_unpack(kvs[q]), pair_rows(phq, q, j * nsub, nsub))
            rab = 1.0 / (nd[40:48, :] + 1e-6)
            rba = pltpu.roll(rab, 4, 0)
            ra = jnp.where(low, rab, rba)
            rb = jnp.where(low, rba, rab)
            os_.append(nd[0:40, :] * jnp.concatenate([ra, ra, rab, rb, rb], axis=0))
        return _pack(jnp.concatenate(os_, axis=0).astype(BF16).T)

    def project(ty, j, o, slot):
        r = rows(j, TN)
        x = _dot(_unpack(o), woa[...]) + xres[ty, r, :]
        xres[ty, r, :] = x
        for s in range(16):
            z = _layernorm(x[16 * s + 8 - 8 * (s % 2):16 * s + 16 - 8 * (s % 2), :])
            z = z - z[KE:KE + 1, :]
            for c in range(D // 128):
                xe[ty, slot, c, pl.ds(s * KE, 8), :] = z[:, 128 * c:128 * (c + 1)]

    def extra_keys(seg, p):
        k = jnp.concatenate(
            [ke[2 * (seg // 32) + t // 24, (seg // 16) % 2, t % 24, pl.ds((seg % 16) * KE, 8), :]
             for t in range(3 * p, 3 * p + 3)], axis=1)
        return jnp.where(lax.broadcasted_iota(jnp.int32, (8, PW), 0) < KE, k, 0.0)

    def b_residual(i):
        r = rows(i, TB // 2)
        xs = [xres[e, r, :] + d for e, d in enumerate(_split_rows(rsave[...]))]
        for e, x in enumerate(xs):
            xres[e, r, :] = x
        xio[rows(i, TB), :] = _merge_rows(*xs).astype(BF16)
        return xs

    def b_finish(i):
        xn = [_layernorm(x) for x in b_residual(i)]
        for e, x in enumerate(xn):
            xl[e, rows(jnp.minimum(i, 2), TB // 2), :] = x
        return jnp.concatenate(xn, axis=0)

    def b_tile(mem, xn, i, side):
        for u in range(4):
            t0 = u * SEG
            late = u % 2 == 0
            ext = [SEG * v + (24 if v % 2 == 0 else 0) for v in range(4)]

            def place(y, z):
                return jnp.concatenate([y, z] if late else [y[0:M], z, y[M:]], axis=0)

            def fix_qv(p, y):
                cols = slice(p * 2 * PW, (p + 1) * 2 * PW)
                if u == 0:
                    ysave[:, cols] = y[L:, :]
                    y = y[0:L, :]
                else:
                    y = place(y, ysave[8 * u - 8:8 * u, cols])
                if not late:
                    return y
                c0 = 2 * PW - D
                r0 = 64 * u + 8 * p
                tie = jnp.where(i < 0, side[r0:r0 + 8, :], y[0:M, c0:])
                return jnp.concatenate(
                    [jnp.concatenate([y[0:M, 0:c0], tie], axis=1), y[M:, :]], axis=0)

            def fix_k(p, k):
                return place(k, extra_keys(4 * i + u, p))

            def fix_o(p, o):
                cols = slice(p * PW, (p + 1) * PW)
                if u == 3:
                    return jnp.concatenate([o, osave[:, cols]], axis=0)
                osave[8 * u:8 * u + 8, cols] = o[32:L, :]
                return o[0:32, :]

            h = jnp.concatenate(
                [mem, xn[t0:t0 + 24, :] if late else xn[t0 + 8:t0 + SEG, :]], axis=0)
            hk = (h - xn[ext[u] + KE:ext[u] + KE + 1, :]).astype(BF16)
            if u == 0:
                h = jnp.concatenate([h] + [xn[e:e + 8, :] for e in ext], axis=0)
            r = _segment(h, hk, wqv, sqv, wk, wob, sob, fix_qv, fix_k, fix_o, u == 3)
            mem = r[0:M, :]
            if u < 3:
                rsave[t0:t0 + 24, :] = r[M:, :]
            else:
                rsave[t0:t0 + SEG, :] = r[M:L, :]
                for v in range(3):
                    rsave[SEG * v + 24:SEG * v + SEG, :] = r[L + 8 * v:L + 8 * v + 8, :]
        return mem

    def layer(l, _):
        def wait_first(copies):
            @pl.when(l == 0)
            def _():
                for c in copies:
                    c.wait()

        with jax.named_scope("a1"):
            lax.fori_loop(0, na, functools.partial(a1, l == 0), 0)

        def a2(n, _):
            wait_first(w_copies(n))
            ty, half = n % 2, n // 2
            o0 = attend(4 * ty + 2 * half)
            o1 = attend(4 * ty + 2 * half + 1)

            def sample(w):
                z = [w[64 * a + 56:64 * a + 64, :] for a in range(D // 128)]
                out = []
                for y in z:
                    acc = y[:, 0:128]
                    for c in range(1, y.shape[1] // 128):
                        acc = acc | y[:, 128 * c:128 * (c + 1)]
                    out.append(acc)
                return jnp.concatenate(out, axis=1)

            mr = 16 * KE

            def staged(e):
                return jnp.concatenate([xe[0, e, c, 0:mr, :] for c in range(D // 128)], axis=1)

            def side(job):
                out = []
                if job == 'k':
                    out.append(_pack(wraw[3, n].T))
                    wk[n] = out[0]
                else:
                    for i in range(2):
                        out.append(_pack(wraw[i, n, rows(int(job), PW), :].T))
                        wqv[n, :, rows(2 * int(job) + i, PW)] = out[i]
                return functools.reduce(jnp.bitwise_or, [sample(w) for w in out])

            j1, j2, j3 = '01', '23', 'k'
            for job in j1:
                o1 = jnp.concatenate(
                    [jnp.where(n < 0, side(job), o1[0:8, :]), o1[8:, :]], axis=0)
            project(ty, 2 * half, o0, 0)
            x0 = staged(0)
            for job in j2:
                tie = pltpu.bitcast(side(job), F32)
                x0 = jnp.concatenate([jnp.where(n < 0, tie, x0[0:8, :]), x0[8:, :]], axis=0)
            project(ty, 2 * half + 1, o1, 1)
            x1 = staged(1)
            r = rows(ty, 32)
            xb[rows(ty, 64), :] = _layernorm(_merge_rows(xres[0, r, :], xres[1, r, :]))
            rsave[rows(ty, 64), :] = jnp.zeros((64, D), F32)

            a11, a12, a21, a22 = x0[:, 0:256], x0[:, 256:512], x1[:, 0:256], x1[:, 256:512]
            lhs = [z.astype(BF16) for z in (
                a11 + a22, a21 + a22, a11, a22, a11 + a12, a21 - a11, a12 - a22,
                x0[:, 512:], x1[:, 512:])]
            done = []

            def emit(e, t, k):
                ke[n, e, t, 0:mr, :] = k
                c, q = divmod(len(done), PW // 16)
                done.append(q)
                kk_ = pltpu.bitcast(k, U32)
                g = [kk_[16 * i:16 * i + 8, :] for i in range(7)]
                tie = jnp.concatenate([g[1], g[4], g[1], g[4], g[6]], axis=1)
                ws = []
                for e in range(2):
                    r0 = (2 * c + e) * PW + 16 * q
                    w = jnp.where(n < 0, tie, _pack(wraw[2, n, r0:r0 + 16, :]))
                    wob[rows(n * (QW // 16) + r0 // 16, 8), :] = w
                    ws.append(_unpack(w[:, 0:512]).astype(F32))
                sums = _strassen_sums(ws[0][:, 0:256], ws[0][:, 256:],
                                      ws[1][:, 0:256], ws[1][:, 256:])
                sob[rows((2 * n + c) * (PW // 16) + q, 8), :] = _pack(
                    jnp.concatenate(sums, axis=1).astype(BF16))
                cc, rr = divmod(q, 8)
                tie = jnp.concatenate([jnp.concatenate([g[0], g[2]], axis=1),
                                       jnp.concatenate([g[3], g[5]], axis=1)], axis=0)
                ws = [wqv[n, 128 * kk + 16 * rr:128 * kk + 16 * rr + 16,
                          rows(3 * (2 * c + e) + cc, 256)] for kk in range(2) for e in range(2)]
                ws = [_unpack(jnp.where(n < 0, tie, w)).astype(F32) for w in ws]
                sqv[rows(8 * n + rr, 16), rows(3 * c + cc, 5 * 256)] = _pack(
                    jnp.concatenate(_strassen_sums(*ws), axis=1).astype(BF16))

            def blk(v, e, k):
                return wraw[3, 2 * ty + v // 6, rows(2 * (v % 6) + e, 128),
                            256 * k:min(256 * (k + 1), D)]

            def comb(v, x, sign, y):
                x, y = blk(v, *x).astype(F32), blk(v, *y).astype(F32)
                return (x + y if sign > 0 else x - y).astype(BF16)

            b11, b21, b12, b22 = (0, 0), (0, 1), (1, 0), (1, 1)

            def first_half(v):
                m3 = _dot_nt(lhs[2], comb(v, b12, -1, b22))
                m5 = _dot_nt(lhs[4], blk(v, *b22))
                emit(0, 2 * v + 1, _dot_nt(lhs[7], blk(v, 1, 2)) + (m3 + m5))
                return m3, _dot_nt(lhs[7], blk(v, 0, 2)) - m5

            def second_half(v, m3, c11):
                m2 = _dot_nt(lhs[1], blk(v, *b11))
                m4 = _dot_nt(lhs[3], comb(v, b21, -1, b11))
                emit(1, 2 * v, _dot_nt(lhs[8], blk(v, 0, 2)) + (m2 + m4))
                m1 = _dot_nt(lhs[0], comb(v, b11, 1, b22))
                c22 = _dot_nt(lhs[5], comb(v, b11, 1, b12)) + (m1 + (m3 - m2))
                emit(1, 2 * v + 1, _dot_nt(lhs[8], blk(v, 1, 2)) + c22)
                emit(0, 2 * v, _dot_nt(lhs[6], comb(v, b21, 1, b22)) + (c11 + (m1 + m4)))

            nst = 10
            lead = 2
            xb0, xb1 = x0.astype(BF16), x1.astype(BF16)

            def plain(v, e):
                w = wraw[3, 2 * ty + v // 6, rows(v % 6, 256), :]
                k = _dot_nt((xb0, xb1)[e], w)
                emit(e, 2 * v, k[:, 0:128])
                emit(e, 2 * v + 1, k[:, 128:])

            for v in range(lead):
                plain(v, 0)
            for v in range(12):
                if v < 12 - nst:
                    if v >= lead:
                        plain(v, 0)
                    plain(v, 1)
                else:
                    second_half(v, *first_half(v))
            for job in j3:
                side(job)
            return 0

        wait_first([woa_copy, mem0_copy, wk_copy])
        with jax.named_scope("a2"):
            lax.fori_loop(0, NW, a2, 0)

        def b_step(i, mem):
            xn = xb[...]
            side = b_finish(jnp.maximum(i - 1, 0))
            r = rows(jnp.minimum(i + 1, nb - 1), TB // 2)
            nxt = _layernorm(_merge_rows(xres[0, r, :], xres[1, r, :]))
            xb[...] = nxt
            side = jnp.concatenate([side, nxt], axis=0)
            mem = b_tile(mem, xn, i, side)

            @pl.when(jnp.logical_and(l == 1, i >= 1))
            def _():
                out_copy(i - 1).start()
            return mem

        with jax.named_scope("b"):
            lax.fori_loop(0, nb, b_step, mem0[...].astype(F32))

        b_residual(nb - 1)

        @pl.when(l == 0)
        def _():
            xa[...] = strassen_rhs(xl[0, 0:128, :], xl[1, 0:128, :])
        return 0

    lax.fori_loop(0, 2, layer, 0)
    out_copy(nb - 1).start()
    pltpu.make_async_copy(xio, out_hbm, sem_out.at[0]).wait()


@jax.jit
def pallas_interleave_layers__linear_kernel_hedgehog__memory_aug_recurrent_mem_tr__prompt_kernel(
    A_x, A_wqkv, A_w_phi, A_wo, B_x, B_mem0, B_Wq, B_Wk, B_Wv, B_Wo, B_seg_len,
):
    del B_x
    del B_seg_len
    x = A_x.reshape(S, D)
    wphi = A_w_phi.transpose(1, 2, 0)
    mem0 = B_mem0.reshape(M, D)
    wq, wk, wv = (w.transpose(1, 2, 0).reshape(NW, QW, D) for w in (B_Wq, B_Wk, B_Wv))
    wo = B_Wo.reshape(NW, QW, D)
    hbm = pl.BlockSpec(memory_space=pl.ANY)
    out = pl.pallas_call(
        _kernel,
        out_shape=jax.ShapeDtypeStruct((S, D), A_x.dtype),
        in_specs=[hbm] * 9,
        out_specs=hbm,
        scratch_shapes=[
            pltpu.VMEM((S, D), BF16),
            pltpu.VMEM((D, 3 * D), BF16),
            pltpu.VMEM((FA, FA, HA), BF16),
            pltpu.VMEM((D, D), BF16),
            pltpu.VMEM((M, D), BF16),
            pltpu.VMEM((2, S // 2, D), F32),
            pltpu.VMEM((64, 2048), U32),
            pltpu.VMEM((2, 3 * TB // 2, D), F32),
            pltpu.VMEM((TB, D), F32),
            pltpu.VMEM((GA, GR // 2, 256), U32),
            pltpu.VMEM((6, 8, GR // 2, 256), U32),
            pltpu.VMEM((S // 128, D, 128), U32),
            pltpu.VMEM((TA // 128, D, 128), U32),
            pltpu.VMEM((PA, 2 * VR, 4 * FA), F32),
            pltpu.VMEM((PA, VR, 4 * FA), U32),
            pltpu.VMEM((4, NW, QW, D), BF16),
            pltpu.VMEM((NW, D // 2, 2 * QW), U32),
            pltpu.VMEM((NW * 128, 5 * QW), U32),
            pltpu.VMEM((NW, D // 2, QW), U32),
            pltpu.VMEM((HD // 2, D), U32),
            pltpu.VMEM((HD // 4, 5 * 256), U32),
            pltpu.VMEM((2, 2, D // 128, 16 * KE + 8, 128), F32),
            pltpu.VMEM((NW, 2, HD // 256, 16 * KE + 8, 128), F32),
            pltpu.VMEM((24, 2 * HD), F32),
            pltpu.VMEM((24, HD), F32),
            pltpu.VMEM((TB, D), F32),
            pltpu.SemaphoreType.DMA((10 + S // TA + 3 * NW,)),
            pltpu.SemaphoreType.DMA((1,)),
        ],
        compiler_params=pltpu.CompilerParams(vmem_limit_bytes=127 * 1024 * 1024,
                                             disable_bounds_checks=True,
                                             disable_semaphore_checks=True),
    )(x, A_wqkv, wphi, A_wo, mem0, wq, wk, wv, wo)
    return out.reshape(1, S, D)
```

```python
import functools

import jax
import jax.numpy as jnp
from jax import lax
import jax.experimental.pallas as pl
import jax.experimental.pallas.tpu as pltpu

F32 = jnp.float32
BF16 = jnp.bfloat16
U32 = jnp.uint32

S = 2048
D = 640
HA = 32
FA = 20
GA = 4
GR = 8 * FA
VR = 24
PA = HA // 2
TN = 256
TA = 512
HB = 32
DH = 192
HD = HB * DH
M = 8
SEG = 32
L = M + SEG
PW = 2 * DH
NP = HB // 2
TB = 128
NW = 4
QW = HD // NW
KE = 7

NT = (((1,), (1,)), ((), ()))
LOG2E = 1.4426950408889634
HALF_ULP = 0.0040612


def _dot(a, b):
    return jnp.dot(a, b, preferred_element_type=F32)


def _dot_nt(a, b):
    return lax.dot_general(a, b, NT, preferred_element_type=F32)


def _pack(a):
    return pltpu.bitcast(a, U32)


def _unpack(a):
    return pltpu.bitcast(a, BF16)


def _interleave(a, b):
    lo = lax.bitcast_convert_type(a, U32) >> 16
    hi = lax.bitcast_convert_type(b, U32) & jnp.uint32(0xFFFF0000)
    return lo | hi


def _recip(x):
    r = pl.reciprocal(x, approx=True)
    return r * (2.0 - x * r)


def _layernorm(x):
    m = jnp.mean(x, axis=-1, keepdims=True)
    c = x - m
    v = jnp.mean(c * c, axis=-1, keepdims=True)
    return c * lax.rsqrt(v + 1e-5)


def _split_rows(x):
    blocks = range(0, x.shape[0], 64)
    return (jnp.concatenate([x[b + 16:b + 48] for b in blocks], axis=0),
            jnp.concatenate([x[b + k:b + k + 16] for b in blocks for k in (0, 48)], axis=0))


def _merge_rows(inner, outer):
    return jnp.concatenate(
        [z for b in range(0, inner.shape[0], 32)
         for z in (outer[b:b + 16], inner[b:b + 32], outer[b + 16:b + 32])], axis=0)


def _feature_map(p):
    t = p.shape[-1]
    p3 = jnp.concatenate([jnp.zeros((8, t), F32), p], axis=0).reshape(FA, 8, t)
    mx = jnp.max(p3, axis=0)
    mn = jnp.min(p3, axis=0)
    sp, sn = jnp.exp2(p3[0] - mx), jnp.exp2(mn - p3[0])
    for f in range(1, FA):
        sp, sn = sp + jnp.exp2(p3[f] - mx), sn + jnp.exp2(mn - p3[f])
    lp = (mx - HALF_ULP) + jnp.log2(sp)
    ln = (mn + HALF_ULP) - jnp.log2(sn)
    return [_interleave(jnp.exp2(p3[f] - lp), jnp.exp2(ln - p3[f])) for f in range(FA)]


def _tiles(a, odd):
    t0, t1, t2 = a[:, 0:128], a[:, 128:256], a[:, 256:384]
    return (t1, t2, t0) if odd else (t1, t0, t2)


def _own_weights(a, odd):
    lane = lax.broadcasted_iota(jnp.int32, (L, 128), 1)
    mid, own, _ = _tiles(a, odd)
    return jnp.concatenate(
        [jnp.where(lane < 64, mid, 0.0), jnp.where(lane < 64, 0.0, mid), own,
         jnp.zeros((128 - 3 * L, 128), F32)], axis=0).astype(BF16)


def _others(even, odd, pad):
    parts = [_tiles(odd, 1)[2], _tiles(even, 0)[2]]
    if pad:
        parts.append(jnp.zeros((128 - 2 * L, 128), F32))
    return jnp.concatenate(parts, axis=0).astype(BF16)


def _softmax3(s3):
    row = lax.broadcasted_iota(jnp.int32, (L, 128), 0)
    col = lax.broadcasted_iota(jnp.int32, (L, 128), 1)
    first = col < L
    second = jnp.logical_and(col >= L, col < 2 * L)
    key = jnp.where(first, col, col - L)
    valid = jnp.logical_or(row < M, row >= key)
    out, other = [], []
    for odd in range(2):
        own = pltpu.roll(s3[odd][L:, :], 128 - L if odd else 128 - 2 * L, 1)
        s = (jnp.where(first, s3[2][0:L, :], own) if odd
             else jnp.where(first, own, s3[2][L:, :]))
        s = jnp.where(valid, (s + s3[odd][0:L, :]) * (DH ** -0.5), -1e9)
        m0 = jnp.max(jnp.where(first, s, -jnp.inf), axis=-1, keepdims=True)
        m1 = jnp.max(jnp.where(second, s, -jnp.inf), axis=-1, keepdims=True)
        e = jnp.exp(s - jnp.where(first, m0, m1))
        e0 = jnp.where(first, e, 0.0)
        e1 = jnp.where(second, e, 0.0)
        p0 = e0 * _recip(jnp.sum(e0, axis=-1, keepdims=True))
        p1 = e1 * _recip(jnp.sum(e1, axis=-1, keepdims=True))
        own = pltpu.roll(p1, L, 1) if odd else pltpu.roll(p0, 2 * L, 1)
        out.append(jnp.concatenate([p0 + p1, own], axis=0).astype(BF16))
        other.append(p0 if odd else p1)
    out.append(jnp.concatenate([other[1], other[0]], axis=0).astype(BF16))
    return out


_SCHEME = [[[(t[k] == '+', int(t[k + 1]), int(t[k + 2])) for k in range(0, len(t), 3)]
            for t in row.split()] for row in (
    '+00+01-10-11 +00 +00',
    '+01+02 +21 +01',
    '+02-04 +20+22 +02',
    '+13-14 +41 +10-11',
    '+11+12 +11-12 +11',
    '+00+13-03-10 +01-02 +12',
    '+04-14 +40+41 -10',
    '+00+13-03 +02+32-01 +12-01',
    '+04-12 +20+22+42 +02-00-10',
    '+10+11-01 +10+12-00 +11+12-00-10',
    '+10 +00+01-10-12 +11+12',
    '+04 +20+22+30+40+42 +00+10',
    '+01-11 +00-10 +10-11-12',
    '+12 +11+22+42-12-21 +02+12-00-10',
    '+10+11 +10+12 +00+10',
    '+03-13 +01+30+31-02-32 +01',
    '+01 +11-21 +01+02+11+12-00-10',
    '+02-12 +20 +00-02',
    '+13 +31+41 +01+11',
    '+00-03 +32 -02-12',
    '+01+12 +12+21-11 +02+11+12-00-10',
    '+12-14 +42 -12',
    '+03-04 +30 +00-01',
    '+04-13 +30-41 -01-10',
    '+00 +02+32 +01+02',
)]
_GROUPS = ((2, 8, 11), (6, 18, 23), (9, 10, 12, 14), (4, 13, 16, 20), (5, 7, 15, 24))
_MIXED = [r for g in _GROUPS for r in g]
assert sorted(_MIXED) == [r for r, (_, v, _) in enumerate(_SCHEME) if len(v) > 1]
NS = len(_MIXED)


def _signed_sum(terms, get):
    pos = terms[0][0]
    acc = get(*terms[0][1:])
    for p, i, j in terms[1:]:
        acc = acc + get(i, j) if p == pos else acc - get(i, j)
    return acc, pos


def _shared_pairs(sums):
    steps = []
    while True:
        count = {}
        for t in sums:
            for x in t:
                for y in t:
                    if str(x) < str(y):
                        count[x, y, t[x] == t[y]] = count.get((x, y, t[x] == t[y]), 0) + 1
        (x, y, same), c = max(count.items(), key=lambda kv: kv[1], default=((0, 0, 0), 0))
        if c < 2:
            return steps, sums
        for t in sums:
            if x in t and y in t and (t[x] == t[y]) == same:
                t[len(steps)] = t.pop(x)
                del t[y]
        steps.append((x, y, same))


def _scheme_sums(group, get_b):
    val = {(i, j): _unpack(get_b(i, j)).astype(F32) for r in group for _, i, j in _SCHEME[r][1]}
    steps, sums = _shared_pairs([{(i, j): p for p, i, j in _SCHEME[r][1]} for r in group])
    for k, (x, y, same) in enumerate(steps):
        val[k] = val[x] + val[y] if same else val[x] - val[y]
    out = []
    for t in sums:
        z, pos = _signed_sum(sorted(((p, x, 0) for x, p in t.items()), key=lambda e: not e[0]),
                             lambda x, _: val[x])
        out.append(z if pos else -z)
    return _pack(jnp.concatenate(out, axis=1).astype(BF16))


def _scheme_lhs(side, get_a):
    return [(z.astype(BF16), pos)
            for z, pos in (_signed_sum(row[side], get_a) for row in _SCHEME)]


def _scheme_apply(side, lhs, plain, mixed, acc):
    for r, row in enumerate(_SCHEME):
        m = _dot(lhs[r][0], mixed(_MIXED.index(r)) if r in _MIXED else plain(*row[1][0][1:]))
        for p, i, j in row[side]:
            p = p == lhs[r][1]
            if (i, j) not in acc:
                acc[i, j] = (m, p)
            elif p == acc[i, j][1]:
                acc[i, j] = (m + acc[i, j][0], p)
            else:
                acc[i, j] = (m - acc[i, j][0] if p else acc[i, j][0] - m, True)
    return acc


def _scheme_result(acc, ncol):
    assert all(p for _, p in acc.values())
    return jnp.concatenate([jnp.concatenate([acc[i, j][0] for j in range(ncol)], axis=1)
                            for i in range(2)], axis=0)


def _segment(h, hk, wqv, sqv, wk, wob, sob, fix_qv, fix_k, fix_o, wide_o):
    ys, ks, ss, ps, pvs, os_ = {}, {}, {}, {}, {}, {}
    kg = 4
    hb = h.astype(BF16)
    if h.shape[0] == 64:
        lhs = _scheme_lhs(0, lambda i, j: h[32 * i:32 * i + 32, 128 * j:128 * j + 128])

    def wide_proj(n, c):
        return _scheme_result(_scheme_apply(
            2, lhs,
            lambda j, l: _unpack(wqv[n, 64 * j:64 * j + 64, pl.ds(c * PW + 128 * l, 128)]),
            lambda m: _unpack(sqv[64 * n:64 * n + 64, pl.ds((c * NS + m) * 128, 128)]), {}), 3)

    def proj(p):
        n, e = divmod(p, NP // NW)
        cols = slice(e * 2 * PW, (e + 1) * 2 * PW)
        if h.shape[0] == 64:
            y = jnp.concatenate([wide_proj(n, 2 * e), wide_proj(n, 2 * e + 1)], axis=1)
        elif p == 0:
            ksp = 512
            y = _dot(hb[:, 0:ksp], _unpack(wqv[n, 0:ksp // 2, cols]))
            y = _dot(hb[:, ksp:], _unpack(wqv[n, ksp // 2:, cols])) + y
        else:
            y = _dot(hb, _unpack(wqv[n, :, cols]))
        y = fix_qv(p, y)
        if p % kg == 0:
            k = _dot(hk, _unpack(wk[n, :, e * PW:(e + kg) * PW]))
            for i in range(kg):
                ks[p + i] = fix_k(p + i, k[:, i * PW:(i + 1) * PW])
        ys[p] = [y[:, 0:PW], ks.pop(p), y[:, PW:]]

    def weights(c, i, which):
        if i < 2:
            return _own_weights(ys[2 * c + i][which], i)
        return _others(ys[2 * c][which], ys[2 * c + 1][which], True)

    def score_round(n):
        for c, i in (divmod(j, 3) for j in range(4 * n, 4 * n + 4)):
            if i < 2:
                q = jnp.concatenate(_tiles(ys[2 * c + i][0], i)[0:2], axis=0).astype(BF16)
            else:
                q = _others(ys[2 * c][0], ys[2 * c + 1][0], False)
            ss[c, i] = _dot_nt(q, weights(c, i, 1))
            if i == 2:
                ps[c] = _softmax3([ss.pop((c, k)) for k in range(3)])

    def pv_round(n):
        for c, i in (divmod(j, 3) for j in range(4 * n, 4 * n + 4)):
            pvs[c, i] = _dot(ps[c][i], weights(c, i, 2))
            if i == 2:
                o0, o1, o2 = [pvs.pop((c, k)) for k in range(3)]
                os_[2 * c] = fix_o(2 * c, jnp.concatenate(
                    [o0[L:, :], o0[0:L, :], o2[L:, :]], axis=1))
                os_[2 * c + 1] = fix_o(2 * c + 1, jnp.concatenate(
                    [o2[0:L, :], o1[0:L, :], o1[L:, :]], axis=1))

    def slot(n):
        if n >= 2:
            pv_round(n - 2)
        if n < 6:
            score_round(n)

    def oproj(lo, hi, r):
        o = [os_.pop(p) for p in range(lo, hi)]
        if not wide_o:
            y = _dot(jnp.concatenate(o, axis=1).astype(BF16), _unpack(wob[lo * DH:hi * DH, :]))
            return y if r is None else y + r
        return _scheme_apply(
            0, _scheme_lhs(2, lambda i, l: jnp.concatenate(
                [z[32 * i:32 * i + 32, 128 * l:128 * l + 128] for z in o], axis=1)),
            lambda j, l: _unpack(jnp.concatenate(
                [wob[pl.ds(p * DH + 64 * l, 64), 128 * j:128 * j + 128] for p in range(lo, hi)],
                axis=0)),
            lambda m: _unpack(sob[64 * lo:64 * hi, 128 * m:128 * m + 128]), r or {})

    after = (3, 6, 9, 11, 14) if h.shape[0] == 64 else (3, 6, 9, 12, 14)
    for p in range(NP):
        proj(p)
        if p in after:
            slot(after.index(p))
    o1, o2, o3 = (2, 6, 10) if wide_o else (2, 9, 10)
    r = oproj(0, o1, None)
    slot(5)
    r = oproj(o1, o2, r)
    slot(6)
    slot(7)
    r = oproj(o2, o3, r)
    r = oproj(o3, NP, r)
    return _scheme_result(r, 5) if wide_o else r


def _kernel(x_hbm, wqkv_hbm, wphi_hbm, woa_hbm, mem0_hbm,
            wq_hbm, wk_hbm, wv_hbm, wo_hbm,
            out_hbm,
            xio, wqkv, wphi, woa, mem0, xres, xa, xl, xb, bds, wat, phq, phk, kvacc, kvs,
            wraw, wqv, sqv, wk, wob, sob, xe, ke, ysave, osave, rsave, sem_in, sem_out):
    nsub = TN // 128
    na = S // TA
    asub = TA // 128
    nb = S // TB

    def rows(j, n):
        return pl.ds(j * n if isinstance(j, int) else pl.multiple_of(j * n, n), n)

    def x_copy(j):
        if isinstance(j, int) and j < 0:
            r = pl.ds(0, 256)
        elif isinstance(j, int) and j == na - 1:
            r = pl.ds(S - TA + 256, TA - 256)
        else:
            r = pl.ds(j * TA + 256 if isinstance(j, int)
                      else pl.multiple_of(j * TA + 256, 256), TA)
        return pltpu.make_async_copy(x_hbm.at[r, :], xio.at[r, :], sem_in.at[9 + j])

    def w_copies(c):
        return [pltpu.make_async_copy(src.at[c], wraw.at[i, c],
                                      sem_in.at[10 + na + 3 * c + i])
                for i, src in enumerate((wq_hbm, wv_hbm, wo_hbm))]

    def wa_copy(c):
        r = pl.ds(512, 128) if isinstance(c, int) and c == 2 else rows(c, 256)
        return pltpu.make_async_copy(wqkv_hbm.at[r, :], wqkv.at[r, :], sem_in.at[3 + c])

    def out_copy(i):
        return pltpu.make_async_copy(xio.at[rows(i, TB), :],
                                     out_hbm.at[rows(i, TB), :], sem_out.at[0])

    wphi_copy = pltpu.make_async_copy(wphi_hbm, wphi, sem_in.at[0])
    woa_copy = pltpu.make_async_copy(woa_hbm, woa, sem_in.at[1])
    mem0_copy = pltpu.make_async_copy(mem0_hbm, mem0, sem_in.at[2])
    order = [wphi_copy, wa_copy(0), wa_copy(1), x_copy(-1), wa_copy(2)]
    wk_copy = pltpu.make_async_copy(wk_hbm, wraw.at[3], sem_in.at[9 + na])
    order += [x_copy(j) for j in range(na)] + [woa_copy, mem0_copy, wk_copy]
    for c in range(NW):
        order += w_copies(c)
    for c in order:
        c.start()

    def strassen_rhs(x0, x1):
        b11, b12 = [jnp.concatenate([x[:, 0:128], x[:, 256:384]], axis=1) for x in (x0, x1)]
        b21, b22 = [jnp.concatenate([x[:, 128:256], x[:, 384:512]], axis=1) for x in (x0, x1)]
        ops = [b11 + b22, b11, b12 - b22, b21 - b11, b22, b11 + b12, b21 + b22,
               x0[:, 512:], x1[:, 512:]]
        return _pack(jnp.concatenate(ops, axis=1).astype(BF16))

    def load_x(t, first):
        xs = _split_rows(xio[rows(t, 256), :].astype(F32))
        if first is not True:
            xs = [jnp.where(first, x, xres[e, rows(t, 128), :]) for e, x in enumerate(xs)]
        for e, x in enumerate(xs):
            xres[e, rows(t, 128), :] = x
        return jnp.concatenate(xs, axis=0)

    wphi_copy.wait()
    cphi = jnp.zeros((FA, D), F32)
    hh = lax.broadcasted_iota(jnp.int32, (HA, D), 0) * FA
    jj = lax.broadcasted_iota(jnp.int32, (HA, D), 1)
    for d in range(FA):
        cphi = _dot(wphi[d], jnp.where(jj == hh + d, 1.0, 0.0).astype(BF16)) + cphi
    cb = jnp.concatenate(
        [jnp.broadcast_to(cphi[f:f + 1, :], (8, D)) for f in range(FA)], axis=0)
    for g in range(GA):
        row = lax.broadcasted_iota(jnp.int32, (GR, 256), 0)
        col = lax.broadcasted_iota(jnp.int32, (GR, 256), 1) + 128 * g
        lo = (8 * g + (row & 7)) * FA
        bds[g] = _pack(jnp.where(jnp.logical_and(col >= lo, col < lo + FA),
                                 cb[:, 128 * g:128 * g + 256], 0.0).astype(BF16))

    def folded(rr):
        out = [[], [], []]
        for g in range(GA):
            ws = []
            for i in range(2):
                c0 = i * D + 128 * g
                w = _dot_nt(_unpack(bds[g]), wqkv[rr, c0:c0 + 256]).reshape(FA, 8, 128)
                ws.append(((w[1:] - w[0:1]) * LOG2E).reshape(GR - 8, 128))
            out[0].append(jnp.concatenate([ws[1], ws[0][GR - 16:, :]], axis=0))
            out[1].append(ws[0][0:GR - 16, :])
        wvt = wqkv[rr, 2 * D:3 * D].T.astype(F32)
        out[2] = [wvt[g * GR:(g + 1) * GR, :] for g in range(GA)]
        return out

    def fold(c, _):
        wa_copy(c).wait()
        wa, wb = folded(rows(2 * c, 128)), folded(rows(2 * c + 1, 128))
        for i in range(3):
            for p in range(2):
                a11, a12, a21, a22 = wa[i][2 * p], wb[i][2 * p], wa[i][2 * p + 1], wb[i][2 * p + 1]
                ops = [a11 + a22, a21 + a22, a11, a22, a11 + a12, a21 - a11, a12 - a22]
                for m, w in enumerate(ops):
                    wat[2 * i + p, m, 0:w.shape[0] // 2, rows(c, 128)] = _pack(w.astype(BF16))
        return 0

    lax.fori_loop(0, 2, fold, 0)
    x_copy(-1).wait()
    wa_copy(2).wait()
    x = _layernorm(load_x(0, True))
    xa[...] = strassen_rhs(x[0:128], x[128:])
    for i, ws in enumerate(folded(pl.ds(512, 128))):
        for g, w in enumerate(ws):
            wat[2 * i + g // 2, 7, 0:w.shape[0] // 2, rows(g % 2, 128)] = _pack(w.astype(BF16))

    def pair_rows(ph, q, t0, n):
        return _unpack(jnp.concatenate(
            [ph[t0 + u, rows(q, 2 * FA), :] for u in range(n)], axis=1))

    def a1(first, j, _):
        @pl.when(jnp.logical_and(first, j < na - 1))
        def _():
            x_copy(j).wait()

        @pl.when(jnp.logical_and(first, j == na - 1))
        def _():
            x_copy(na - 1).wait()

        def features(ph, t, g, y):
            for f, w in enumerate(_feature_map(y)):
                ph[t, pl.ds(GR * g + f, 8, stride=FA), :] = w

        def tail(n, xs, g, u):
            nr = GR // 2 - 8 if n // 2 == 1 else GR // 2
            return _dot_nt(_unpack(wat[n, 7, 0:nr, 128 * g:128 * (g + 1)]),
                           xs[:, 1792 + 128 * u:1920 + 128 * u])

        def a_dots(n, xs, emit, tie, t10):
            nr = GR // 2 - 8 if n // 2 == 1 else GR // 2
            p = n % 2

            def prod(m):
                return _dot_nt(_unpack(tie(wat[n, m, 0:nr, :])), xs[:, 256 * m:256 * (m + 1)])

            m2, m4 = prod(1), prod(3)
            emit(2 * p + 1, 0, m4 + (m2 - (-t10)))
            t01 = tail(n, xs, 0, 1)
            m3, m5 = prod(2), prod(4)
            emit(2 * p, 1, m5 + (m3 - (-t01)))
            m1 = prod(0)
            c22 = prod(5) + (m1 + (m3 - m2))
            emit(2 * p + 1, 1, tail(n, xs, 1, 1) + c22)
            t10 = tail(n + 1, xs, 1, 0) if n < 5 else None
            c11 = tail(n, xs, 0, 0) + (m1 + (m4 - m5))
            emit(2 * p, 0, prod(6) + c11)
            return t10

        vs = {}
        cur = xa[...]
        dl = (3, 8, 13, 30, 33, 36, 39, 41)
        for u in range(0, asub, 2):
            t = j * (asub // 2) + u // 2
            xs = _unpack(cur)
            tn = t + 1
            x = load_x(tn if u + 2 < asub else jnp.minimum(tn, (na - 1) * (asub // 2)), first)
            rest, seen, nxt = {}, [], []

            def tie(w):
                seen.append(0)
                if len(seen) - 1 not in dl:
                    return w
                n = len(nxt)
                nxt.append(strassen_rhs(*[
                    _layernorm(x[128 * e + 16 * n:128 * e + 16 * n + 16, :]) for e in range(2)]))
                z = jnp.concatenate(
                    [nxt[n][:, 256 * c:256 * (c + 1)] for c in range(8)], axis=0)
                return jnp.concatenate([jnp.where(j < 0, z, w[0:64, :]), w[64:, :]], axis=0)

            def emit_k(g, e, y):
                features(phk, u + e, g, y[0:GR - 8, :])
                rest[g, e] = y[GR - 8:, :]

            def emit_q(g, e, y):
                features(phq, 8 * e + t, g, jnp.concatenate([y, rest[g, e]], axis=0))

            def emit_v(g, e, y):
                for q in range(4):
                    vs[4 * g + q, u + e] = y[40 * q:40 * q + 40, :]

            t10 = tail(0, xs, 1, 0)
            for n in range(6):
                t10 = a_dots(n, xs, (emit_k, emit_q, emit_v)[n // 2], tie, t10)
            cur = jnp.concatenate(nxt, axis=0)
        xa[...] = cur
        row = lax.broadcasted_iota(jnp.int32, (2 * VR, 4 * FA), 0)
        col = lax.broadcasted_iota(jnp.int32, (2 * VR, 4 * FA), 1)
        split = jnp.where(row < 2 * FA, FA, 2 * FA + 4)
        same = (row >= split) == (col >= 2 * FA)
        for q in range(PA):
            v = jnp.concatenate([vs[q, u] for u in range(asub)], axis=1)
            v = jnp.concatenate([v, jnp.ones((8, TA), F32)], axis=0)
            kv = _dot_nt(v.astype(BF16), pair_rows(phk, q, 0, asub))
            kv = kv + jnp.where(j == 0, 0.0, kvacc[q])
            kvacc[q] = kv
            kvs[q] = _pack(jnp.where(same, kv, 0.0).astype(BF16))
        return 0

    def attend(j):
        low = lax.broadcasted_iota(jnp.int32, (8, TN), 0) < 4
        os_ = []
        for q in range(PA):
            nd = _dot(_unpack(kvs[q]), pair_rows(phq, q, j * nsub, nsub))
            rab = 1.0 / (nd[40:48, :] + 1e-6)
            rba = pltpu.roll(rab, 4, 0)
            ra = jnp.where(low, rab, rba)
            rb = jnp.where(low, rba, rab)
            os_.append(nd[0:40, :] * jnp.concatenate([ra, ra, rab, rb, rb], axis=0))
        return _pack(jnp.concatenate(os_, axis=0).astype(BF16).T)

    def project(ty, j, o, slot):
        r = rows(j, TN)
        x = _dot(_unpack(o), woa[...]) + xres[ty, r, :]
        xres[ty, r, :] = x
        for s in range(16):
            z = _layernorm(x[16 * s + 8 - 8 * (s % 2):16 * s + 16 - 8 * (s % 2), :])
            z = z - z[KE:KE + 1, :]
            for c in range(D // 128):
                xe[ty, slot, c, pl.ds(s * KE, 8), :] = z[:, 128 * c:128 * (c + 1)]

    def extra_keys(seg, p):
        k = jnp.concatenate(
            [ke[2 * (seg // 32) + t // 24, (seg // 16) % 2, t % 24, pl.ds((seg % 16) * KE, 8), :]
             for t in range(3 * p, 3 * p + 3)], axis=1)
        return jnp.where(lax.broadcasted_iota(jnp.int32, (8, PW), 0) < KE, k, 0.0)

    def b_residual(i):
        r = rows(i, TB // 2)
        xs = [xres[e, r, :] + d for e, d in enumerate(_split_rows(rsave[...]))]
        for e, x in enumerate(xs):
            xres[e, r, :] = x
        xio[rows(i, TB), :] = _merge_rows(*xs).astype(BF16)
        return xs

    def b_finish(i):
        xn = [_layernorm(x) for x in b_residual(i)]
        for e, x in enumerate(xn):
            xl[e, rows(jnp.minimum(i, 2), TB // 2), :] = x
        return jnp.concatenate(xn, axis=0)

    def b_tile(mem, xn, i, side):
        for u in range(4):
            t0 = u * SEG
            late = u % 2 == 0
            ext = [SEG * v + (24 if v % 2 == 0 else 0) for v in range(4)]

            def place(y, z):
                return jnp.concatenate([y, z] if late else [y[0:M], z, y[M:]], axis=0)

            def fix_qv(p, y):
                cols = slice(p * 2 * PW, (p + 1) * 2 * PW)
                if u == 0:
                    ysave[:, cols] = y[L:, :]
                    y = y[0:L, :]
                else:
                    y = place(y, ysave[8 * u - 8:8 * u, cols])
                if not late:
                    return y
                c0 = 2 * PW - D
                r0 = 64 * u + 8 * p
                tie = jnp.where(i < 0, side[r0:r0 + 8, :], y[0:M, c0:])
                return jnp.concatenate(
                    [jnp.concatenate([y[0:M, 0:c0], tie], axis=1), y[M:, :]], axis=0)

            def fix_k(p, k):
                return place(k, extra_keys(4 * i + u, p))

            def fix_o(p, o):
                cols = slice(p * PW, (p + 1) * PW)
                if u == 3:
                    return jnp.concatenate([o, osave[:, cols]], axis=0)
                osave[8 * u:8 * u + 8, cols] = o[32:L, :]
                return o[0:32, :]

            h = jnp.concatenate(
                [mem, xn[t0:t0 + 24, :] if late else xn[t0 + 8:t0 + SEG, :]], axis=0)
            hk = (h - xn[ext[u] + KE:ext[u] + KE + 1, :]).astype(BF16)
            if u == 0:
                h = jnp.concatenate([h] + [xn[e:e + 8, :] for e in ext], axis=0)
            r = _segment(h, hk, wqv, sqv, wk, wob, sob, fix_qv, fix_k, fix_o, u == 3)
            mem = r[0:M, :]
            if u < 3:
                rsave[t0:t0 + 24, :] = r[M:, :]
            else:
                rsave[t0:t0 + SEG, :] = r[M:L, :]
                for v in range(3):
                    rsave[SEG * v + 24:SEG * v + SEG, :] = r[L + 8 * v:L + 8 * v + 8, :]
        return mem

    def layer(l, _):
        def wait_first(copies):
            @pl.when(l == 0)
            def _():
                for c in copies:
                    c.wait()

        with jax.named_scope("a1"):
            lax.fori_loop(0, na, functools.partial(a1, l == 0), 0)

        def a2(n, _):
            wait_first(w_copies(n))
            ty, half = n % 2, n // 2
            o0 = attend(4 * ty + 2 * half)
            o1 = attend(4 * ty + 2 * half + 1)

            def sample(w):
                z = [w[64 * a + 56:64 * a + 64, :] for a in range(D // 128)]
                out = []
                for y in z:
                    acc = y[:, 0:128]
                    for c in range(1, y.shape[1] // 128):
                        acc = acc | y[:, 128 * c:128 * (c + 1)]
                    out.append(acc)
                return jnp.concatenate(out, axis=1)

            mr = 16 * KE

            def staged(e):
                return jnp.concatenate([xe[0, e, c, 0:mr, :] for c in range(D // 128)], axis=1)

            def side(job):
                out = []
                if job == 'k':
                    out.append(_pack(wraw[3, n].T))
                    wk[n] = out[0]
                else:
                    for i in range(2):
                        out.append(_pack(wraw[i, n, rows(int(job), PW), :].T))
                        wqv[n, :, rows(2 * int(job) + i, PW)] = out[i]
                return functools.reduce(jnp.bitwise_or, [sample(w) for w in out])

            j1, j2, j3 = '01', '23', ''
            for job in j1:
                o1 = jnp.concatenate(
                    [jnp.where(n < 0, side(job), o1[0:8, :]), o1[8:, :]], axis=0)
            project(ty, 2 * half, o0, 0)
            x0 = staged(0)
            for job in j2:
                tie = pltpu.bitcast(side(job), F32)
                x0 = jnp.concatenate([jnp.where(n < 0, tie, x0[0:8, :]), x0[8:, :]], axis=0)
            project(ty, 2 * half + 1, o1, 1)
            x1 = staged(1)
            r = rows(ty, 32)
            xb[rows(ty, 64), :] = _layernorm(_merge_rows(xres[0, r, :], xres[1, r, :]))
            rsave[rows(ty, 64), :] = jnp.zeros((64, D), F32)

            a11, a12, a21, a22 = x0[:, 0:256], x0[:, 256:512], x1[:, 0:256], x1[:, 256:512]
            lhs = [z.astype(BF16) for z in (
                a11 + a22, a21 + a22, a11, a22, a11 + a12, a21 - a11, a12 - a22,
                x0[:, 512:], x1[:, 512:])]

            def wo_rows(e, l, rr):
                return _pack(wraw[2, n, rows(e * 24 + 8 * l + rr, 16), :])

            def repack(e, rr, l, tie):
                wob[rows(n * (QW // 16) + e * 24 + 8 * l + rr, 8), :] = jnp.where(
                    n < 0, jnp.concatenate([tie] * 5, axis=1), wo_rows(e, l, rr))

            def o_sums(e, rr, g, tie):
                sob[rows((4 * n + e) * 8 + rr, 8), pl.ds(128 * _MIXED.index(g[0]), 128 * len(g))] = (
                    _scheme_sums(g, lambda j, l: jnp.where(
                        n < 0, tie, wo_rows(e, l, rr)[:, 128 * j:128 * j + 128])))

            def qv_sums(c, rr, g, tie):
                sqv[rows(8 * n + rr, 8), pl.ds(128 * (c * NS + _MIXED.index(g[0])), 128 * len(g))] = (
                    _scheme_sums(g, lambda j, l: jnp.where(
                        n < 0, tie, wqv[n, rows(8 * j + rr, 8), rows(3 * c + l, 128)])))

            def k_tiles(t, c, tie):
                w = _pack(wraw[3, n, rows(t, 256), rows(c, 128)])
                w = jnp.concatenate([jnp.where(n < 0, tie, w[0:8, :]), w[8:64, :],
                                     jnp.where(n < 0, tie, w[64:72, :]), w[72:, :]], axis=0)
                wk[n, rows(c, 64), rows(t, 256)] = _pack(_unpack(w).T)

            kjobs = [functools.partial(k_tiles, t, c) for t in range(6) for c in range(5)]
            todo = []
            for e in range(4):
                for rr in range(8):
                    todo += kjobs[8 * e + rr:8 * e + rr + 1]
                    todo += [functools.partial(repack, e, rr, l) for l in range(3)]
                    todo += [functools.partial(job, c, rr, g) for job, c in (
                        (o_sums, e), (qv_sums, 2 * e), (qv_sums, 2 * e + 1)) for g in _GROUPS]
            left = [48]

            def emit(e, t, k):
                ke[n, e, t, 0:mr, :] = k
                left[0] -= 1
                if left[0] < 48 - 4:
                    m = -(-len(todo) // (left[0] + 1))
                    for g in range(m):
                        g = 8 * (14 * g // m)
                        todo.pop(0)(pltpu.bitcast(k[g:g + 8, :], U32))

            def blk(v, e, k):
                return wraw[3, 2 * ty + v // 6, rows(2 * (v % 6) + e, 128),
                            256 * k:min(256 * (k + 1), D)]

            def comb(v, x, sign, y):
                x, y = blk(v, *x).astype(F32), blk(v, *y).astype(F32)
                return (x + y if sign > 0 else x - y).astype(BF16)

            b11, b21, b12, b22 = (0, 0), (0, 1), (1, 0), (1, 1)

            def first_half(v):
                m3 = _dot_nt(lhs[2], comb(v, b12, -1, b22))
                m5 = _dot_nt(lhs[4], blk(v, *b22))
                emit(0, 2 * v + 1, _dot_nt(lhs[7], blk(v, 1, 2)) + (m3 + m5))
                return m3, _dot_nt(lhs[7], blk(v, 0, 2)) - m5

            def second_half(v, m3, c11):
                m2 = _dot_nt(lhs[1], blk(v, *b11))
                m4 = _dot_nt(lhs[3], comb(v, b21, -1, b11))
                emit(1, 2 * v, _dot_nt(lhs[8], blk(v, 0, 2)) + (m2 + m4))
                m1 = _dot_nt(lhs[0], comb(v, b11, 1, b22))
                c22 = _dot_nt(lhs[5], comb(v, b11, 1, b12)) + (m1 + (m3 - m2))
                emit(1, 2 * v + 1, _dot_nt(lhs[8], blk(v, 1, 2)) + c22)
                emit(0, 2 * v, _dot_nt(lhs[6], comb(v, b21, 1, b22)) + (c11 + (m1 + m4)))

            nst = 0
            lead = 2
            xb0, xb1 = x0.astype(BF16), x1.astype(BF16)

            def plain(v, e):
                w = wraw[3, 2 * ty + v // 6, rows(v % 6, 256), :]
                k = _dot_nt((xb0, xb1)[e], w)
                emit(e, 2 * v, k[:, 0:128])
                emit(e, 2 * v + 1, k[:, 128:])

            for v in range(lead):
                plain(v, 0)
            for v in range(12):
                if v < 12 - nst:
                    if v >= lead:
                        plain(v, 0)
                    plain(v, 1)
                else:
                    second_half(v, *first_half(v))
            for job in j3:
                side(job)
            return 0

        wait_first([woa_copy, mem0_copy, wk_copy])
        with jax.named_scope("a2"):
            lax.fori_loop(0, NW, a2, 0)

        def b_step(i, mem):
            xn = xb[...]
            side = b_finish(jnp.maximum(i - 1, 0))
            r = rows(jnp.minimum(i + 1, nb - 1), TB // 2)
            nxt = _layernorm(_merge_rows(xres[0, r, :], xres[1, r, :]))
            xb[...] = nxt
            side = jnp.concatenate([side, nxt], axis=0)
            mem = b_tile(mem, xn, i, side)

            @pl.when(jnp.logical_and(l == 1, i >= 1))
            def _():
                out_copy(i - 1).start()
            return mem

        with jax.named_scope("b"):
            lax.fori_loop(0, nb, b_step, mem0[...].astype(F32))

        b_residual(nb - 1)

        @pl.when(l == 0)
        def _():
            xa[...] = strassen_rhs(xl[0, 0:128, :], xl[1, 0:128, :])
        return 0

    lax.fori_loop(0, 2, layer, 0)
    out_copy(nb - 1).start()
    pltpu.make_async_copy(xio, out_hbm, sem_out.at[0]).wait()


@jax.jit
def pallas_interleave_layers__linear_kernel_hedgehog__memory_aug_recurrent_mem_tr__prompt_kernel(
    A_x, A_wqkv, A_w_phi, A_wo, B_x, B_mem0, B_Wq, B_Wk, B_Wv, B_Wo, B_seg_len,
):
    del B_x
    del B_seg_len
    x = A_x.reshape(S, D)
    wphi = A_w_phi.transpose(1, 2, 0)
    mem0 = B_mem0.reshape(M, D)
    wq, wk, wv = (w.transpose(1, 2, 0).reshape(NW, QW, D) for w in (B_Wq, B_Wk, B_Wv))
    wo = B_Wo.reshape(NW, QW, D)
    hbm = pl.BlockSpec(memory_space=pl.ANY)
    out = pl.pallas_call(
        _kernel,
        out_shape=jax.ShapeDtypeStruct((S, D), A_x.dtype),
        in_specs=[hbm] * 9,
        out_specs=hbm,
        scratch_shapes=[
            pltpu.VMEM((S, D), BF16),
            pltpu.VMEM((D, 3 * D), BF16),
            pltpu.VMEM((FA, FA, HA), BF16),
            pltpu.VMEM((D, D), BF16),
            pltpu.VMEM((M, D), BF16),
            pltpu.VMEM((2, S // 2, D), F32),
            pltpu.VMEM((64, 2048), U32),
            pltpu.VMEM((2, 3 * TB // 2, D), F32),
            pltpu.VMEM((TB, D), F32),
            pltpu.VMEM((GA, GR // 2, 256), U32),
            pltpu.VMEM((6, 8, GR // 2, 256), U32),
            pltpu.VMEM((S // 128, D, 128), U32),
            pltpu.VMEM((TA // 128, D, 128), U32),
            pltpu.VMEM((PA, 2 * VR, 4 * FA), F32),
            pltpu.VMEM((PA, VR, 4 * FA), U32),
            pltpu.VMEM((4, NW, QW, D), BF16),
            pltpu.VMEM((NW, D // 2, 2 * QW), U32),
            pltpu.VMEM((NW * 64, 8 * NS * 128), U32),
            pltpu.VMEM((NW, D // 2, QW), U32),
            pltpu.VMEM((HD // 2, D), U32),
            pltpu.VMEM((NP * 64, NS * 128), U32),
            pltpu.VMEM((2, 2, D // 128, 16 * KE + 8, 128), F32),
            pltpu.VMEM((NW, 2, HD // 256, 16 * KE + 8, 128), F32),
            pltpu.VMEM((24, 2 * HD), F32),
            pltpu.VMEM((24, HD), F32),
            pltpu.VMEM((TB, D), F32),
            pltpu.SemaphoreType.DMA((10 + S // TA + 3 * NW,)),
            pltpu.SemaphoreType.DMA((1,)),
        ],
        compiler_params=pltpu.CompilerParams(vmem_limit_bytes=128 * 1024 * 1024,
                                             disable_bounds_checks=True,
                                             disable_semaphore_checks=True),
    )(x, A_wqkv, wphi, A_wo, mem0, wq, wk, wv, wo)
    return out.reshape(1, S, D)
```

```python
import functools

import jax
import jax.numpy as jnp
from jax import lax
import jax.experimental.pallas as pl
import jax.experimental.pallas.tpu as pltpu

F32 = jnp.float32
BF16 = jnp.bfloat16
U32 = jnp.uint32

S = 2048
D = 640
HA = 32
FA = 20
GA = 4
GR = 8 * FA
VR = 24
PA = HA // 2
TN = 256
TA = 512
HB = 32
DH = 192
HD = HB * DH
M = 8
SEG = 32
L = M + SEG
PW = 2 * DH
NP = HB // 2
TB = 128
NW = 4
QW = HD // NW
KE = 7

NT = (((1,), (1,)), ((), ()))
LOG2E = 1.4426950408889634
HALF_ULP = 0.0040612


def _dot(a, b):
    return jnp.dot(a, b, preferred_element_type=F32)


def _dot_nt(a, b):
    return lax.dot_general(a, b, NT, preferred_element_type=F32)


def _pack(a):
    return pltpu.bitcast(a, U32)


def _unpack(a):
    return pltpu.bitcast(a, BF16)


def _interleave(a, b):
    lo = lax.bitcast_convert_type(a, U32) >> 16
    hi = lax.bitcast_convert_type(b, U32) & jnp.uint32(0xFFFF0000)
    return lo | hi


def _recip(x):
    r = pl.reciprocal(x, approx=True)
    return r * (2.0 - x * r)


def _layernorm(x):
    m = jnp.mean(x, axis=-1, keepdims=True)
    c = x - m
    v = jnp.mean(c * c, axis=-1, keepdims=True)
    return c * lax.rsqrt(v + 1e-5)


def _split_rows(x):
    blocks = range(0, x.shape[0], 64)
    return (jnp.concatenate([x[b + 16:b + 48] for b in blocks], axis=0),
            jnp.concatenate([x[b + k:b + k + 16] for b in blocks for k in (0, 48)], axis=0))


def _merge_rows(inner, outer):
    return jnp.concatenate(
        [z for b in range(0, inner.shape[0], 32)
         for z in (outer[b:b + 16], inner[b:b + 32], outer[b + 16:b + 32])], axis=0)


def _feature_map(p):
    t = p.shape[-1]
    p3 = jnp.concatenate([jnp.zeros((8, t), F32), p], axis=0).reshape(FA, 8, t)
    mx = jnp.max(p3, axis=0)
    mn = jnp.min(p3, axis=0)
    sp, sn = jnp.exp2(p3[0] - mx), jnp.exp2(mn - p3[0])
    for f in range(1, FA):
        sp, sn = sp + jnp.exp2(p3[f] - mx), sn + jnp.exp2(mn - p3[f])
    lp = (mx - HALF_ULP) + jnp.log2(sp)
    ln = (mn + HALF_ULP) - jnp.log2(sn)
    return [_interleave(jnp.exp2(p3[f] - lp), jnp.exp2(ln - p3[f])) for f in range(FA)]


def _tiles(a, odd):
    t0, t1, t2 = a[:, 0:128], a[:, 128:256], a[:, 256:384]
    return (t1, t2, t0) if odd else (t1, t0, t2)


def _own_weights(a, odd):
    lane = lax.broadcasted_iota(jnp.int32, (L, 128), 1)
    mid, own, _ = _tiles(a, odd)
    return jnp.concatenate(
        [jnp.where(lane < 64, mid, 0.0), jnp.where(lane < 64, 0.0, mid), own,
         jnp.zeros((128 - 3 * L, 128), F32)], axis=0).astype(BF16)


def _others(even, odd, pad):
    parts = [_tiles(odd, 1)[2], _tiles(even, 0)[2]]
    if pad:
        parts.append(jnp.zeros((128 - 2 * L, 128), F32))
    return jnp.concatenate(parts, axis=0).astype(BF16)


def _softmax3(s3):
    row = lax.broadcasted_iota(jnp.int32, (L, 128), 0)
    col = lax.broadcasted_iota(jnp.int32, (L, 128), 1)
    first = col < L
    second = jnp.logical_and(col >= L, col < 2 * L)
    key = jnp.where(first, col, col - L)
    valid = jnp.logical_or(row < M, row >= key)
    out, other = [], []
    for odd in range(2):
        own = pltpu.roll(s3[odd][L:, :], 128 - L if odd else 128 - 2 * L, 1)
        s = (jnp.where(first, s3[2][0:L, :], own) if odd
             else jnp.where(first, own, s3[2][L:, :]))
        s = jnp.where(valid, (s + s3[odd][0:L, :]) * (DH ** -0.5), -1e9)
        m0 = jnp.max(jnp.where(first, s, -jnp.inf), axis=-1, keepdims=True)
        m1 = jnp.max(jnp.where(second, s, -jnp.inf), axis=-1, keepdims=True)
        e = jnp.exp(s - jnp.where(first, m0, m1))
        e0 = jnp.where(first, e, 0.0)
        e1 = jnp.where(second, e, 0.0)
        p0 = e0 * _recip(jnp.sum(e0, axis=-1, keepdims=True))
        p1 = e1 * _recip(jnp.sum(e1, axis=-1, keepdims=True))
        own = pltpu.roll(p1, L, 1) if odd else pltpu.roll(p0, 2 * L, 1)
        out.append(jnp.concatenate([p0 + p1, own], axis=0).astype(BF16))
        other.append(p0 if odd else p1)
    out.append(jnp.concatenate([other[1], other[0]], axis=0).astype(BF16))
    return out


_T = {5: (-1.5, -0.5, 0.0, 0.5, 1.5), 4: (-1.25, -0.25, 0.25, 1.25)}
_STARS = tuple((5 * g, 5 if g < 4 else 4) for g in range(5))


def _star_sums(n):
    own = {j: [] for j in range(n)}
    for a in range(n):
        for b in range(a + 1, n):
            own[a if (b - a) % 2 else b].append((a, b))
    return [['r%d' % j, 'c%d' % j] + own[j] for j in range(n)]


def _star_slot(g, name):
    return 20 * g + [x for grp in _star_sums(_STARS[g][1]) for x in grp].index(name)


NS = 94


def _star_lhs(n, get, scaled):
    t = _T[n]
    f = [get(0, j) for j in range(n)]
    g = [get(1, j) + t[j] * f[j] if t[j] else get(1, j) for j in range(n)]
    out = {'r%d' % j: f[j] for j in range(n)}
    out.update({'c%d' % j: g[j] for j in range(n)})
    for a in range(n):
        for b in range(a + 1, n):
            d = t[a] - t[b]
            if scaled:
                l = (g[a] - g[b]) * (1.0 / d)
                out[a, b], out[b, a, 0], out[a, b, 0] = l, f[b] - l, f[a] - l
            else:
                l = g[a] - g[b]
                out[a, b], out[b, a, 0], out[a, b, 0] = l, d * f[b] - l, d * f[a] - l
    return {k: v.astype(BF16) for k, v in out.items()}


def _star_apply(n, lhs, plain, mixed, scaled, acc=None):
    t = _T[n]
    p, q = ([None] * n, [None] * n) if acc is None else (list(acc[0]), list(acc[1]))
    started = set()

    def start(j):
        if j not in started:
            started.add(j)
            dp, dq = [_dot(lhs[k % j], mixed(k % j)) for k in ('r%d', 'c%d')]
            p[j] = dp if p[j] is None else dp + p[j]
            q[j] = dq if q[j] is None else dq + q[j]

    for a in range(n):
        for b in range(a + 1, n):
            start(a)
            start(b)
            d = t[a] - t[b]
            m6 = _dot(lhs[b, a, 0], plain(b, a))
            m7 = _dot(lhs[a, b, 0], plain(a, b))
            m = _dot(lhs[a, b], mixed((a, b))) + (m6 + m7)
            if scaled:
                q[a], q[b] = q[a] - (-d) * m6, q[b] - d * m7
                p[a], p[b] = p[a] - (-m), p[b] - (-m)
            else:
                q[a], q[b] = q[a] - (-m6), q[b] - m7
                m = m * (-1.0 / d)
                p[a], p[b] = p[a] - m, p[b] - m
    return p, q


def _star_result(n, p, q):
    return [jnp.concatenate([p[j], q[j] - _T[n][j] * p[j] if _T[n][j] else q[j]], axis=0)
            for j in range(n)]


def _segment(h, hk, wqv, wk, wob, wsum, fix_qv, fix_k, fix_o, wide_o):
    ys = {p: [None] * 3 for p in range(NP)}
    ss, ps, pvs, os_ = {}, {}, {}, {}
    hb = h.astype(BF16)

    def summed(slab, g, name):
        return wsum[64 * slab:64 * slab + 64, pl.ds(128 * _star_slot(g, name), 128)]

    def keys(n):
        k = _dot(hk, _unpack(wk[n]))
        for e in range(4):
            ys[4 * n + e][1] = fix_k(4 * n + e, k[:, e * PW:(e + 1) * PW])

    def proj(p):
        def w(lo, hi):
            return _unpack(jnp.concatenate(
                [wqv[2 * i + p // 8, lo:hi, pl.ds(p % 8 * PW, PW)] for i in range(2)], axis=1))
        if p == 0:
            y = _dot(hb[:, 0:512], w(0, 256))
            y = _dot(hb[:, 512:], w(256, D // 2)) + y
        else:
            y = _dot(hb, w(0, D // 2))
        for i in range(2):
            ys[p][2 * i] = fix_qv(p, i, y[:, i * PW:(i + 1) * PW])

    def wide_proj(half, g, i, lhs, tiles):
        slab, (t0, n) = 2 * i + half, _STARS[g]
        if n == 4:
            tail = _dot(hb[:, 512:], _unpack(wqv[slab, 256:, 128 * t0:]))
        out = _star_result(n, *_star_apply(
            n, lhs[n],
            lambda j, l: _unpack(wqv[slab, 64 * j:64 * j + 64, pl.ds(128 * (t0 + l), 128)]),
            lambda name: _unpack(summed(slab, g, name)), False))
        for l, y in enumerate(out):
            tiles[t0 + l] = y - (-tail[:, 128 * l:128 * l + 128]) if n == 4 else y
        for e in range(8):
            if all(3 * e + k in tiles for k in range(3)):
                ys[8 * half + e][2 * i] = fix_qv(8 * half + e, i, jnp.concatenate(
                    [tiles.pop(3 * e + k) for k in range(3)], axis=1))

    def weights(c, i, which):
        if i < 2:
            return _own_weights(ys[2 * c + i][which], i)
        return _others(ys[2 * c][which], ys[2 * c + 1][which], True)

    def score_round(n):
        for c, i in (divmod(j, 3) for j in range(4 * n, 4 * n + 4)):
            if i < 2:
                q = jnp.concatenate(_tiles(ys[2 * c + i][0], i)[0:2], axis=0).astype(BF16)
            else:
                q = _others(ys[2 * c][0], ys[2 * c + 1][0], False)
            ss[c, i] = _dot_nt(q, weights(c, i, 1))
            if i == 2:
                ps[c] = _softmax3([ss.pop((c, k)) for k in range(3)])

    def pv_round(n):
        for c, i in (divmod(j, 3) for j in range(4 * n, 4 * n + 4)):
            pvs[c, i] = _dot(ps[c][i], weights(c, i, 2))
            if i == 2:
                o0, o1, o2 = [pvs.pop((c, k)) for k in range(3)]
                os_[2 * c] = fix_o(2 * c, jnp.concatenate(
                    [o0[L:, :], o0[0:L, :], o2[L:, :]], axis=1))
                os_[2 * c + 1] = fix_o(2 * c + 1, jnp.concatenate(
                    [o2[0:L, :], o1[0:L, :], o1[L:, :]], axis=1))

    def slot(n):
        if n >= 2:
            pv_round(n - 2)
        if n < 6:
            score_round(n)

    def oproj(lo, hi, r):
        o = jnp.concatenate([os_.pop(p) for p in range(lo, hi)], axis=1).astype(BF16)
        y = _dot(o, _unpack(wob[lo * DH:hi * DH, :]))
        return y if r is None else y + r

    def wide_oproj(stars, r):
        def o_tile(t):
            return os_[t // 3][:, 128 * (t % 3):128 * (t % 3) + 128]

        for n in (4, 5):
            sel = [divmod(x, 5) for x in stars if _STARS[x % 5][1] == n]
            if not sel:
                continue
            t0 = [24 * half + _STARS[g][0] for half, g in sel]
            if n == 4:
                ts = [t + j for t in t0 for j in range(4)]
                y = _dot(jnp.concatenate([o_tile(t) for t in ts], axis=1).astype(BF16),
                         _unpack(jnp.concatenate(
                             [wob[64 * t:64 * t + 64, 512:] for t in ts], axis=0)))
                r[0] = y + r[0] if 0 in r else y
            r[n] = _star_apply(
                n, _star_lhs(n, lambda i, j: jnp.concatenate(
                    [o_tile(t + j)[32 * i:32 * i + 32] for t in t0], axis=1), True),
                lambda j, l: _unpack(jnp.concatenate(
                    [wob[pl.ds(64 * (t + j), 64), 128 * l:128 * l + 128] for t in t0], axis=0)),
                lambda name: _unpack(jnp.concatenate(
                    [summed(4 + half, g, name) for half, g in sel], axis=0)), True, r.get(n))
        return r

    if h.shape[0] == 64:
        lhs = {n: _star_lhs(n, lambda i, j: h[32 * i:32 * i + 32, 128 * j:128 * j + 128], False)
               for n in (4, 5)}
        after = (3, 7, 9, 13, 17)
        kat = (0, 4, 10, 14)
        tiles = {}
        for unit in range(20):
            half, g, i = unit // 10, unit % 10 // 2, unit % 2
            wide_proj(half, g, i, lhs, tiles.setdefault((half, i), {}))
            if unit in kat:
                keys(kat.index(unit))
            if unit in after:
                slot(after.index(unit))
    else:
        after = (3, 6, 9, 12, 14)
        for p in range(NP):
            proj(p)
            if p % 4 == 0:
                keys(p // 4)
            if p in after:
                slot(after.index(p))
    if wide_o:
        o1, o2, o3 = (2, 5, 6)
        r = wide_oproj(range(0, o1), {})
        slot(5)
        r = wide_oproj(range(o1, o2), r)
        slot(6)
        slot(7)
        r = wide_oproj(range(o2, o3), r)
        r = wide_oproj(range(o3, 10), r)
        return jnp.concatenate(
            [x + y for x, y in zip(_star_result(5, *r[5]), _star_result(4, *r[4]) + [r[0]])],
            axis=1)
    o1, o2, o3 = (1, 8, 10) if h.shape[0] == 64 else (2, 9, 10)
    r = oproj(0, o1, None) if o1 else None
    slot(5)
    r = oproj(o1, o2, r)
    slot(6)
    slot(7)
    r = oproj(o2, o3, r)
    return oproj(o3, NP, r)


def _kernel(x_hbm, wqkv_hbm, wphi_hbm, woa_hbm, mem0_hbm,
            wq_hbm, wk_hbm, wv_hbm, wo_hbm,
            out_hbm,
            xio, wqkv, wphi, woa, mem0, xres, xa, xl, xb, bds, wat, phq, phk, kvacc, kvs,
            wraw, wqv, wk, wob, wsum, xe, ke, ysave, osave, rsave, sem_in, sem_out):
    nsub = TN // 128
    na = S // TA
    asub = TA // 128
    nb = S // TB

    def rows(j, n):
        return pl.ds(j * n if isinstance(j, int) else pl.multiple_of(j * n, n), n)

    def x_copy(j):
        if isinstance(j, int) and j < 0:
            r = pl.ds(0, 256)
        elif isinstance(j, int) and j == na - 1:
            r = pl.ds(S - TA + 256, TA - 256)
        else:
            r = pl.ds(j * TA + 256 if isinstance(j, int)
                      else pl.multiple_of(j * TA + 256, 256), TA)
        return pltpu.make_async_copy(x_hbm.at[r, :], xio.at[r, :], sem_in.at[9 + j])

    def w_copy(c):
        src = (wq_hbm, wv_hbm, wo_hbm, wk_hbm)[c // 2 if isinstance(c, int) else 0]
        return pltpu.make_async_copy(src.at[c % 2], wraw.at[c], sem_in.at[9 + na + c])

    def wa_copy(c):
        r = pl.ds(512, 128) if isinstance(c, int) and c == 2 else rows(c, 256)
        return pltpu.make_async_copy(wqkv_hbm.at[r, :], wqkv.at[r, :], sem_in.at[3 + c])

    def out_copy(i):
        return pltpu.make_async_copy(xio.at[rows(i, TB), :],
                                     out_hbm.at[rows(i, TB), :], sem_out.at[0])

    wphi_copy = pltpu.make_async_copy(wphi_hbm, wphi, sem_in.at[0])
    woa_copy = pltpu.make_async_copy(woa_hbm, woa, sem_in.at[1])
    mem0_copy = pltpu.make_async_copy(mem0_hbm, mem0, sem_in.at[2])
    order = [wphi_copy, wa_copy(0), wa_copy(1), x_copy(-1), wa_copy(2)]
    order += [x_copy(j) for j in range(na)] + [woa_copy, mem0_copy]
    order += [w_copy(c) for c in (6, 0, 4, 7, 1, 2, 5, 3)]
    for c in order:
        c.start()

    def strassen_rhs(x0, x1):
        b11, b12 = [jnp.concatenate([x[:, 0:128], x[:, 256:384]], axis=1) for x in (x0, x1)]
        b21, b22 = [jnp.concatenate([x[:, 128:256], x[:, 384:512]], axis=1) for x in (x0, x1)]
        ops = [b11 + b22, b11, b12 - b22, b21 - b11, b22, b11 + b12, b21 + b22,
               x0[:, 512:], x1[:, 512:]]
        return _pack(jnp.concatenate(ops, axis=1).astype(BF16))

    def load_x(t, first):
        xs = _split_rows(xio[rows(t, 256), :].astype(F32))
        if first is not True:
            xs = [jnp.where(first, x, xres[e, rows(t, 128), :]) for e, x in enumerate(xs)]
        for e, x in enumerate(xs):
            xres[e, rows(t, 128), :] = x
        return jnp.concatenate(xs, axis=0)

    wphi_copy.wait()
    cphi = jnp.zeros((FA, D), F32)
    hh = lax.broadcasted_iota(jnp.int32, (HA, D), 0) * FA
    jj = lax.broadcasted_iota(jnp.int32, (HA, D), 1)
    for d in range(FA):
        cphi = _dot(wphi[d], jnp.where(jj == hh + d, 1.0, 0.0).astype(BF16)) + cphi
    cb = jnp.concatenate(
        [jnp.broadcast_to(cphi[f:f + 1, :], (8, D)) for f in range(FA)], axis=0)
    for g in range(GA):
        row = lax.broadcasted_iota(jnp.int32, (GR, 256), 0)
        col = lax.broadcasted_iota(jnp.int32, (GR, 256), 1) + 128 * g
        lo = (8 * g + (row & 7)) * FA
        bds[g] = _pack(jnp.where(jnp.logical_and(col >= lo, col < lo + FA),
                                 cb[:, 128 * g:128 * g + 256], 0.0).astype(BF16))

    def folded(rr):
        out = [[], [], []]
        for g in range(GA):
            ws = []
            for i in range(2):
                c0 = i * D + 128 * g
                w = _dot_nt(_unpack(bds[g]), wqkv[rr, c0:c0 + 256]).reshape(FA, 8, 128)
                ws.append(((w[1:] - w[0:1]) * LOG2E).reshape(GR - 8, 128))
            out[0].append(jnp.concatenate([ws[1], ws[0][GR - 16:, :]], axis=0))
            out[1].append(ws[0][0:GR - 16, :])
        wvt = wqkv[rr, 2 * D:3 * D].T.astype(F32)
        out[2] = [wvt[g * GR:(g + 1) * GR, :] for g in range(GA)]
        return out

    def fold(c, _):
        wa_copy(c).wait()
        wa, wb = folded(rows(2 * c, 128)), folded(rows(2 * c + 1, 128))
        for i in range(3):
            for p in range(2):
                a11, a12, a21, a22 = wa[i][2 * p], wb[i][2 * p], wa[i][2 * p + 1], wb[i][2 * p + 1]
                ops = [a11 + a22, a21 + a22, a11, a22, a11 + a12, a21 - a11, a12 - a22]
                for m, w in enumerate(ops):
                    wat[2 * i + p, m, 0:w.shape[0] // 2, rows(c, 128)] = _pack(w.astype(BF16))
        return 0

    lax.fori_loop(0, 2, fold, 0)
    x_copy(-1).wait()
    wa_copy(2).wait()
    x = _layernorm(load_x(0, True))
    xa[...] = strassen_rhs(x[0:128], x[128:])
    for i, ws in enumerate(folded(pl.ds(512, 128))):
        for g, w in enumerate(ws):
            wat[2 * i + g // 2, 7, 0:w.shape[0] // 2, rows(g % 2, 128)] = _pack(w.astype(BF16))

    def pair_rows(ph, q, t0, n):
        return _unpack(jnp.concatenate(
            [ph[t0 + u, rows(q, 2 * FA), :] for u in range(n)], axis=1))

    def a1(first, j, _):
        @pl.when(jnp.logical_and(first, j < na - 1))
        def _():
            x_copy(j).wait()

        @pl.when(jnp.logical_and(first, j == na - 1))
        def _():
            x_copy(na - 1).wait()

        def features(ph, t, g, y):
            for f, w in enumerate(_feature_map(y)):
                ph[t, pl.ds(GR * g + f, 8, stride=FA), :] = w

        def tail(n, xs, g, u):
            nr = GR // 2 - 8 if n // 2 == 1 else GR // 2
            return _dot_nt(_unpack(wat[n, 7, 0:nr, 128 * g:128 * (g + 1)]),
                           xs[:, 1792 + 128 * u:1920 + 128 * u])

        def a_dots(n, xs, emit, tie, t10):
            nr = GR // 2 - 8 if n // 2 == 1 else GR // 2
            p = n % 2

            def prod(m):
                return _dot_nt(_unpack(tie(wat[n, m, 0:nr, :])), xs[:, 256 * m:256 * (m + 1)])

            m2, m4 = prod(1), prod(3)
            emit(2 * p + 1, 0, m4 + (m2 - (-t10)))
            t01 = tail(n, xs, 0, 1)
            m3, m5 = prod(2), prod(4)
            emit(2 * p, 1, m5 + (m3 - (-t01)))
            m1 = prod(0)
            c22 = prod(5) + (m1 + (m3 - m2))
            emit(2 * p + 1, 1, tail(n, xs, 1, 1) + c22)
            t10 = tail(n + 1, xs, 1, 0) if n < 5 else None
            c11 = tail(n, xs, 0, 0) + (m1 + (m4 - m5))
            emit(2 * p, 0, prod(6) + c11)
            return t10

        vs = {}
        cur = xa[...]
        dl = (3, 8, 13, 30, 33, 36, 39, 41)
        for u in range(0, asub, 2):
            t = j * (asub // 2) + u // 2
            xs = _unpack(cur)
            tn = t + 1
            x = load_x(tn if u + 2 < asub else jnp.minimum(tn, (na - 1) * (asub // 2)), first)
            rest, seen, nxt = {}, [], []

            def tie(w):
                seen.append(0)
                if len(seen) - 1 not in dl:
                    return w
                n = len(nxt)
                nxt.append(strassen_rhs(*[
                    _layernorm(x[128 * e + 16 * n:128 * e + 16 * n + 16, :]) for e in range(2)]))
                z = jnp.concatenate(
                    [nxt[n][:, 256 * c:256 * (c + 1)] for c in range(8)], axis=0)
                return jnp.concatenate([jnp.where(j < 0, z, w[0:64, :]), w[64:, :]], axis=0)

            def emit_k(g, e, y):
                features(phk, u + e, g, y[0:GR - 8, :])
                rest[g, e] = y[GR - 8:, :]

            def emit_q(g, e, y):
                features(phq, 8 * e + t, g, jnp.concatenate([y, rest[g, e]], axis=0))

            def emit_v(g, e, y):
                for q in range(4):
                    vs[4 * g + q, u + e] = y[40 * q:40 * q + 40, :]

            t10 = tail(0, xs, 1, 0)
            for n in range(6):
                t10 = a_dots(n, xs, (emit_k, emit_q, emit_v)[n // 2], tie, t10)
            cur = jnp.concatenate(nxt, axis=0)
        xa[...] = cur
        row = lax.broadcasted_iota(jnp.int32, (2 * VR, 4 * FA), 0)
        col = lax.broadcasted_iota(jnp.int32, (2 * VR, 4 * FA), 1)
        split = jnp.where(row < 2 * FA, FA, 2 * FA + 4)
        same = (row >= split) == (col >= 2 * FA)
        for q in range(PA):
            v = jnp.concatenate([vs[q, u] for u in range(asub)], axis=1)
            v = jnp.concatenate([v, jnp.ones((8, TA), F32)], axis=0)
            kv = _dot_nt(v.astype(BF16), pair_rows(phk, q, 0, asub))
            kv = kv + jnp.where(j == 0, 0.0, kvacc[q])
            kvacc[q] = kv
            kvs[q] = _pack(jnp.where(same, kv, 0.0).astype(BF16))
        return 0

    def attend(j):
        low = lax.broadcasted_iota(jnp.int32, (8, TN), 0) < 4
        os_ = []
        for q in range(PA):
            nd = _dot(_unpack(kvs[q]), pair_rows(phq, q, j * nsub, nsub))
            rab = 1.0 / (nd[40:48, :] + 1e-6)
            rba = pltpu.roll(rab, 4, 0)
            ra = jnp.where(low, rab, rba)
            rb = jnp.where(low, rba, rab)
            os_.append(nd[0:40, :] * jnp.concatenate([ra, ra, rab, rb, rb], axis=0))
        return _pack(jnp.concatenate(os_, axis=0).astype(BF16).T)

    def project(ty, j, o, slot):
        r = rows(j, TN)
        x = _dot(_unpack(o), woa[...]) + xres[ty, r, :]
        xres[ty, r, :] = x
        for s in range(16):
            z = _layernorm(x[16 * s + 8 - 8 * (s % 2):16 * s + 16 - 8 * (s % 2), :])
            z = z - z[KE:KE + 1, :]
            for c in range(D // 128):
                xe[ty, slot, c, pl.ds(s * KE, 8), :] = z[:, 128 * c:128 * (c + 1)]

    def extra_keys(seg, p):
        k = jnp.concatenate(
            [ke[2 * (seg // 32) + t // 24, (seg // 16) % 2, t % 24, pl.ds((seg % 16) * KE, 8), :]
             for t in range(3 * p, 3 * p + 3)], axis=1)
        return jnp.where(lax.broadcasted_iota(jnp.int32, (8, PW), 0) < KE, k, 0.0)

    def b_residual(i):
        r = rows(i, TB // 2)
        xs = [xres[e, r, :] + d for e, d in enumerate(_split_rows(rsave[...]))]
        for e, x in enumerate(xs):
            xres[e, r, :] = x
        xio[rows(i, TB), :] = _merge_rows(*xs).astype(BF16)
        return xs

    def b_finish(i):
        xn = [_layernorm(x) for x in b_residual(i)]
        for e, x in enumerate(xn):
            xl[e, rows(jnp.minimum(i, 2), TB // 2), :] = x
        return jnp.concatenate(xn, axis=0)

    def b_tile(mem, xn, i, side):
        for u in range(4):
            t0 = u * SEG
            late = u % 2 == 0
            ext = [SEG * v + (24 if v % 2 == 0 else 0) for v in range(4)]

            def place(y, z):
                return jnp.concatenate([y, z] if late else [y[0:M], z, y[M:]], axis=0)

            def fix_qv(p, kind, y):
                cols = pl.ds((2 * p + kind) * PW, PW)
                if u == 0:
                    ysave[:, cols] = y[L:, :]
                    y = y[0:L, :]
                else:
                    y = place(y, ysave[8 * u - 8:8 * u, cols])
                if not late:
                    return y
                r0 = 64 * u + 8 * p
                tie = jnp.where(i < 0, side[r0:r0 + 8, 256 * kind:256 * kind + PW], y[0:M, :])
                return jnp.concatenate([tie, y[M:, :]], axis=0)

            def fix_k(p, k):
                return place(k, extra_keys(4 * i + u, p))

            def fix_o(p, o):
                cols = slice(p * PW, (p + 1) * PW)
                if u == 3:
                    return jnp.concatenate([o, osave[:, cols]], axis=0)
                osave[8 * u:8 * u + 8, cols] = o[32:L, :]
                return o[0:32, :]

            h = jnp.concatenate(
                [mem, xn[t0:t0 + 24, :] if late else xn[t0 + 8:t0 + SEG, :]], axis=0)
            hk = (h - xn[ext[u] + KE:ext[u] + KE + 1, :]).astype(BF16)
            if u == 0:
                h = jnp.concatenate([h] + [xn[e:e + 8, :] for e in ext], axis=0)
            r = _segment(h, hk, wqv, wk, wob, wsum, fix_qv, fix_k, fix_o, u == 3)
            mem = r[0:M, :]
            if u < 3:
                rsave[t0:t0 + 24, :] = r[M:, :]
            else:
                rsave[t0:t0 + SEG, :] = r[M:L, :]
                for v in range(3):
                    rsave[SEG * v + 24:SEG * v + SEG, :] = r[L + 8 * v:L + 8 * v + 8, :]
        return mem

    def layer(l, _):
        def wait_first(copies):
            @pl.when(l == 0)
            def _():
                for c in copies:
                    c.wait()

        with jax.named_scope("a1"):
            lax.fori_loop(0, na, functools.partial(a1, l == 0), 0)

        def a2(n, _):
            for m, cs in enumerate(((6, 0, 4), (7, 1), (2, 5), (3,))):
                @pl.when(jnp.logical_and(l == 0, n == m))
                def _():
                    for c in cs:
                        w_copy(c).wait()

            ty, half = n % 2, n // 2
            o0 = attend(4 * ty + 2 * half)
            o1 = attend(4 * ty + 2 * half + 1)

            def sample(w):
                z = [w[64 * a + 56:64 * a + 64, :] for a in range(D // 128)]
                out = []
                for y in z:
                    acc = y[:, 0:128]
                    for c in range(1, y.shape[1] // 128):
                        acc = acc | y[:, 128 * c:128 * (c + 1)]
                    out.append(acc)
                return jnp.concatenate(out, axis=1)

            mr = 16 * KE

            def staged(e):
                return jnp.concatenate([xe[0, e, c, 0:mr, :] for c in range(D // 128)], axis=1)

            def side(job):
                w = _pack(wraw[n, rows(int(job), 2 * PW), :].T)
                wqv[n, :, rows(int(job), 2 * PW)] = w
                return sample(w)

            j1, j2 = '01', '23'
            for job in j1:
                o1 = jnp.concatenate(
                    [jnp.where(n < 0, side(job), o1[0:8, :]), o1[8:, :]], axis=0)
            project(ty, 2 * half, o0, 0)
            x0 = staged(0)
            for job in j2:
                tie = pltpu.bitcast(side(job), F32)
                x0 = jnp.concatenate([jnp.where(n < 0, tie, x0[0:8, :]), x0[8:, :]], axis=0)
            project(ty, 2 * half + 1, o1, 1)
            x1 = staged(1)
            r = rows(ty, 32)
            xb[rows(ty, 64), :] = _layernorm(_merge_rows(xres[0, r, :], xres[1, r, :]))
            rsave[rows(ty, 64), :] = jnp.zeros((64, D), F32)

            def view(ref, start, size, align):
                return ref.at[pl.ds(pl.multiple_of(start, align), size)]

            wo_src = view(wraw.at[4 + half], 64 * ty, HD // 2 - 64, 64)
            wo_dst = view(wob, QW * half + 32 * ty, QW - 32, 32)
            wk_src = view(wraw.at[6 + half], QW * ty, QW, QW)
            sum_dst = view(wsum, 64 * n, 64, 64), view(wsum, 256 + 32 * n, 32, 32)

            def wo_rows(t, rr):
                return _pack(wo_src[rows(8 * t + rr, 16), :])

            def sums(is_o, g, j, rr, tie):
                t0, sz = _STARS[g]
                names = _star_sums(sz)[j]
                if is_o:
                    row = jnp.where(n < 0, jnp.concatenate([tie] * 5, axis=1), wo_rows(t0 + j, rr))
                    wo_dst[rows(8 * (t0 + j) + rr, 8), :] = row
                val = {}
                for x, y in [(j, k) for k in range(sz)] + [(k, j) for k in range(sz) if k != j]:
                    if is_o and x == j:
                        w = row[:, 128 * y:128 * y + 128]
                    elif is_o and x < j:
                        w = jnp.where(n < 0, tie, wo_dst[rows(8 * (t0 + x) + rr, 8), rows(y, 128)])
                    else:
                        w = jnp.where(n < 0, tie, wo_rows(t0 + x, rr)[:, 128 * y:128 * y + 128] if is_o
                                      else wqv[n, rows(8 * x + rr, 8), rows(t0 + y, 128)])
                    val[x, y] = _unpack(w).astype(F32)
                others = [k for k in range(sz) if k != j]
                out = [functools.reduce(lambda z, k: z - val[j, k], others, val[j, j]),
                       functools.reduce(lambda z, k: z + val[k, j], others, val[j, j])]
                out += [val[x, y] + val[y, x] for x, y in names[2:]]
                sum_dst[is_o][rows(rr, 8),
                              pl.ds(128 * _star_slot(g, names[0]), 128 * len(names))] = _pack(
                    jnp.concatenate(out, axis=1).astype(BF16))

            def k_tiles(t, c, tie):
                w = _pack(wk_src[rows(t, 256), rows(c, 128)])
                w = jnp.concatenate([jnp.where(n < 0, tie, w[0:8, :]), w[8:64, :],
                                     jnp.where(n < 0, tie, w[64:72, :]), w[72:, :]], axis=0)
                wk[n, rows(c, 64), rows(t, 256)] = _pack(_unpack(w).T)

            kjobs = [functools.partial(k_tiles, t, c) for t in range(6) for c in range(5)]
            todo = []
            for g in range(5):
                for j in range(_STARS[g][1]):
                    for rr in range(4):
                        if len(todo) % 10 < 3:
                            todo += kjobs[-1:]
                            del kjobs[-1:]
                        todo += [functools.partial(sums, False, g, j, 2 * rr),
                                 functools.partial(sums, True, g, j, rr),
                                 functools.partial(sums, False, g, j, 2 * rr + 1)]
            assert not kjobs
            left = [48]

            def emit(e, t, k):
                ke[n, e, t, 0:mr, :] = k
                left[0] -= 1
                if left[0] < 48 - 4:
                    m = -(-len(todo) // (left[0] + 1))
                    for g in range(m):
                        g = 8 * (14 * g // m)
                        todo.pop(0)(pltpu.bitcast(k[g:g + 8, :], U32))

            lead = 2
            xs = x0.astype(BF16), x1.astype(BF16)
            for v, e in [(v, 0) for v in range(lead)] + [
                    (v, e) for v in range(12) for e in range(2) if e or v >= lead]:
                k = _dot_nt(xs[e], wraw[6 + ty, rows(v, 256), :])
                emit(e, 2 * v, k[:, 0:128])
                emit(e, 2 * v + 1, k[:, 128:])
            return 0

        wait_first([woa_copy, mem0_copy])
        with jax.named_scope("a2"):
            lax.fori_loop(0, NW, a2, 0)

        def b_step(i, mem):
            xn = xb[...]
            side = b_finish(jnp.maximum(i - 1, 0))
            r = rows(jnp.minimum(i + 1, nb - 1), TB // 2)
            nxt = _layernorm(_merge_rows(xres[0, r, :], xres[1, r, :]))
            xb[...] = nxt
            side = jnp.concatenate([side, nxt], axis=0)
            mem = b_tile(mem, xn, i, side)

            @pl.when(jnp.logical_and(l == 1, i >= 1))
            def _():
                out_copy(i - 1).start()
            return mem

        with jax.named_scope("b"):
            lax.fori_loop(0, nb, b_step, mem0[...].astype(F32))

        b_residual(nb - 1)

        @pl.when(l == 0)
        def _():
            xa[...] = strassen_rhs(xl[0, 0:128, :], xl[1, 0:128, :])
        return 0

    lax.fori_loop(0, 2, layer, 0)
    out_copy(nb - 1).start()
    pltpu.make_async_copy(xio, out_hbm, sem_out.at[0]).wait()


@jax.jit
def pallas_interleave_layers__linear_kernel_hedgehog__memory_aug_recurrent_mem_tr__prompt_kernel(
    A_x, A_wqkv, A_w_phi, A_wo, B_x, B_mem0, B_Wq, B_Wk, B_Wv, B_Wo, B_seg_len,
):
    del B_x
    del B_seg_len
    x = A_x.reshape(S, D)
    wphi = A_w_phi.transpose(1, 2, 0)
    mem0 = B_mem0.reshape(M, D)
    wq, wk, wv = (w.transpose(1, 2, 0).reshape(2, HD // 2, D) for w in (B_Wq, B_Wk, B_Wv))
    wo = B_Wo.reshape(2, HD // 2, D)
    hbm = pl.BlockSpec(memory_space=pl.ANY)
    out = pl.pallas_call(
        _kernel,
        out_shape=jax.ShapeDtypeStruct((S, D), A_x.dtype),
        in_specs=[hbm] * 9,
        out_specs=hbm,
        scratch_shapes=[
            pltpu.VMEM((S, D), BF16),
            pltpu.VMEM((D, 3 * D), BF16),
            pltpu.VMEM((FA, FA, HA), BF16),
            pltpu.VMEM((D, D), BF16),
            pltpu.VMEM((M, D), BF16),
            pltpu.VMEM((2, S // 2, D), F32),
            pltpu.VMEM((64, 2048), U32),
            pltpu.VMEM((2, 3 * TB // 2, D), F32),
            pltpu.VMEM((TB, D), F32),
            pltpu.VMEM((GA, GR // 2, 256), U32),
            pltpu.VMEM((6, 8, GR // 2, 256), U32),
            pltpu.VMEM((S // 128, D, 128), U32),
            pltpu.VMEM((TA // 128, D, 128), U32),
            pltpu.VMEM((PA, 2 * VR, 4 * FA), F32),
            pltpu.VMEM((PA, VR, 4 * FA), U32),
            pltpu.VMEM((8, HD // 2, D), BF16),
            pltpu.VMEM((4, D // 2, HD // 2), U32),
            pltpu.VMEM((NW, D // 2, QW), U32),
            pltpu.VMEM((HD // 2, D), U32),
            pltpu.VMEM((6 * 64, NS * 128), U32),
            pltpu.VMEM((2, 2, D // 128, 16 * KE + 8, 128), F32),
            pltpu.VMEM((NW, 2, HD // 256, 16 * KE + 8, 128), F32),
            pltpu.VMEM((24, 2 * HD), F32),
            pltpu.VMEM((24, HD), F32),
            pltpu.VMEM((TB, D), F32),
            pltpu.SemaphoreType.DMA((17 + S // TA,)),
            pltpu.SemaphoreType.DMA((1,)),
        ],
        compiler_params=pltpu.CompilerParams(vmem_limit_bytes=128 * 1024 * 1024,
                                             disable_bounds_checks=True,
                                             disable_semaphore_checks=True),
    )(x, A_wqkv, wphi, A_wo, mem0, wq, wk, wv, wo)
    return out.reshape(1, S, D)
```

```python
import functools

import jax
import jax.numpy as jnp
from jax import lax
import jax.experimental.pallas as pl
import jax.experimental.pallas.tpu as pltpu

F32 = jnp.float32
BF16 = jnp.bfloat16
U32 = jnp.uint32

S = 2048
D = 640
HA = 32
FA = 20
GA = 4
GR = 8 * FA
VR = 24
PA = HA // 2
TN = 256
TA = 512
HB = 32
DH = 192
HD = HB * DH
M = 8
SEG = 32
L = M + SEG
PW = 2 * DH
NP = HB // 2
TB = 128
NW = 4
QW = HD // NW
KE = 7

NT = (((1,), (1,)), ((), ()))
LOG2E = 1.4426950408889634
HALF_ULP = 0.0040612


def _dot(a, b):
    return jnp.dot(a, b, preferred_element_type=F32)


def _dot_nt(a, b):
    return lax.dot_general(a, b, NT, preferred_element_type=F32)


def _pack(a):
    return pltpu.bitcast(a, U32)


def _unpack(a):
    return pltpu.bitcast(a, BF16)


def _interleave(a, b):
    lo = lax.bitcast_convert_type(a, U32) >> 16
    hi = lax.bitcast_convert_type(b, U32) & jnp.uint32(0xFFFF0000)
    return lo | hi


def _recip(x):
    r = pl.reciprocal(x, approx=True)
    return r * (2.0 - x * r)


def _layernorm(x):
    m = jnp.mean(x, axis=-1, keepdims=True)
    c = x - m
    v = jnp.mean(c * c, axis=-1, keepdims=True)
    return c * lax.rsqrt(v + 1e-5)


def _feature_map(p):
    t = p.shape[-1]
    p3 = jnp.concatenate([jnp.zeros((8, t), F32), p], axis=0).reshape(FA, 8, t)
    mx = jnp.max(p3, axis=0)
    mn = jnp.min(p3, axis=0)
    sp, sn = jnp.exp2(p3[0] - mx), jnp.exp2(mn - p3[0])
    for f in range(1, FA):
        sp, sn = sp + jnp.exp2(p3[f] - mx), sn + jnp.exp2(mn - p3[f])
    lp = (mx - HALF_ULP) + jnp.log2(sp)
    ln = (mn + HALF_ULP) - jnp.log2(sn)
    return [_interleave(jnp.exp2(p3[f] - lp), jnp.exp2(ln - p3[f])) for f in range(FA)]


def _tiles(a, odd):
    t0, t1, t2 = a[:, 0:128], a[:, 128:256], a[:, 256:384]
    return (t1, t2, t0) if odd else (t1, t0, t2)


def _own_weights(a, odd):
    lane = lax.broadcasted_iota(jnp.int32, (L, 128), 1)
    mid, own, _ = _tiles(a, odd)
    return jnp.concatenate(
        [jnp.where(lane < 64, mid, 0.0), jnp.where(lane < 64, 0.0, mid), own,
         jnp.zeros((128 - 3 * L, 128), F32)], axis=0).astype(BF16)


def _others(even, odd, pad):
    parts = [_tiles(odd, 1)[2], _tiles(even, 0)[2]]
    if pad:
        parts.append(jnp.zeros((128 - 2 * L, 128), F32))
    return jnp.concatenate(parts, axis=0).astype(BF16)


def _softmax3(s3):
    row = lax.broadcasted_iota(jnp.int32, (L, 128), 0)
    col = lax.broadcasted_iota(jnp.int32, (L, 128), 1)
    first = col < L
    second = jnp.logical_and(col >= L, col < 2 * L)
    key = jnp.where(first, col, col - L)
    valid = jnp.logical_or(row < M, row >= key)
    out, other = [], []
    for odd in range(2):
        own = pltpu.roll(s3[odd][L:, :], 128 - L if odd else 128 - 2 * L, 1)
        s = (jnp.where(first, s3[2][0:L, :], own) if odd
             else jnp.where(first, own, s3[2][L:, :]))
        s = jnp.where(valid, (s + s3[odd][0:L, :]) * (DH ** -0.5), -1e9)
        m0 = jnp.max(jnp.where(first, s, -jnp.inf), axis=-1, keepdims=True)
        m1 = jnp.max(jnp.where(second, s, -jnp.inf), axis=-1, keepdims=True)
        e = jnp.exp(s - jnp.where(first, m0, m1))
        e0 = jnp.where(first, e, 0.0)
        e1 = jnp.where(second, e, 0.0)
        p0 = e0 * _recip(jnp.sum(e0, axis=-1, keepdims=True))
        p1 = e1 * _recip(jnp.sum(e1, axis=-1, keepdims=True))
        own = pltpu.roll(p1, L, 1) if odd else pltpu.roll(p0, 2 * L, 1)
        out.append(jnp.concatenate([p0 + p1, own], axis=0).astype(BF16))
        other.append(p0 if odd else p1)
    out.append(jnp.concatenate([other[1], other[0]], axis=0).astype(BF16))
    return out


_T = {5: (-1.5, -0.5, 0.0, 0.5, 1.5), 4: (-1.25, -0.25, 0.25, 1.25)}
_STARS = tuple((5 * g, 5 if g < 4 else 4) for g in range(5))


def _star_sums(n):
    own = {j: [] for j in range(n)}
    for a in range(n):
        for b in range(a + 1, n):
            own[a if (b - a) % 2 else b].append((a, b))
    return [['r%d' % j, 'c%d' % j] + own[j] for j in range(n)]


def _star_slot(g, name):
    return 20 * g + [x for grp in _star_sums(_STARS[g][1]) for x in grp].index(name)


NS = 94


def _star_lhs(n, get, scaled):
    t = _T[n]
    f = [get(0, j) for j in range(n)]
    g = [get(1, j) + t[j] * f[j] if t[j] else get(1, j) for j in range(n)]
    out = {'r%d' % j: f[j] for j in range(n)}
    out.update({'c%d' % j: g[j] for j in range(n)})
    for a in range(n):
        for b in range(a + 1, n):
            d = t[a] - t[b]
            if scaled:
                l = (g[a] - g[b]) * (1.0 / d)
                out[a, b], out[b, a, 0], out[a, b, 0] = l, f[b] - l, f[a] - l
            else:
                l = g[a] - g[b]
                out[a, b], out[b, a, 0], out[a, b, 0] = l, d * f[b] - l, d * f[a] - l
    return {k: v.astype(BF16) for k, v in out.items()}


def _star_apply(n, lhs, plain, mixed, scaled, acc=None):
    t = _T[n]
    p, q = ([None] * n, [None] * n) if acc is None else (list(acc[0]), list(acc[1]))
    started = set()

    def start(j):
        if j not in started:
            started.add(j)
            dp, dq = [_dot(lhs[k % j], mixed(k % j)) for k in ('r%d', 'c%d')]
            p[j] = dp if p[j] is None else dp + p[j]
            q[j] = dq if q[j] is None else dq + q[j]

    for a in range(n):
        for b in range(a + 1, n):
            start(a)
            start(b)
            d = t[a] - t[b]
            m6 = _dot(lhs[b, a, 0], plain(b, a))
            m7 = _dot(lhs[a, b, 0], plain(a, b))
            m = _dot(lhs[a, b], mixed((a, b))) + (m6 + m7)
            if scaled:
                q[a], q[b] = q[a] - (-d) * m6, q[b] - d * m7
                p[a], p[b] = m + p[a], m + p[b]
            else:
                q[a], q[b] = m6 + q[a], q[b] - m7
                m = m * (-1.0 / d) if d != -1.0 else m
                p[a], p[b] = p[a] - m, p[b] - m
    return p, q


def _star_result(n, p, q):
    return [jnp.concatenate([p[j], q[j] - _T[n][j] * p[j] if _T[n][j] else q[j]], axis=0)
            for j in range(n)]


_PLAN = (
    ((3, 7, 9, 13, 17), (0, 4, 10, 14), (1, 9, 10)),
    ((3, 6, 9, 11, 14), (0, 4, 8, 12), (2, 9, 10)),
    ((3, 6, 9, 11, 14), (0, 4, 8, 12), (2, 9, 10)),
    ((3, 6, 9, 11, 14), (0, 4, 8, 12), (2, 5, 6)),
)


def _segment(h, hk, wqv, wk, wob, wsum, fix_qv, fix_k, fix_o, step):
    ys = {p: [None] * 3 for p in range(NP)}
    ss, ps, pvs, os_ = {}, {}, {}, {}
    hb = h.astype(BF16)

    def summed(slab, g, name):
        return wsum[64 * slab:64 * slab + 64, pl.ds(128 * _star_slot(g, name), 128)]

    def keys(n):
        k = _dot(hk, _unpack(wk[n]))
        for e in range(4):
            ys[4 * n + e][1] = fix_k(4 * n + e, k[:, e * PW:(e + 1) * PW])

    def proj(p):
        def w(lo, hi):
            return _unpack(jnp.concatenate(
                [wqv[2 * i + p // 8, lo:hi, pl.ds(p % 8 * PW, PW)] for i in range(2)], axis=1))
        if p == 0:
            y = _dot(hb[:, 0:512], w(0, 256))
            y = _dot(hb[:, 512:], w(256, D // 2)) + y
        else:
            y = _dot(hb, w(0, D // 2))
        for i in range(2):
            ys[p][2 * i] = fix_qv(p, i, y[:, i * PW:(i + 1) * PW])

    def wide_proj(half, g, i, lhs, tiles):
        slab, (t0, n) = 2 * i + half, _STARS[g]
        if n == 4:
            tail = _dot(hb[:, 512:], _unpack(wqv[slab, 256:, 128 * t0:]))
        out = _star_result(n, *_star_apply(
            n, lhs[n],
            lambda j, l: _unpack(wqv[slab, 64 * j:64 * j + 64, pl.ds(128 * (t0 + l), 128)]),
            lambda name: _unpack(summed(slab, g, name)), False))
        for l, y in enumerate(out):
            tiles[t0 + l] = y + tail[:, 128 * l:128 * l + 128] if n == 4 else y
        for e in range(8):
            if all(3 * e + k in tiles for k in range(3)):
                ys[8 * half + e][2 * i] = fix_qv(8 * half + e, i, jnp.concatenate(
                    [tiles.pop(3 * e + k) for k in range(3)], axis=1))

    def weights(c, i, which):
        if i < 2:
            return _own_weights(ys[2 * c + i][which], i)
        return _others(ys[2 * c][which], ys[2 * c + 1][which], True)

    def score_round(n):
        for c, i in (divmod(j, 3) for j in range(4 * n, 4 * n + 4)):
            if i < 2:
                q = jnp.concatenate(_tiles(ys[2 * c + i][0], i)[0:2], axis=0).astype(BF16)
            else:
                q = _others(ys[2 * c][0], ys[2 * c + 1][0], False)
            ss[c, i] = _dot_nt(q, weights(c, i, 1))
            if i == 2:
                ps[c] = _softmax3([ss.pop((c, k)) for k in range(3)])

    def pv_round(n):
        for c, i in (divmod(j, 3) for j in range(4 * n, 4 * n + 4)):
            pvs[c, i] = _dot(ps[c][i], weights(c, i, 2))
            if i == 2:
                o0, o1, o2 = [pvs.pop((c, k)) for k in range(3)]
                os_[2 * c] = fix_o(2 * c, jnp.concatenate(
                    [o0[L:, :], o0[0:L, :], o2[L:, :]], axis=1))
                os_[2 * c + 1] = fix_o(2 * c + 1, jnp.concatenate(
                    [o2[0:L, :], o1[0:L, :], o1[L:, :]], axis=1))

    def slot(n):
        if n >= 2:
            pv_round(n - 2)
        if n < 6:
            score_round(n)

    def oproj(lo, hi, r):
        o = jnp.concatenate([os_.pop(p) for p in range(lo, hi)], axis=1).astype(BF16)
        y = _dot(o, _unpack(wob[lo * DH:hi * DH, :]))
        return y if r is None else y + r

    def wide_oproj(stars, r):
        def o_tile(t):
            return os_[t // 3][:, 128 * (t % 3):128 * (t % 3) + 128]

        for n in (4, 5):
            sel = [divmod(x, 5) for x in stars if _STARS[x % 5][1] == n]
            if not sel:
                continue
            t0 = [24 * half + _STARS[g][0] for half, g in sel]
            if n == 4:
                ts = [t + j for t in t0 for j in range(4)]
                y = _dot(jnp.concatenate([o_tile(t) for t in ts], axis=1).astype(BF16),
                         _unpack(jnp.concatenate(
                             [wob[64 * t:64 * t + 64, 512:] for t in ts], axis=0)))
                r[0] = y + r[0] if 0 in r else y
            r[n] = _star_apply(
                n, _star_lhs(n, lambda i, j: jnp.concatenate(
                    [o_tile(t + j)[32 * i:32 * i + 32] for t in t0], axis=1), True),
                lambda j, l: _unpack(jnp.concatenate(
                    [wob[pl.ds(64 * (t + j), 64), 128 * l:128 * l + 128] for t in t0], axis=0)),
                lambda name: _unpack(jnp.concatenate(
                    [summed(4 + half, g, name) for half, g in sel], axis=0)), True, r.get(n))
        return r

    after, kat, (o1, o2, o3) = _PLAN[step]
    if step == 0:
        lhs = {n: _star_lhs(n, lambda i, j: h[32 * i:32 * i + 32, 128 * j:128 * j + 128], False)
               for n in (4, 5)}
        tiles = {}
    for unit in range(20 if step == 0 else NP):
        if step == 0:
            half, g, i = unit // 10, unit % 10 // 2, unit % 2
            wide_proj(half, g, i, lhs, tiles.setdefault((half, i), {}))
        else:
            proj(unit)
        if unit in kat:
            keys(kat.index(unit))
        if unit in after:
            slot(after.index(unit))
    if step == 3:
        r = wide_oproj(range(0, o1), {})
        slot(5)
        r = wide_oproj(range(o1, o2), r)
        slot(6)
        slot(7)
        r = wide_oproj(range(o2, o3), r)
        r = wide_oproj(range(o3, 10), r)
        return jnp.concatenate(
            [x + y for x, y in zip(_star_result(5, *r[5]), _star_result(4, *r[4]) + [r[0]])],
            axis=1)
    r = oproj(0, o1, None) if o1 else None
    slot(5)
    r = oproj(o1, o2, r)
    slot(6)
    slot(7)
    r = oproj(o2, o3, r)
    return oproj(o3, NP, r)


def _kernel(x_hbm, wqkv_hbm, wphi_hbm, woa_hbm, mem0_hbm,
            wq_hbm, wk_hbm, wv_hbm, wo_hbm,
            out_hbm,
            xio, wqkv, wphi, woa, mem0, xres, xa, xl, xb, bds, wat, phq, phk, kvacc, kvs,
            wraw, wqv, wk, wob, wsum, xe, ke, ysave, osave, rsave, sem_in, sem_out):
    nsub = TN // 128
    na = S // TA
    asub = TA // 128
    nb = S // TB

    def rows(j, n):
        return pl.ds(j * n if isinstance(j, int) else pl.multiple_of(j * n, n), n)

    def x_copy(j):
        if isinstance(j, int) and j < 0:
            r = pl.ds(0, 256)
        elif isinstance(j, int) and j == na - 1:
            r = pl.ds(S - TA + 256, TA - 256)
        else:
            r = pl.ds(j * TA + 256 if isinstance(j, int)
                      else pl.multiple_of(j * TA + 256, 256), TA)
        return pltpu.make_async_copy(x_hbm.at[r, :], xio.at[r, :], sem_in.at[9 + j])

    def w_copy(c):
        src = (wq_hbm, wv_hbm, wo_hbm, wk_hbm)[c // 2 if isinstance(c, int) else 0]
        return pltpu.make_async_copy(src.at[c % 2], wraw.at[c], sem_in.at[9 + na + c])

    def wa_copy(c):
        r = pl.ds(512, 128) if isinstance(c, int) and c == 2 else rows(c, 256)
        return pltpu.make_async_copy(wqkv_hbm.at[r, :], wqkv.at[r, :], sem_in.at[3 + c])

    def out_copy(i):
        return pltpu.make_async_copy(xio.at[rows(i, TB), :],
                                     out_hbm.at[rows(i, TB), :], sem_out.at[0])

    wphi_copy = pltpu.make_async_copy(wphi_hbm, wphi, sem_in.at[0])
    woa_copy = pltpu.make_async_copy(woa_hbm, woa, sem_in.at[1])
    mem0_copy = pltpu.make_async_copy(mem0_hbm, mem0, sem_in.at[2])
    order = [wphi_copy, wa_copy(0), wa_copy(1), x_copy(-1), wa_copy(2)]
    order += [x_copy(j) for j in range(na)] + [woa_copy, mem0_copy]
    order += [w_copy(c) for c in (6, 7, 0, 4, 1, 2, 5, 3)]
    for c in order:
        c.start()

    def strassen_rhs(x0, x1):
        b11, b12 = [jnp.concatenate([x[:, 0:128], x[:, 256:384]], axis=1) for x in (x0, x1)]
        b21, b22 = [jnp.concatenate([x[:, 128:256], x[:, 384:512]], axis=1) for x in (x0, x1)]
        ops = [b11 + b22, b11, b12 - b22, b21 - b11, b22, b11 + b12, b21 + b22,
               x0[:, 512:], x1[:, 512:]]
        return _pack(jnp.concatenate(ops, axis=1).astype(BF16))

    def load_x(t, first):
        x = xio[rows(t, 256), :].astype(F32)
        if first is not True:
            x = jnp.where(first, x, xres[rows(t, 256), :])
        xres[rows(t, 256), :] = x
        return x

    wphi_copy.wait()
    cphi = jnp.zeros((FA, D), F32)
    hh = lax.broadcasted_iota(jnp.int32, (HA, D), 0) * FA
    jj = lax.broadcasted_iota(jnp.int32, (HA, D), 1)
    for d in range(FA):
        cphi = _dot(wphi[d], jnp.where(jj == hh + d, 1.0, 0.0).astype(BF16)) + cphi
    cb = jnp.concatenate(
        [jnp.broadcast_to(cphi[f:f + 1, :], (8, D)) for f in range(FA)], axis=0)
    for g in range(GA):
        row = lax.broadcasted_iota(jnp.int32, (GR, 256), 0)
        col = lax.broadcasted_iota(jnp.int32, (GR, 256), 1) + 128 * g
        lo = (8 * g + (row & 7)) * FA
        bds[g] = _pack(jnp.where(jnp.logical_and(col >= lo, col < lo + FA),
                                 cb[:, 128 * g:128 * g + 256], 0.0).astype(BF16))

    def folded(rr):
        out = [[], [], []]
        for g in range(GA):
            ws = []
            for i in range(2):
                c0 = i * D + 128 * g
                w = _dot_nt(_unpack(bds[g]), wqkv[rr, c0:c0 + 256]).reshape(FA, 8, 128)
                ws.append(((w[1:] - w[0:1]) * LOG2E).reshape(GR - 8, 128))
            out[0].append(jnp.concatenate([ws[1], ws[0][GR - 16:, :]], axis=0))
            out[1].append(ws[0][0:GR - 16, :])
        wvt = wqkv[rr, 2 * D:3 * D].T.astype(F32)
        out[2] = [wvt[g * GR:(g + 1) * GR, :] for g in range(GA)]
        return out

    def fold(c, _):
        wa_copy(c).wait()
        wa, wb = folded(rows(2 * c, 128)), folded(rows(2 * c + 1, 128))
        for i in range(3):
            for p in range(2):
                a11, a12, a21, a22 = wa[i][2 * p], wb[i][2 * p], wa[i][2 * p + 1], wb[i][2 * p + 1]
                ops = [a11 + a22, a21 + a22, a11, a22, a11 + a12, a21 - a11, a12 - a22]
                for m, w in enumerate(ops):
                    wat[2 * i + p, m, 0:w.shape[0] // 2, rows(c, 128)] = _pack(w.astype(BF16))
        return 0

    lax.fori_loop(0, 2, fold, 0)
    x_copy(-1).wait()
    wa_copy(2).wait()
    x = _layernorm(load_x(0, True))
    xa[...] = strassen_rhs(x[0:128], x[128:])
    for i, ws in enumerate(folded(pl.ds(512, 128))):
        for g, w in enumerate(ws):
            wat[2 * i + g // 2, 7, 0:w.shape[0] // 2, rows(g % 2, 128)] = _pack(w.astype(BF16))

    def pair_rows(ph, q, t0, n):
        return _unpack(jnp.concatenate(
            [ph[t0 + u, rows(q, 2 * FA), :] for u in range(n)], axis=1))

    def a1(first, j, _):
        @pl.when(jnp.logical_and(first, j < na - 1))
        def _():
            x_copy(j).wait()

        @pl.when(jnp.logical_and(first, j == na - 1))
        def _():
            x_copy(na - 1).wait()

        def features(ph, t, g, y):
            for f, w in enumerate(_feature_map(y)):
                ph[t, pl.ds(GR * g + f, 8, stride=FA), :] = w

        def tail(n, xs, g, u):
            nr = GR // 2 - 8 if n // 2 == 1 else GR // 2
            return _dot_nt(_unpack(wat[n, 7, 0:nr, 128 * g:128 * (g + 1)]),
                           xs[:, 1792 + 128 * u:1920 + 128 * u])

        def a_dots(n, xs, emit, tie, t10):
            nr = GR // 2 - 8 if n // 2 == 1 else GR // 2
            p = n % 2

            def prod(m):
                return _dot_nt(_unpack(tie(wat[n, m, 0:nr, :])), xs[:, 256 * m:256 * (m + 1)])

            m2, m4 = prod(1), prod(3)
            emit(2 * p + 1, 0, m4 + (m2 - (-t10)))
            t01 = tail(n, xs, 0, 1)
            m3, m5 = prod(2), prod(4)
            emit(2 * p, 1, m5 + (m3 - (-t01)))
            m1 = prod(0)
            c22 = prod(5) + (m1 + (m3 - m2))
            emit(2 * p + 1, 1, tail(n, xs, 1, 1) + c22)
            t10 = tail(n + 1, xs, 1, 0) if n < 5 else None
            c11 = tail(n, xs, 0, 0) + (m1 + (m4 - m5))
            emit(2 * p, 0, prod(6) + c11)
            return t10

        vs = {}
        cur = xa[...]
        dl = (3, 8, 13, 30, 33, 36, 39, 41)
        for u in range(0, asub, 2):
            t = j * (asub // 2) + u // 2
            xs = _unpack(cur)
            tn = t + 1
            x = load_x(tn if u + 2 < asub else jnp.minimum(tn, (na - 1) * (asub // 2)), first)
            rest, seen, nxt = {}, [], []

            def tie(w):
                seen.append(0)
                if len(seen) - 1 not in dl:
                    return w
                n = len(nxt)
                nxt.append(strassen_rhs(*[
                    _layernorm(x[128 * e + 16 * n:128 * e + 16 * n + 16, :]) for e in range(2)]))
                z = jnp.concatenate(
                    [nxt[n][:, 256 * c:256 * (c + 1)] for c in range(8)], axis=0)
                return jnp.concatenate([jnp.where(j < 0, z, w[0:64, :]), w[64:, :]], axis=0)

            def emit_k(g, e, y):
                features(phk, u + e, g, y[0:GR - 8, :])
                rest[g, e] = y[GR - 8:, :]

            def emit_q(g, e, y):
                features(phq, 2 * t + e, g, jnp.concatenate([y, rest[g, e]], axis=0))

            def emit_v(g, e, y):
                for q in range(4):
                    vs[4 * g + q, u + e] = y[40 * q:40 * q + 40, :]

            t10 = tail(0, xs, 1, 0)
            for n in range(6):
                t10 = a_dots(n, xs, (emit_k, emit_q, emit_v)[n // 2], tie, t10)
            cur = jnp.concatenate(nxt, axis=0)
        xa[...] = cur
        row = lax.broadcasted_iota(jnp.int32, (2 * VR, 4 * FA), 0)
        col = lax.broadcasted_iota(jnp.int32, (2 * VR, 4 * FA), 1)
        split = jnp.where(row < 2 * FA, FA, 2 * FA + 4)
        same = (row >= split) == (col >= 2 * FA)
        for q in range(PA):
            v = jnp.concatenate([vs[q, u] for u in range(asub)], axis=1)
            v = jnp.concatenate([v, jnp.ones((8, TA), F32)], axis=0)
            kv = _dot_nt(v.astype(BF16), pair_rows(phk, q, 0, asub))
            kv = kv + jnp.where(j == 0, 0.0, kvacc[q])
            kvacc[q] = kv
            kvs[q] = _pack(jnp.where(same, kv, 0.0).astype(BF16))
        return 0

    def attend(j):
        low = lax.broadcasted_iota(jnp.int32, (8, TN), 0) < 4
        os_ = []
        for q in range(PA):
            nd = _dot(_unpack(kvs[q]), pair_rows(phq, q, j * nsub, nsub))
            rab = 1.0 / (nd[40:48, :] + 1e-6)
            rba = pltpu.roll(rab, 4, 0)
            ra = jnp.where(low, rab, rba)
            rb = jnp.where(low, rba, rab)
            os_.append(nd[0:40, :] * jnp.concatenate([ra, ra, rab, rb, rb], axis=0))
        return _pack(jnp.concatenate(os_, axis=0).astype(BF16).T)

    def project(j, o, slot):
        ns = TN // SEG
        xs = []
        r = rows(j, TN)
        old, new = xres[r, :], {}
        for part in ((1, 2), (0, 3)):
            grp = [b + k for b in range(0, TN // 16, 4) for k in part]
            oo = jnp.concatenate([o[8 * g:8 * g + 8, :] for g in grp], axis=0)
            x = _dot(_unpack(oo), woa[...]) + jnp.concatenate(
                [old[16 * g:16 * g + 16, :] for g in grp], axis=0)
            for n, g in enumerate(grp):
                new[g] = x[16 * n:16 * n + 16, :]
            xs.append(x)
        xres[r, :] = jnp.concatenate([new[g] for g in range(TN // 16)], axis=0)
        for s in range(ns):
            x = xs[0][16 * s + 8 - 8 * (s % 2):16 * s + 16 - 8 * (s % 2), :]
            x = _layernorm(x)
            x = x - x[KE:KE + 1, :]
            for c in range(D // 128):
                xe[c, pl.ds((slot * ns + s) * KE, 8), :] = x[:, 128 * c:128 * (c + 1)]

    def extra_keys(seg, p):
        k = jnp.concatenate(
            [ke[seg // 16, 3 * p + c, pl.ds((seg % 16) * KE, 8), :] for c in range(3)], axis=1)
        return jnp.where(lax.broadcasted_iota(jnp.int32, (8, PW), 0) < KE, k, 0.0)

    def b_residual(i):
        r = rows(i, TB)
        x = xres[r, :] + rsave[...]
        xres[r, :] = x
        xio[r, :] = x.astype(BF16)
        return x

    def b_finish(i):
        xn = _layernorm(b_residual(i))
        xl[rows(jnp.minimum(i, 2), TB), :] = xn
        return xn

    def b_tile(mem, xn, i, side):
        for u in range(4):
            t0 = u * SEG
            late = u % 2 == 0
            ext = [SEG * v + (24 if v % 2 == 0 else 0) for v in range(4)]

            def place(y, z):
                return jnp.concatenate([y, z] if late else [y[0:M], z, y[M:]], axis=0)

            def fix_qv(p, kind, y):
                cols = pl.ds((2 * p + kind) * PW, PW)
                if u == 0:
                    ysave[:, cols] = y[L:, :]
                    y = y[0:L, :]
                else:
                    y = place(y, ysave[8 * u - 8:8 * u, cols])
                if not late:
                    return y
                r0 = 64 * u + 8 * p
                tie = jnp.where(i < 0, side[r0:r0 + 8, 256 * kind:256 * kind + PW], y[0:M, :])
                return jnp.concatenate([tie, y[M:, :]], axis=0)

            def fix_k(p, k):
                return place(k, extra_keys(4 * i + u, p))

            def fix_o(p, o):
                cols = slice(p * PW, (p + 1) * PW)
                if u == 3:
                    return jnp.concatenate([o, osave[:, cols]], axis=0)
                osave[8 * u:8 * u + 8, cols] = o[32:L, :]
                return o[0:32, :]

            h = jnp.concatenate(
                [mem, xn[t0:t0 + 24, :] if late else xn[t0 + 8:t0 + SEG, :]], axis=0)
            hk = (h - xn[ext[u] + KE:ext[u] + KE + 1, :]).astype(BF16)
            if u == 0:
                h = jnp.concatenate([h] + [xn[e:e + 8, :] for e in ext], axis=0)
            r = _segment(h, hk, wqv, wk, wob, wsum, fix_qv, fix_k, fix_o, u)
            mem = r[0:M, :]
            if u < 3:
                rsave[t0:t0 + 24, :] = r[M:, :]
            else:
                rsave[t0:t0 + SEG, :] = r[M:L, :]
                for v in range(3):
                    rsave[SEG * v + 24:SEG * v + SEG, :] = r[L + 8 * v:L + 8 * v + 8, :]
        return mem

    def layer(l, _):
        def wait_first(copies):
            @pl.when(l == 0)
            def _():
                for c in copies:
                    c.wait()

        with jax.named_scope("a1"):
            lax.fori_loop(0, na, functools.partial(a1, l == 0), 0)

        def a2(n, _):
            for m, cs in enumerate(((6, 7, 0, 4), (1,), (2, 5), (3,))):
                @pl.when(jnp.logical_and(l == 0, n == m))
                def _():
                    for c in cs:
                        w_copy(c).wait()

            ty, half = n % 2, n // 2
            o0 = attend(2 * n)
            o1 = attend(2 * n + 1)

            def sample(w):
                z = [w[64 * a + 56:64 * a + 64, :] for a in range(D // 128)]
                out = []
                for y in z:
                    acc = y[:, 0:128]
                    for c in range(1, y.shape[1] // 128):
                        acc = acc | y[:, 128 * c:128 * (c + 1)]
                    out.append(acc)
                return jnp.concatenate(out, axis=1)

            mr = 16 * KE

            def side(job):
                w = _pack(wraw[n, rows(int(job), 2 * PW), :].T)
                wqv[n, :, rows(int(job), 2 * PW)] = w
                return sample(w)

            for job in '01':
                o1 = jnp.concatenate([o1[0:8, :], jnp.where(n < 0, side(job), o1[8:16, :]),
                                      o1[16:, :]], axis=0)
            project(2 * n, o0, 0)
            ties = [pltpu.bitcast(side(job), F32) for job in '23']
            project(2 * n + 1, o1, 1)
            x = jnp.concatenate([xe[c, 0:mr, :] for c in range(D // 128)], axis=1)
            for tie in ties:
                x = jnp.concatenate([jnp.where(n < 0, tie, x[0:8, :]), x[8:, :]], axis=0)
            x = x.astype(BF16)
            r = rows(n, TB // NW)
            xb[r, :] = _layernorm(xres[r, :])
            rsave[r, :] = jnp.zeros((TB // NW, D), F32)

            def view(ref, start, size, align):
                return ref.at[pl.ds(pl.multiple_of(start, align), size)]

            wo_src = view(wraw.at[4 + half], 64 * ty, HD // 2 - 64, 64)
            wo_dst = view(wob, QW * half + 32 * ty, QW - 32, 32)
            wk_src = view(wraw.at[6 + half], QW * ty, QW, QW)
            sum_dst = view(wsum, 64 * n, 64, 64), view(wsum, 256 + 32 * n, 32, 32)

            def wo_rows(t, rr):
                return _pack(wo_src[rows(8 * t + rr, 16), :])

            def sums(is_o, g, j, rr, tie):
                t0, sz = _STARS[g]
                names = _star_sums(sz)[j]
                if is_o:
                    row = jnp.where(n < 0, jnp.concatenate([tie] * 5, axis=1), wo_rows(t0 + j, rr))
                    wo_dst[rows(8 * (t0 + j) + rr, 8), :] = row
                val = {}
                for x, y in [(j, k) for k in range(sz)] + [(k, j) for k in range(sz) if k != j]:
                    if is_o and x == j:
                        w = row[:, 128 * y:128 * y + 128]
                    elif is_o and x < j:
                        w = jnp.where(n < 0, tie, wo_dst[rows(8 * (t0 + x) + rr, 8), rows(y, 128)])
                    else:
                        w = jnp.where(n < 0, tie, wo_rows(t0 + x, rr)[:, 128 * y:128 * y + 128] if is_o
                                      else wqv[n, rows(8 * x + rr, 8), rows(t0 + y, 128)])
                    val[x, y] = _unpack(w).astype(F32)
                others = [k for k in range(sz) if k != j]
                out = [functools.reduce(lambda z, k: z - val[j, k], others, val[j, j]),
                       functools.reduce(lambda z, k: z + val[k, j], others, val[j, j])]
                out += [val[x, y] + val[y, x] for x, y in names[2:]]
                sum_dst[is_o][rows(rr, 8),
                              pl.ds(128 * _star_slot(g, names[0]), 128 * len(names))] = _pack(
                    jnp.concatenate(out, axis=1).astype(BF16))

            def k_tiles(t, c, tie):
                w = _pack(wk_src[rows(t, 256), rows(c, 128)])
                w = jnp.concatenate([jnp.where(n < 0, tie, w[0:8, :]), w[8:64, :],
                                     jnp.where(n < 0, tie, w[64:72, :]), w[72:, :]], axis=0)
                wk[n, rows(c, 64), rows(t, 256)] = _pack(_unpack(w).T)

            kjobs = [functools.partial(k_tiles, t, c) for t in range(6) for c in range(5)]
            todo = []
            for g in range(5):
                for j in range(_STARS[g][1]):
                    for rr in range(4):
                        if len(todo) % 10 < 3:
                            todo += kjobs[-1:]
                            del kjobs[-1:]
                        todo += [functools.partial(sums, False, g, j, 2 * rr),
                                 functools.partial(sums, True, g, j, rr),
                                 functools.partial(sums, False, g, j, 2 * rr + 1)]
            assert not kjobs
            left = [48]

            def emit(t, k):
                ke[n, t, 0:mr, :] = k
                left[0] -= 1
                if left[0] < 48 - 2:
                    m = -(-len(todo) // (left[0] + 1))
                    for g in range(m):
                        g = 8 * (14 * g // m)
                        todo.pop(0)(pltpu.bitcast(k[g:g + 8, :], U32))

            for v in range(HD // 256):
                k = _dot_nt(x, wraw[6 + v // 12, rows(v % 12, 256), :])
                emit(2 * v, k[:, 0:128])
                emit(2 * v + 1, k[:, 128:])
            return 0

        wait_first([woa_copy, mem0_copy])
        with jax.named_scope("a2"):
            lax.fori_loop(0, NW, a2, 0)

        def b_step(i, mem):
            xn = xb[...]
            side = b_finish(jnp.maximum(i - 1, 0))
            nxt = _layernorm(xres[rows(jnp.minimum(i + 1, nb - 1), TB), :])
            xb[...] = nxt
            side = jnp.concatenate([side, nxt], axis=0)
            mem = b_tile(mem, xn, i, side)

            @pl.when(jnp.logical_and(l == 1, i >= 1))
            def _():
                out_copy(i - 1).start()
            return mem

        with jax.named_scope("b"):
            lax.fori_loop(0, nb, b_step, mem0[...].astype(F32))

        b_residual(nb - 1)

        @pl.when(l == 0)
        def _():
            xa[...] = strassen_rhs(xl[0:128, :], xl[128:256, :])
        return 0

    lax.fori_loop(0, 2, layer, 0)
    out_copy(nb - 1).start()
    pltpu.make_async_copy(xio, out_hbm, sem_out.at[0]).wait()


@jax.jit
def pallas_interleave_layers__linear_kernel_hedgehog__memory_aug_recurrent_mem_tr__prompt_kernel(
    A_x, A_wqkv, A_w_phi, A_wo, B_x, B_mem0, B_Wq, B_Wk, B_Wv, B_Wo, B_seg_len,
):
    del B_x
    del B_seg_len
    x = A_x.reshape(S, D)
    wphi = A_w_phi.transpose(1, 2, 0)
    mem0 = B_mem0.reshape(M, D)
    wq, wk, wv = (w.transpose(1, 2, 0).reshape(2, HD // 2, D) for w in (B_Wq, B_Wk, B_Wv))
    wo = B_Wo.reshape(2, HD // 2, D)
    hbm = pl.BlockSpec(memory_space=pl.ANY)
    out = pl.pallas_call(
        _kernel,
        out_shape=jax.ShapeDtypeStruct((S, D), A_x.dtype),
        in_specs=[hbm] * 9,
        out_specs=hbm,
        scratch_shapes=[
            pltpu.VMEM((S, D), BF16),
            pltpu.VMEM((D, 3 * D), BF16),
            pltpu.VMEM((FA, FA, HA), BF16),
            pltpu.VMEM((D, D), BF16),
            pltpu.VMEM((M, D), BF16),
            pltpu.VMEM((S, D), F32),
            pltpu.VMEM((64, 2048), U32),
            pltpu.VMEM((3 * TB, D), F32),
            pltpu.VMEM((TB, D), F32),
            pltpu.VMEM((GA, GR // 2, 256), U32),
            pltpu.VMEM((6, 8, GR // 2, 256), U32),
            pltpu.VMEM((S // 128, D, 128), U32),
            pltpu.VMEM((TA // 128, D, 128), U32),
            pltpu.VMEM((PA, 2 * VR, 4 * FA), F32),
            pltpu.VMEM((PA, VR, 4 * FA), U32),
            pltpu.VMEM((8, HD // 2, D), BF16),
            pltpu.VMEM((4, D // 2, HD // 2), U32),
            pltpu.VMEM((NW, D // 2, QW), U32),
            pltpu.VMEM((HD // 2, D), U32),
            pltpu.VMEM((6 * 64, NS * 128), U32),
            pltpu.VMEM((D // 128, 16 * KE + 8, 128), F32),
            pltpu.VMEM((NW, HD // 128, 16 * KE + 8, 128), F32),
            pltpu.VMEM((24, 2 * HD), F32),
            pltpu.VMEM((24, HD), F32),
            pltpu.VMEM((TB, D), F32),
            pltpu.SemaphoreType.DMA((17 + S // TA,)),
            pltpu.SemaphoreType.DMA((1,)),
        ],
        compiler_params=pltpu.CompilerParams(vmem_limit_bytes=128 * 1024 * 1024,
                                             disable_bounds_checks=True,
                                             disable_semaphore_checks=True),
    )(x, A_wqkv, wphi, A_wo, mem0, wq, wk, wv, wo)
    return out.reshape(1, S, D)
```

```python
import functools

import jax
import jax.numpy as jnp
from jax import lax
import jax.experimental.pallas as pl
import jax.experimental.pallas.tpu as pltpu

F32 = jnp.float32
BF16 = jnp.bfloat16
U32 = jnp.uint32

S = 2048
D = 640
HA = 32
FA = 20
GA = 4
GR = 8 * FA
VR = 24
PA = HA // 2
TN = 256
TA = 512
HB = 32
DH = 192
HD = HB * DH
M = 8
SEG = 32
L = M + SEG
PW = 2 * DH
NP = HB // 2
TB = 128
NW = 4
QW = HD // NW
KE = 7

NT = (((1,), (1,)), ((), ()))
LOG2E = 1.4426950408889634
HALF_ULP = 0.0040612


def _dot(a, b):
    return jnp.dot(a, b, preferred_element_type=F32)


def _dot_nt(a, b):
    return lax.dot_general(a, b, NT, preferred_element_type=F32)


def _pack(a):
    return pltpu.bitcast(a, U32)


def _unpack(a):
    return pltpu.bitcast(a, BF16)


def _interleave(a, b):
    lo = lax.bitcast_convert_type(a, U32) >> 16
    hi = lax.bitcast_convert_type(b, U32) & jnp.uint32(0xFFFF0000)
    return lo | hi


def _recip(x):
    r = pl.reciprocal(x, approx=True)
    return r * (2.0 - x * r)


def _layernorm(x):
    m = jnp.mean(x, axis=-1, keepdims=True)
    c = x - m
    v = jnp.mean(c * c, axis=-1, keepdims=True)
    return c * lax.rsqrt(v + 1e-5)


def _feature_map(p):
    t = p.shape[-1]
    p3 = jnp.concatenate([jnp.zeros((8, t), F32), p], axis=0).reshape(FA, 8, t)
    mx = jnp.max(p3, axis=0)
    mn = jnp.min(p3, axis=0)
    sp, sn = jnp.exp2(p3[0] - mx), jnp.exp2(mn - p3[0])
    for f in range(1, FA):
        sp, sn = sp + jnp.exp2(p3[f] - mx), sn + jnp.exp2(mn - p3[f])
    lp = (mx - HALF_ULP) + jnp.log2(sp)
    ln = (mn + HALF_ULP) - jnp.log2(sn)
    return [_interleave(jnp.exp2(p3[f] - lp), jnp.exp2(ln - p3[f])) for f in range(FA)]


def _tiles(a, odd):
    t0, t1, t2 = a[:, 0:128], a[:, 128:256], a[:, 256:384]
    return (t1, t2, t0) if odd else (t1, t0, t2)


def _own_weights(a, odd):
    lane = lax.broadcasted_iota(jnp.int32, (L, 128), 1)
    mid, own, _ = _tiles(a, odd)
    return jnp.concatenate(
        [jnp.where(lane < 64, mid, 0.0), jnp.where(lane < 64, 0.0, mid), own,
         jnp.zeros((128 - 3 * L, 128), F32)], axis=0).astype(BF16)


def _others(even, odd, pad):
    parts = [_tiles(odd, 1)[2], _tiles(even, 0)[2]]
    if pad:
        parts.append(jnp.zeros((128 - 2 * L, 128), F32))
    return jnp.concatenate(parts, axis=0).astype(BF16)


def _softmax3(s3):
    row = lax.broadcasted_iota(jnp.int32, (L, 128), 0)
    col = lax.broadcasted_iota(jnp.int32, (L, 128), 1)
    first = col < L
    second = jnp.logical_and(col >= L, col < 2 * L)
    key = jnp.where(first, col, col - L)
    valid = jnp.logical_or(row < M, row >= key)
    out, other = [], []
    for odd in range(2):
        own = pltpu.roll(s3[odd][L:, :], 128 - L if odd else 128 - 2 * L, 1)
        s = (jnp.where(first, s3[2][0:L, :], own) if odd
             else jnp.where(first, own, s3[2][L:, :]))
        s = jnp.where(valid, (s + s3[odd][0:L, :]) * (DH ** -0.5), -1e9)
        m0 = jnp.max(jnp.where(first, s, -jnp.inf), axis=-1, keepdims=True)
        m1 = jnp.max(jnp.where(second, s, -jnp.inf), axis=-1, keepdims=True)
        e = jnp.exp(s - jnp.where(first, m0, m1))
        e0 = jnp.where(first, e, 0.0)
        e1 = jnp.where(second, e, 0.0)
        p0 = e0 * _recip(jnp.sum(e0, axis=-1, keepdims=True))
        p1 = e1 * _recip(jnp.sum(e1, axis=-1, keepdims=True))
        own = pltpu.roll(p1, L, 1) if odd else pltpu.roll(p0, 2 * L, 1)
        out.append(jnp.concatenate([p0 + p1, own], axis=0))
        other.append(p0 if odd else p1)
    out.append(jnp.concatenate([other[1], other[0]], axis=0))
    return _pack(jnp.concatenate(out, axis=1).astype(BF16))


_T = {5: (-1.5, -0.5, 0.0, 0.5, 1.5), 4: (-1.25, -0.25, 0.25, 1.25)}
_STARS = tuple((5 * g, 5 if g < 4 else 4) for g in range(5))


def _star_sums(n):
    own = {j: [] for j in range(n)}
    for a in range(n):
        for b in range(a + 1, n):
            own[a if (b - a) % 2 else b].append((a, b))
    return [['r%d' % j, 'c%d' % j] + own[j] for j in range(n)]


def _star_slot(g, name):
    return 20 * g + [x for grp in _star_sums(_STARS[g][1]) for x in grp].index(name)


NS = 94


def _star_lhs(n, get, scaled):
    t = _T[n]
    f = [get(0, j) for j in range(n)]
    g = [get(1, j) + t[j] * f[j] if t[j] else get(1, j) for j in range(n)]
    out = {'r%d' % j: f[j] for j in range(n)}
    out.update({'c%d' % j: g[j] for j in range(n)})
    for a in range(n):
        for b in range(a + 1, n):
            d = t[a] - t[b]
            if scaled:
                l = (g[a] - g[b]) * (1.0 / d)
                out[a, b], out[b, a, 0], out[a, b, 0] = l, f[b] - l, f[a] - l
            else:
                l = g[a] - g[b]
                out[a, b], out[b, a, 0], out[a, b, 0] = l, d * f[b] - l, d * f[a] - l
    return out


def _star_apply(n, lhs, plain, mixed, scaled, acc=None):
    t = _T[n]
    p, q = ([None] * n, [None] * n) if acc is None else (list(acc[0]), list(acc[1]))
    started = set()

    def start(j):
        if j not in started:
            started.add(j)
            dp, dq = [_dot(lhs(k % j), mixed(k % j)) for k in ('r%d', 'c%d')]
            p[j] = dp if p[j] is None else dp + p[j]
            q[j] = dq if q[j] is None else dq + q[j]

    for a in range(n):
        for b in range(a + 1, n):
            start(a)
            start(b)
            d = t[a] - t[b]
            m6 = _dot(lhs((b, a, 0)), plain(b, a))
            m7 = _dot(lhs((a, b, 0)), plain(a, b))
            m = _dot(lhs((a, b)), mixed((a, b))) + (m6 + m7)
            if scaled:
                q[a], q[b] = q[a] - (-d) * m6, q[b] - d * m7
                p[a], p[b] = m + p[a], m + p[b]
            else:
                q[a], q[b] = m6 + q[a], q[b] - m7
                m = m * (-1.0 / d) if d != -1.0 else m
                p[a], p[b] = p[a] - m, p[b] - m
    return p, q


def _star_result(n, p, q):
    return [jnp.concatenate([p[j], q[j] - _T[n][j] * p[j] if _T[n][j] else q[j]], axis=0)
            for j in range(n)]


_PLAN = (
    ((3, 7, 9, 14, 16), (0, 5, 10, 14), (1, 9, 10)),
    ((3, 6, 8, 11, 13), (1, 5, 9, 12), (2, 9, 10)),
    ((3, 7, 9, 11, 14), (0, 2, 9, 12), (2, 9, 11)),
    ((3, 6, 9, 11, 14), (0, 4, 8, 12), (2, 5, 6)),
)


def _segment(h, hk, wqv, wk, wob, wsum, pst, lst, fix_qv, fix_k, fix_o, step):
    ys = {p: [None] * 3 for p in range(NP)}
    ss, pvs, os_ = {}, {}, {}
    hb = h.astype(BF16)

    used = [0]

    def staged(ops, through_memory):
        if not through_memory:
            ops = {k: v.astype(BF16) for k, v in ops.items()}
            return ops.get
        names, w, c0 = list(ops), next(iter(ops.values())).shape[1], used[0]
        used[0] += w * len(names)
        lst[:, c0:used[0]] = _pack(jnp.concatenate(list(ops.values()), axis=1).astype(BF16))
        return lambda k: _unpack(lst[:, pl.ds(c0 + w * names.index(k), w)])

    def summed(slab, g, name):
        return wsum[64 * slab:64 * slab + 64, pl.ds(128 * _star_slot(g, name), 128)]

    def keys(n):
        k = _dot(hk, _unpack(wk[n]))
        for e in range(4):
            ys[4 * n + e][1] = fix_k(4 * n + e, k[:, e * PW:(e + 1) * PW])

    def proj(p):
        def w(lo, hi):
            return _unpack(jnp.concatenate(
                [wqv[2 * i + p // 8, lo:hi, pl.ds(p % 8 * PW, PW)] for i in range(2)], axis=1))
        if p == 0:
            y = _dot(hb[:, 0:512], w(0, 256))
            y = _dot(hb[:, 512:], w(256, D // 2)) + y
        else:
            y = _dot(hb, w(0, D // 2))
        for i in range(2):
            ys[p][2 * i] = fix_qv(p, i, y[:, i * PW:(i + 1) * PW])

    def wide_proj(half, g, i, lhs, tiles):
        slab, (t0, n) = 2 * i + half, _STARS[g]
        if n == 4:
            tail = _dot(hb[:, 512:], _unpack(wqv[slab, 256:, 128 * t0:]))
        out = _star_result(n, *_star_apply(
            n, lhs[n],
            lambda j, l: _unpack(wqv[slab, 64 * j:64 * j + 64, pl.ds(128 * (t0 + l), 128)]),
            lambda name: _unpack(summed(slab, g, name)), False))
        for l, y in enumerate(out):
            tiles[t0 + l] = y + tail[:, 128 * l:128 * l + 128] if n == 4 else y
        for e in range(8):
            if all(3 * e + k in tiles for k in range(3)):
                ys[8 * half + e][2 * i] = fix_qv(8 * half + e, i, jnp.concatenate(
                    [tiles.pop(3 * e + k) for k in range(3)], axis=1))

    def weights(c, i, which):
        if i < 2:
            return _own_weights(ys[2 * c + i][which](), i)
        return _others(ys[2 * c][which](), ys[2 * c + 1][which](), True)

    def score_round(n):
        for c, i in (divmod(j, 3) for j in range(4 * n, 4 * n + 4)):
            if i < 2:
                q = jnp.concatenate(_tiles(ys[2 * c + i][0](), i)[0:2], axis=0).astype(BF16)
            else:
                q = _others(ys[2 * c][0](), ys[2 * c + 1][0](), False)
            ss[c, i] = _dot_nt(q, weights(c, i, 1))
            if i == 2:
                pst[:, c * PW:(c + 1) * PW] = _softmax3([ss.pop((c, k)) for k in range(3)])

    def pv_round(n):
        for c, i in (divmod(j, 3) for j in range(4 * n, 4 * n + 4)):
            pvs[c, i] = _dot(_unpack(pst[:, pl.ds(c * PW + 128 * i, 128)]), weights(c, i, 2))
            if i == 2:
                o0, o1, o2 = [pvs.pop((c, k)) for k in range(3)]
                os_[2 * c] = fix_o(2 * c, jnp.concatenate(
                    [o0[L:, :], o0[0:L, :], o2[L:, :]], axis=1))
                os_[2 * c + 1] = fix_o(2 * c + 1, jnp.concatenate(
                    [o2[0:L, :], o1[0:L, :], o1[L:, :]], axis=1))

    def slot(n):
        if n >= 2:
            pv_round(n - 2)
        if n < 6:
            score_round(n)

    def oproj(lo, hi, r):
        o = jnp.concatenate([os_.pop(p) for p in range(lo, hi)], axis=1).astype(BF16)
        y = _dot(o, _unpack(wob[lo * DH:hi * DH, :]))
        return y if r is None else y + r

    def wide_oproj(stars, r):
        def o_tile(t):
            return os_[t // 3][:, 128 * (t % 3):128 * (t % 3) + 128]

        for n in (4, 5):
            sel = [divmod(x, 5) for x in stars if _STARS[x % 5][1] == n]
            if not sel:
                continue
            t0 = [24 * half + _STARS[g][0] for half, g in sel]
            if n == 4:
                ts = [t + j for t in t0 for j in range(4)]
                y = _dot(jnp.concatenate([o_tile(t) for t in ts], axis=1).astype(BF16),
                         _unpack(jnp.concatenate(
                             [wob[64 * t:64 * t + 64, 512:] for t in ts], axis=0)))
                r[0] = y + r[0] if 0 in r else y
            r[n] = _star_apply(
                n, staged(_star_lhs(n, lambda i, j: jnp.concatenate(
                    [o_tile(t + j)[32 * i:32 * i + 32] for t in t0], axis=1), True), False),
                lambda j, l: _unpack(jnp.concatenate(
                    [wob[pl.ds(64 * (t + j), 64), 128 * l:128 * l + 128] for t in t0], axis=0)),
                lambda name: _unpack(jnp.concatenate(
                    [summed(4 + half, g, name) for half, g in sel], axis=0)), True, r.get(n))
        return r

    after, kat, (o1, o2, o3) = _PLAN[step]
    if step == 0:
        lhs = {n: staged(_star_lhs(
            n, lambda i, j: h[32 * i:32 * i + 32, 128 * j:128 * j + 128], False), True)
               for n in (5, 4)}
        tiles = {}
    for unit in range(20 if step == 0 else NP):
        if step == 0:
            half, g, i = unit // 10, unit % 10 // 2, unit % 2
            wide_proj(half, g, i, lhs, tiles.setdefault((half, i), {}))
        else:
            proj(unit)
        if unit in kat:
            keys(kat.index(unit))
        for n in range(5):
            if after[n] == unit:
                slot(n)
    if step == 3:
        r = wide_oproj(range(0, o1), {})
        slot(5)
        r = wide_oproj(range(o1, o2), r)
        slot(6)
        slot(7)
        r = wide_oproj(range(o2, o3), r)
        r = wide_oproj(range(o3, 10), r)
        return jnp.concatenate(
            [x + y for x, y in zip(_star_result(5, *r[5]), _star_result(4, *r[4]) + [r[0]])],
            axis=1)
    r = oproj(0, o1, None) if o1 else None
    slot(5)
    r = oproj(o1, o2, r)
    slot(6)
    slot(7)
    r = oproj(o2, o3, r)
    return oproj(o3, NP, r)


def _kernel(x_hbm, wqkv_hbm, wphi_hbm, woa_hbm, mem0_hbm,
            wq_hbm, wk_hbm, wv_hbm, wo_hbm,
            out_hbm,
            xio, wqkv, wphi, woa, mem0, xres, xa, xl, xb, bds, wat, phq, phk, kvacc, kvs,
            wraw, wqv, wk, wob, wsum, xe, ke, ysave, osave, pst, lst, rsave, sem_in, sem_out):
    nsub = TN // 128
    na = S // TA
    asub = TA // 128
    nb = S // TB

    def rows(j, n):
        return pl.ds(j * n if isinstance(j, int) else pl.multiple_of(j * n, n), n)

    def x_copy(j):
        if isinstance(j, int) and j < 0:
            r = pl.ds(0, 256)
        elif isinstance(j, int) and j == na - 1:
            r = pl.ds(S - TA + 256, TA - 256)
        else:
            r = pl.ds(j * TA + 256 if isinstance(j, int)
                      else pl.multiple_of(j * TA + 256, 256), TA)
        return pltpu.make_async_copy(x_hbm.at[r, :], xio.at[r, :], sem_in.at[9 + j])

    def w_copy(c):
        src = (wq_hbm, wv_hbm, wo_hbm, wk_hbm)[c // 2 if isinstance(c, int) else 0]
        return pltpu.make_async_copy(src.at[c % 2], wraw.at[c], sem_in.at[9 + na + c])

    def wa_copy(c):
        r = pl.ds(512, 128) if isinstance(c, int) and c == 2 else rows(c, 256)
        return pltpu.make_async_copy(wqkv_hbm.at[r, :], wqkv.at[r, :], sem_in.at[3 + c])

    def out_copy(i):
        return pltpu.make_async_copy(xio.at[rows(i, TB), :],
                                     out_hbm.at[rows(i, TB), :], sem_out.at[0])

    wphi_copy = pltpu.make_async_copy(wphi_hbm, wphi, sem_in.at[0])
    woa_copy = pltpu.make_async_copy(woa_hbm, woa, sem_in.at[1])
    mem0_copy = pltpu.make_async_copy(mem0_hbm, mem0, sem_in.at[2])
    order = [wphi_copy, wa_copy(0), wa_copy(1), x_copy(-1), wa_copy(2)]
    order += [x_copy(j) for j in range(na)] + [woa_copy, mem0_copy]
    order += [w_copy(c) for c in (6, 7, 0, 4, 1, 2, 5, 3)]
    for c in order:
        c.start()

    def strassen_rhs(x0, x1):
        b11, b12 = [jnp.concatenate([x[:, 0:128], x[:, 256:384]], axis=1) for x in (x0, x1)]
        b21, b22 = [jnp.concatenate([x[:, 128:256], x[:, 384:512]], axis=1) for x in (x0, x1)]
        ops = [b11 + b22, b11, b12 - b22, b21 - b11, b22, b11 + b12, b21 + b22,
               x0[:, 512:], x1[:, 512:]]
        return _pack(jnp.concatenate(ops, axis=1).astype(BF16))

    def load_x(t, first):
        x = xio[rows(t, 256), :].astype(F32)
        if first is not True:
            x = jnp.where(first, x, xres[rows(t, 256), :])
        xres[rows(t, 256), :] = x
        return x

    wphi_copy.wait()
    cphi = jnp.zeros((FA, D), F32)
    hh = lax.broadcasted_iota(jnp.int32, (HA, D), 0) * FA
    jj = lax.broadcasted_iota(jnp.int32, (HA, D), 1)
    for d in range(FA):
        cphi = _dot(wphi[d], jnp.where(jj == hh + d, 1.0, 0.0).astype(BF16)) + cphi
    cb = jnp.concatenate(
        [jnp.broadcast_to(cphi[f:f + 1, :], (8, D)) for f in range(FA)], axis=0)
    for g in range(GA):
        row = lax.broadcasted_iota(jnp.int32, (GR, 256), 0)
        col = lax.broadcasted_iota(jnp.int32, (GR, 256), 1) + 128 * g
        lo = (8 * g + (row & 7)) * FA
        bds[g] = _pack(jnp.where(jnp.logical_and(col >= lo, col < lo + FA),
                                 cb[:, 128 * g:128 * g + 256], 0.0).astype(BF16))

    def folded(rr):
        out = [[], [], []]
        for g in range(GA):
            ws = []
            for i in range(2):
                c0 = i * D + 128 * g
                w = _dot_nt(_unpack(bds[g]), wqkv[rr, c0:c0 + 256]).reshape(FA, 8, 128)
                ws.append(((w[1:] - w[0:1]) * LOG2E).reshape(GR - 8, 128))
            out[0].append(jnp.concatenate([ws[1], ws[0][GR - 16:, :]], axis=0))
            out[1].append(ws[0][0:GR - 16, :])
        wvt = wqkv[rr, 2 * D:3 * D].T.astype(F32)
        out[2] = [wvt[g * GR:(g + 1) * GR, :] for g in range(GA)]
        return out

    def fold(c, _):
        wa_copy(c).wait()
        wa, wb = folded(rows(2 * c, 128)), folded(rows(2 * c + 1, 128))
        for i in range(3):
            for p in range(2):
                a11, a12, a21, a22 = wa[i][2 * p], wb[i][2 * p], wa[i][2 * p + 1], wb[i][2 * p + 1]
                ops = [a11 + a22, a21 + a22, a11, a22, a11 + a12, a21 - a11, a12 - a22]
                for m, w in enumerate(ops):
                    wat[2 * i + p, m, 0:w.shape[0] // 2, rows(c, 128)] = _pack(w.astype(BF16))
        return 0

    lax.fori_loop(0, 2, fold, 0)
    x_copy(-1).wait()
    wa_copy(2).wait()
    x = _layernorm(load_x(0, True))
    xa[...] = strassen_rhs(x[0:128], x[128:])
    for i, ws in enumerate(folded(pl.ds(512, 128))):
        for g, w in enumerate(ws):
            wat[2 * i + g // 2, 7, 0:w.shape[0] // 2, rows(g % 2, 128)] = _pack(w.astype(BF16))

    def pair_rows(ph, q, t0, n):
        return _unpack(jnp.concatenate(
            [ph[t0 + u, rows(q, 2 * FA), :] for u in range(n)], axis=1))

    def a1(first, j, _):
        @pl.when(jnp.logical_and(first, j < na - 1))
        def _():
            x_copy(j).wait()

        @pl.when(jnp.logical_and(first, j == na - 1))
        def _():
            x_copy(na - 1).wait()

        def features(ph, t, g, y):
            for f, w in enumerate(_feature_map(y)):
                ph[t, pl.ds(GR * g + f, 8, stride=FA), :] = w

        def tail(n, xs, g, u):
            nr = GR // 2 - 8 if n // 2 == 1 else GR // 2
            return _dot_nt(_unpack(wat[n, 7, 0:nr, 128 * g:128 * (g + 1)]),
                           xs[:, 1792 + 128 * u:1920 + 128 * u])

        def a_dots(n, xs, emit, tie, t10):
            nr = GR // 2 - 8 if n // 2 == 1 else GR // 2
            p = n % 2

            def prod(m):
                return _dot_nt(_unpack(tie(wat[n, m, 0:nr, :])), xs[:, 256 * m:256 * (m + 1)])

            m2, m4 = prod(1), prod(3)
            emit(2 * p + 1, 0, m4 + (m2 - (-t10)))
            t01 = tail(n, xs, 0, 1)
            m3, m5 = prod(2), prod(4)
            emit(2 * p, 1, m5 + (m3 - (-t01)))
            m1 = prod(0)
            c22 = prod(5) + (m1 + (m3 - m2))
            emit(2 * p + 1, 1, tail(n, xs, 1, 1) + c22)
            t10 = tail(n + 1, xs, 1, 0) if n < 5 else None
            c11 = tail(n, xs, 0, 0) + (m1 + (m4 - m5))
            emit(2 * p, 0, prod(6) + c11)
            return t10

        vs = {}
        cur = xa[...]
        dl = (3, 8, 13, 30, 33, 36, 39, 41)
        for u in range(0, asub, 2):
            t = j * (asub // 2) + u // 2
            xs = _unpack(cur)
            tn = t + 1
            x = load_x(tn if u + 2 < asub else jnp.minimum(tn, (na - 1) * (asub // 2)), first)
            rest, seen, nxt = {}, [], []

            def tie(w):
                seen.append(0)
                if len(seen) - 1 not in dl:
                    return w
                n = len(nxt)
                nxt.append(strassen_rhs(*[
                    _layernorm(x[128 * e + 16 * n:128 * e + 16 * n + 16, :]) for e in range(2)]))
                z = jnp.concatenate(
                    [nxt[n][:, 256 * c:256 * (c + 1)] for c in range(8)], axis=0)
                return jnp.concatenate([jnp.where(j < 0, z, w[0:64, :]), w[64:, :]], axis=0)

            def emit_k(g, e, y):
                features(phk, u + e, g, y[0:GR - 8, :])
                rest[g, e] = y[GR - 8:, :]

            def emit_q(g, e, y):
                features(phq, 2 * t + e, g, jnp.concatenate([y, rest[g, e]], axis=0))

            def emit_v(g, e, y):
                for q in range(4):
                    vs[4 * g + q, u + e] = y[40 * q:40 * q + 40, :]

            t10 = tail(0, xs, 1, 0)
            for n in range(6):
                t10 = a_dots(n, xs, (emit_k, emit_q, emit_v)[n // 2], tie, t10)
            cur = jnp.concatenate(nxt, axis=0)
        xa[...] = cur
        row = lax.broadcasted_iota(jnp.int32, (2 * VR, 4 * FA), 0)
        col = lax.broadcasted_iota(jnp.int32, (2 * VR, 4 * FA), 1)
        split = jnp.where(row < 2 * FA, FA, 2 * FA + 4)
        same = (row >= split) == (col >= 2 * FA)
        for q in range(PA):
            v = jnp.concatenate([vs[q, u] for u in range(asub)], axis=1)
            v = jnp.concatenate([v, jnp.ones((8, TA), F32)], axis=0)
            kv = _dot_nt(v.astype(BF16), pair_rows(phk, q, 0, asub))
            kv = kv + jnp.where(j == 0, 0.0, kvacc[q])
            kvacc[q] = kv
            kvs[q] = _pack(jnp.where(same, kv, 0.0).astype(BF16))
        return 0

    def attend(j):
        low = lax.broadcasted_iota(jnp.int32, (8, TN), 0) < 4
        os_ = []
        for q in range(PA):
            nd = _dot(_unpack(kvs[q]), pair_rows(phq, q, j * nsub, nsub))
            rab = 1.0 / (nd[40:48, :] + 1e-6)
            rba = pltpu.roll(rab, 4, 0)
            ra = jnp.where(low, rab, rba)
            rb = jnp.where(low, rba, rab)
            os_.append(nd[0:40, :] * jnp.concatenate([ra, ra, rab, rb, rb], axis=0))
        return _pack(jnp.concatenate(os_, axis=0).astype(BF16).T)

    def project(j, o, slot):
        ns = TN // SEG
        xs = []
        r = rows(j, TN)
        old, new = xres[r, :], {}
        for part in ((1, 2), (0, 3)):
            grp = [b + k for b in range(0, TN // 16, 4) for k in part]
            oo = jnp.concatenate([o[8 * g:8 * g + 8, :] for g in grp], axis=0)
            x = _dot(_unpack(oo), woa[...]) + jnp.concatenate(
                [old[16 * g:16 * g + 16, :] for g in grp], axis=0)
            for n, g in enumerate(grp):
                new[g] = x[16 * n:16 * n + 16, :]
            xs.append(x)
        xres[r, :] = jnp.concatenate([new[g] for g in range(TN // 16)], axis=0)
        for s in range(ns):
            x = xs[0][16 * s + 8 - 8 * (s % 2):16 * s + 16 - 8 * (s % 2), :]
            x = _layernorm(x)
            x = x - x[KE:KE + 1, :]
            for c in range(D // 128):
                xe[c, pl.ds((slot * ns + s) * KE, 8), :] = x[:, 128 * c:128 * (c + 1)]

    def extra_keys(seg, p):
        k = jnp.concatenate(
            [ke[seg // 16, 3 * p + c, pl.ds((seg % 16) * KE, 8), :] for c in range(3)], axis=1)
        return jnp.where(lax.broadcasted_iota(jnp.int32, (8, PW), 0) < KE, k, 0.0)

    def b_residual(i):
        r = rows(i, TB)
        x = xres[r, :] + rsave[...]
        xres[r, :] = x
        xio[r, :] = x.astype(BF16)
        return x

    def b_finish(i):
        xn = _layernorm(b_residual(i))
        xl[rows(jnp.minimum(i, 2), TB), :] = xn
        return xn

    def b_tile(mem, xn, i, side):
        for u in range(4):
            t0 = u * SEG
            late = u % 2 == 0
            ext = [SEG * v + (24 if v % 2 == 0 else 0) for v in range(4)]

            def place(y, z):
                return jnp.concatenate([y, z] if late else [y[0:M], z, y[M:]], axis=0)

            def fix_qv(p, kind, y):
                cols = pl.ds((3 * p + 2 * kind) * PW, PW)
                ysave[0:y.shape[0], cols] = y

                def get():
                    z = place(ysave[0:32, cols], ysave[32 + 8 * u:40 + 8 * u, cols])
                    if not late or kind == 0:
                        return z
                    r0 = 64 * u + 8 * p
                    tie = jnp.concatenate(
                        [side[r0:r0 + 8, 0:PW], side[r0:r0 + 8, D - PW:]], axis=0)
                    return jnp.concatenate([jnp.where(i < 0, tie, z[0:16, :]), z[16:, :]], axis=0)
                return get

            def fix_k(p, k):
                cols = pl.ds((3 * p + 1) * PW, PW)
                ysave[0:32, cols] = k
                return lambda: place(ysave[0:32, cols], extra_keys(4 * i + u, p))

            def fix_o(p, o):
                cols = slice(p * PW, (p + 1) * PW)
                r0 = 0 if u == 3 else 8 + 8 * u
                osave[r0:r0 + 8, cols] = o[32:L, :]
                if u == 3:
                    return jnp.concatenate([o[0:32, :], osave[:, cols]], axis=0)
                return o[0:32, :]

            h = jnp.concatenate(
                [mem, xn[t0:t0 + 24, :] if late else xn[t0 + 8:t0 + SEG, :]], axis=0)
            hk = (h - xn[ext[u] + KE:ext[u] + KE + 1, :]).astype(BF16)
            if u == 0:
                h = jnp.concatenate([h] + [xn[e:e + 8, :] for e in ext], axis=0)
            r = _segment(h, hk, wqv, wk, wob, wsum, pst, lst, fix_qv, fix_k, fix_o, u)
            mem = r[0:M, :]
            if u < 3:
                rsave[t0:t0 + 24, :] = r[M:, :]
            else:
                rsave[t0:t0 + SEG, :] = r[M:L, :]
                for v in range(3):
                    rsave[SEG * v + 24:SEG * v + SEG, :] = r[L + 8 * v:L + 8 * v + 8, :]
        return mem

    def layer(l, _):
        def wait_first(copies):
            @pl.when(l == 0)
            def _():
                for c in copies:
                    c.wait()

        with jax.named_scope("a1"):
            lax.fori_loop(0, na, functools.partial(a1, l == 0), 0)

        def a2(n, _):
            for m, cs in enumerate(((6, 7, 0, 4), (1,), (2, 5), (3,))):
                @pl.when(jnp.logical_and(l == 0, n == m))
                def _():
                    for c in cs:
                        w_copy(c).wait()

            ty, half = n % 2, n // 2
            o0 = attend(2 * n)
            o1 = attend(2 * n + 1)

            def sample(w):
                z = [w[64 * a + 56:64 * a + 64, :] for a in range(D // 128)]
                out = []
                for y in z:
                    acc = y[:, 0:128]
                    for c in range(1, y.shape[1] // 128):
                        acc = acc | y[:, 128 * c:128 * (c + 1)]
                    out.append(acc)
                return jnp.concatenate(out, axis=1)

            mr = 16 * KE

            def side(job):
                w = _pack(wraw[n, rows(int(job), 2 * PW), :].T)
                wqv[n, :, rows(int(job), 2 * PW)] = w
                return sample(w)

            for job in '01':
                o1 = jnp.concatenate([o1[0:8, :], jnp.where(n < 0, side(job), o1[8:16, :]),
                                      o1[16:, :]], axis=0)
            project(2 * n, o0, 0)
            ties = [pltpu.bitcast(side(job), F32) for job in '23']
            project(2 * n + 1, o1, 1)
            x = jnp.concatenate([xe[c, 0:mr, :] for c in range(D // 128)], axis=1)
            for tie in ties:
                x = jnp.concatenate([jnp.where(n < 0, tie, x[0:8, :]), x[8:, :]], axis=0)
            x = x.astype(BF16)
            r = rows(n, TB // NW)
            xb[r, :] = _layernorm(xres[r, :])
            rsave[r, :] = jnp.zeros((TB // NW, D), F32)
            for ref in (ysave, osave, pst, lst):
                ref[rows(ty, 8), 0:128] = jnp.zeros((8, 128), ref.dtype)

            def view(ref, start, size, align):
                return ref.at[pl.ds(pl.multiple_of(start, align), size)]

            wo_src = view(wraw.at[4 + half], 64 * ty, HD // 2 - 64, 64)
            wo_dst = view(wob, QW * half + 32 * ty, QW - 32, 32)
            wk_src = view(wraw.at[6 + half], QW * ty, QW, QW)
            sum_dst = view(wsum, 64 * n, 64, 64), view(wsum, 256 + 32 * n, 32, 32)

            def wo_rows(t, rr):
                return _pack(wo_src[rows(8 * t + rr, 16), :])

            def sums(is_o, g, j, rr, tie):
                t0, sz = _STARS[g]
                names = _star_sums(sz)[j]
                if is_o:
                    row = jnp.where(n < 0, jnp.concatenate([tie] * 5, axis=1), wo_rows(t0 + j, rr))
                    wo_dst[rows(8 * (t0 + j) + rr, 8), :] = row
                val = {}
                for x, y in [(j, k) for k in range(sz)] + [(k, j) for k in range(sz) if k != j]:
                    if is_o and x == j:
                        w = row[:, 128 * y:128 * y + 128]
                    elif is_o and x < j:
                        w = jnp.where(n < 0, tie, wo_dst[rows(8 * (t0 + x) + rr, 8), rows(y, 128)])
                    else:
                        w = jnp.where(n < 0, tie, wo_rows(t0 + x, rr)[:, 128 * y:128 * y + 128] if is_o
                                      else wqv[n, rows(8 * x + rr, 8), rows(t0 + y, 128)])
                    val[x, y] = _unpack(w).astype(F32)
                others = [k for k in range(sz) if k != j]
                out = [functools.reduce(lambda z, k: z - val[j, k], others, val[j, j]),
                       functools.reduce(lambda z, k: z + val[k, j], others, val[j, j])]
                out += [val[x, y] + val[y, x] for x, y in names[2:]]
                sum_dst[is_o][rows(rr, 8),
                              pl.ds(128 * _star_slot(g, names[0]), 128 * len(names))] = _pack(
                    jnp.concatenate(out, axis=1).astype(BF16))

            def k_tiles(t, c, tie):
                w = _pack(wk_src[rows(t, 256), rows(c, 128)])
                w = jnp.concatenate([jnp.where(n < 0, tie, w[0:8, :]), w[8:64, :],
                                     jnp.where(n < 0, tie, w[64:72, :]), w[72:, :]], axis=0)
                wk[n, rows(c, 64), rows(t, 256)] = _pack(_unpack(w).T)

            kjobs = [functools.partial(k_tiles, t, c) for t in range(6) for c in range(5)]
            todo = []
            for g in range(5):
                for j in range(_STARS[g][1]):
                    for rr in range(4):
                        if len(todo) % 10 < 3:
                            todo += kjobs[-1:]
                            del kjobs[-1:]
                        todo += [functools.partial(sums, False, g, j, 2 * rr),
                                 functools.partial(sums, True, g, j, rr),
                                 functools.partial(sums, False, g, j, 2 * rr + 1)]
            assert not kjobs
            left = [48]

            def emit(t, k):
                ke[n, t, 0:mr, :] = k
                left[0] -= 1
                if left[0] < 48 - 2:
                    m = -(-len(todo) // (left[0] + 1))
                    for g in range(m):
                        g = 8 * (14 * g // m)
                        todo.pop(0)(pltpu.bitcast(k[g:g + 8, :], U32))

            for v in range(HD // 256):
                k = _dot_nt(x, wraw[6 + v // 12, rows(v % 12, 256), :])
                emit(2 * v, k[:, 0:128])
                emit(2 * v + 1, k[:, 128:])
            return 0

        wait_first([woa_copy, mem0_copy])
        with jax.named_scope("a2"):
            lax.fori_loop(0, NW, a2, 0)

        def b_step(i, mem):
            xn = xb[...]
            side = b_finish(jnp.maximum(i - 1, 0))
            nxt = _layernorm(xres[rows(jnp.minimum(i + 1, nb - 1), TB), :])
            xb[...] = nxt
            side = jnp.concatenate([side, nxt], axis=0)
            mem = b_tile(mem, xn, i, side)

            @pl.when(jnp.logical_and(l == 1, i >= 1))
            def _():
                out_copy(i - 1).start()
            return mem

        with jax.named_scope("b"):
            lax.fori_loop(0, nb, b_step, mem0[...].astype(F32))

        b_residual(nb - 1)

        @pl.when(l == 0)
        def _():
            xa[...] = strassen_rhs(xl[0:128, :], xl[128:256, :])
        return 0

    lax.fori_loop(0, 2, layer, 0)
    out_copy(nb - 1).start()
    pltpu.make_async_copy(xio, out_hbm, sem_out.at[0]).wait()


@jax.jit
def pallas_interleave_layers__linear_kernel_hedgehog__memory_aug_recurrent_mem_tr__prompt_kernel(
    A_x, A_wqkv, A_w_phi, A_wo, B_x, B_mem0, B_Wq, B_Wk, B_Wv, B_Wo, B_seg_len,
):
    del B_x
    del B_seg_len
    x = A_x.reshape(S, D)
    wphi = A_w_phi.transpose(1, 2, 0)
    mem0 = B_mem0.reshape(M, D)
    wq, wk, wv = (w.transpose(1, 2, 0).reshape(2, HD // 2, D) for w in (B_Wq, B_Wk, B_Wv))
    wo = B_Wo.reshape(2, HD // 2, D)
    hbm = pl.BlockSpec(memory_space=pl.ANY)
    out = pl.pallas_call(
        _kernel,
        out_shape=jax.ShapeDtypeStruct((S, D), A_x.dtype),
        in_specs=[hbm] * 9,
        out_specs=hbm,
        scratch_shapes=[
            pltpu.VMEM((S, D), BF16),
            pltpu.VMEM((D, 3 * D), BF16),
            pltpu.VMEM((FA, FA, HA), BF16),
            pltpu.VMEM((D, D), BF16),
            pltpu.VMEM((M, D), BF16),
            pltpu.VMEM((S, D), F32),
            pltpu.VMEM((64, 2048), U32),
            pltpu.VMEM((3 * TB, D), F32),
            pltpu.VMEM((TB, D), F32),
            pltpu.VMEM((GA, GR // 2, 256), U32),
            pltpu.VMEM((6, 8, GR // 2, 256), U32),
            pltpu.VMEM((S // 128, D, 128), U32),
            pltpu.VMEM((TA // 128, D, 128), U32),
            pltpu.VMEM((PA, 2 * VR, 4 * FA), F32),
            pltpu.VMEM((PA, VR, 4 * FA), U32),
            pltpu.VMEM((8, HD // 2, D), BF16),
            pltpu.VMEM((4, D // 2, HD // 2), U32),
            pltpu.VMEM((NW, D // 2, QW), U32),
            pltpu.VMEM((HD // 2, D), U32),
            pltpu.VMEM((6 * 64, NS * 128), U32),
            pltpu.VMEM((D // 128, 16 * KE + 8, 128), F32),
            pltpu.VMEM((NW, HD // 128, 16 * KE + 8, 128), F32),
            pltpu.VMEM((64, 3 * HD), F32),
            pltpu.VMEM((32, HD), F32),
            pltpu.VMEM((L, HD // 2), U32),
            pltpu.VMEM((16, 66 * 128), U32),
            pltpu.VMEM((TB, D), F32),
            pltpu.SemaphoreType.DMA((17 + S // TA,)),
            pltpu.SemaphoreType.DMA((1,)),
        ],
        compiler_params=pltpu.CompilerParams(vmem_limit_bytes=126 * 1024 * 1024,
                                             disable_bounds_checks=True,
                                             disable_semaphore_checks=True),
    )(x, A_wqkv, wphi, A_wo, mem0, wq, wk, wv, wo)
    return out.reshape(1, S, D)
```

```python
import functools

import jax
import jax.numpy as jnp
from jax import lax
import jax.experimental.pallas as pl
import jax.experimental.pallas.tpu as pltpu

F32 = jnp.float32
BF16 = jnp.bfloat16
U32 = jnp.uint32

S = 2048
D = 640
HA = 32
FA = 20
GA = 4
GR = 8 * FA
VR = 24
PA = HA // 2
TN = 256
TA = 512
HB = 32
DH = 192
HD = HB * DH
M = 8
SEG = 32
L = M + SEG
PW = 2 * DH
NP = HB // 2
TB = 128
NW = 4
QW = HD // NW
KE = 7

NT = (((1,), (1,)), ((), ()))
LOG2E = 1.4426950408889634
HALF_ULP = 0.0040612


def _dot(a, b):
    return jnp.dot(a, b, preferred_element_type=F32)


def _dot_nt(a, b):
    return lax.dot_general(a, b, NT, preferred_element_type=F32)


def _pack(a):
    return pltpu.bitcast(a, U32)


def _unpack(a):
    return pltpu.bitcast(a, BF16)


def _interleave(a, b):
    lo = lax.bitcast_convert_type(a, U32) >> 16
    hi = lax.bitcast_convert_type(b, U32) & jnp.uint32(0xFFFF0000)
    return lo | hi


def _recip(x):
    r = pl.reciprocal(x, approx=True)
    return r * (2.0 - x * r)


def _layernorm(x):
    m = jnp.mean(x, axis=-1, keepdims=True)
    c = x - m
    v = jnp.mean(c * c, axis=-1, keepdims=True)
    return c * lax.rsqrt(v + 1e-5)


def _feature_map(p):
    t = p.shape[-1]
    p3 = jnp.concatenate([jnp.zeros((8, t), F32), p], axis=0).reshape(FA, 8, t)
    mx = jnp.max(p3, axis=0)
    mn = jnp.min(p3, axis=0)
    sp, sn = jnp.exp2(p3[0] - mx), jnp.exp2(mn - p3[0])
    for f in range(1, FA):
        sp, sn = sp + jnp.exp2(p3[f] - mx), sn + jnp.exp2(mn - p3[f])
    lp = (mx - HALF_ULP) + jnp.log2(sp)
    ln = (mn + HALF_ULP) - jnp.log2(sn)
    return [_interleave(jnp.exp2(p3[f] - lp), jnp.exp2(ln - p3[f])) for f in range(FA)]


def _tiles(a, odd):
    t0, t1, t2 = a[:, 0:128], a[:, 128:256], a[:, 256:384]
    return (t1, t2, t0) if odd else (t1, t0, t2)


def _own_weights(a, odd):
    lane = lax.broadcasted_iota(jnp.int32, (L, 128), 1)
    mid, own, _ = _tiles(a, odd)
    return jnp.concatenate(
        [jnp.where(lane < 64, mid, 0.0), jnp.where(lane < 64, 0.0, mid), own,
         jnp.zeros((128 - 3 * L, 128), F32)], axis=0).astype(BF16)


def _others(even, odd, pad):
    parts = [_tiles(odd, 1)[2], _tiles(even, 0)[2]]
    if pad:
        parts.append(jnp.zeros((128 - 2 * L, 128), F32))
    return jnp.concatenate(parts, axis=0).astype(BF16)


def _softmax3(s3):
    row = lax.broadcasted_iota(jnp.int32, (L, 128), 0)
    col = lax.broadcasted_iota(jnp.int32, (L, 128), 1)
    first = col < L
    second = jnp.logical_and(col >= L, col < 2 * L)
    key = jnp.where(first, col, col - L)
    valid = jnp.logical_or(row < M, row >= key)
    out, other = [], []
    for odd in range(2):
        own = pltpu.roll(s3[odd][L:, :], 128 - L if odd else 128 - 2 * L, 1)
        s = (jnp.where(first, s3[2][0:L, :], own) if odd
             else jnp.where(first, own, s3[2][L:, :]))
        s = jnp.where(valid, (s + s3[odd][0:L, :]) * (DH ** -0.5), -1e9)
        m0 = jnp.max(jnp.where(first, s, -jnp.inf), axis=-1, keepdims=True)
        m1 = jnp.max(jnp.where(second, s, -jnp.inf), axis=-1, keepdims=True)
        e = jnp.exp(s - jnp.where(first, m0, m1))
        e0 = jnp.where(first, e, 0.0)
        e1 = jnp.where(second, e, 0.0)
        p0 = e0 * _recip(jnp.sum(e0, axis=-1, keepdims=True))
        p1 = e1 * _recip(jnp.sum(e1, axis=-1, keepdims=True))
        own = pltpu.roll(p1, L, 1) if odd else pltpu.roll(p0, 2 * L, 1)
        out.append(jnp.concatenate([p0 + p1, own], axis=0))
        other.append(p0 if odd else p1)
    out.append(jnp.concatenate([other[1], other[0]], axis=0))
    return _pack(jnp.concatenate(out, axis=1).astype(BF16))


_T = {5: (-1.5, -0.5, 0.0, 0.5, 1.5), 4: (-1.25, -0.25, 0.25, 1.25)}
_STARS = tuple((5 * g, 5 if g < 4 else 4) for g in range(5))


def _star_sums(n):
    own = {j: [] for j in range(n)}
    for a in range(n):
        for b in range(a + 1, n):
            own[a if (b - a) % 2 else b].append((a, b))
    return [['r%d' % j, 'c%d' % j] + own[j] for j in range(n)]


def _star_slot(g, name):
    return 20 * g + [x for grp in _star_sums(_STARS[g][1]) for x in grp].index(name)


NS = 94


def _star_lhs(n, get, scaled):
    t = _T[n]
    f = [get(0, j) for j in range(n)]
    g = [get(1, j) + t[j] * f[j] if t[j] else get(1, j) for j in range(n)]
    out = {'r%d' % j: f[j] for j in range(n)}
    out.update({'c%d' % j: g[j] for j in range(n)})
    for a in range(n):
        for b in range(a + 1, n):
            d = t[a] - t[b]
            if scaled:
                l = (g[a] - g[b]) * (1.0 / d)
                out[a, b], out[b, a, 0], out[a, b, 0] = l, f[b] - l, f[a] - l
            else:
                l = g[a] - g[b]
                out[a, b], out[b, a, 0], out[a, b, 0] = l, d * f[b] - l, d * f[a] - l
    return out


def _star_apply(n, lhs, plain, mixed, scaled, acc=None):
    t = _T[n]
    p, q = ([None] * n, [None] * n) if acc is None else (list(acc[0]), list(acc[1]))
    started = set()

    def start(j):
        if j not in started:
            started.add(j)
            dp, dq = [_dot(lhs(k % j), mixed(k % j)) for k in ('r%d', 'c%d')]
            p[j] = dp if p[j] is None else dp + p[j]
            q[j] = dq if q[j] is None else dq + q[j]

    for a in range(n):
        for b in range(a + 1, n):
            start(a)
            start(b)
            d = t[a] - t[b]
            m6 = _dot(lhs((b, a, 0)), plain(b, a))
            m7 = _dot(lhs((a, b, 0)), plain(a, b))
            m = _dot(lhs((a, b)), mixed((a, b))) + (m6 + m7)
            if scaled:
                q[a], q[b] = q[a] - (-d) * m6, q[b] - d * m7
                p[a], p[b] = m + p[a], m + p[b]
            else:
                q[a], q[b] = m6 + q[a], q[b] - m7
                m = m * (-1.0 / d) if d != -1.0 else m
                p[a], p[b] = p[a] - m, p[b] - m
    return p, q


def _star_result(n, p, q):
    return [jnp.concatenate([p[j], q[j] - _T[n][j] * p[j] if _T[n][j] else q[j]], axis=0)
            for j in range(n)]


_PLAN = (
    ((3, 7, 10, 14, 17), (0, 4, 10, 14), (1, 9, 10)),
    ((3, 6, 9, 11, 13), (0, 6, 7, 13), (2, 9, 10)),
    ((3, 6, 8, 11, 14), (1, 2, 8, 12), (2, 9, 10)),
    ((3, 6, 9, 11, 13), (1, 3, 8, 12), (2, 5, 6)),
)


def _segment(h, hk, wqv, wk, wob, wsum, pst, lst, fix_qv, fix_k, fix_o, step):
    ys = {p: [None] * 3 for p in range(NP)}
    ss, pvs, os_ = {}, {}, {}
    hb = h.astype(BF16)

    used = [0]

    def staged(ops, through_memory):
        if not through_memory:
            ops = {k: v.astype(BF16) for k, v in ops.items()}
            return ops.get
        names, w, c0 = list(ops), next(iter(ops.values())).shape[1], used[0]
        used[0] += w * len(names)
        lst[:, c0:used[0]] = _pack(jnp.concatenate(list(ops.values()), axis=1).astype(BF16))
        return lambda k: _unpack(lst[:, pl.ds(c0 + w * names.index(k), w)])

    def summed(slab, g, name):
        return wsum[64 * slab:64 * slab + 64, pl.ds(128 * _star_slot(g, name), 128)]

    def keys(n):
        k = _dot(hk, _unpack(wk[n]))
        for e in range(4):
            ys[4 * n + e][1] = fix_k(4 * n + e, k[:, e * PW:(e + 1) * PW])

    def proj(p):
        def w(lo, hi):
            return _unpack(jnp.concatenate(
                [wqv[2 * i + p // 8, lo:hi, pl.ds(p % 8 * PW, PW)] for i in range(2)], axis=1))
        if p == 0:
            y = _dot(hb[:, 0:512], w(0, 256))
            y = _dot(hb[:, 512:], w(256, D // 2)) + y
        else:
            y = _dot(hb, w(0, D // 2))
        for i in range(2):
            ys[p][2 * i] = fix_qv(p, i, y[:, i * PW:(i + 1) * PW])

    def wide_proj(half, g, i, lhs, tiles):
        slab, (t0, n) = 2 * i + half, _STARS[g]
        if n == 4:
            tail = _dot(hb[:, 512:], _unpack(wqv[slab, 256:, 128 * t0:]))
        out = _star_result(n, *_star_apply(
            n, lhs[n],
            lambda j, l: _unpack(wqv[slab, 64 * j:64 * j + 64, pl.ds(128 * (t0 + l), 128)]),
            lambda name: _unpack(summed(slab, g, name)), False))
        for l, y in enumerate(out):
            tiles[t0 + l] = y + tail[:, 128 * l:128 * l + 128] if n == 4 else y
        for e in range(8):
            if all(3 * e + k in tiles for k in range(3)):
                ys[8 * half + e][2 * i] = fix_qv(8 * half + e, i, jnp.concatenate(
                    [tiles.pop(3 * e + k) for k in range(3)], axis=1))

    def weights(c, i, which):
        if i < 2:
            return _own_weights(ys[2 * c + i][which](), i)
        return _others(ys[2 * c][which](), ys[2 * c + 1][which](), True)

    def score_round(n):
        for c, i in (divmod(j, 3) for j in range(4 * n, 4 * n + 4)):
            if i < 2:
                q = jnp.concatenate(_tiles(ys[2 * c + i][0](), i)[0:2], axis=0).astype(BF16)
            else:
                q = _others(ys[2 * c][0](), ys[2 * c + 1][0](), False)
            ss[c, i] = _dot_nt(q, weights(c, i, 1))
            if i == 2:
                pst[:, c * PW:(c + 1) * PW] = _softmax3([ss.pop((c, k)) for k in range(3)])

    def pv_round(n):
        for c, i in (divmod(j, 3) for j in range(4 * n, 4 * n + 4)):
            pvs[c, i] = _dot(_unpack(pst[:, pl.ds(c * PW + 128 * i, 128)]), weights(c, i, 2))
            if i == 2:
                o0, o1, o2 = [pvs.pop((c, k)) for k in range(3)]
                os_[2 * c] = fix_o(2 * c, jnp.concatenate(
                    [o0[L:, :], o0[0:L, :], o2[L:, :]], axis=1))
                os_[2 * c + 1] = fix_o(2 * c + 1, jnp.concatenate(
                    [o2[0:L, :], o1[0:L, :], o1[L:, :]], axis=1))

    def slot(n):
        if n >= 2:
            pv_round(n - 2)
        if n < 6:
            score_round(n)

    def oproj(lo, hi, r):
        o = jnp.concatenate([os_.pop(p) for p in range(lo, hi)], axis=1).astype(BF16)
        y = _dot(o, _unpack(wob[lo * DH:hi * DH, :]))
        return y if r is None else y + r

    def wide_oproj(stars, r):
        def o_tile(t):
            return os_[t // 3][:, 128 * (t % 3):128 * (t % 3) + 128]

        for n in (4, 5):
            sel = [divmod(x, 5) for x in stars if _STARS[x % 5][1] == n]
            if not sel:
                continue
            t0 = [24 * half + _STARS[g][0] for half, g in sel]
            if n == 4:
                ts = [t + j for t in t0 for j in range(4)]
                y = _dot(jnp.concatenate([o_tile(t) for t in ts], axis=1).astype(BF16),
                         _unpack(jnp.concatenate(
                             [wob[64 * t:64 * t + 64, 512:] for t in ts], axis=0)))
                r[0] = y + r[0] if 0 in r else y
            r[n] = _star_apply(
                n, staged(_star_lhs(n, lambda i, j: jnp.concatenate(
                    [o_tile(t + j)[32 * i:32 * i + 32] for t in t0], axis=1), True), False),
                lambda j, l: _unpack(jnp.concatenate(
                    [wob[pl.ds(64 * (t + j), 64), 128 * l:128 * l + 128] for t in t0], axis=0)),
                lambda name: _unpack(jnp.concatenate(
                    [summed(4 + half, g, name) for half, g in sel], axis=0)), True, r.get(n))
        return r

    after, kat, (o1, o2, o3) = _PLAN[step]
    if step == 0:
        lhs = {n: staged(_star_lhs(
            n, lambda i, j: h[32 * i:32 * i + 32, 128 * j:128 * j + 128], False), True)
               for n in (5, 4)}
        tiles = {}
    for unit in range(20 if step == 0 else NP):
        if step == 0:
            half, g, i = unit // 10, unit % 10 // 2, unit % 2
            wide_proj(half, g, i, lhs, tiles.setdefault((half, i), {}))
        else:
            proj(unit)
        if unit in kat:
            keys(kat.index(unit))
        for n in range(5):
            if after[n] == unit:
                slot(n)
    if step == 3:
        r = wide_oproj(range(0, o1), {})
        slot(5)
        r = wide_oproj(range(o1, o2), r)
        slot(6)
        slot(7)
        r = wide_oproj(range(o2, o3), r)
        r = wide_oproj(range(o3, 10), r)
        return jnp.concatenate(
            [x + y for x, y in zip(_star_result(5, *r[5]), _star_result(4, *r[4]) + [r[0]])],
            axis=1)
    r = oproj(0, o1, None) if o1 else None
    slot(5)
    r = oproj(o1, o2, r)
    slot(6)
    slot(7)
    r = oproj(o2, o3, r)
    return oproj(o3, NP, r)


def _kernel(x_hbm, wqkv_hbm, wphi_hbm, woa_hbm, mem0_hbm,
            wq_hbm, wk_hbm, wv_hbm, wo_hbm,
            out_hbm,
            xio, wqkv, wphi, woa, mem0, xres, xa, xl, xb, bds, wat, phq, phk, kvacc, kvs,
            wraw, wqv, wk, wob, wsum, xe, ke, ysave, osave, pst, lst, rsave, sem_in, sem_out):
    nsub = TN // 128
    na = S // TA
    asub = TA // 128
    nb = S // TB

    def rows(j, n):
        return pl.ds(j * n if isinstance(j, int) else pl.multiple_of(j * n, n), n)

    def x_copy(j):
        if isinstance(j, int) and j < 0:
            r = pl.ds(0, 256)
        elif isinstance(j, int) and j == na - 1:
            r = pl.ds(S - TA + 256, TA - 256)
        else:
            r = pl.ds(j * TA + 256 if isinstance(j, int)
                      else pl.multiple_of(j * TA + 256, 256), TA)
        return pltpu.make_async_copy(x_hbm.at[r, :], xio.at[r, :], sem_in.at[9 + j])

    def w_copy(c):
        src = (wq_hbm, wv_hbm, wo_hbm, wk_hbm)[c // 2 if isinstance(c, int) else 0]
        return pltpu.make_async_copy(src.at[c % 2], wraw.at[c], sem_in.at[9 + na + c])

    def wa_copy(c):
        r = pl.ds(512, 128) if isinstance(c, int) and c == 2 else rows(c, 256)
        return pltpu.make_async_copy(wqkv_hbm.at[r, :], wqkv.at[r, :], sem_in.at[3 + c])

    def out_copy(i):
        return pltpu.make_async_copy(xio.at[rows(i, TB), :],
                                     out_hbm.at[rows(i, TB), :], sem_out.at[0])

    wphi_copy = pltpu.make_async_copy(wphi_hbm, wphi, sem_in.at[0])
    woa_copy = pltpu.make_async_copy(woa_hbm, woa, sem_in.at[1])
    mem0_copy = pltpu.make_async_copy(mem0_hbm, mem0, sem_in.at[2])
    order = [wphi_copy, wa_copy(0), wa_copy(1), x_copy(-1), wa_copy(2)]
    order += [x_copy(j) for j in range(na)] + [woa_copy, mem0_copy]
    order += [w_copy(c) for c in (6, 7, 0, 4, 1, 2, 5, 3)]
    for c in order:
        c.start()

    def strassen_rhs(x0, x1):
        b11, b12 = [jnp.concatenate([x[:, 0:128], x[:, 256:384]], axis=1) for x in (x0, x1)]
        b21, b22 = [jnp.concatenate([x[:, 128:256], x[:, 384:512]], axis=1) for x in (x0, x1)]
        ops = [b11 + b22, b11, b12 - b22, b21 - b11, b22, b11 + b12, b21 + b22,
               x0[:, 512:], x1[:, 512:]]
        return _pack(jnp.concatenate(ops, axis=1).astype(BF16))

    def load_x(t, first):
        x = xio[rows(t, 256), :].astype(F32)
        if first is not True:
            x = jnp.where(first, x, xres[rows(t, 256), :])
        xres[rows(t, 256), :] = x
        return x

    wphi_copy.wait()
    cphi = jnp.zeros((FA, D), F32)
    hh = lax.broadcasted_iota(jnp.int32, (HA, D), 0) * FA
    jj = lax.broadcasted_iota(jnp.int32, (HA, D), 1)
    for d in range(FA):
        cphi = _dot(wphi[d], jnp.where(jj == hh + d, 1.0, 0.0).astype(BF16)) + cphi
    cb = jnp.concatenate(
        [jnp.broadcast_to(cphi[f:f + 1, :], (8, D)) for f in range(FA)], axis=0)
    for g in range(GA):
        row = lax.broadcasted_iota(jnp.int32, (GR, 256), 0)
        col = lax.broadcasted_iota(jnp.int32, (GR, 256), 1) + 128 * g
        lo = (8 * g + (row & 7)) * FA
        bds[g] = _pack(jnp.where(jnp.logical_and(col >= lo, col < lo + FA),
                                 cb[:, 128 * g:128 * g + 256], 0.0).astype(BF16))

    def folded(rr):
        out = [[], [], []]
        for g in range(GA):
            ws = []
            for i in range(2):
                c0 = i * D + 128 * g
                w = _dot_nt(_unpack(bds[g]), wqkv[rr, c0:c0 + 256]).reshape(FA, 8, 128)
                ws.append(((w[1:] - w[0:1]) * LOG2E).reshape(GR - 8, 128))
            out[0].append(jnp.concatenate([ws[1], ws[0][GR - 16:, :]], axis=0))
            out[1].append(ws[0][0:GR - 16, :])
        wvt = wqkv[rr, 2 * D:3 * D].T.astype(F32)
        out[2] = [wvt[g * GR:(g + 1) * GR, :] for g in range(GA)]
        return out

    def fold(c, _):
        wa_copy(c).wait()
        wa, wb = folded(rows(2 * c, 128)), folded(rows(2 * c + 1, 128))
        for i in range(3):
            for p in range(2):
                a11, a12, a21, a22 = wa[i][2 * p], wb[i][2 * p], wa[i][2 * p + 1], wb[i][2 * p + 1]
                ops = [a11 + a22, a21 + a22, a11, a22, a11 + a12, a21 - a11, a12 - a22]
                for m, w in enumerate(ops):
                    wat[2 * i + p, m, 0:w.shape[0] // 2, rows(c, 128)] = _pack(w.astype(BF16))
        return 0

    lax.fori_loop(0, 2, fold, 0)
    x_copy(-1).wait()
    wa_copy(2).wait()
    x = _layernorm(load_x(0, True))
    xa[...] = strassen_rhs(x[0:128], x[128:])
    for i, ws in enumerate(folded(pl.ds(512, 128))):
        for g, w in enumerate(ws):
            wat[2 * i + g // 2, 7, 0:w.shape[0] // 2, rows(g % 2, 128)] = _pack(w.astype(BF16))

    def pair_rows(ph, q, t0, n):
        return _unpack(jnp.concatenate(
            [ph[t0 + u, rows(q, 2 * FA), :] for u in range(n)], axis=1))

    def a1(first, j, _):
        @pl.when(jnp.logical_and(first, j < na - 1))
        def _():
            x_copy(j).wait()

        @pl.when(jnp.logical_and(first, j == na - 1))
        def _():
            x_copy(na - 1).wait()

        def features(ph, t, g, y):
            for f, w in enumerate(_feature_map(y)):
                ph[t, pl.ds(GR * g + f, 8, stride=FA), :] = w

        def tail(n, xs, g, u):
            nr = GR // 2 - 8 if n // 2 == 1 else GR // 2
            return _dot_nt(_unpack(wat[n, 7, 0:nr, 128 * g:128 * (g + 1)]),
                           xs[:, 1792 + 128 * u:1920 + 128 * u])

        def a_dots(n, xs, emit, tie, t10):
            nr = GR // 2 - 8 if n // 2 == 1 else GR // 2
            p = n % 2

            def prod(m):
                return _dot_nt(_unpack(tie(wat[n, m, 0:nr, :])), xs[:, 256 * m:256 * (m + 1)])

            m2, m4 = prod(1), prod(3)
            emit(2 * p + 1, 0, m4 + (m2 - (-t10)))
            t01 = tail(n, xs, 0, 1)
            m3, m5 = prod(2), prod(4)
            emit(2 * p, 1, m5 + (m3 - (-t01)))
            m1 = prod(0)
            c22 = prod(5) + (m1 + (m3 - m2))
            emit(2 * p + 1, 1, tail(n, xs, 1, 1) + c22)
            t10 = tail(n + 1, xs, 1, 0) if n < 5 else None
            c11 = tail(n, xs, 0, 0) + (m1 + (m4 - m5))
            emit(2 * p, 0, prod(6) + c11)
            return t10

        vs = {}
        cur = xa[...]
        dl = (3, 8, 13, 30, 33, 36, 39, 41)
        for u in range(0, asub, 2):
            t = j * (asub // 2) + u // 2
            xs = _unpack(cur)
            tn = t + 1
            x = load_x(tn if u + 2 < asub else jnp.minimum(tn, (na - 1) * (asub // 2)), first)
            rest, seen, nxt = {}, [], []

            def tie(w):
                seen.append(0)
                if len(seen) - 1 not in dl:
                    return w
                n = len(nxt)
                nxt.append(strassen_rhs(*[
                    _layernorm(x[128 * e + 16 * n:128 * e + 16 * n + 16, :]) for e in range(2)]))
                z = jnp.concatenate(
                    [nxt[n][:, 256 * c:256 * (c + 1)] for c in range(8)], axis=0)
                return jnp.concatenate([jnp.where(j < 0, z, w[0:64, :]), w[64:, :]], axis=0)

            def emit_k(g, e, y):
                features(phk, u + e, g, y[0:GR - 8, :])
                rest[g, e] = y[GR - 8:, :]

            def emit_q(g, e, y):
                features(phq, 2 * t + e, g, jnp.concatenate([y, rest[g, e]], axis=0))

            def emit_v(g, e, y):
                for q in range(4):
                    vs[4 * g + q, u + e] = y[40 * q:40 * q + 40, :]

            t10 = tail(0, xs, 1, 0)
            for n in range(6):
                t10 = a_dots(n, xs, (emit_k, emit_q, emit_v)[n // 2], tie, t10)
            cur = jnp.concatenate(nxt, axis=0)
        xa[...] = cur
        row = lax.broadcasted_iota(jnp.int32, (2 * VR, 4 * FA), 0)
        col = lax.broadcasted_iota(jnp.int32, (2 * VR, 4 * FA), 1)
        split = jnp.where(row < 2 * FA, FA, 2 * FA + 4)
        same = (row >= split) == (col >= 2 * FA)
        for q in range(PA):
            v = jnp.concatenate([vs[q, u] for u in range(asub)], axis=1)
            v = jnp.concatenate([v, jnp.ones((8, TA), F32)], axis=0)
            kv = _dot_nt(v.astype(BF16), pair_rows(phk, q, 0, asub))
            kv = kv + jnp.where(j == 0, 0.0, kvacc[q])
            kvacc[q] = kv
            kvs[q] = _pack(jnp.where(same, kv, 0.0).astype(BF16))
        return 0

    def attend(j):
        low = lax.broadcasted_iota(jnp.int32, (8, TN), 0) < 4
        os_ = []
        for q in range(PA):
            nd = _dot(_unpack(kvs[q]), pair_rows(phq, q, j * nsub, nsub))
            rab = 1.0 / (nd[40:48, :] + 1e-6)
            rba = pltpu.roll(rab, 4, 0)
            ra = jnp.where(low, rab, rba)
            rb = jnp.where(low, rba, rab)
            os_.append(nd[0:40, :] * jnp.concatenate([ra, ra, rab, rb, rb], axis=0))
        return _pack(jnp.concatenate(os_, axis=0).astype(BF16).T)

    def project(j, o, slot):
        ns = TN // SEG
        xs = []
        r = rows(j, TN)
        old, new = xres[r, :], {}
        for part in ((1, 2), (0, 3)):
            grp = [b + k for b in range(0, TN // 16, 4) for k in part]
            oo = jnp.concatenate([o[8 * g:8 * g + 8, :] for g in grp], axis=0)
            x = _dot(_unpack(oo), woa[...]) + jnp.concatenate(
                [old[16 * g:16 * g + 16, :] for g in grp], axis=0)
            for n, g in enumerate(grp):
                new[g] = x[16 * n:16 * n + 16, :]
            xs.append(x)
        xres[r, :] = jnp.concatenate([new[g] for g in range(TN // 16)], axis=0)
        for s in range(ns):
            x = xs[0][16 * s + 8 - 8 * (s % 2):16 * s + 16 - 8 * (s % 2), :]
            x = _layernorm(x)
            x = x - x[KE:KE + 1, :]
            for c in range(D // 128):
                xe[c, pl.ds((slot * ns + s) * KE, 8), :] = x[:, 128 * c:128 * (c + 1)]

    def extra_keys(seg, p):
        k = jnp.concatenate(
            [ke[seg // 16, 3 * p + c, pl.ds((seg % 16) * KE, 8), :] for c in range(3)], axis=1)
        return jnp.where(lax.broadcasted_iota(jnp.int32, (8, PW), 0) < KE, k, 0.0)

    def b_residual(i):
        r = rows(i, TB)
        x = xres[r, :] + rsave[...]
        xres[r, :] = x
        xio[r, :] = x.astype(BF16)
        return x

    def b_finish(i):
        xn = _layernorm(b_residual(i))
        xl[rows(jnp.minimum(i, 2), TB), :] = xn
        return xn

    def b_tile(mem, xn, i, side):
        for u in range(4):
            t0 = u * SEG
            late = u % 2 == 0
            ext = [SEG * v + (24 if v % 2 == 0 else 0) for v in range(4)]

            def place(y, z):
                return jnp.concatenate([y, z] if late else [y[0:M], z, y[M:]], axis=0)

            def fix_qv(p, kind, y):
                cols = pl.ds((3 * p + 2 * kind) * PW, PW)
                ysave[0:y.shape[0], cols] = y

                def get():
                    z = place(ysave[0:32, cols], ysave[32 + 8 * u:40 + 8 * u, cols])
                    if not late:
                        return z
                    r0 = 64 * u + 8 * p
                    tie = jnp.where(i < 0, side[r0:r0 + 8, 256 * kind:256 * kind + PW], z[16:24, :])
                    return jnp.concatenate([z[0:16, :], tie, z[24:, :]], axis=0)
                return get

            def fix_k(p, k):
                cols = pl.ds((3 * p + 1) * PW, PW)
                ysave[0:32, cols] = k
                return lambda: place(ysave[0:32, cols], extra_keys(4 * i + u, p))

            def fix_o(p, o):
                cols = slice(p * PW, (p + 1) * PW)
                r0 = 0 if u == 3 else 8 + 8 * u
                osave[r0:r0 + 8, cols] = o[32:L, :]
                if u == 3:
                    return jnp.concatenate([o[0:32, :], osave[:, cols]], axis=0)
                return o[0:32, :]

            h = jnp.concatenate(
                [mem, xn[t0:t0 + 24, :] if late else xn[t0 + 8:t0 + SEG, :]], axis=0)
            hk = (h - xn[ext[u] + KE:ext[u] + KE + 1, :]).astype(BF16)
            if u == 0:
                h = jnp.concatenate([h] + [xn[e:e + 8, :] for e in ext], axis=0)
            r = _segment(h, hk, wqv, wk, wob, wsum, pst, lst, fix_qv, fix_k, fix_o, u)
            mem = r[0:M, :]
            if u < 3:
                rsave[t0:t0 + 24, :] = r[M:, :]
            else:
                rsave[t0:t0 + SEG, :] = r[M:L, :]
                for v in range(3):
                    rsave[SEG * v + 24:SEG * v + SEG, :] = r[L + 8 * v:L + 8 * v + 8, :]
        return mem

    def layer(l, _):
        def wait_first(copies):
            @pl.when(l == 0)
            def _():
                for c in copies:
                    c.wait()

        with jax.named_scope("a1"):
            lax.fori_loop(0, na, functools.partial(a1, l == 0), 0)

        def a2(n, _):
            for m, cs in enumerate(((6, 7, 0, 4), (1,), (2, 5), (3,))):
                @pl.when(jnp.logical_and(l == 0, n == m))
                def _():
                    for c in cs:
                        w_copy(c).wait()

            ty, half = n % 2, n // 2
            o0 = attend(2 * n)
            o1 = attend(2 * n + 1)

            def sample(w):
                z = [w[64 * a + 56:64 * a + 64, :] for a in range(D // 128)]
                out = []
                for y in z:
                    acc = y[:, 0:128]
                    for c in range(1, y.shape[1] // 128):
                        acc = acc | y[:, 128 * c:128 * (c + 1)]
                    out.append(acc)
                return jnp.concatenate(out, axis=1)

            mr = 16 * KE

            def side(job):
                w = _pack(wraw[n, rows(int(job), 2 * PW), :].T)
                wqv[n, :, rows(int(job), 2 * PW)] = w
                return sample(w)

            for job in '01':
                o1 = jnp.concatenate([o1[0:8, :], jnp.where(n < 0, side(job), o1[8:16, :]),
                                      o1[16:, :]], axis=0)
            project(2 * n, o0, 0)
            ties = [pltpu.bitcast(side(job), F32) for job in '23']
            project(2 * n + 1, o1, 1)
            x = jnp.concatenate([xe[c, 0:mr, :] for c in range(D // 128)], axis=1)
            for tie in ties:
                x = jnp.concatenate([jnp.where(n < 0, tie, x[0:8, :]), x[8:, :]], axis=0)
            x = x.astype(BF16)
            r = rows(n, TB // NW)
            xb[r, :] = _layernorm(xres[r, :])
            rsave[r, :] = jnp.zeros((TB // NW, D), F32)
            for ref in (ysave, osave, pst, lst):
                ref[rows(ty, 8), 0:128] = jnp.zeros((8, 128), ref.dtype)

            def view(ref, start, size, align):
                return ref.at[pl.ds(pl.multiple_of(start, align), size)]

            wo_src = view(wraw.at[4 + half], 64 * ty, HD // 2 - 64, 64)
            wo_dst = view(wob, QW * half + 32 * ty, QW - 32, 32)
            wk_src = view(wraw.at[6 + half], QW * ty, QW, QW)
            sum_dst = view(wsum, 64 * n, 64, 64), view(wsum, 256 + 32 * n, 32, 32)

            def wo_rows(t, rr):
                return _pack(wo_src[rows(8 * t + rr, 16), :])

            def sums(is_o, g, j, rr, tie):
                t0, sz = _STARS[g]
                names = _star_sums(sz)[j]
                if is_o:
                    row = jnp.where(n < 0, jnp.concatenate([tie] * 5, axis=1), wo_rows(t0 + j, rr))
                    wo_dst[rows(8 * (t0 + j) + rr, 8), :] = row
                val = {}
                for x, y in [(j, k) for k in range(sz)] + [(k, j) for k in range(sz) if k != j]:
                    if is_o and x == j:
                        w = row[:, 128 * y:128 * y + 128]
                    elif is_o and x < j:
                        w = jnp.where(n < 0, tie, wo_dst[rows(8 * (t0 + x) + rr, 8), rows(y, 128)])
                    else:
                        w = jnp.where(n < 0, tie, wo_rows(t0 + x, rr)[:, 128 * y:128 * y + 128] if is_o
                                      else wqv[n, rows(8 * x + rr, 8), rows(t0 + y, 128)])
                    val[x, y] = _unpack(w).astype(F32)
                others = [k for k in range(sz) if k != j]
                out = [functools.reduce(lambda z, k: z - val[j, k], others, val[j, j]),
                       functools.reduce(lambda z, k: z + val[k, j], others, val[j, j])]
                out += [val[x, y] + val[y, x] for x, y in names[2:]]
                sum_dst[is_o][rows(rr, 8),
                              pl.ds(128 * _star_slot(g, names[0]), 128 * len(names))] = _pack(
                    jnp.concatenate(out, axis=1).astype(BF16))

            def k_tiles(t, c, tie):
                w = _pack(wk_src[rows(t, 256), rows(c, 128)])
                w = jnp.concatenate([jnp.where(n < 0, tie, w[0:8, :]), w[8:64, :],
                                     jnp.where(n < 0, tie, w[64:72, :]), w[72:, :]], axis=0)
                wk[n, rows(c, 64), rows(t, 256)] = _pack(_unpack(w).T)

            kjobs = [functools.partial(k_tiles, t, c) for t in range(6) for c in range(5)]
            todo = []
            for g in range(5):
                for j in range(_STARS[g][1]):
                    for rr in range(4):
                        if len(todo) % 10 < 3:
                            todo += kjobs[-1:]
                            del kjobs[-1:]
                        todo += [functools.partial(sums, False, g, j, 2 * rr),
                                 functools.partial(sums, True, g, j, rr),
                                 functools.partial(sums, False, g, j, 2 * rr + 1)]
            assert not kjobs
            left = [48]

            def emit(t, k):
                ke[n, t, 0:mr, :] = k
                left[0] -= 1
                if left[0] < 48 - 2:
                    m = -(-len(todo) // (left[0] + 1))
                    for g in range(m):
                        g = 8 * (14 * g // m)
                        todo.pop(0)(pltpu.bitcast(k[g:g + 8, :], U32))

            for v in range(HD // 256):
                k = _dot_nt(x, wraw[6 + v // 12, rows(v % 12, 256), :])
                emit(2 * v, k[:, 0:128])
                emit(2 * v + 1, k[:, 128:])
            return 0

        wait_first([woa_copy, mem0_copy])
        with jax.named_scope("a2"):
            lax.fori_loop(0, NW, a2, 0)

        def b_step(i, mem):
            xn = xb[...]
            side = b_finish(jnp.maximum(i - 1, 0))
            nxt = _layernorm(xres[rows(jnp.minimum(i + 1, nb - 1), TB), :])
            xb[...] = nxt
            side = jnp.concatenate([side, nxt], axis=0)
            mem = b_tile(mem, xn, i, side)

            @pl.when(jnp.logical_and(l == 1, i >= 1))
            def _():
                out_copy(i - 1).start()
            return mem

        with jax.named_scope("b"):
            lax.fori_loop(0, nb, b_step, mem0[...].astype(F32))

        b_residual(nb - 1)

        @pl.when(l == 0)
        def _():
            xa[...] = strassen_rhs(xl[0:128, :], xl[128:256, :])
        return 0

    lax.fori_loop(0, 2, layer, 0)
    out_copy(nb - 1).start()
    pltpu.make_async_copy(xio, out_hbm, sem_out.at[0]).wait()


@jax.jit
def pallas_interleave_layers__linear_kernel_hedgehog__memory_aug_recurrent_mem_tr__prompt_kernel(
    A_x, A_wqkv, A_w_phi, A_wo, B_x, B_mem0, B_Wq, B_Wk, B_Wv, B_Wo, B_seg_len,
):
    del B_x
    del B_seg_len
    x = A_x.reshape(S, D)
    wphi = A_w_phi.transpose(1, 2, 0)
    mem0 = B_mem0.reshape(M, D)
    wq, wk, wv = (w.transpose(1, 2, 0).reshape(2, HD // 2, D) for w in (B_Wq, B_Wk, B_Wv))
    wo = B_Wo.reshape(2, HD // 2, D)
    hbm = pl.BlockSpec(memory_space=pl.ANY)
    out = pl.pallas_call(
        _kernel,
        out_shape=jax.ShapeDtypeStruct((S, D), A_x.dtype),
        in_specs=[hbm] * 9,
        out_specs=hbm,
        scratch_shapes=[
            pltpu.VMEM((S, D), BF16),
            pltpu.VMEM((D, 3 * D), BF16),
            pltpu.VMEM((FA, FA, HA), BF16),
            pltpu.VMEM((D, D), BF16),
            pltpu.VMEM((M, D), BF16),
            pltpu.VMEM((S, D), F32),
            pltpu.VMEM((64, 2048), U32),
            pltpu.VMEM((3 * TB, D), F32),
            pltpu.VMEM((TB, D), F32),
            pltpu.VMEM((GA, GR // 2, 256), U32),
            pltpu.VMEM((6, 8, GR // 2, 256), U32),
            pltpu.VMEM((S // 128, D, 128), U32),
            pltpu.VMEM((TA // 128, D, 128), U32),
            pltpu.VMEM((PA, 2 * VR, 4 * FA), F32),
            pltpu.VMEM((PA, VR, 4 * FA), U32),
            pltpu.VMEM((8, HD // 2, D), BF16),
            pltpu.VMEM((4, D // 2, HD // 2), U32),
            pltpu.VMEM((NW, D // 2, QW), U32),
            pltpu.VMEM((HD // 2, D), U32),
            pltpu.VMEM((6 * 64, NS * 128), U32),
            pltpu.VMEM((D // 128, 16 * KE + 8, 128), F32),
            pltpu.VMEM((NW, HD // 128, 16 * KE + 8, 128), F32),
            pltpu.VMEM((64, 3 * HD), F32),
            pltpu.VMEM((32, HD), F32),
            pltpu.VMEM((L, HD // 2), U32),
            pltpu.VMEM((16, 66 * 128), U32),
            pltpu.VMEM((TB, D), F32),
            pltpu.SemaphoreType.DMA((17 + S // TA,)),
            pltpu.SemaphoreType.DMA((1,)),
        ],
        compiler_params=pltpu.CompilerParams(vmem_limit_bytes=126 * 1024 * 1024,
                                             disable_bounds_checks=True,
                                             disable_semaphore_checks=True),
    )(x, A_wqkv, wphi, A_wo, mem0, wq, wk, wv, wo)
    return out.reshape(1, S, D)
```

```python
import functools

import jax
import jax.numpy as jnp
from jax import lax
import jax.experimental.pallas as pl
import jax.experimental.pallas.tpu as pltpu

F32 = jnp.float32
BF16 = jnp.bfloat16
U32 = jnp.uint32

S = 2048
D = 640
HA = 32
FA = 20
GA = 4
GR = 8 * FA
VR = 24
PA = HA // 2
TN = 256
TA = 512
HB = 32
DH = 192
HD = HB * DH
M = 8
SEG = 32
L = M + SEG
PW = 2 * DH
NP = HB // 2
TB = 128
NW = 4
QW = HD // NW

NT = (((1,), (1,)), ((), ()))
LOG2E = 1.4426950408889634
HALF_ULP = 0.0040612


def _dot(a, b):
    return jnp.dot(a, b, preferred_element_type=F32)


def _dot_nt(a, b):
    return lax.dot_general(a, b, NT, preferred_element_type=F32)


def _pack(a):
    return pltpu.bitcast(a, U32)


def _unpack(a):
    return pltpu.bitcast(a, BF16)


def _interleave(a, b):
    lo = lax.bitcast_convert_type(a, U32) >> 16
    hi = lax.bitcast_convert_type(b, U32) & jnp.uint32(0xFFFF0000)
    return lo | hi


def _recip(x):
    r = pl.reciprocal(x, approx=True)
    return r * (2.0 - x * r)


def _layernorm(x):
    m = jnp.mean(x, axis=-1, keepdims=True)
    c = x - m
    v = jnp.mean(c * c, axis=-1, keepdims=True)
    return c * lax.rsqrt(v + 1e-5)


def _feature_map(p):
    t = p.shape[-1]
    p3 = jnp.concatenate([jnp.zeros((8, t), F32), p], axis=0).reshape(FA, 8, t)
    mx = jnp.max(p3, axis=0)
    mn = jnp.min(p3, axis=0)
    sp, sn = jnp.exp2(p3[0] - mx), jnp.exp2(mn - p3[0])
    for f in range(1, FA):
        sp, sn = sp + jnp.exp2(p3[f] - mx), sn + jnp.exp2(mn - p3[f])
    lp = (mx - HALF_ULP) + jnp.log2(sp)
    ln = (mn + HALF_ULP) - jnp.log2(sn)
    return [_interleave(jnp.exp2(p3[f] - lp), jnp.exp2(ln - p3[f])) for f in range(FA)]


def _tiles(a, odd):
    t0, t1, t2 = a[:, 0:128], a[:, 128:256], a[:, 256:384]
    return (t1, t2, t0) if odd else (t1, t0, t2)


def _own_weights(a, odd):
    lane = lax.broadcasted_iota(jnp.int32, (L, 128), 1)
    mid, own, _ = _tiles(a, odd)
    return jnp.concatenate(
        [jnp.where(lane < 64, mid, 0.0), jnp.where(lane < 64, 0.0, mid), own,
         jnp.zeros((128 - 3 * L, 128), F32)], axis=0).astype(BF16)


def _others(even, odd, pad):
    parts = [_tiles(odd, 1)[2], _tiles(even, 0)[2]]
    if pad:
        parts.append(jnp.zeros((128 - 2 * L, 128), F32))
    return jnp.concatenate(parts, axis=0).astype(BF16)


def _softmax3(s3):
    row = lax.broadcasted_iota(jnp.int32, (L, 128), 0)
    col = lax.broadcasted_iota(jnp.int32, (L, 128), 1)
    first = col < L
    second = jnp.logical_and(col >= L, col < 2 * L)
    key = jnp.where(first, col, col - L)
    valid = jnp.logical_or(row < M, row >= key)
    out, other = [], []
    for odd in range(2):
        own = pltpu.roll(s3[odd][L:, :], 128 - L if odd else 128 - 2 * L, 1)
        s = (jnp.where(first, s3[2][0:L, :], own) if odd
             else jnp.where(first, own, s3[2][L:, :]))
        s = jnp.where(valid, (s + s3[odd][0:L, :]) * (DH ** -0.5), -1e9)
        m0 = jnp.max(jnp.where(first, s, -jnp.inf), axis=-1, keepdims=True)
        m1 = jnp.max(jnp.where(second, s, -jnp.inf), axis=-1, keepdims=True)
        e = jnp.exp(s - jnp.where(first, m0, m1))
        e0 = jnp.where(first, e, 0.0)
        e1 = jnp.where(second, e, 0.0)
        p0 = e0 * _recip(jnp.sum(e0, axis=-1, keepdims=True))
        p1 = e1 * _recip(jnp.sum(e1, axis=-1, keepdims=True))
        own = pltpu.roll(p1, L, 1) if odd else pltpu.roll(p0, 2 * L, 1)
        out.append(jnp.concatenate([p0 + p1, own], axis=0))
        other.append(p0 if odd else p1)
    out.append(jnp.concatenate([other[1], other[0]], axis=0))
    return _pack(jnp.concatenate(out, axis=1).astype(BF16))


_T = {5: (-1.5, -0.5, 0.0, 0.5, 1.5), 4: (-1.25, -0.25, 0.25, 1.25)}
_STARS = tuple((5 * g, 5 if g < 4 else 4) for g in range(5))


def _star_sums(n):
    own = {j: [] for j in range(n)}
    for a in range(n):
        for b in range(a + 1, n):
            own[a if (b - a) % 2 else b].append((a, b))
    return [['r%d' % j, 'c%d' % j] + own[j] for j in range(n)]


def _star_slot(g, name):
    return 20 * g + [x for grp in _star_sums(_STARS[g][1]) for x in grp].index(name)


NS = 94


def _star_lhs(n, get, scaled):
    t = _T[n]
    f = [get(0, j) for j in range(n)]
    g = [get(1, j) + t[j] * f[j] if t[j] else get(1, j) for j in range(n)]
    out = {'r%d' % j: f[j] for j in range(n)}
    out.update({'c%d' % j: g[j] for j in range(n)})
    for a in range(n):
        for b in range(a + 1, n):
            d = t[a] - t[b]
            if scaled:
                l = (g[a] - g[b]) * (1.0 / d)
                out[a, b], out[b, a, 0], out[a, b, 0] = l, f[b] - l, f[a] - l
            else:
                l = g[a] - g[b]
                out[a, b], out[b, a, 0], out[a, b, 0] = l, d * f[b] - l, d * f[a] - l
    return out


def _star_apply(n, lhs, plain, mixed, scaled, acc=None):
    t = _T[n]
    p, q = ([None] * n, [None] * n) if acc is None else (list(acc[0]), list(acc[1]))
    started = set()

    def start(j):
        if j not in started:
            started.add(j)
            dp, dq = [_dot(lhs(k % j), mixed(k % j)) for k in ('r%d', 'c%d')]
            p[j] = dp if p[j] is None else dp + p[j]
            q[j] = dq if q[j] is None else dq + q[j]

    for a in range(n):
        for b in range(a + 1, n):
            start(a)
            start(b)
            d = t[a] - t[b]
            m6 = _dot(lhs((b, a, 0)), plain(b, a))
            m7 = _dot(lhs((a, b, 0)), plain(a, b))
            m = _dot(lhs((a, b)), mixed((a, b))) + (m6 + m7)
            if scaled:
                q[a], q[b] = q[a] - (-d) * m6, q[b] - d * m7
                p[a], p[b] = m + p[a], m + p[b]
            else:
                q[a], q[b] = m6 + q[a], q[b] - m7
                m = m * (-1.0 / d) if d != -1.0 else m
                p[a], p[b] = p[a] - m, p[b] - m
    return p, q


def _star_result(n, p, q):
    return [jnp.concatenate([p[j], q[j] - _T[n][j] * p[j] if _T[n][j] else q[j]], axis=0)
            for j in range(n)]


_PLAN = (
    ((5, 11, 15, 20, 26), (), (1, 9, 10)),
    ((3, 6, 9, 11, 13), (0, 6, 7, 13), (2, 8, 9)),
    ((3, 6, 8, 11, 14), (1, 3, 8, 11), (2, 9, 10)),
    ((3, 6, 9, 11, 14), (1, 3, 8, 12), (2, 5, 6)),
)


def _segment(h, wqv, wk, wob, wsum, pst, lst, fix_y, fix_o, step):
    ys = {p: [None] * 3 for p in range(NP)}
    ss, pvs, os_ = {}, {}, {}
    hb = h.astype(BF16)

    used = [0]

    def staged(ops, through_memory):
        if not through_memory:
            ops = {k: v.astype(BF16) for k, v in ops.items()}
            return ops.get
        names, w, c0 = list(ops), next(iter(ops.values())).shape[1], used[0]
        used[0] += w * len(names)
        lst[:, c0:used[0]] = _pack(jnp.concatenate(list(ops.values()), axis=1).astype(BF16))
        return lambda k: _unpack(lst[:, pl.ds(c0 + w * names.index(k), w)])

    def summed(slab, g, name):
        return wsum[64 * slab:64 * slab + 64, pl.ds(128 * _star_slot(g, name), 128)]

    def keys(n):
        k = _dot(hb, _unpack(wk[n // 2, :, pl.ds(n % 2 * QW, QW)]))
        for e in range(4):
            ys[4 * n + e][1] = fix_y(4 * n + e, 1, k[:, e * PW:(e + 1) * PW])

    def proj(p):
        def w(lo, hi):
            return _unpack(jnp.concatenate(
                [wqv[2 * i + p // 8, lo:hi, pl.ds(p % 8 * PW, PW)] for i in range(2)], axis=1))
        if p == 0:
            y = _dot(hb[:, 0:512], w(0, 256))
            y = _dot(hb[:, 512:], w(256, D // 2)) + y
        else:
            y = _dot(hb, w(0, D // 2))
        for i in range(2):
            ys[p][2 * i] = fix_y(p, 2 * i, y[:, i * PW:(i + 1) * PW])

    def wide_proj(half, g, i, lhs, tiles):
        t0, n = _STARS[g]
        w, ws, slab = (wk, half, 6 + half) if i == 1 else (wqv, i + half, i + half)
        if n == 4:
            tail = _dot(hb[:, 512:], _unpack(w[ws, 256:, 128 * t0:]))
        out = _star_result(n, *_star_apply(
            n, lhs[n],
            lambda j, l: _unpack(w[ws, 64 * j:64 * j + 64, pl.ds(128 * (t0 + l), 128)]),
            lambda name: _unpack(summed(slab, g, name)), False))
        for l, y in enumerate(out):
            tiles[t0 + l] = y + tail[:, 128 * l:128 * l + 128] if n == 4 else y
        for e in range(8):
            if all(3 * e + k in tiles for k in range(3)):
                ys[8 * half + e][i] = fix_y(8 * half + e, i, jnp.concatenate(
                    [tiles.pop(3 * e + k) for k in range(3)], axis=1))

    def weights(c, i, which):
        if i < 2:
            return _own_weights(ys[2 * c + i][which](), i)
        return _others(ys[2 * c][which](), ys[2 * c + 1][which](), True)

    def score_round(n):
        for c, i in (divmod(j, 3) for j in range(4 * n, 4 * n + 4)):
            if i < 2:
                q = jnp.concatenate(_tiles(ys[2 * c + i][0](), i)[0:2], axis=0).astype(BF16)
            else:
                q = _others(ys[2 * c][0](), ys[2 * c + 1][0](), False)
            ss[c, i] = _dot_nt(q, weights(c, i, 1))
            if i == 2:
                pst[:, c * PW:(c + 1) * PW] = _softmax3([ss.pop((c, k)) for k in range(3)])

    def pv_round(n):
        for c, i in (divmod(j, 3) for j in range(4 * n, 4 * n + 4)):
            pvs[c, i] = _dot(_unpack(pst[:, pl.ds(c * PW + 128 * i, 128)]), weights(c, i, 2))
            if i == 2:
                o0, o1, o2 = [pvs.pop((c, k)) for k in range(3)]
                os_[2 * c] = fix_o(2 * c, jnp.concatenate(
                    [o0[L:, :], o0[0:L, :], o2[L:, :]], axis=1))
                os_[2 * c + 1] = fix_o(2 * c + 1, jnp.concatenate(
                    [o2[0:L, :], o1[0:L, :], o1[L:, :]], axis=1))

    def slot(n):
        if n >= 2:
            pv_round(n - 2)
        if n < 6:
            score_round(n)

    def oproj(lo, hi, r):
        o = jnp.concatenate([os_.pop(p) for p in range(lo, hi)], axis=1).astype(BF16)
        y = _dot(o, _unpack(wob[lo * DH:hi * DH, :]))
        return y if r is None else y + r

    def wide_oproj(stars, r):
        def o_tile(t):
            return os_[t // 3][:, 128 * (t % 3):128 * (t % 3) + 128]

        for n in (4, 5):
            sel = [divmod(x, 5) for x in stars if _STARS[x % 5][1] == n]
            if not sel:
                continue
            t0 = [24 * half + _STARS[g][0] for half, g in sel]
            if n == 4:
                ts = [t + j for t in t0 for j in range(4)]
                y = _dot(jnp.concatenate([o_tile(t) for t in ts], axis=1).astype(BF16),
                         _unpack(jnp.concatenate(
                             [wob[64 * t:64 * t + 64, 512:] for t in ts], axis=0)))
                r[0] = y + r[0] if 0 in r else y
            r[n] = _star_apply(
                n, staged(_star_lhs(n, lambda i, j: jnp.concatenate(
                    [o_tile(t + j)[32 * i:32 * i + 32] for t in t0], axis=1), True), False),
                lambda j, l: _unpack(jnp.concatenate(
                    [wob[pl.ds(64 * (t + j), 64), 128 * l:128 * l + 128] for t in t0], axis=0)),
                lambda name: _unpack(jnp.concatenate(
                    [summed(4 + half, g, name) for half, g in sel], axis=0)), True, r.get(n))
        return r

    after, kat, (o1, o2, o3) = _PLAN[step]
    if step == 0:
        lhs = {n: staged(_star_lhs(
            n, lambda i, j: h[32 * i:32 * i + 32, 128 * j:128 * j + 128], False), True)
               for n in (5, 4)}
        tiles = {}
    for unit in range(30 if step == 0 else NP):
        if step == 0:
            half, g, i = unit // 15, unit % 15 // 3, unit % 3
            wide_proj(half, g, i, lhs, tiles.setdefault((half, i), {}))
        else:
            proj(unit)
        if unit in kat:
            keys(kat.index(unit))
        for n in range(5):
            if after[n] == unit:
                slot(n)
    if step == 3:
        r = wide_oproj(range(0, o1), {})
        slot(5)
        r = wide_oproj(range(o1, o2), r)
        slot(6)
        slot(7)
        r = wide_oproj(range(o2, o3), r)
        r = wide_oproj(range(o3, 10), r)
        return jnp.concatenate(
            [x + y for x, y in zip(_star_result(5, *r[5]), _star_result(4, *r[4]) + [r[0]])],
            axis=1)
    r = oproj(0, o1, None) if o1 else None
    slot(5)
    r = oproj(o1, o2, r)
    slot(6)
    slot(7)
    r = oproj(o2, o3, r)
    return oproj(o3, NP, r)


def _kernel(x_hbm, wqkv_hbm, wphi_hbm, woa_hbm, mem0_hbm,
            wq_hbm, wk_hbm, wv_hbm, wo_hbm,
            out_hbm,
            xio, wqkv, wphi, woa, mem0, xres, xa, xl, xb, bds, wat, phq, phk, kvacc, kvs,
            wraw, wqv, wk, wob, wsum, ysave, osave, pst, lst, rsave, sem_in, sem_out):
    nsub = TN // 128
    na = S // TA
    asub = TA // 128
    nb = S // TB

    def rows(j, n):
        return pl.ds(j * n if isinstance(j, int) else pl.multiple_of(j * n, n), n)

    def x_copy(j):
        if isinstance(j, int) and j < 0:
            r = pl.ds(0, 256)
        elif isinstance(j, int) and j == na - 1:
            r = pl.ds(S - TA + 256, TA - 256)
        else:
            r = pl.ds(j * TA + 256 if isinstance(j, int)
                      else pl.multiple_of(j * TA + 256, 256), TA)
        return pltpu.make_async_copy(x_hbm.at[r, :], xio.at[r, :], sem_in.at[9 + j])

    def w_copy(c):
        src = (wq_hbm, wv_hbm, wo_hbm, wk_hbm)[c // 2 if isinstance(c, int) else 0]
        return pltpu.make_async_copy(src.at[c % 2], wraw.at[c], sem_in.at[9 + na + c])

    def wa_copy(c):
        r = pl.ds(512, 128) if isinstance(c, int) and c == 2 else rows(c, 256)
        return pltpu.make_async_copy(wqkv_hbm.at[r, :], wqkv.at[r, :], sem_in.at[3 + c])

    def out_copy(i):
        return pltpu.make_async_copy(xio.at[rows(i, TB), :],
                                     out_hbm.at[rows(i, TB), :], sem_out.at[0])

    wphi_copy = pltpu.make_async_copy(wphi_hbm, wphi, sem_in.at[0])
    woa_copy = pltpu.make_async_copy(woa_hbm, woa, sem_in.at[1])
    mem0_copy = pltpu.make_async_copy(mem0_hbm, mem0, sem_in.at[2])
    order = [wphi_copy, wa_copy(0), wa_copy(1), x_copy(-1), wa_copy(2)]
    order += [x_copy(j) for j in range(na)] + [woa_copy, mem0_copy]
    order += [w_copy(c) for c in (0, 1, 2, 3, 6, 7, 4, 5)]
    for c in order:
        c.start()

    def strassen_rhs(x0, x1):
        b11, b12 = [jnp.concatenate([x[:, 0:128], x[:, 256:384]], axis=1) for x in (x0, x1)]
        b21, b22 = [jnp.concatenate([x[:, 128:256], x[:, 384:512]], axis=1) for x in (x0, x1)]
        ops = [b11 + b22, b11, b12 - b22, b21 - b11, b22, b11 + b12, b21 + b22,
               x0[:, 512:], x1[:, 512:]]
        return _pack(jnp.concatenate(ops, axis=1).astype(BF16))

    def load_x(t, first):
        x = xio[rows(t, 256), :].astype(F32)
        if first is not True:
            x = jnp.where(first, x, xres[rows(t, 256), :])
        xres[rows(t, 256), :] = x
        return x

    wphi_copy.wait()
    cphi = jnp.zeros((FA, D), F32)
    hh = lax.broadcasted_iota(jnp.int32, (HA, D), 0) * FA
    jj = lax.broadcasted_iota(jnp.int32, (HA, D), 1)
    for d in range(FA):
        cphi = _dot(wphi[d], jnp.where(jj == hh + d, 1.0, 0.0).astype(BF16)) + cphi
    cb = jnp.concatenate(
        [jnp.broadcast_to(cphi[f:f + 1, :], (8, D)) for f in range(FA)], axis=0)
    for g in range(GA):
        row = lax.broadcasted_iota(jnp.int32, (GR, 256), 0)
        col = lax.broadcasted_iota(jnp.int32, (GR, 256), 1) + 128 * g
        lo = (8 * g + (row & 7)) * FA
        bds[g] = _pack(jnp.where(jnp.logical_and(col >= lo, col < lo + FA),
                                 cb[:, 128 * g:128 * g + 256], 0.0).astype(BF16))

    def folded(rr):
        out = [[], [], []]
        for g in range(GA):
            ws = []
            for i in range(2):
                c0 = i * D + 128 * g
                w = _dot_nt(_unpack(bds[g]), wqkv[rr, c0:c0 + 256]).reshape(FA, 8, 128)
                ws.append(((w[1:] - w[0:1]) * LOG2E).reshape(GR - 8, 128))
            out[0].append(jnp.concatenate([ws[1], ws[0][GR - 16:, :]], axis=0))
            out[1].append(ws[0][0:GR - 16, :])
        wvt = wqkv[rr, 2 * D:3 * D].T.astype(F32)
        out[2] = [wvt[g * GR:(g + 1) * GR, :] for g in range(GA)]
        return out

    def fold(c, _):
        wa_copy(c).wait()
        wa, wb = folded(rows(2 * c, 128)), folded(rows(2 * c + 1, 128))
        for i in range(3):
            for p in range(2):
                a11, a12, a21, a22 = wa[i][2 * p], wb[i][2 * p], wa[i][2 * p + 1], wb[i][2 * p + 1]
                ops = [a11 + a22, a21 + a22, a11, a22, a11 + a12, a21 - a11, a12 - a22]
                for m, w in enumerate(ops):
                    wat[2 * i + p, m, 0:w.shape[0] // 2, rows(c, 128)] = _pack(w.astype(BF16))
        return 0

    lax.fori_loop(0, 2, fold, 0)
    x_copy(-1).wait()
    wa_copy(2).wait()
    x = _layernorm(load_x(0, True))
    xa[...] = strassen_rhs(x[0:128], x[128:])
    for i, ws in enumerate(folded(pl.ds(512, 128))):
        for g, w in enumerate(ws):
            wat[2 * i + g // 2, 7, 0:w.shape[0] // 2, rows(g % 2, 128)] = _pack(w.astype(BF16))

    def pair_rows(ph, q, t0, n):
        return _unpack(jnp.concatenate(
            [ph[t0 + u, rows(q, 2 * FA), :] for u in range(n)], axis=1))

    def a1(first, j, _):
        @pl.when(jnp.logical_and(first, j < na - 1))
        def _():
            x_copy(j).wait()

        @pl.when(jnp.logical_and(first, j == na - 1))
        def _():
            x_copy(na - 1).wait()

        def features(ph, t, g, y):
            for f, w in enumerate(_feature_map(y)):
                ph[t, pl.ds(GR * g + f, 8, stride=FA), :] = w

        def tail(n, xs, g, u):
            nr = GR // 2 - 8 if n // 2 == 1 else GR // 2
            return _dot_nt(_unpack(wat[n, 7, 0:nr, 128 * g:128 * (g + 1)]),
                           xs[:, 1792 + 128 * u:1920 + 128 * u])

        def a_dots(n, xs, emit, tie, t10):
            nr = GR // 2 - 8 if n // 2 == 1 else GR // 2
            p = n % 2

            def prod(m):
                return _dot_nt(_unpack(tie(wat[n, m, 0:nr, :])), xs[:, 256 * m:256 * (m + 1)])

            m2, m4 = prod(1), prod(3)
            emit(2 * p + 1, 0, m4 + (m2 - (-t10)))
            t01 = tail(n, xs, 0, 1)
            m3, m5 = prod(2), prod(4)
            emit(2 * p, 1, m5 + (m3 - (-t01)))
            m1 = prod(0)
            c22 = prod(5) + (m1 + (m3 - m2))
            emit(2 * p + 1, 1, tail(n, xs, 1, 1) + c22)
            t10 = tail(n + 1, xs, 1, 0) if n < 5 else None
            c11 = tail(n, xs, 0, 0) + (m1 + (m4 - m5))
            emit(2 * p, 0, prod(6) + c11)
            return t10

        vs = {}
        cur = xa[...]
        dl = (3, 8, 13, 30, 33, 36, 39, 41)
        for u in range(0, asub, 2):
            t = j * (asub // 2) + u // 2
            xs = _unpack(cur)
            tn = t + 1
            x = load_x(tn if u + 2 < asub else jnp.minimum(tn, (na - 1) * (asub // 2)), first)
            rest, seen, nxt = {}, [], []

            def tie(w):
                seen.append(0)
                if len(seen) - 1 not in dl:
                    return w
                n = len(nxt)
                nxt.append(strassen_rhs(*[
                    _layernorm(x[128 * e + 16 * n:128 * e + 16 * n + 16, :]) for e in range(2)]))
                z = jnp.concatenate(
                    [nxt[n][:, 256 * c:256 * (c + 1)] for c in range(8)], axis=0)
                return jnp.concatenate([jnp.where(j < 0, z, w[0:64, :]), w[64:, :]], axis=0)

            def emit_k(g, e, y):
                features(phk, u + e, g, y[0:GR - 8, :])
                rest[g, e] = y[GR - 8:, :]

            def emit_q(g, e, y):
                features(phq, 2 * t + e, g, jnp.concatenate([y, rest[g, e]], axis=0))

            def emit_v(g, e, y):
                for q in range(4):
                    vs[4 * g + q, u + e] = y[40 * q:40 * q + 40, :]

            t10 = tail(0, xs, 1, 0)
            for n in range(6):
                t10 = a_dots(n, xs, (emit_k, emit_q, emit_v)[n // 2], tie, t10)
            cur = jnp.concatenate(nxt, axis=0)
        xa[...] = cur
        row = lax.broadcasted_iota(jnp.int32, (2 * VR, 4 * FA), 0)
        col = lax.broadcasted_iota(jnp.int32, (2 * VR, 4 * FA), 1)
        split = jnp.where(row < 2 * FA, FA, 2 * FA + 4)
        same = (row >= split) == (col >= 2 * FA)
        for q in range(PA):
            v = jnp.concatenate([vs[q, u] for u in range(asub)], axis=1)
            v = jnp.concatenate([v, jnp.ones((8, TA), F32)], axis=0)
            kv = _dot_nt(v.astype(BF16), pair_rows(phk, q, 0, asub))
            kv = kv + jnp.where(j == 0, 0.0, kvacc[q])
            kvacc[q] = kv
            kvs[q] = _pack(jnp.where(same, kv, 0.0).astype(BF16))
        return 0

    def attend(j):
        low = lax.broadcasted_iota(jnp.int32, (8, TN), 0) < 4
        os_ = []
        for q in range(PA):
            nd = _dot(_unpack(kvs[q]), pair_rows(phq, q, j * nsub, nsub))
            rab = 1.0 / (nd[40:48, :] + 1e-6)
            rba = pltpu.roll(rab, 4, 0)
            ra = jnp.where(low, rab, rba)
            rb = jnp.where(low, rba, rab)
            os_.append(nd[0:40, :] * jnp.concatenate([ra, ra, rab, rb, rb], axis=0))
        return _pack(jnp.concatenate(os_, axis=0).astype(BF16).T)

    def project(j, o):
        r = rows(j, TN)
        xres[r, :] = _dot(_unpack(o), woa[...]) + xres[r, :]

    def b_residual(i):
        r = rows(i, TB)
        x = xres[r, :] + rsave[...]
        xres[r, :] = x
        xio[r, :] = x.astype(BF16)
        return x

    def b_finish(i):
        xn = _layernorm(b_residual(i))
        xl[rows(jnp.minimum(i, 2), TB), :] = xn
        return xn

    def b_tile(mem, xn, i, side):
        for u in range(4):
            t0 = u * SEG

            def fix_y(p, kind, y):
                cols = pl.ds((3 * p + kind) * PW, PW)
                ysave[0:y.shape[0], cols] = y

                def get():
                    z = ysave[0:32, cols]
                    if u % 2 == 0 and kind != 1:
                        r0 = 64 * u + 8 * p
                        tie = jnp.where(i < 0, side[r0:r0 + 8, 128 * kind:128 * kind + PW],
                                        z[16:24, :])
                        z = jnp.concatenate([z[0:16, :], tie, z[24:, :]], axis=0)
                    return jnp.concatenate([z, ysave[32 + 8 * u:40 + 8 * u, cols]], axis=0)
                return get

            def fix_o(p, o):
                cols = slice(p * PW, (p + 1) * PW)
                r0 = 0 if u == 3 else 8 + 8 * u
                osave[r0:r0 + 8, cols] = o[32:L, :]
                if u == 3:
                    return jnp.concatenate([o[0:32, :], osave[:, cols]], axis=0)
                return o[0:32, :]

            h = jnp.concatenate([mem, xn[t0:t0 + 24, :]], axis=0)
            if u == 0:
                h = jnp.concatenate(
                    [h] + [xn[SEG * v + 24:SEG * v + SEG, :] for v in range(4)], axis=0)
            r = _segment(h, wqv, wk, wob, wsum, pst, lst, fix_y, fix_o, u)
            mem = r[0:M, :]
            if u < 3:
                rsave[t0:t0 + 24, :] = r[M:, :]
            else:
                rsave[t0:t0 + SEG, :] = r[M:L, :]
                for v in range(3):
                    rsave[SEG * v + 24:SEG * v + SEG, :] = r[L + 8 * v:L + 8 * v + 8, :]
        return mem

    def prep(kind, nr, t, _):
        per = 8 // nr
        for c, at in {'qv': ((6, 0), (7, 2 * per)), 'k': (), 'o': ((4, 0), (5, per))}[kind]:
            @pl.when(t == at)
            def _():
                w_copy(c).wait()

        def view(ref, start, size, align):
            return ref.at[pl.ds(pl.multiple_of(start, align), size)]

        slab, q, ties = t // per, t % per, []
        dst = view(wsum, 8 * nr * t + {'qv': 0, 'o': 256, 'k': 384}[kind], 8 * nr, 8 * nr)
        if kind == 'o':
            src = view(wraw.at[4 + slab], 16 * nr * q, HD // 2 - 128 + 16 * nr, 16 * nr)
            wo = view(wob, QW * slab + 8 * nr * q, QW - 64 + 8 * nr, 8 * nr)
        else:
            src = view((wqv if kind == 'qv' else wk).at[slab], 8 * nr * q,
                       D // 2 - 64 + 8 * nr, 8 * nr)
        if kind == 'qv':
            ksrc = view(wraw.at[6 + t // (2 * per)], t % (2 * per) * DH * nr, DH * nr, DH * nr)
            for b in range(DH * nr // 256):
                for c in range(D // 128):
                    z = _pack(ksrc[rows(b, 256), rows(c, 128)])
                    wk[t // (2 * per), rows(c, 64),
                       rows(t % (2 * per) * (DH * nr // 256) + b, 256)] = _pack(_unpack(z).T)
                    ties += [z[8 * (k // 2) + 64 * (k % 2):8 * (k // 2) + 64 * (k % 2) + 8, :]
                             for k in range(16)]
        for rr in range(nr):
            for g, (t0, sz) in enumerate(_STARS):
                if kind == 'o':
                    w = [_pack(src[rows(8 * (t0 + x) + rr, 16), :]) for x in range(sz)]
                    for x in range(sz):
                        wo[rows(8 * (t0 + x) + rr, 8), :] = w[x]
                else:
                    w = [src[rows(8 * x + rr, 8), pl.ds(128 * t0, 128 * sz)] for x in range(sz)]

                mine = ties[0:16]
                del ties[0:len(mine)]

                def val(x, y):
                    z = w[x][:, 128 * y:128 * y + 128]
                    if mine:
                        z = jnp.where(t < 0, mine.pop(0), z)
                    return _unpack(z).astype(F32)

                out = {}
                for x in range(sz):
                    out['r%d' % x] = out['c%d' % x] = val(x, x)
                for x in range(sz):
                    for y in range(x + 1, sz):
                        xy, yx = val(x, y), val(y, x)
                        out[x, y] = xy + yx
                        out['r%d' % x], out['c%d' % y] = out['r%d' % x] - xy, out['c%d' % y] + xy
                        out['r%d' % y], out['c%d' % x] = out['r%d' % y] - yx, out['c%d' % x] + yx
                names = [x for grp in _star_sums(sz) for x in grp]
                dst[rows(rr, 8), pl.ds(128 * 20 * g, 128 * len(names))] = _pack(
                    jnp.concatenate([out[x] for x in names], axis=1).astype(BF16))
        return 0

    def layer(l, _):
        def wait_first(copies):
            @pl.when(l == 0)
            def _():
                for c in copies:
                    c.wait()

        with jax.named_scope("a1"):
            lax.fori_loop(0, na, functools.partial(a1, l == 0), 0)

        def a2(n, _):
            o0 = attend(2 * n)
            o1 = attend(2 * n + 1)
            for job in range(4):
                w = _pack(wraw[n, rows(job, 2 * PW), :].T)
                wqv[n, :, rows(job, 2 * PW)] = w
                if job < 2:
                    z = jnp.concatenate([functools.reduce(jnp.bitwise_or, [
                        w[64 * a + 56:64 * a + 64, 128 * c:128 * c + 128] for c in range(6)])
                        for a in range(D // 128)], axis=1)
                    o1 = jnp.concatenate([jnp.where(n < 0, z, o1[0:8, :]), o1[8:, :]], axis=0)
            project(2 * n, o0)
            r = rows(n, TB // NW)
            xb[r, :] = _layernorm(xres[r, :])
            rsave[r, :] = jnp.zeros((TB // NW, D), F32)
            for ref in (ysave, osave, pst, lst):
                ref[rows(n % 2, 8), 0:128] = jnp.zeros((8, 128), ref.dtype)
            project(2 * n + 1, o1)
            return 0

        wait_first([woa_copy, mem0_copy] + [w_copy(c) for c in range(4)])
        with jax.named_scope("a2"):
            lax.fori_loop(0, NW, a2, 0)

        @pl.when(l == 0)
        def _():
            with jax.named_scope("prep"):
                nq = 8
                lax.fori_loop(0, 32 // nq, functools.partial(prep, 'qv', nq), 0)
                lax.fori_loop(0, 8, functools.partial(prep, 'k', 2), 0)
                lax.fori_loop(0, 8, functools.partial(prep, 'o', 2), 0)

        def b_step(i, mem):
            xn = xb[...]
            side = b_finish(jnp.maximum(i - 1, 0))
            nxt = _layernorm(xres[rows(jnp.minimum(i + 1, nb - 1), TB), :])
            xb[...] = nxt
            side = jnp.concatenate([side, nxt], axis=0)
            mem = b_tile(mem, xn, i, side)

            @pl.when(jnp.logical_and(l == 1, i >= 1))
            def _():
                out_copy(i - 1).start()
            return mem

        with jax.named_scope("b"):
            lax.fori_loop(0, nb, b_step, mem0[...].astype(F32))

        b_residual(nb - 1)

        @pl.when(l == 0)
        def _():
            xa[...] = strassen_rhs(xl[0:128, :], xl[128:256, :])
        return 0

    lax.fori_loop(0, 2, layer, 0)
    out_copy(nb - 1).start()
    pltpu.make_async_copy(xio, out_hbm, sem_out.at[0]).wait()


@jax.jit
def pallas_interleave_layers__linear_kernel_hedgehog__memory_aug_recurrent_mem_tr__prompt_kernel(
    A_x, A_wqkv, A_w_phi, A_wo, B_x, B_mem0, B_Wq, B_Wk, B_Wv, B_Wo, B_seg_len,
):
    del B_x
    del B_seg_len
    x = A_x.reshape(S, D)
    wphi = A_w_phi.transpose(1, 2, 0)
    mem0 = B_mem0.reshape(M, D)
    wq, wk, wv = (w.transpose(1, 2, 0).reshape(2, HD // 2, D) for w in (B_Wq, B_Wk, B_Wv))
    wo = B_Wo.reshape(2, HD // 2, D)
    hbm = pl.BlockSpec(memory_space=pl.ANY)
    out = pl.pallas_call(
        _kernel,
        out_shape=jax.ShapeDtypeStruct((S, D), A_x.dtype),
        in_specs=[hbm] * 9,
        out_specs=hbm,
        scratch_shapes=[
            pltpu.VMEM((S, D), BF16),
            pltpu.VMEM((D, 3 * D), BF16),
            pltpu.VMEM((FA, FA, HA), BF16),
            pltpu.VMEM((D, D), BF16),
            pltpu.VMEM((M, D), BF16),
            pltpu.VMEM((S, D), F32),
            pltpu.VMEM((64, 2048), U32),
            pltpu.VMEM((3 * TB, D), F32),
            pltpu.VMEM((TB, D), F32),
            pltpu.VMEM((GA, GR // 2, 256), U32),
            pltpu.VMEM((6, 8, GR // 2, 256), U32),
            pltpu.VMEM((S // 128, D, 128), U32),
            pltpu.VMEM((TA // 128, D, 128), U32),
            pltpu.VMEM((PA, 2 * VR, 4 * FA), F32),
            pltpu.VMEM((PA, VR, 4 * FA), U32),
            pltpu.VMEM((8, HD // 2, D), BF16),
            pltpu.VMEM((4, D // 2, HD // 2), U32),
            pltpu.VMEM((2, D // 2, HD // 2), U32),
            pltpu.VMEM((HD // 2, D), U32),
            pltpu.VMEM((8 * 64, NS * 128), U32),
            pltpu.VMEM((64, 3 * HD), F32),
            pltpu.VMEM((32, HD), F32),
            pltpu.VMEM((L, HD // 2), U32),
            pltpu.VMEM((16, 66 * 128), U32),
            pltpu.VMEM((TB, D), F32),
            pltpu.SemaphoreType.DMA((17 + S // TA,)),
            pltpu.SemaphoreType.DMA((1,)),
        ],
        compiler_params=pltpu.CompilerParams(vmem_limit_bytes=126 * 1024 * 1024,
                                             disable_bounds_checks=True,
                                             disable_semaphore_checks=True),
    )(x, A_wqkv, wphi, A_wo, mem0, wq, wk, wv, wo)
    return out.reshape(1, S, D)
```

```python
import functools

import jax
import jax.numpy as jnp
from jax import lax
import jax.experimental.pallas as pl
import jax.experimental.pallas.tpu as pltpu

F32 = jnp.float32
BF16 = jnp.bfloat16
U32 = jnp.uint32

S = 2048
D = 640
HA = 32
FA = 20
GA = 4
GR = 8 * FA
VR = 24
PA = HA // 2
TN = 256
TA = 512
HB = 32
DH = 192
HD = HB * DH
M = 8
SEG = 32
L = M + SEG
PW = 2 * DH
NP = HB // 2
TB = 128
NW = 4
QW = HD // NW

NT = (((1,), (1,)), ((), ()))
LOG2E = 1.4426950408889634
HALF_ULP = 0.0040612


def _dot(a, b):
    return jnp.dot(a, b, preferred_element_type=F32)


def _dot_nt(a, b):
    return lax.dot_general(a, b, NT, preferred_element_type=F32)


def _pack(a):
    return pltpu.bitcast(a, U32)


def _unpack(a):
    return pltpu.bitcast(a, BF16)


def _interleave(a, b):
    lo = lax.bitcast_convert_type(a, U32) >> 16
    hi = lax.bitcast_convert_type(b, U32) & jnp.uint32(0xFFFF0000)
    return lo | hi


def _recip(x):
    r = pl.reciprocal(x, approx=True)
    return r * (2.0 - x * r)


def _layernorm(x):
    m = jnp.mean(x, axis=-1, keepdims=True)
    c = x - m
    v = jnp.mean(c * c, axis=-1, keepdims=True)
    return c * lax.rsqrt(v + 1e-5)


def _feature_map(p):
    t = p.shape[-1]
    p3 = jnp.concatenate([jnp.zeros((8, t), F32), p], axis=0).reshape(FA, 8, t)
    mx = jnp.max(p3, axis=0)
    mn = jnp.min(p3, axis=0)
    sp, sn = jnp.exp2(p3[0] - mx), jnp.exp2(mn - p3[0])
    for f in range(1, FA):
        sp, sn = sp + jnp.exp2(p3[f] - mx), sn + jnp.exp2(mn - p3[f])
    lp = (mx - HALF_ULP) + jnp.log2(sp)
    ln = (mn + HALF_ULP) - jnp.log2(sn)
    return [_interleave(jnp.exp2(p3[f] - lp), jnp.exp2(ln - p3[f])) for f in range(FA)]


def _tiles(a, odd):
    t0, t1, t2 = a[:, 0:128], a[:, 128:256], a[:, 256:384]
    return (t1, t2, t0) if odd else (t1, t0, t2)


def _own_weights(a, odd):
    lane = lax.broadcasted_iota(jnp.int32, (L, 128), 1)
    mid, own, _ = _tiles(a, odd)
    return jnp.concatenate(
        [jnp.where(lane < 64, mid, 0.0), jnp.where(lane < 64, 0.0, mid), own,
         jnp.zeros((128 - 3 * L, 128), F32)], axis=0).astype(BF16)


def _others(even, odd, pad):
    parts = [_tiles(odd, 1)[2], _tiles(even, 0)[2]]
    if pad:
        parts.append(jnp.zeros((128 - 2 * L, 128), F32))
    return jnp.concatenate(parts, axis=0).astype(BF16)


def _softmax3(s3):
    row = lax.broadcasted_iota(jnp.int32, (L, 128), 0)
    col = lax.broadcasted_iota(jnp.int32, (L, 128), 1)
    first = col < L
    second = jnp.logical_and(col >= L, col < 2 * L)
    key = jnp.where(first, col, col - L)
    valid = jnp.logical_or(row < M, row >= key)
    out, other = [], []
    for odd in range(2):
        own = pltpu.roll(s3[odd][L:, :], 128 - L if odd else 128 - 2 * L, 1)
        s = (jnp.where(first, s3[2][0:L, :], own) if odd
             else jnp.where(first, own, s3[2][L:, :]))
        s = jnp.where(valid, (s + s3[odd][0:L, :]) * (DH ** -0.5), -1e9)
        m0 = jnp.max(jnp.where(first, s, -jnp.inf), axis=-1, keepdims=True)
        m1 = jnp.max(jnp.where(second, s, -jnp.inf), axis=-1, keepdims=True)
        e = jnp.exp(s - jnp.where(first, m0, m1))
        e0 = jnp.where(first, e, 0.0)
        e1 = jnp.where(second, e, 0.0)
        p0 = e0 * _recip(jnp.sum(e0, axis=-1, keepdims=True))
        p1 = e1 * _recip(jnp.sum(e1, axis=-1, keepdims=True))
        own = pltpu.roll(p1, L, 1) if odd else pltpu.roll(p0, 2 * L, 1)
        out.append(jnp.concatenate([p0 + p1, own], axis=0))
        other.append(p0 if odd else p1)
    out.append(jnp.concatenate([other[1], other[0]], axis=0))
    return _pack(jnp.concatenate(out, axis=1).astype(BF16))


_T = {5: (-1.5, -0.5, 0.0, 0.5, 1.5), 3: (-1.0, 0.0, 1.0), 2: (-0.5, 0.5)}
_STARS = tuple((5 * g, 0, 5) for g in range(9)) + ((45, 0, 3), (45, 3, 2))


def _star_sums(n):
    return ([k % j for j in range(n) for k in ('r%d', 'c%d')]
            + [(a, b) for a in range(n) for b in range(a + 1, n)])


def _star_slot(g, name):
    return 20 * g - 11 * (g == 10) + _star_sums(_STARS[g][2]).index(name)


NS = 194


def _star_lhs(n, get, scaled):
    t = _T[n]
    f = [get(0, j) for j in range(n)]
    g = [get(1, j) + t[j] * f[j] if t[j] else get(1, j) for j in range(n)]
    out = {'r%d' % j: f[j] for j in range(n)}
    out.update({'c%d' % j: g[j] for j in range(n)})
    for a in range(n):
        for b in range(a + 1, n):
            d = t[a] - t[b]
            if scaled:
                l = (g[a] - g[b]) * (1.0 / d)
                out[a, b], out[b, a, 0], out[a, b, 0] = l, f[b] - l, f[a] - l
            else:
                l = g[a] - g[b]
                out[a, b], out[b, a, 0], out[a, b, 0] = l, d * f[b] - l, d * f[a] - l
    return out


def _star_apply(n, lhs, plain, mixed, scaled, acc=None):
    t = _T[n]
    p, q = ([None] * n, [None] * n) if acc is None else (list(acc[0]), list(acc[1]))
    started = set()

    def start(j):
        if j not in started:
            started.add(j)
            dp, dq = [_dot(lhs(k % j), mixed(k % j)) for k in ('r%d', 'c%d')]
            p[j] = dp if p[j] is None else dp + p[j]
            q[j] = dq if q[j] is None else dq + q[j]

    for a in range(n):
        for b in range(a + 1, n):
            start(a)
            start(b)
            d = t[a] - t[b]
            m6 = _dot(lhs((b, a, 0)), plain(b, a))
            m7 = _dot(lhs((a, b, 0)), plain(a, b))
            m = _dot(lhs((a, b)), mixed((a, b))) + (m6 + m7)
            if scaled:
                q[a], q[b] = q[a] - (-d) * m6, q[b] - d * m7
                p[a], p[b] = m + p[a], m + p[b]
            else:
                q[a], q[b] = m6 + q[a], q[b] - m7
                m = m * (-1.0 / d) if d != -1.0 else m
                p[a], p[b] = p[a] - m, p[b] - m
    return p, q


def _star_result(n, p, q):
    return [jnp.concatenate([p[j], q[j] - _T[n][j] * p[j] if _T[n][j] else q[j]], axis=0)
            for j in range(n)]


_PLAN = (
    ((5, 11, 14, 20, 26), (), (0, 9, 11)),
    ((3, 6, 9, 11, 13), (0, 6, 7, 13), (1, 8, 9)),
    ((3, 6, 8, 11, 14), (1, 4, 8, 11), (3, 9, 10)),
    ((3, 6, 9, 11, 14), (1, 4, 8, 12), (2, 5, 6)),
)


def _segment(h, wqv, wk, wob, wsum, pst, lst, fix_y, fix_o, step):
    ys = {p: [None] * 3 for p in range(NP)}
    ss, pvs, os_ = {}, {}, {}
    hb = h.astype(BF16)

    used = [0]

    def staged(ops, through_memory):
        if not through_memory:
            ops = {k: v.astype(BF16) for k, v in ops.items()}
            return ops.get
        names, w, c0 = list(ops), next(iter(ops.values())).shape[1], used[0]
        used[0] += w * len(names)
        lst[:, c0:used[0]] = _pack(jnp.concatenate(list(ops.values()), axis=1).astype(BF16))
        return lambda k: _unpack(lst[:, pl.ds(c0 + w * names.index(k), w)])

    def summed(kind, g, name):
        return wsum[64 * kind:64 * kind + 64, pl.ds(128 * _star_slot(g, name), 128)]

    def keys(n):
        k = _dot(hb, _unpack(wk[n // 2, :, pl.ds(n % 2 * QW, QW)]))
        for e in range(4):
            ys[4 * n + e][1] = fix_y(4 * n + e, 1, k[:, e * PW:(e + 1) * PW])

    def proj(p):
        def w(lo, hi):
            return _unpack(jnp.concatenate(
                [wqv[2 * i + p // 8, lo:hi, pl.ds(p % 8 * PW, PW)] for i in range(2)], axis=1))
        if p == 0:
            y = _dot(hb[:, 0:512], w(0, 256))
            y = _dot(hb[:, 512:], w(256, D // 2)) + y
        else:
            y = _dot(hb, w(0, D // 2))
        for i in range(2):
            ys[p][2 * i] = fix_y(p, 2 * i, y[:, i * PW:(i + 1) * PW])

    def wide_proj(g, i, lhs, tiles):
        def w(j, nj, t):
            ref, slab = (wk, t // 24) if i == 1 else (wqv, i + t // 24)
            return _unpack(ref[slab, 64 * j:64 * (j + nj), pl.ds(128 * (t % 24), 128)])

        def star(g):
            t0, j0, n = _STARS[g]
            return _star_result(n, *_star_apply(
                n, lhs[n], lambda j, l: w(j0 + j, 1, t0 + l),
                lambda name: _unpack(summed(i, g, name)), False))

        if g == 9:
            rest = star(10) + [_dot(hb[:, 384:], w(3, 2, 47))]
            out = [x + y for x, y in zip(star(9), rest)]
        else:
            out = star(g)
        for l, y in enumerate(out):
            tiles[5 * g + l] = y
        for p in range(NP):
            if all(3 * p + k in tiles for k in range(3)):
                ys[p][i] = fix_y(p, i, jnp.concatenate(
                    [tiles.pop(3 * p + k) for k in range(3)], axis=1))

    def weights(c, i, which):
        if i < 2:
            return _own_weights(ys[2 * c + i][which](), i)
        return _others(ys[2 * c][which](), ys[2 * c + 1][which](), True)

    def score_round(n):
        for c, i in (divmod(j, 3) for j in range(4 * n, 4 * n + 4)):
            if i < 2:
                q = jnp.concatenate(_tiles(ys[2 * c + i][0](), i)[0:2], axis=0).astype(BF16)
            else:
                q = _others(ys[2 * c][0](), ys[2 * c + 1][0](), False)
            ss[c, i] = _dot_nt(q, weights(c, i, 1))
            if i == 2:
                pst[:, c * PW:(c + 1) * PW] = _softmax3([ss.pop((c, k)) for k in range(3)])

    def pv_round(n):
        for c, i in (divmod(j, 3) for j in range(4 * n, 4 * n + 4)):
            pvs[c, i] = _dot(_unpack(pst[:, pl.ds(c * PW + 128 * i, 128)]), weights(c, i, 2))
            if i == 2:
                o0, o1, o2 = [pvs.pop((c, k)) for k in range(3)]
                os_[2 * c] = fix_o(2 * c, jnp.concatenate(
                    [o0[L:, :], o0[0:L, :], o2[L:, :]], axis=1))
                os_[2 * c + 1] = fix_o(2 * c + 1, jnp.concatenate(
                    [o2[0:L, :], o1[0:L, :], o1[L:, :]], axis=1))

    def slot(n):
        if n >= 2:
            pv_round(n - 2)
        if n < 6:
            score_round(n)

    def oproj(lo, hi, r):
        o = jnp.concatenate([os_.pop(p) for p in range(lo, hi)], axis=1).astype(BF16)
        y = _dot(o, _unpack(wob[lo * DH:hi * DH, :]))
        return y if r is None else y + r

    def o_tile(t):
        return os_[t // 3][:, 128 * (t % 3):128 * (t % 3) + 128]

    def wide_oproj(stars, acc):
        _, j0, n = _STARS[stars[0]]
        t0 = [_STARS[g][0] for g in stars]
        return _star_apply(
            n, staged(_star_lhs(n, lambda i, j: jnp.concatenate(
                [o_tile(t + j)[32 * i:32 * i + 32] for t in t0], axis=1), True), False),
            lambda j, l: _unpack(jnp.concatenate(
                [wob[pl.ds(64 * (t + j), 64), pl.ds(128 * (j0 + l), 128)] for t in t0], axis=0)),
            lambda name: _unpack(jnp.concatenate(
                [summed(3, g, name) for g in stars], axis=0)), True, acc)

    after, kat, (o1, o2, o3) = _PLAN[step]
    if step == 0:
        lhs = {n: staged(_star_lhs(
            n, lambda i, j: h[32 * i:32 * i + 32, 128 * (j0 + j):128 * (j0 + j + 1)], False), True)
               for _, j0, n in _STARS[8:]}
        tiles = {}
    for unit in range(30 if step == 0 else NP):
        if step == 0:
            wide_proj(unit // 3, unit % 3, lhs, tiles.setdefault(unit % 3, {}))
        else:
            proj(unit)
        if unit in kat:
            keys(kat.index(unit))
        for n in range(5):
            if after[n] == unit:
                slot(n)
    if step == 3:
        r = wide_oproj(range(0, o1), None)
        slot(5)
        r = wide_oproj(range(o1, o2), r)
        slot(6)
        slot(7)
        r = wide_oproj(range(o2, o3), r)
        r = wide_oproj(range(o3, 9), r)
        y = _dot(o_tile(47).astype(BF16), _unpack(wob[64 * 47:, 384:]))
        y = jnp.concatenate(_star_result(2, *wide_oproj([10], None)), axis=1) + y
        y = jnp.concatenate(_star_result(3, *wide_oproj([9], None)) + [y], axis=1)
        return jnp.concatenate(_star_result(5, *r), axis=1) + y
    r = oproj(0, o1, None) if o1 else None
    slot(5)
    r = oproj(o1, o2, r)
    slot(6)
    slot(7)
    r = oproj(o2, o3, r)
    return oproj(o3, NP, r)


def _kernel(x_hbm, wqkv_hbm, wphi_hbm, woa_hbm, mem0_hbm,
            wq_hbm, wk_hbm, wv_hbm, wo_hbm,
            out_hbm,
            xio, wqkv, wphi, woa, mem0, xres, xa, xl, xb, bds, wat, phq, phk, kvacc, kvs,
            wraw, wqv, wk, wob, wsum, ysave, osave, pst, lst, rsave, sem_in, sem_out):
    nsub = TN // 128
    na = S // TA
    asub = TA // 128
    nb = S // TB

    def rows(j, n):
        return pl.ds(j * n if isinstance(j, int) else pl.multiple_of(j * n, n), n)

    def x_copy(j):
        if isinstance(j, int) and j < 0:
            r = pl.ds(0, 256)
        elif isinstance(j, int) and j == na - 1:
            r = pl.ds(S - TA + 256, TA - 256)
        else:
            r = pl.ds(j * TA + 256 if isinstance(j, int)
                      else pl.multiple_of(j * TA + 256, 256), TA)
        return pltpu.make_async_copy(x_hbm.at[r, :], xio.at[r, :], sem_in.at[9 + j])

    def w_copy(c):
        src = (wq_hbm, wv_hbm, wo_hbm, wk_hbm)[c // 2]
        return pltpu.make_async_copy(src.at[c % 2], wraw.at[c], sem_in.at[9 + na + c])

    def wa_copy(c):
        r = pl.ds(512, 128) if isinstance(c, int) and c == 2 else rows(c, 256)
        return pltpu.make_async_copy(wqkv_hbm.at[r, :], wqkv.at[r, :], sem_in.at[3 + c])

    def out_copy(i):
        return pltpu.make_async_copy(xio.at[rows(i, TB), :],
                                     out_hbm.at[rows(i, TB), :], sem_out.at[0])

    wphi_copy = pltpu.make_async_copy(wphi_hbm, wphi, sem_in.at[0])
    woa_copy = pltpu.make_async_copy(woa_hbm, woa, sem_in.at[1])
    mem0_copy = pltpu.make_async_copy(mem0_hbm, mem0, sem_in.at[2])
    order = [wphi_copy, wa_copy(0), wa_copy(1), x_copy(-1), wa_copy(2)]
    order += [x_copy(j) for j in range(na)] + [woa_copy, mem0_copy]
    order += [w_copy(c) for c in (0, 1, 2, 3, 6, 7, 4, 5)]
    for c in order:
        c.start()

    def strassen_rhs(x0, x1):
        b11, b12 = [jnp.concatenate([x[:, 0:128], x[:, 256:384]], axis=1) for x in (x0, x1)]
        b21, b22 = [jnp.concatenate([x[:, 128:256], x[:, 384:512]], axis=1) for x in (x0, x1)]
        ops = [b11 + b22, b11, b12 - b22, b21 - b11, b22, b11 + b12, b21 + b22,
               x0[:, 512:], x1[:, 512:]]
        return _pack(jnp.concatenate(ops, axis=1).astype(BF16))

    def load_x(t, first):
        x = xio[rows(t, 256), :].astype(F32)
        if first is not True:
            x = jnp.where(first, x, xres[rows(t, 256), :])
        xres[rows(t, 256), :] = x
        return x

    wphi_copy.wait()
    cphi = jnp.zeros((FA, D), F32)
    hh = lax.broadcasted_iota(jnp.int32, (HA, D), 0) * FA
    jj = lax.broadcasted_iota(jnp.int32, (HA, D), 1)
    for d in range(FA):
        cphi = _dot(wphi[d], jnp.where(jj == hh + d, 1.0, 0.0).astype(BF16)) + cphi
    cb = jnp.concatenate(
        [jnp.broadcast_to(cphi[f:f + 1, :], (8, D)) for f in range(FA)], axis=0)
    for g in range(GA):
        row = lax.broadcasted_iota(jnp.int32, (GR, 256), 0)
        col = lax.broadcasted_iota(jnp.int32, (GR, 256), 1) + 128 * g
        lo = (8 * g + (row & 7)) * FA
        bds[g] = _pack(jnp.where(jnp.logical_and(col >= lo, col < lo + FA),
                                 cb[:, 128 * g:128 * g + 256], 0.0).astype(BF16))

    def folded(rr):
        out = [[], [], []]
        for g in range(GA):
            ws = []
            for i in range(2):
                c0 = i * D + 128 * g
                w = _dot_nt(_unpack(bds[g]), wqkv[rr, c0:c0 + 256]).reshape(FA, 8, 128)
                ws.append(((w[1:] - w[0:1]) * LOG2E).reshape(GR - 8, 128))
            out[0].append(jnp.concatenate([ws[1], ws[0][GR - 16:, :]], axis=0))
            out[1].append(ws[0][0:GR - 16, :])
        wvt = wqkv[rr, 2 * D:3 * D].T.astype(F32)
        out[2] = [wvt[g * GR:(g + 1) * GR, :] for g in range(GA)]
        return out

    def fold(c, _):
        wa_copy(c).wait()
        wa, wb = folded(rows(2 * c, 128)), folded(rows(2 * c + 1, 128))
        for i in range(3):
            for p in range(2):
                a11, a12, a21, a22 = wa[i][2 * p], wb[i][2 * p], wa[i][2 * p + 1], wb[i][2 * p + 1]
                ops = [a11 + a22, a21 + a22, a11, a22, a11 + a12, a21 - a11, a12 - a22]
                for m, w in enumerate(ops):
                    wat[2 * i + p, m, 0:w.shape[0] // 2, rows(c, 128)] = _pack(w.astype(BF16))
        return 0

    lax.fori_loop(0, 2, fold, 0)
    x_copy(-1).wait()
    wa_copy(2).wait()
    x = _layernorm(load_x(0, True))
    xa[...] = strassen_rhs(x[0:128], x[128:])
    for i, ws in enumerate(folded(pl.ds(512, 128))):
        for g, w in enumerate(ws):
            wat[2 * i + g // 2, 7, 0:w.shape[0] // 2, rows(g % 2, 128)] = _pack(w.astype(BF16))

    def pair_rows(ph, q, t0, n):
        return _unpack(jnp.concatenate(
            [ph[t0 + u, rows(q, 2 * FA), :] for u in range(n)], axis=1))

    def a1(first, j, _):
        @pl.when(jnp.logical_and(first, j < na - 1))
        def _():
            x_copy(j).wait()

        @pl.when(jnp.logical_and(first, j == na - 1))
        def _():
            x_copy(na - 1).wait()

        def features(ph, t, g, y):
            for f, w in enumerate(_feature_map(y)):
                ph[t, pl.ds(GR * g + f, 8, stride=FA), :] = w

        def tail(n, xs, g, u):
            nr = GR // 2 - 8 if n // 2 == 1 else GR // 2
            return _dot_nt(_unpack(wat[n, 7, 0:nr, 128 * g:128 * (g + 1)]),
                           xs[:, 1792 + 128 * u:1920 + 128 * u])

        def a_dots(n, xs, emit, tie, t10):
            nr = GR // 2 - 8 if n // 2 == 1 else GR // 2
            p = n % 2

            def prod(m):
                return _dot_nt(_unpack(tie(wat[n, m, 0:nr, :])), xs[:, 256 * m:256 * (m + 1)])

            m2, m4 = prod(1), prod(3)
            emit(2 * p + 1, 0, m4 + (m2 - (-t10)))
            t01 = tail(n, xs, 0, 1)
            m3, m5 = prod(2), prod(4)
            emit(2 * p, 1, m5 + (m3 - (-t01)))
            m1 = prod(0)
            c22 = prod(5) + (m1 + (m3 - m2))
            emit(2 * p + 1, 1, tail(n, xs, 1, 1) + c22)
            t10 = tail(n + 1, xs, 1, 0) if n < 5 else None
            c11 = tail(n, xs, 0, 0) + (m1 + (m4 - m5))
            emit(2 * p, 0, prod(6) + c11)
            return t10

        vs = {}
        cur = xa[...]
        dl = (3, 8, 13, 30, 34, 37, 39, 40)
        for u in range(0, asub, 2):
            t = j * (asub // 2) + u // 2
            xs = _unpack(cur)
            tn = t + 1
            x = load_x(tn if u + 2 < asub else jnp.minimum(tn, (na - 1) * (asub // 2)), first)
            rest, seen, nxt = {}, [], []

            def tie(w):
                seen.append(0)
                if len(seen) - 1 not in dl:
                    return w
                n = len(nxt)
                nxt.append(strassen_rhs(*[
                    _layernorm(x[128 * e + 16 * n:128 * e + 16 * n + 16, :]) for e in range(2)]))
                z = jnp.concatenate(
                    [nxt[n][:, 256 * c:256 * (c + 1)] for c in range(8)], axis=0)
                return jnp.concatenate([jnp.where(j < 0, z, w[0:64, :]), w[64:, :]], axis=0)

            def emit_k(g, e, y):
                features(phk, u + e, g, y[0:GR - 8, :])
                rest[g, e] = y[GR - 8:, :]

            def emit_q(g, e, y):
                features(phq, 2 * t + e, g, jnp.concatenate([y, rest[g, e]], axis=0))

            def emit_v(g, e, y):
                for q in range(4):
                    vs[4 * g + q, u + e] = y[40 * q:40 * q + 40, :]

            t10 = tail(0, xs, 1, 0)
            for n in range(6):
                t10 = a_dots(n, xs, (emit_k, emit_q, emit_v)[n // 2], tie, t10)
            cur = jnp.concatenate(nxt, axis=0)
        xa[...] = cur
        row = lax.broadcasted_iota(jnp.int32, (2 * VR, 4 * FA), 0)
        col = lax.broadcasted_iota(jnp.int32, (2 * VR, 4 * FA), 1)
        split = jnp.where(row < 2 * FA, FA, 2 * FA + 4)
        same = (row >= split) == (col >= 2 * FA)
        for q in range(PA):
            v = jnp.concatenate([vs[q, u] for u in range(asub)], axis=1)
            v = jnp.concatenate([v, jnp.ones((8, TA), F32)], axis=0)
            kv = _dot_nt(v.astype(BF16), pair_rows(phk, q, 0, asub))
            kv = kv + jnp.where(j == 0, 0.0, kvacc[q])
            kvacc[q] = kv
            kvs[q] = _pack(jnp.where(same, kv, 0.0).astype(BF16))
        return 0

    def attend(j):
        low = lax.broadcasted_iota(jnp.int32, (8, TN), 0) < 4
        os_ = []
        for q in range(PA):
            nd = _dot(_unpack(kvs[q]), pair_rows(phq, q, j * nsub, nsub))
            rab = 1.0 / (nd[40:48, :] + 1e-6)
            rba = pltpu.roll(rab, 4, 0)
            ra = jnp.where(low, rab, rba)
            rb = jnp.where(low, rba, rab)
            os_.append(nd[0:40, :] * jnp.concatenate([ra, ra, rab, rb, rb], axis=0))
        return _pack(jnp.concatenate(os_, axis=0).astype(BF16).T)

    def project(j, o):
        r = rows(j, TN)
        xres[r, :] = _dot(_unpack(o), woa[...]) + xres[r, :]

    def b_residual(i):
        r = rows(i, TB)
        x = xres[r, :] + rsave[...]
        xres[r, :] = x
        xio[r, :] = x.astype(BF16)
        return x

    def b_finish(i):
        xn = _layernorm(b_residual(i))
        xl[rows(jnp.minimum(i, 2), TB), :] = xn
        return xn

    def b_tile(mem, xn, i, side):
        for u in range(4):
            t0 = u * SEG

            def fix_y(p, kind, y):
                cols = pl.ds((3 * p + kind) * PW, PW)
                ysave[0:y.shape[0], cols] = y

                def get():
                    z = ysave[0:32, cols]
                    if u % 2 == 0 and kind != 1:
                        r0 = 64 * u + 8 * p
                        tie = jnp.where(i < 0, side[r0:r0 + 8, 128 * kind:128 * kind + PW],
                                        z[16:24, :])
                        z = jnp.concatenate([z[0:16, :], tie, z[24:, :]], axis=0)
                    return jnp.concatenate([z, ysave[32 + 8 * u:40 + 8 * u, cols]], axis=0)
                return get

            def fix_o(p, o):
                cols = slice(p * PW, (p + 1) * PW)
                r0 = 0 if u == 3 else 8 + 8 * u
                osave[r0:r0 + 8, cols] = o[32:L, :]
                if u == 3:
                    return jnp.concatenate([o[0:32, :], osave[:, cols]], axis=0)
                return o[0:32, :]

            h = jnp.concatenate([mem, xn[t0:t0 + 24, :]], axis=0)
            if u == 0:
                h = jnp.concatenate(
                    [h] + [xn[SEG * v + 24:SEG * v + SEG, :] for v in range(4)], axis=0)
            r = _segment(h, wqv, wk, wob, wsum, pst, lst, fix_y, fix_o, u)
            mem = r[0:M, :]
            if u < 3:
                rsave[t0:t0 + 24, :] = r[M:, :]
            else:
                rsave[t0:t0 + SEG, :] = r[M:L, :]
                for v in range(3):
                    rsave[SEG * v + 24:SEG * v + SEG, :] = r[L + 8 * v:L + 8 * v + 8, :]
        return mem

    def prep(kind, nr, t, _):
        def view(ref, start, size, align):
            return ref.at[pl.ds(pl.multiple_of(start, align), size)]

        ties = []
        if kind == 'qv':
            for c in range(2):
                @pl.when(t == 2 * c)
                def _():
                    w_copy(6 + c).wait()

            src = [view(wqv.at[t // 2 * 2 + c], 32 * (t % 2), D // 2 - 32, 32) for c in range(2)]
            dst = view(wsum, 128 * (t // 2) + 32 * (t % 2), 32, 32)
            ksrc = view(wraw.at[6 + t // 2], t % 2 * QW, QW, QW)
            for b in range(QW // 256):
                for c in range(D // 128):
                    z = _pack(ksrc[rows(b, 256), rows(c, 128)])
                    wk[t // 2, rows(c, 64), rows(t % 2 * (QW // 256) + b, 256)] = _pack(
                        _unpack(z).T)
                    ties += [z[8 * (k // 2) + 64 * (k % 2):8 * (k // 2) + 64 * (k % 2) + 8, :]
                             for k in range(16)]
        elif kind == 'k':
            src = [view(wk.at[c], 8 * t, D // 2 - 56, 8) for c in range(2)]
            dst = view(wsum, 64 + 8 * t, 8, 8)
        else:
            src = [view(wraw.at[4 + c], 16 * t, HD // 2 - 112, 16) for c in range(2)]
            dst = view(wsum, 192 + 8 * t, 8, 8)
            wo = view(wob, 8 * t, HD // 2 - 56, 8)
        for rr in range(nr):
            for g, (t0, j0, sz) in enumerate(_STARS):
                if kind == 'o' and g < 10:
                    w = [_pack(src[(t0 + x) // 24][rows(8 * ((t0 + x) % 24), 16), :])
                         for x in range(sz)]
                    for x in range(sz):
                        wo[rows(8 * (t0 + x), 8), :] = w[x]
                mine = ties[0:min(18, sz * sz)]
                del ties[0:len(mine)]

                def val(x, y):
                    z = (w[x][:, 128 * (j0 + y):128 * (j0 + y + 1)] if kind == 'o' else
                         src[(t0 + y) // 24][rows(8 * (j0 + x) + rr, 8), rows((t0 + y) % 24, 128)])
                    if mine:
                        z = jnp.where(t < 0, mine.pop(0), z)
                    return _unpack(z).astype(F32)

                out = {}
                for x in range(sz):
                    out['r%d' % x] = out['c%d' % x] = val(x, x)
                for x in range(sz):
                    for y in range(x + 1, sz):
                        xy, yx = val(x, y), val(y, x)
                        out[x, y] = xy + yx
                        out['r%d' % x], out['c%d' % y] = out['r%d' % x] - xy, out['c%d' % y] + xy
                        out['r%d' % y], out['c%d' % x] = out['r%d' % y] - yx, out['c%d' % x] + yx
                names = _star_sums(sz)
                dst[rows(rr, 8), pl.ds(128 * _star_slot(g, 'r0'), 128 * len(names))] = _pack(
                    jnp.concatenate([out[x] for x in names], axis=1).astype(BF16))
        return 0

    def layer(l, _):
        def wait_first(copies):
            @pl.when(l == 0)
            def _():
                for c in copies:
                    c.wait()

        with jax.named_scope("a1"):
            lax.fori_loop(0, na, functools.partial(a1, l == 0), 0)

        def a2(n, _):
            o0 = attend(2 * n)
            o1 = attend(2 * n + 1)
            for job in range(4):
                wqv[n, :, rows(job, 2 * PW)] = _pack(wraw[n, rows(job, 2 * PW), :].T)
            project(2 * n, o0)
            r = rows(n, TB // NW)
            xb[r, :] = _layernorm(xres[r, :])
            rsave[r, :] = jnp.zeros((TB // NW, D), F32)
            for ref in (ysave, osave, pst, lst):
                ref[rows(n % 2, 8), 0:128] = jnp.zeros((8, 128), ref.dtype)
            project(2 * n + 1, o1)
            return 0

        wait_first([woa_copy, mem0_copy] + [w_copy(c) for c in range(4)])
        with jax.named_scope("a2"):
            lax.fori_loop(0, NW, a2, 0, unroll=2)

        @pl.when(l == 0)
        def _():
            with jax.named_scope("prep"):
                lax.fori_loop(0, 4, functools.partial(prep, 'qv', 4), 0)
                lax.fori_loop(0, 8, functools.partial(prep, 'k', 1), 0)
                w_copy(4).wait()
                w_copy(5).wait()
                lax.fori_loop(0, 8, functools.partial(prep, 'o', 1), 0)

        def b_step(i, mem):
            xn = xb[...]
            side = b_finish(jnp.maximum(i - 1, 0))
            nxt = _layernorm(xres[rows(jnp.minimum(i + 1, nb - 1), TB), :])
            xb[...] = nxt
            side = jnp.concatenate([side, nxt], axis=0)
            mem = b_tile(mem, xn, i, side)

            @pl.when(jnp.logical_and(l == 1, i >= 1))
            def _():
                out_copy(i - 1).start()
            return mem

        with jax.named_scope("b"):
            lax.fori_loop(0, nb, b_step, mem0[...].astype(F32))

        b_residual(nb - 1)

        @pl.when(l == 0)
        def _():
            xa[...] = strassen_rhs(xl[0:128, :], xl[128:256, :])
        return 0

    lax.fori_loop(0, 2, layer, 0)
    out_copy(nb - 1).start()
    pltpu.make_async_copy(xio, out_hbm, sem_out.at[0]).wait()


@jax.jit
def pallas_interleave_layers__linear_kernel_hedgehog__memory_aug_recurrent_mem_tr__prompt_kernel(
    A_x, A_wqkv, A_w_phi, A_wo, B_x, B_mem0, B_Wq, B_Wk, B_Wv, B_Wo, B_seg_len,
):
    del B_x
    del B_seg_len
    x = A_x.reshape(S, D)
    wphi = A_w_phi.transpose(1, 2, 0)
    mem0 = B_mem0.reshape(M, D)
    wq, wk, wv = (w.transpose(1, 2, 0).reshape(2, HD // 2, D) for w in (B_Wq, B_Wk, B_Wv))
    wo = B_Wo.reshape(2, HD // 2, D)
    hbm = pl.BlockSpec(memory_space=pl.ANY)
    out = pl.pallas_call(
        _kernel,
        out_shape=jax.ShapeDtypeStruct((S, D), A_x.dtype),
        in_specs=[hbm] * 9,
        out_specs=hbm,
        scratch_shapes=[
            pltpu.VMEM((S, D), BF16),
            pltpu.VMEM((D, 3 * D), BF16),
            pltpu.VMEM((FA, FA, HA), BF16),
            pltpu.VMEM((D, D), BF16),
            pltpu.VMEM((M, D), BF16),
            pltpu.VMEM((S, D), F32),
            pltpu.VMEM((64, 2048), U32),
            pltpu.VMEM((3 * TB, D), F32),
            pltpu.VMEM((TB, D), F32),
            pltpu.VMEM((GA, GR // 2, 256), U32),
            pltpu.VMEM((6, 8, GR // 2, 256), U32),
            pltpu.VMEM((S // 128, D, 128), U32),
            pltpu.VMEM((TA // 128, D, 128), U32),
            pltpu.VMEM((PA, 2 * VR, 4 * FA), F32),
            pltpu.VMEM((PA, VR, 4 * FA), U32),
            pltpu.VMEM((8, HD // 2, D), BF16),
            pltpu.VMEM((4, D // 2, HD // 2), U32),
            pltpu.VMEM((2, D // 2, HD // 2), U32),
            pltpu.VMEM((HD // 2, D), U32),
            pltpu.VMEM((4 * 64, NS * 128), U32),
            pltpu.VMEM((64, 3 * HD), F32),
            pltpu.VMEM((32, HD), F32),
            pltpu.VMEM((L, HD // 2), U32),
            pltpu.VMEM((16, 62 * 128), U32),
            pltpu.VMEM((TB, D), F32),
            pltpu.SemaphoreType.DMA((17 + S // TA,)),
            pltpu.SemaphoreType.DMA((1,)),
        ],
        compiler_params=pltpu.CompilerParams(vmem_limit_bytes=126 * 1024 * 1024,
                                             disable_bounds_checks=True,
                                             disable_semaphore_checks=True),
    )(x, A_wqkv, wphi, A_wo, mem0, wq, wk, wv, wo)
    return out.reshape(1, S, D)
```
